```python
import jax
import jax.numpy as jnp

def _softmax(x, axis=-1):
    return jax.nn.softmax(x, axis=axis)

def _gelu(x):
    return jax.nn.gelu(x, approximate=True)

def _silu(x):
    return jax.nn.silu(x)

def _sigmoid(x):
    return jax.nn.sigmoid(x)

def _layernorm(x, axis=-1, eps=1e-05):
    m = jnp.mean(x, axis=axis, keepdims=True)
    v = jnp.var(x, axis=axis, keepdims=True)
    return (x - m) / jnp.sqrt(v + eps)

def _scatter_add(tgt, idx, src, axis=0):
    return tgt.at[idx].add(src)

def _segment_sum(src, seg, n):
    return jax.ops.segment_sum(src, seg, n)

class _Rng:

    def __init__(self, key):
        self._k = key

    def _next(self):
        self._k, sub = jax.random.split(self._k)
        return sub

    def normal(self, shape):
        return jax.random.normal(self._next(), shape, dtype=jnp.bfloat16)

    def randint(self, lo, hi, shape):
        return jax.random.randint(self._next(), shape, lo, hi, dtype=jnp.int32)

    def uniform(self, shape, lo=0.0, hi=1.0):
        return jax.random.uniform(self._next(), shape, jnp.bfloat16, lo, hi)

    def permutation(self, n):
        return jax.random.permutation(self._next(), n)
kernel_name = 'concat_heads__memory_aug_recurrent_mem_tr__spectral_gfnet__prompt'

def setup_inputs():
    _rng = _Rng(jax.random.key(int.from_bytes(__import__("os").urandom(4), "little")))
    _w = lambda a: (lambda t: t.astype(jnp.bfloat16) if jnp.issubdtype(t.dtype, jnp.floating) else t)(jnp.asarray(a))

    def _A_setup():
        B, S, Dm = (1, 2048, 1024)
        H, Dh = (32, 128)
        M, seg = (8, 32)
        seg = min(seg, S)
        S = S // seg * seg
        return {'x': _w((lambda *s: _rng.normal(s) * 0.05)(B, S, Dm)), 'mem0': _w((lambda *s: _rng.normal(s) * 0.05)(B, M, Dm)), 'Wq': _w((lambda *s: _rng.normal(s) * 0.05)(Dm, H, Dh) * Dm ** (-0.5)), 'Wk': _w((lambda *s: _rng.normal(s) * 0.05)(Dm, H, Dh) * Dm ** (-0.5)), 'Wv': _w((lambda *s: _rng.normal(s) * 0.05)(Dm, H, Dh) * Dm ** (-0.5)), 'Wo': _w((lambda *s: _rng.normal(s) * 0.05)(H, Dh, Dm) * (H * Dh) ** (-0.5)), 'seg_len': seg}
    _A_in = _A_setup()

    def _B_setup():
        B, S, D = (1, 2048, 1024)
        Df = D // 2 + 1
        return {'x': _w((lambda *s: _rng.normal(s) * 0.05)(B, S, D)), 'w_r': _w((lambda *s: _rng.normal(s) * 0.05)(S, Df) * 0.02), 'w_i': _w((lambda *s: _rng.normal(s) * 0.05)(S, Df) * 0.02)}
    _B_in = _B_setup()
    return {'A_x': _A_in['x'], 'A_mem0': _A_in['mem0'], 'A_Wq': _A_in['Wq'], 'A_Wk': _A_in['Wk'], 'A_Wv': _A_in['Wv'], 'A_Wo': _A_in['Wo'], 'A_seg_len': _A_in['seg_len'], 'B_x': _B_in['x'], 'B_w_r': _B_in['w_r'], 'B_w_i': _B_in['w_i']}

def reference(A_x, A_mem0, A_Wq, A_Wk, A_Wv, A_Wo, A_seg_len, B_x, B_w_r, B_w_i):

    def _A_ref(x, mem0, Wq, Wk, Wv, Wo, seg_len):
        B, S, Dm = x.shape
        H, Dh = (Wq.shape[1], Wq.shape[2])
        M = mem0.shape[1]
        scale = Dh ** (-0.5)
        n_seg = S // seg_len
        L = M + seg_len
        idx = jnp.arange(L)
        mask = (idx[:, None] < M) | (idx[:, None] >= idx[None, :])
        mem = mem0
        outs = []
        for s in range(n_seg):
            xs = x[:, s * seg_len:(s + 1) * seg_len, :].copy()
            h = jnp.concatenate([mem, xs], axis=1)
            q = jnp.einsum('btd,dhe->bhte', h, Wq)
            k = jnp.einsum('btd,dhe->bhte', h, Wk)
            v = jnp.einsum('btd,dhe->bhte', h, Wv)
            scores = jnp.einsum('bhqe,bhke->bhqk', q, k) * scale
            scores = jnp.where(mask[None, None], scores, -1000000000.0)
            p = _softmax(scores, axis=-1)
            o = jnp.einsum('bhqk,bhke->bhqe', p, v)
            o = jnp.einsum('bhte,hed->btd', o, Wo)
            mem = o[:, :M, :].copy()
            outs.append(o[:, M:, :])
        return jnp.concatenate(outs, axis=1)

    def _B_ref(x, w_r, w_i):
        B, S, D = x.shape
        X = (lambda x, axes=(-2, -1): jnp.fft.rfft2(x.astype(jnp.float32), axes=axes))(x, axes=(-2, -1))
        W = w_r + 1j * w_i
        X = X * W
        y = (lambda x, s, axes=(-2, -1): jnp.fft.irfft2(x, s=s, axes=axes).astype(jnp.bfloat16))(X, (S, D), axes=(-2, -1))
        return y
    a = _A_ref(A_x, A_mem0, A_Wq, A_Wk, A_Wv, A_Wo, A_seg_len)
    b = _B_ref(B_x, B_w_r, B_w_i)
    return jnp.concatenate([a, b], axis=-1)
```

```python
import functools

import jax
import jax.numpy as jnp
import numpy as np
from jax import lax
from jax.experimental import pallas as pl
from jax.experimental.pallas import tpu as pltpu

S, D, H, E, M, SEG = 2048, 1024, 32, 128, 8, 32
NSEG = S // SEG
WP = 516
XP = 132
YR = 520
bf16, f32, u32 = jnp.bfloat16, jnp.float32, jnp.uint32
RES = ((0, 4), (2, 6), (1, 7), (3, 5))
RC = float(np.sqrt(0.5))


def _fwd8(x):
    s04, d04 = x[0] + x[4], x[0] - x[4]
    s26, d26 = x[2] + x[6], x[2] - x[6]
    s15, d15 = x[1] + x[5], x[1] - x[5]
    s37, d37 = x[3] + x[7], x[3] - x[7]
    t1, t2 = (d15 - d37) * RC, (d15 + d37) * RC
    return [s04 + s26, s15 + s37, s04 - s26, s15 - s37, d04 + t1, d26 + t2, d04 - t1, d26 - t2]


def _inv8(z):
    e0, o0, e1, o1, r1, i1, r3, i3 = z
    s04, s26, s15, s37 = e0 + e1, e0 - e1, o0 + o1, o0 - o1
    d04, d26 = r1 + r3, i1 + i3
    t1, t2 = (r1 - r3) * RC, (i1 - i3) * RC
    d15, d37 = t1 + t2, t2 - t1
    return [s04 + d04, s15 + d15, s26 + d26, s37 + d37, s04 - d04, s15 - d15, s26 - d26, s37 - d37]


def _twiddle16(z, k):
    re, im = z
    k = k % 16
    if k == 0:
        return z
    if k == 4:
        return (im, -re)
    if k == 12:
        return (-im, re)
    if k == 2:
        return ((re + im) * RC, (im - re) * RC)
    if k == 14:
        return ((re - im) * RC, (re + im) * RC)
    if k == 6:
        return ((im - re) * RC, (re + im) * -RC)
    if k == 10:
        return ((re + im) * -RC, (re - im) * RC)
    c, s = float(np.cos(2 * np.pi * k / 16)), float(-np.sin(2 * np.pi * k / 16))
    return (re * c - im * s, re * s + im * c)


def _bfly4(z, sign):
    (ar, ai), (br, bi), (cr, ci), (dr, di) = z
    sr, si, tr, ti = ar + cr, ai + ci, ar - cr, ai - ci
    ur, ui, vr, vi = br + dr, bi + di, br - dr, bi - di
    o0, o2 = (sr + ur, si + ui), (sr - ur, si - ui)
    p, q = (tr + vi, ti - vr), (tr - vi, ti + vr)
    return [o0, p, o2, q] if sign > 0 else [o0, q, o2, p]


def _filter16(z, wfn):
    st = [None] * 16
    for b0 in range(4):
        o = _bfly4([z[4 * b1 + b0] for b1 in range(4)], 1)
        for d0 in range(4):
            st[4 * d0 + b0] = _twiddle16(o[d0], b0 * d0)
    for d0 in range(4):
        o = _bfly4([st[4 * d0 + b0] for b0 in range(4)], 1)
        y = []
        for d1 in range(4):
            wr, wi = wfn(d0 + 4 * d1)
            xr, xi = o[d1]
            y.append((xr * wr - xi * wi, xr * wi + xi * wr))
        o = _bfly4(y, -1)
        for b0 in range(4):
            st[4 * d0 + b0] = _twiddle16(o[b0], -b0 * d0)
    out = [None] * 16
    for b0 in range(4):
        o = _bfly4([st[4 * d0 + b0] for d0 in range(4)], -1)
        for b1 in range(4):
            out[4 * b1 + b0] = o[b1]
    return out


def _pack_rows(m):
    b = np.asarray(m, np.float32).astype(jnp.bfloat16).view(np.uint16).astype(np.uint32)
    return b[..., 0::2, :] | (b[..., 1::2, :] << 16)


@functools.lru_cache(maxsize=None)
def _dft_constants():
    b8 = np.array(_fwd8(list(np.eye(8)))).T
    n = np.arange(D)
    fw = np.zeros((D, D))
    bw = np.zeros((D, D))
    for g in range(4):
        k = np.concatenate([8 * np.arange(64) + r for r in RES[g]])
        ang = 2 * np.pi * ((n[:, None] * k[None, :]) % D) / D
        wgt = np.where(k == 0, 1.0, 2.0) / (D * S)
        fw[:, 256 * g:256 * g + 128] = np.cos(ang)
        fw[:, 256 * g + 128:256 * g + 256] = -np.sin(ang)
        bw[256 * g:256 * g + 128] = (np.cos(ang) * wgt).T
        bw[256 * g + 128:256 * g + 256] = (-np.sin(ang) * wgt).T
    bw[128, :] = (-1.0) ** n / (D * S)
    binv = np.kron(np.linalg.inv(b8), np.eye(128))
    gall = binv @ fw
    giall = bw @ binv.T
    gf = np.zeros((4, 272, 256))
    gi = np.zeros((4, 256, 256))
    for g in range(4):
        sl = slice(256 * g, 256 * g + 256)
        gf[g, :256] = gall[sl, sl].T
        gi[g] = giall[sl, sl]
    gf[0, 256] = (-1.0) ** np.arange(256)
    split = lambda m: np.stack([m[..., :128], m[..., 128:]], axis=1)
    a = np.arange(128)
    mt = np.zeros((16, 256, 128))
    for b in range(16):
        ang = 2 * np.pi * (((16 * a[:, None] + b) * a[None, :]) % S) / S
        mt[b, :128], mt[b, 128:] = np.cos(ang), -np.sin(ang)
    return _pack_rows(split(gf)), _pack_rows(split(gi)), _pack_rows(mt)


def _attn_fill():
    head = np.concatenate([np.zeros(32), np.ones(32), np.zeros(8), np.ones(8)]).astype(int)
    pos32 = np.concatenate([np.arange(8), np.arange(16, 40)])
    pos = np.concatenate([pos32, pos32, np.arange(8, 16), np.arange(8, 16)])
    ok = (pos[:, None] < M) | (pos[:, None] >= pos[None, :])
    fill = np.where(ok, 0.0, -1e9)
    fill = np.where(head[:, None] == head[None, :], fill, -np.inf)
    return fill.astype(np.float32)


def _kernel(x_hbm, mem_hbm, wq_hbm, wk_hbm, wv_hbm, wo_hbm, bx_hbm, wr_hbm, wi_hbm,
            gf_hbm, gi_hbm, mt_hbm, fill_hbm, out_hbm,
            wraw, w32, wo, xbuf, x8, pre, odef, outbuf, fill_ref,
            xb, wt, wl, gf, gi, mt, xd, yb, sems):
    def start(src, dst, i):
        c = pltpu.make_async_copy(src, dst, sems.at[i])
        c.start()
        return c

    def wait_all(cs):
        for c in cs:
            c.wait()

    dot = functools.partial(jnp.dot, preferred_element_type=f32)
    dot_nt = lambda a, b: lax.dot_general(a, b, (((1,), (1,)), ((), ())), preferred_element_type=f32)
    as_bf16 = lambda w: pltpu.bitcast(w, bf16)
    lo_f32 = lambda w: pltpu.bitcast(w << 16, f32)
    hi_f32 = lambda w: pltpu.bitcast(w & u32(0xFFFF0000), f32)
    out3 = out_hbm.reshape(NSEG, SEG, 2 * D)

    c_b1 = [start(bx_hbm.at[:, pl.ds(128 * j, 128)], xb.at[j], 0) for j in range(8)]
    c_b1 += [start(gf_hbm, gf, 1), start(mt_hbm, mt, 2)]
    c_x8 = start(x_hbm.at[:, pl.ds(0, M), :], x8, 3)
    c_wq = start(wq_hbm, wraw.at[0], 4)
    c_wk = start(wk_hbm, wraw.at[1], 5)
    c_flt = []
    for t, w in enumerate((wr_hbm, wi_hbm)):
        for d in range(16):
            c_flt.append(start(w.at[pl.ds(0, 512), pl.ds(128 * d, 128)], wt.at[t, d], 6))
        c_flt.append(start(w.at[pl.ds(512, 1), :], wl.at[t], 7 + t))
    c_gi = start(gi_hbm, gi, 9)

    xb32 = xb.bitcast(u32)

    def b_dfwd(b):
        un = lo_f32 if b % 2 == 0 else hi_f32
        z = _fwd8([un(xb32[j, pl.ds(b // 2, 128, stride=8), :]) for j in range(8)])
        ts = []
        for g in range(4):
            rows = 136 if g == 0 else 128
            t = (dot_nt(as_bf16(gf[g, 0, 0:rows]), z[2 * g].astype(bf16))
                 + dot_nt(as_bf16(gf[g, 1, 0:rows]), z[2 * g + 1].astype(bf16)))
            ts.append(t.astype(bf16))
        return ts

    def b_sfwd(b, ts):
        mr, mi = as_bf16(mt[b, 0:64]), as_bf16(mt[b, 64:128])
        for g in range(4):
            pa, pb = dot(ts[g], mr), dot(ts[g], mi)
            yb[0, b, pl.ds(128 * g, 128), :] = pa[0:128] - pb[128:256]
            yb[1, b, pl.ds(128 * g, 128), :] = pb[0:128] + pa[128:256]
            if g == 0:
                yb[0, b, pl.ds(512, 8), :] = pa[256:264]
                yb[1, b, pl.ds(512, 8), :] = pb[256:264]

    wait_all(c_b1)
    prev = None
    for b in range(16):
        ts = b_dfwd(b)
        if prev is not None:
            b_sfwd(b - 1, prev)
        prev = ts
    b_sfwd(15, prev)

    wraw32 = wraw.bitcast(u32)

    def relayout(i, slot):
        def body(t, c):
            off = pl.multiple_of(t * 8, 8)
            ov = w32.at[i, pl.ds(off, 31 * WP + 12)]
            for u in range(8):
                a = wraw32[slot, off + u, 0:16, :]
                b = wraw32[slot, off + u, 16:32, :]
                ov[pl.ds(u, 16, stride=WP), :] = (a & u32(0xFFFF)) | (b << 16)
                ov[pl.ds(u + 16 * WP, 16, stride=WP), :] = (a >> 16) | (b & u32(0xFFFF0000))
            return c
        lax.fori_loop(0, D // 16, body, 0)

    def wqkv(i, p, second):
        return as_bf16(w32[i, pl.ds((p + 16 * second) * WP, D // 2), :])

    def batch_proj(i):
        for p in range(16):
            lhs = x8[...].reshape(NSEG * M, D)
            r1 = dot(lhs, wqkv(i, p, 0))
            r2 = dot(lhs, wqkv(i, p, 1))
            st = jnp.concatenate([r1.reshape(NSEG, M, E), r2.reshape(NSEG, M, E)], axis=1)
            pre[i, p] = pltpu.bitcast(st.reshape(NSEG * 2 * M, E).astype(bf16), u32)

    c_x8.wait()
    c_wq.wait()
    relayout(0, 0)
    c_wv = start(wv_hbm, wraw.at[0], 10)
    c_x = [start(x_hbm.at[:, pl.ds(M, SEG - M), :], xbuf.at[:, pl.ds(M, SEG - M), :], 11),
           start(mem_hbm, xbuf.at[0, pl.ds(0, M), :], 12), start(fill_hbm, fill_ref, 13)]
    c_wo = [start(wo_hbm.at[:, pl.ds(128 * j, 128)], wo.at[j], 14) for j in range(8)]
    batch_proj(0)
    c_wk.wait()
    relayout(1, 1)
    batch_proj(1)

    wait_all(c_flt)
    wt32 = wt.bitcast(u32)

    def mid_block(rows, wfn):
        z = [(yb[0, b, rows, :], yb[1, b, rows, :]) for b in range(16)]
        o = _filter16(z, wfn)
        for b in range(16):
            yb[0, b, rows, :] = o[b][0]
            yb[1, b, rows, :] = o[b][1]

    def mid(i, c):
        for g in range(4):
            for q in range(2):
                r = RES[g][q]
                un = lo_f32 if r % 2 == 0 else hi_f32

                def wfn(d, r=r, un=un):
                    blk = pl.ds(pl.multiple_of(32 * i, 32), 32)
                    return [un(wt32.at[t, d, blk][pl.ds(r // 2, 8, stride=4), :]) for t in range(2)]
                mid_block(pl.ds(pl.multiple_of(128 * g + 64 * q + 8 * i, 8), 8), wfn)
        return c
    lax.fori_loop(0, 8, mid, 0)
    mid_block(pl.ds(512, 8), lambda d: [wl[t, :, pl.ds(128 * d, 128)].astype(f32) for t in range(2)])

    c_gi.wait()
    row0 = lax.broadcasted_iota(jnp.int32, (8, 128), 0) == 0
    for b in range(16):
        m = as_bf16(mt[b])
        for g in range(4):
            yr, yi = yb[0, b, pl.ds(128 * g, 128), :], yb[1, b, pl.ds(128 * g, 128), :]
            if g == 0:
                v2 = jnp.concatenate([jnp.where(row0, yb[0, b, pl.ds(512, 8), :], yi[0:8]), yi[8:]], axis=0)
                u2 = jnp.concatenate([jnp.where(row0, -yb[1, b, pl.ds(512, 8), :], yr[0:8]), yr[8:]], axis=0)
                tr = dot_nt(m[:128], yr.astype(bf16)) + dot_nt(m[128:], yi.astype(bf16))
                ti = dot_nt(m[:128], v2.astype(bf16)) - dot_nt(m[128:], u2.astype(bf16))
            else:
                pa, pb = dot_nt(m, yr.astype(bf16)), dot_nt(m, yi.astype(bf16))
                tr = pa[:128] + pb[128:]
                ti = pb[:128] - pa[128:]
            xd[2 * g, pl.ds(XP * b, 128), :] = tr
            xd[2 * g + 1, pl.ds(XP * b, 128), :] = ti
    for t in range(16):
        z = []
        for g in range(4):
            zz = jnp.concatenate(
                [jnp.concatenate([xd[2 * g + h, pl.ds(8 * t + u, 16, stride=XP), :] for u in range(8)], axis=0)
                 for h in range(2)], axis=1).astype(bf16)
            z += [dot(zz, as_bf16(gi[g, 0])), dot(zz, as_bf16(gi[g, 1]))]
        y = _inv8(z)
        for j in range(8):
            xb32[j, pl.ds(64 * t, 64), :] = pltpu.bitcast(y[j].astype(bf16), u32)
    c_out = [start(xb.at[j], out_hbm.at[:, pl.ds(D + 128 * j, 128)], 15) for j in range(8)]

    c_wv.wait()
    relayout(2, 0)
    batch_proj(2)
    wait_all(c_x)
    wait_all(c_wo)

    wo32 = wo.bitcast(u32)
    scale = E ** -0.5

    def step(s, mem):
        top = jnp.concatenate([mem, xbuf[s, pl.ds(M, M), :].astype(f32)], axis=0).astype(bf16)
        lhs = jnp.concatenate([top, xbuf[s, pl.ds(2 * M, 2 * M), :]], axis=0)
        r8 = pl.multiple_of(M * s, M)
        fill = fill_ref[...]
        heads = [None] * H

        def proj(i, p):
            a = dot(lhs, wqkv(i, p, 0))
            b = dot(lhs, wqkv(i, p, 1))
            return jnp.concatenate([a.astype(bf16), b.astype(bf16), as_bf16(pre[i, p, pl.ds(r8, M), :])], axis=0)

        def probs(q, k):
            sc = dot_nt(q, k) * scale
            sc = jnp.where(fill == 0.0, sc, fill)
            e = jnp.exp(sc - jnp.max(sc, axis=1, keepdims=True))
            return (e * (1.0 / jnp.sum(e, axis=1, keepdims=True))).astype(bf16)

        def pv(p, pr, v):
            o = dot(pr, v)
            heads[2 * p] = o[0:32].astype(bf16)
            heads[2 * p + 1] = o[32:64].astype(bf16)
            odef[2 * p, pl.ds(r8, M), :] = o[64:72].astype(bf16)
            odef[2 * p + 1, pl.ds(r8, M), :] = o[72:80].astype(bf16)

        pend = []
        for g in range(8):
            ps = (2 * g, 2 * g + 1)
            qk = [(proj(0, p), proj(1, p)) for p in ps]
            vs = [proj(2, p) for p in ps]
            new = [(p, probs(*qk[t]), vs[t]) for t, p in enumerate(ps)]
            for a in pend:
                pv(*a)
            pend = new

        def wo_part(j, h0, h1):
            oc = jnp.concatenate(heads[h0:h1], axis=1)
            return dot(oc, as_bf16(wo32[j, pl.ds(64 * h0, 64 * (h1 - h0)), :]))

        acc = []
        for j in range(8):
            acc.append(wo_part(j, 0, 24))
            if j == 3:
                for a in pend:
                    pv(*a)
        nxt = []
        for j in range(8):
            r = wo_part(j, 24, 32) + acc[j]
            outbuf[s, pl.ds(M, SEG - M), pl.ds(128 * j, 128)] = r[M:].astype(bf16)
            nxt.append(r[0:M])
        return jnp.concatenate(nxt, axis=1)
    lax.fori_loop(0, NSEG, step, xbuf[0, pl.ds(0, M), :].astype(f32))
    c_out.append(start(outbuf.at[:, pl.ds(M, SEG - M), :], out3.at[:, pl.ds(M, SEG - M), pl.ds(0, D)], 16))

    for t in range(4):
        lhs = jnp.concatenate([odef[h, pl.ds(128 * t, 128), :] for h in range(H)], axis=1)
        for j in range(8):
            r = dot(lhs, as_bf16(wo32[j]))
            outbuf[pl.ds(16 * t, 16), pl.ds(0, M), pl.ds(128 * j, 128)] = r.reshape(16, M, 128).astype(bf16)
        c_out.append(start(outbuf.at[pl.ds(16 * t, 16), pl.ds(0, M), :],
                           out3.at[pl.ds(16 * t, 16), pl.ds(0, M), pl.ds(0, D)], 17 + t))
    wait_all(c_out)


@functools.partial(jax.jit, static_argnames=("A_seg_len",))
def pallas_concat_heads__memory_aug_recurrent_mem_tr__spectral_gfnet__prompt_kernel(
    A_x: jax.Array,
    A_mem0: jax.Array,
    A_Wq: jax.Array,
    A_Wk: jax.Array,
    A_Wv: jax.Array,
    A_Wo: jax.Array,
    A_seg_len,
    B_x: jax.Array,
    B_w_r: jax.Array,
    B_w_i: jax.Array,
):
    assert A_seg_len == SEG
    assert A_x.shape == (1, S, D) and A_mem0.shape == (1, M, D) and B_x.shape == (1, S, D)
    assert A_Wq.shape == (D, H, E) and A_Wo.shape == (H, E, D) and B_w_r.shape == (S, D // 2 + 1)
    gf, gi, mt = _dft_constants()
    fill = _attn_fill()
    hbm = pl.BlockSpec(memory_space=pltpu.HBM)
    out = pl.pallas_call(
        _kernel,
        out_shape=jax.ShapeDtypeStruct((S, 2 * D), bf16),
        in_specs=[hbm] * 13,
        out_specs=hbm,
        scratch_shapes=[
            pltpu.VMEM((2, D // 2, 2 * H, E), bf16),
            pltpu.VMEM((3, H * WP, E), u32),
            pltpu.VMEM((8, H * E, 128), bf16),
            pltpu.VMEM((NSEG, SEG, D), bf16),
            pltpu.VMEM((NSEG, M, D), bf16),
            pltpu.VMEM((3, 16, NSEG * M, E), u32),
            pltpu.VMEM((H, NSEG * M, E), bf16),
            pltpu.VMEM((NSEG, SEG, D), bf16),
            pltpu.VMEM(fill.shape, f32),
            pltpu.VMEM((8, S, 128), bf16),
            pltpu.VMEM((2, 16, 512, 128), bf16),
            pltpu.VMEM((2, 1, S), bf16),
            pltpu.VMEM(gf.shape, u32),
            pltpu.VMEM(gi.shape, u32),
            pltpu.VMEM(mt.shape, u32),
            pltpu.VMEM((8, 16 * XP, 128), f32),
            pltpu.VMEM((2, 16, YR, 128), f32),
            pltpu.SemaphoreType.DMA((21,)),
        ],
        compiler_params=pltpu.CompilerParams(vmem_limit_bytes=120 * 1024 * 1024),
    )(A_x.reshape(NSEG, SEG, D), A_mem0.reshape(M, D),
      A_Wq.reshape(D // 2, 2 * H, E), A_Wk.reshape(D // 2, 2 * H, E), A_Wv.reshape(D // 2, 2 * H, E),
      A_Wo.reshape(H * E, D), B_x.reshape(S, D), B_w_r.T, B_w_i.T, gf, gi, mt, fill)
    return out.reshape(1, S, 2 * D)
```

```python
import functools

import jax
import jax.numpy as jnp
import numpy as np
from jax import lax
from jax.experimental import pallas as pl
from jax.experimental.pallas import tpu as pltpu

S, D, H, E, M, SEG = 2048, 1024, 32, 128, 8, 32
NSEG = S // SEG
WP = 516
XP = 132
YR = 520
NRAW = 4
BM = 128
B1_SPLIT = 10
bf16, f32, u32 = jnp.bfloat16, jnp.float32, jnp.uint32
RES = ((0, 4), (2, 6), (1, 7), (3, 5))
RC = float(np.sqrt(0.5))


def _fwd8(x):
    s04, d04 = x[0] + x[4], x[0] - x[4]
    s26, d26 = x[2] + x[6], x[2] - x[6]
    s15, d15 = x[1] + x[5], x[1] - x[5]
    s37, d37 = x[3] + x[7], x[3] - x[7]
    t1, t2 = (d15 - d37) * RC, (d15 + d37) * RC
    return [s04 + s26, s15 + s37, s04 - s26, s15 - s37, d04 + t1, d26 + t2, d04 - t1, d26 - t2]


def _inv8(z):
    e0, o0, e1, o1, r1, i1, r3, i3 = z
    s04, s26, s15, s37 = e0 + e1, e0 - e1, o0 + o1, o0 - o1
    d04, d26 = r1 + r3, i1 + i3
    t1, t2 = (r1 - r3) * RC, (i1 - i3) * RC
    d15, d37 = t1 + t2, t2 - t1
    return [s04 + d04, s15 + d15, s26 + d26, s37 + d37, s04 - d04, s15 - d15, s26 - d26, s37 - d37]


def _twiddle16(z, k):
    re, im = z
    k = k % 16
    if k == 0:
        return z
    if k == 4:
        return (im, -re)
    if k == 12:
        return (-im, re)
    if k == 2:
        return ((re + im) * RC, (im - re) * RC)
    if k == 14:
        return ((re - im) * RC, (re + im) * RC)
    if k == 6:
        return ((im - re) * RC, (re + im) * -RC)
    if k == 10:
        return ((re + im) * -RC, (re - im) * RC)
    c, s = float(np.cos(2 * np.pi * k / 16)), float(-np.sin(2 * np.pi * k / 16))
    return (re * c - im * s, re * s + im * c)


def _bfly4(z, sign):
    (ar, ai), (br, bi), (cr, ci), (dr, di) = z
    sr, si, tr, ti = ar + cr, ai + ci, ar - cr, ai - ci
    ur, ui, vr, vi = br + dr, bi + di, br - dr, bi - di
    o0, o2 = (sr + ur, si + ui), (sr - ur, si - ui)
    p, q = (tr + vi, ti - vr), (tr - vi, ti + vr)
    return [o0, p, o2, q] if sign > 0 else [o0, q, o2, p]


class _Pacer:
    def __init__(self, tasks, ntokens):
        self.slots = {}
        for n, task in enumerate(tasks):
            self.slots.setdefault(n * ntokens // len(tasks), []).append(task)
        self.pos = 0
        self.ntokens = ntokens

    def feed(self, r):
        for j in range(r.shape[0] // 8):
            for task in self.slots.pop(self.pos, []):
                task(pltpu.bitcast(r[8 * j:8 * j + 8], u32))
            self.pos += 1

    def done(self):
        assert not self.slots and self.pos == self.ntokens


def _pack_rows(m):
    b = np.asarray(m, np.float32).astype(jnp.bfloat16).view(np.uint16).astype(np.uint32)
    return b[..., 0::2, :] | (b[..., 1::2, :] << 16)


@functools.lru_cache(maxsize=None)
def _dft_constants():
    b8 = np.array(_fwd8(list(np.eye(8)))).T
    n = np.arange(D)
    fw = np.zeros((D, D))
    bw = np.zeros((D, D))
    for g in range(4):
        k = np.concatenate([8 * np.arange(64) + r for r in RES[g]])
        ang = 2 * np.pi * ((n[:, None] * k[None, :]) % D) / D
        wgt = np.where(k == 0, 1.0, 2.0) / (D * S)
        fw[:, 256 * g:256 * g + 128] = np.cos(ang)
        fw[:, 256 * g + 128:256 * g + 256] = -np.sin(ang)
        bw[256 * g:256 * g + 128] = (np.cos(ang) * wgt).T
        bw[256 * g + 128:256 * g + 256] = (-np.sin(ang) * wgt).T
    bw[128, :] = (-1.0) ** n / (D * S)
    binv = np.kron(np.linalg.inv(b8), np.eye(128))
    gall = binv @ fw
    giall = bw @ binv.T
    gf = np.zeros((4, 272, 256))
    gi = np.zeros((4, 256, 256))
    for g in range(4):
        sl = slice(256 * g, 256 * g + 256)
        gf[g, :256] = gall[sl, sl].T
        gi[g] = giall[sl, sl]
    gf[0, 256] = (-1.0) ** np.arange(256)
    split = lambda m: np.stack([m[..., :128], m[..., 128:]], axis=1)
    a = np.arange(128)
    mt = np.zeros((16, 256, 128))
    for b in range(16):
        ang = 2 * np.pi * (((16 * a[:, None] + b) * a[None, :]) % S) / S
        mt[b, :128], mt[b, 128:] = np.cos(ang), -np.sin(ang)
    return _pack_rows(split(gf)), _pack_rows(split(gi)), _pack_rows(mt)


def _attn_fill():
    head = np.concatenate([np.zeros(32), np.ones(32), np.zeros(8), np.ones(8)]).astype(int)
    pos32 = np.concatenate([np.arange(8), np.arange(16, 40)])
    pos = np.concatenate([pos32, pos32, np.arange(8, 16), np.arange(8, 16)])
    ok = (pos[:, None] < M) | (pos[:, None] >= pos[None, :])
    fill = np.where(ok, 0.0, -1e9)
    fill = np.where(head[:, None] == head[None, :], fill, -np.inf)
    return fill.astype(np.float32)


def _kernel(x_hbm, mem_hbm, wq_hbm, wk_hbm, wv_hbm, wo_hbm, bx_hbm, wr_hbm, wi_hbm,
            gf_hbm, gi_hbm, mt_hbm, fill_hbm, out_hbm,
            wraw, w0, w1, w2, w3, w4, w5, wo, xbuf, x8, x8c, pre, odef, outbuf, fill_ref,
            xb, wt, wl, gf, gi, mt, xd, yb, sems):
    def start(src, dst, i):
        c = pltpu.make_async_copy(src, dst, sems.at[i])
        c.start()
        return c

    def wait_all(cs):
        for c in cs:
            c.wait()

    dot = functools.partial(jnp.dot, preferred_element_type=f32)
    dot_nt = lambda a, b: lax.dot_general(a, b, (((1,), (1,)), ((), ())), preferred_element_type=f32)
    as_bf16 = lambda w: pltpu.bitcast(w, bf16)
    lo_f32 = lambda w: pltpu.bitcast(w << 16, f32)
    hi_f32 = lambda w: pltpu.bitcast(w & u32(0xFFFF0000), f32)
    out3 = out_hbm.reshape(NSEG, SEG, 2 * D)
    w_hbm = (wq_hbm, wk_hbm, wv_hbm)
    w32 = (w0, w1, w2, w3, w4, w5)

    def start_unit(u):
        return start(w_hbm[u // 2].at[:, :, u % 2], wraw.at[u % NRAW], 4 + u)

    c_b1 = [start(bx_hbm.at[:, pl.ds(128 * j, 128)], xb.at[j], 0) for j in range(8)]
    c_b1 += [start(gf_hbm, gf, 1), start(mt_hbm, mt, 2)]
    c_x8 = start(x_hbm.at[:, pl.ds(0, M), :], x8, 3)
    c_w = [start_unit(u) for u in range(3)]
    c_flt = []
    for t, w in enumerate((wr_hbm, wi_hbm)):
        for d in range(16):
            c_flt.append(start(w.at[pl.ds(0, 512), pl.ds(128 * d, 128)], wt.at[t, d], 10))
        c_flt.append(start(w.at[pl.ds(512, 1), :], wl.at[t], 11 + t))
    c_w.append(start_unit(3))

    wraw32 = wraw.bitcast(u32)
    wt32 = wt.bitcast(u32)

    def relayout_tasks(u):
        def make(r0):
            def task(tok):
                lo = (tok >> 16) | u32(0xFFFF)
                hi = (tok << 16) | u32(0xFFFF0000)
                for r in range(r0, r0 + 2):
                    a, b = wraw32[u % NRAW, r, 0], wraw32[u % NRAW, r, 1]
                    w32[u][pl.ds(r, 8, stride=WP), :] = (a & lo) | (b << 16)
                    w32[u][pl.ds(r + 8 * WP, 8, stride=WP), :] = (a >> 16) | (b & hi)
            return task
        return [make(r0) for r0 in range(0, D // 2, 2)]

    def filter_tasks(rows, wfn):
        def make(phase, k):
            slots = [4 * k + j for j in range(4)] if phase == 1 else [4 * j + k for j in range(4)]

            def task(tok):
                ones = ((tok >> 16) | u32(0xFFFF)) | u32(0xFFFF0000)
                z = [(yb[0, b, rows, :], yb[1, b, rows, :]) for b in slots]
                z[0] = tuple(pltpu.bitcast(pltpu.bitcast(v, u32) & ones, f32) for v in z[0])
                if phase == 0:
                    o = _bfly4(z, 1)
                    o = [_twiddle16(o[j], k * j) for j in range(4)]
                elif phase == 1:
                    o = _bfly4(z, 1)
                    y = []
                    for j in range(4):
                        wr, wi = wfn(k + 4 * j)
                        xr, xi = o[j]
                        y.append((xr * wr - xi * wi, xr * wi + xi * wr))
                    o = _bfly4(y, -1)
                    o = [_twiddle16(o[j], -k * j) for j in range(4)]
                else:
                    o = _bfly4(z, -1)
                for b, v in zip(slots, o):
                    yb[0, b, rows, :] = v[0]
                    yb[1, b, rows, :] = v[1]
            return task
        return [make(phase, k) for phase in range(3) for k in range(4)]

    def all_filter_tasks():
        tasks = []
        for i in range(8):
            for g in range(4):
                for q in range(2):
                    r = RES[g][q]
                    un = lo_f32 if r % 2 == 0 else hi_f32
                    wrows = pl.ds(32 * i + r // 2, 8, stride=4)
                    tasks += filter_tasks(pl.ds(128 * g + 64 * q + 8 * i, 8),
                                          lambda d, un=un, wrows=wrows: [un(wt32[t, d, wrows, :]) for t in range(2)])
        tasks += filter_tasks(pl.ds(512, 8), lambda d: [wl[t, :, pl.ds(128 * d, 128)].astype(f32) for t in range(2)])
        return tasks

    def merge(a, b):
        keyed = [(n / len(a), 0, n) for n in range(len(a))] + [(n / len(b), 1, n) for n in range(len(b))]
        return [(a, b)[w][n] for _, w, n in sorted(keyed)]

    xb32 = xb.bitcast(u32)

    def b_dfwd(b):
        un = lo_f32 if b % 2 == 0 else hi_f32
        z = _fwd8([un(xb32[j, pl.ds(b // 2, 128, stride=8), :]) for j in range(8)])
        ts = []
        for g in range(4):
            rows = 136 if g == 0 else 128
            t = (dot_nt(as_bf16(gf[g, 0, 0:rows]), z[2 * g].astype(bf16))
                 + dot_nt(as_bf16(gf[g, 1, 0:rows]), z[2 * g + 1].astype(bf16)))
            ts.append(t.astype(bf16))
        return ts

    def b_sfwd(b, ts, pacer=None):
        mr, mi = as_bf16(mt[b, 0:64]), as_bf16(mt[b, 64:128])
        for g in range(4):
            pa, pb = dot(ts[g], mr), dot(ts[g], mi)
            yb[0, b, pl.ds(128 * g, 128), :] = pa[0:128] - pb[128:256]
            yb[1, b, pl.ds(128 * g, 128), :] = pb[0:128] + pa[128:256]
            if g == 0:
                yb[0, b, pl.ds(512, 8), :] = pa[256:264]
                yb[1, b, pl.ds(512, 8), :] = pb[256:264]
            if pacer is not None:
                pacer.feed(pa[0:256])

    def b_stage1(b0, b1, pacer=None):
        prev = None
        for b in range(b0, b1):
            ts = b_dfwd(b)
            if prev is not None:
                b_sfwd(b - 1, prev, pacer)
            prev = ts
        b_sfwd(b1 - 1, prev, None)

    wait_all(c_b1)
    b_stage1(0, B1_SPLIT)
    c_x8.wait()
    c_w[0].wait()
    x8v = x8[...].reshape(NSEG * M, D)
    for k in range(8):
        x8c[k] = pltpu.bitcast(x8v[:, 128 * k:128 * k + 128], u32)
    pacer = _Pacer(relayout_tasks(0), (15 - B1_SPLIT) * 128)
    b_stage1(B1_SPLIT, 16, pacer)
    pacer.done()

    def wqkv(i, p, second):
        return as_bf16(w32[2 * i + p // 8][pl.ds((p % 8 + 8 * second) * WP, D // 2), :])

    def batch_unit(u, tasks):
        pacer = _Pacer(tasks, 7 * 128 + 64) if tasks else None
        for p in range(8 * (u % 2), 8 * (u % 2) + 8):
            for c in range(NSEG * M // BM):
                lhs = jnp.concatenate([as_bf16(x8c[k, pl.ds(c * BM // 2, BM // 2), :]) for k in range(8)], axis=1)
                r1 = dot(lhs, wqkv(u // 2, p, 0))
                r2 = dot(lhs, wqkv(u // 2, p, 1))
                st = jnp.concatenate([r1.reshape(BM // M, M, E), r2.reshape(BM // M, M, E)], axis=1)
                pre[u // 2, p, pl.ds(c * BM, BM), :] = pltpu.bitcast(st.reshape(2 * BM, E).astype(bf16), u32)
                if pacer is not None and pacer.pos < pacer.ntokens:
                    pacer.feed(r1)
                    pacer.feed(r2)
        if pacer is not None:
            pacer.done()

    c_w[1].wait()
    c_w.append(start_unit(4))
    batch_unit(0, relayout_tasks(1))
    c_w[2].wait()
    c_w.append(start_unit(5))
    c_gi = start(gi_hbm, gi, 13)
    c_x = [start(x_hbm.at[:, pl.ds(M, SEG - M), :], xbuf.at[:, pl.ds(M, SEG - M), :], 14),
           start(mem_hbm, xbuf.at[0, pl.ds(0, M), :], 15), start(fill_hbm, fill_ref, 16)]
    c_wo = [start(wo_hbm.at[:, pl.ds(128 * j, 128)], wo.at[j], 17) for j in range(8)]
    batch_unit(1, relayout_tasks(2))
    c_w[3].wait()
    wait_all(c_flt)
    flt = all_filter_tasks()
    third = 12 * 22
    batch_unit(2, merge(relayout_tasks(3), flt[:third]))
    c_w[4].wait()
    c_w[5].wait()
    c_gi.wait()
    batch_unit(3, merge(relayout_tasks(4), flt[third:2 * third]))
    batch_unit(4, merge(relayout_tasks(5), flt[2 * third:]))

    row0 = lax.broadcasted_iota(jnp.int32, (8, 128), 0) == 0
    for b in range(16):
        m = as_bf16(mt[b])
        for g in range(4):
            yr, yi = yb[0, b, pl.ds(128 * g, 128), :], yb[1, b, pl.ds(128 * g, 128), :]
            if g == 0:
                v2 = jnp.concatenate([jnp.where(row0, yb[0, b, pl.ds(512, 8), :], yi[0:8]), yi[8:]], axis=0)
                u2 = jnp.concatenate([jnp.where(row0, -yb[1, b, pl.ds(512, 8), :], yr[0:8]), yr[8:]], axis=0)
                tr = dot_nt(m[:128], yr.astype(bf16)) + dot_nt(m[128:], yi.astype(bf16))
                ti = dot_nt(m[:128], v2.astype(bf16)) - dot_nt(m[128:], u2.astype(bf16))
            else:
                pa, pb = dot_nt(m, yr.astype(bf16)), dot_nt(m, yi.astype(bf16))
                tr = pa[:128] + pb[128:]
                ti = pb[:128] - pa[128:]
            xd[2 * g, pl.ds(XP * b, 128), :] = tr
            xd[2 * g + 1, pl.ds(XP * b, 128), :] = ti
    for t in range(16):
        z = []
        for g in range(4):
            zz = jnp.concatenate(
                [jnp.concatenate([xd[2 * g + h, pl.ds(8 * t + u, 16, stride=XP), :] for u in range(8)], axis=0)
                 for h in range(2)], axis=1).astype(bf16)
            z += [dot(zz, as_bf16(gi[g, 0])), dot(zz, as_bf16(gi[g, 1]))]
        y = _inv8(z)
        for j in range(8):
            xb32[j, pl.ds(64 * t, 64), :] = pltpu.bitcast(y[j].astype(bf16), u32)

    batch_unit(5, None)
    c_out = [start(xb.at[j], out_hbm.at[:, pl.ds(D + 128 * j, 128)], 18) for j in range(8)]
    wait_all(c_x)
    wait_all(c_wo)

    wo32 = wo.bitcast(u32)
    scale = E ** -0.5

    def step(s, mem):
        top = jnp.concatenate([mem, xbuf[s, pl.ds(M, M), :].astype(f32)], axis=0).astype(bf16)
        lhs = jnp.concatenate([top, xbuf[s, pl.ds(2 * M, 2 * M), :]], axis=0)
        r8 = pl.multiple_of(M * s, M)
        fill = fill_ref[...]
        heads = [None] * H

        def proj(i, p):
            a = dot(lhs, wqkv(i, p, 0))
            b = dot(lhs, wqkv(i, p, 1))
            return jnp.concatenate([a.astype(bf16), b.astype(bf16), as_bf16(pre[i, p, pl.ds(r8, M), :])], axis=0)

        def probs(q, k):
            sc = dot_nt(q, k) * scale
            sc = jnp.where(fill == 0.0, sc, fill)
            e = jnp.exp(sc - jnp.max(sc, axis=1, keepdims=True))
            return (e * (1.0 / jnp.sum(e, axis=1, keepdims=True))).astype(bf16)

        def pv(p, pr, v):
            o = dot(pr, v)
            heads[2 * p] = o[0:32].astype(bf16)
            heads[2 * p + 1] = o[32:64].astype(bf16)
            odef[2 * p, pl.ds(r8, M), :] = o[64:72].astype(bf16)
            odef[2 * p + 1, pl.ds(r8, M), :] = o[72:80].astype(bf16)

        pend = []
        for g in range(8):
            ps = (2 * g, 2 * g + 1)
            qk = [(proj(0, p), proj(1, p)) for p in ps]
            vs = [proj(2, p) for p in ps]
            new = [(p, probs(*qk[t]), vs[t]) for t, p in enumerate(ps)]
            for a in pend:
                pv(*a)
            pend = new

        def wo_part(j, h0, h1):
            oc = jnp.concatenate(heads[h0:h1], axis=1)
            return dot(oc, as_bf16(wo32[j, pl.ds(64 * h0, 64 * (h1 - h0)), :]))

        acc = []
        for j in range(8):
            acc.append(wo_part(j, 0, 24))
            if j == 3:
                for a in pend:
                    pv(*a)
        nxt = []
        for j in range(8):
            r = wo_part(j, 24, 32) + acc[j]
            outbuf[s, pl.ds(M, SEG - M), pl.ds(128 * j, 128)] = r[M:].astype(bf16)
            nxt.append(r[0:M])
        return jnp.concatenate(nxt, axis=1)
    lax.fori_loop(0, NSEG, step, xbuf[0, pl.ds(0, M), :].astype(f32))
    c_out.append(start(outbuf.at[:, pl.ds(M, SEG - M), :], out3.at[:, pl.ds(M, SEG - M), pl.ds(0, D)], 19))

    for t in range(4):
        lhs = jnp.concatenate([odef[h, pl.ds(128 * t, 128), :] for h in range(H)], axis=1)
        for j in range(8):
            r = dot(lhs, as_bf16(wo32[j]))
            outbuf[pl.ds(16 * t, 16), pl.ds(0, M), pl.ds(128 * j, 128)] = r.reshape(16, M, 128).astype(bf16)
        c_out.append(start(outbuf.at[pl.ds(16 * t, 16), pl.ds(0, M), :],
                           out3.at[pl.ds(16 * t, 16), pl.ds(0, M), pl.ds(0, D)], 20 + t))
    wait_all(c_out)


@functools.partial(jax.jit, static_argnames=("A_seg_len",))
def pallas_concat_heads__memory_aug_recurrent_mem_tr__spectral_gfnet__prompt_kernel(
    A_x: jax.Array,
    A_mem0: jax.Array,
    A_Wq: jax.Array,
    A_Wk: jax.Array,
    A_Wv: jax.Array,
    A_Wo: jax.Array,
    A_seg_len,
    B_x: jax.Array,
    B_w_r: jax.Array,
    B_w_i: jax.Array,
):
    assert A_seg_len == SEG
    assert A_x.shape == (1, S, D) and A_mem0.shape == (1, M, D) and B_x.shape == (1, S, D)
    assert A_Wq.shape == (D, H, E) and A_Wo.shape == (H, E, D) and B_w_r.shape == (S, D // 2 + 1)
    gf, gi, mt = _dft_constants()
    fill = _attn_fill()
    hbm = pl.BlockSpec(memory_space=pltpu.HBM)
    wshape = (D // 2, 2, 2, 16, E)
    out = pl.pallas_call(
        _kernel,
        out_shape=jax.ShapeDtypeStruct((S, 2 * D), bf16),
        in_specs=[hbm] * 13,
        out_specs=hbm,
        scratch_shapes=[
            pltpu.VMEM((NRAW, D // 2, 2, 16, E), bf16),
            *[pltpu.VMEM((16 * WP, E), u32)] * 6,
            pltpu.VMEM((8, H * E, 128), bf16),
            pltpu.VMEM((NSEG, SEG, D), bf16),
            pltpu.VMEM((NSEG, M, D), bf16),
            pltpu.VMEM((8, NSEG * M // 2, 128), u32),
            pltpu.VMEM((3, 16, NSEG * M, E), u32),
            pltpu.VMEM((H, NSEG * M, E), bf16),
            pltpu.VMEM((NSEG, SEG, D), bf16),
            pltpu.VMEM(fill.shape, f32),
            pltpu.VMEM((8, S, 128), bf16),
            pltpu.VMEM((2, 16, 512, 128), bf16),
            pltpu.VMEM((2, 1, S), bf16),
            pltpu.VMEM(gf.shape, u32),
            pltpu.VMEM(gi.shape, u32),
            pltpu.VMEM(mt.shape, u32),
            pltpu.VMEM((8, 16 * XP, 128), f32),
            pltpu.VMEM((2, 16, YR, 128), f32),
            pltpu.SemaphoreType.DMA((24,)),
        ],
        compiler_params=pltpu.CompilerParams(vmem_limit_bytes=120 * 1024 * 1024),
    )(A_x.reshape(NSEG, SEG, D), A_mem0.reshape(M, D),
      A_Wq.reshape(wshape), A_Wk.reshape(wshape), A_Wv.reshape(wshape),
      A_Wo.reshape(H * E, D), B_x.reshape(S, D), B_w_r.T, B_w_i.T, gf, gi, mt, fill)
    return out.reshape(1, S, 2 * D)
```

```python
import functools

import jax
import jax.numpy as jnp
import numpy as np
from jax import lax
from jax.experimental import pallas as pl
from jax.experimental.pallas import tpu as pltpu

S, D, H, E, M, SEG = 2048, 1024, 32, 128, 8, 32
NSEG = S // SEG
WP = 516
XP = 132
YR = 520
NRAW = 4
BM = 128
B1_SPLIT = 10
UNROLL = 2
EARLY = ((0, 0, 0), (0, 0, 1), (1, 0, 0), (1, 0, 1), (0, 1, 0), (0, 1, 1))
bf16, f32, u32 = jnp.bfloat16, jnp.float32, jnp.uint32
RES = ((0, 4), (2, 6), (1, 7), (3, 5))
RC = float(np.sqrt(0.5))


def _fwd8(x):
    s04, d04 = x[0] + x[4], x[0] - x[4]
    s26, d26 = x[2] + x[6], x[2] - x[6]
    s15, d15 = x[1] + x[5], x[1] - x[5]
    s37, d37 = x[3] + x[7], x[3] - x[7]
    t1, t2 = (d15 - d37) * RC, (d15 + d37) * RC
    return [s04 + s26, s15 + s37, s04 - s26, s15 - s37, d04 + t1, d26 + t2, d04 - t1, d26 - t2]


def _inv8(z):
    e0, o0, e1, o1, r1, i1, r3, i3 = z
    s04, s26, s15, s37 = e0 + e1, e0 - e1, o0 + o1, o0 - o1
    d04, d26 = r1 + r3, i1 + i3
    t1, t2 = (r1 - r3) * RC, (i1 - i3) * RC
    d15, d37 = t1 + t2, t2 - t1
    return [s04 + d04, s15 + d15, s26 + d26, s37 + d37, s04 - d04, s15 - d15, s26 - d26, s37 - d37]


def _twiddle16(z, k):
    re, im = z
    k = k % 16
    if k == 0:
        return z
    if k == 4:
        return (im, -re)
    if k == 12:
        return (-im, re)
    if k == 2:
        return ((re + im) * RC, (im - re) * RC)
    if k == 14:
        return ((re - im) * RC, (re + im) * RC)
    if k == 6:
        return ((im - re) * RC, (re + im) * -RC)
    if k == 10:
        return ((re + im) * -RC, (re - im) * RC)
    c, s = float(np.cos(2 * np.pi * k / 16)), float(-np.sin(2 * np.pi * k / 16))
    return (re * c - im * s, re * s + im * c)


def _bfly4(z, sign):
    (ar, ai), (br, bi), (cr, ci), (dr, di) = z
    sr, si, tr, ti = ar + cr, ai + ci, ar - cr, ai - ci
    ur, ui, vr, vi = br + dr, bi + di, br - dr, bi - di
    o0, o2 = (sr + ur, si + ui), (sr - ur, si - ui)
    p, q = (tr + vi, ti - vr), (tr - vi, ti + vr)
    return [o0, p, o2, q] if sign > 0 else [o0, q, o2, p]


class _Pacer:
    def __init__(self, tasks, ntokens):
        self.slots = {}
        for n, task in enumerate(tasks):
            self.slots.setdefault(n * ntokens // len(tasks), []).append(task)
        self.pos = 0
        self.ntokens = ntokens

    def feed(self, r):
        for j in range(r.shape[0] // 8):
            for task in self.slots.pop(self.pos, []):
                task(pltpu.bitcast(r[8 * j:8 * j + 8], u32))
            self.pos += 1

    def done(self):
        assert not self.slots and self.pos == self.ntokens


def _pack_rows(m):
    b = np.asarray(m, np.float32).astype(jnp.bfloat16).view(np.uint16).astype(np.uint32)
    return b[..., 0::2, :] | (b[..., 1::2, :] << 16)


@functools.lru_cache(maxsize=None)
def _dft_constants():
    b8 = np.array(_fwd8(list(np.eye(8)))).T
    n = np.arange(D)
    fw = np.zeros((D, D))
    bw = np.zeros((D, D))
    for g in range(4):
        k = np.concatenate([8 * np.arange(64) + r for r in RES[g]])
        ang = 2 * np.pi * ((n[:, None] * k[None, :]) % D) / D
        wgt = np.where(k == 0, 1.0, 2.0) / (D * S)
        fw[:, 256 * g:256 * g + 128] = np.cos(ang)
        fw[:, 256 * g + 128:256 * g + 256] = -np.sin(ang)
        bw[256 * g:256 * g + 128] = (np.cos(ang) * wgt).T
        bw[256 * g + 128:256 * g + 256] = (-np.sin(ang) * wgt).T
    bw[128, :] = (-1.0) ** n / (D * S)
    binv = np.kron(np.linalg.inv(b8), np.eye(128))
    gall = binv @ fw
    giall = bw @ binv.T
    gf = np.zeros((4, 272, 256))
    gi = np.zeros((4, 256, 256))
    for g in range(4):
        sl = slice(256 * g, 256 * g + 256)
        gf[g, :256] = gall[sl, sl].T
        gi[g] = giall[sl, sl]
    gf[0, 256] = (-1.0) ** np.arange(256)
    split = lambda m: np.stack([m[..., :128], m[..., 128:]], axis=1)
    a = np.arange(128)
    mt = np.zeros((16, 256, 128))
    for b in range(16):
        ang = 2 * np.pi * (((16 * a[:, None] + b) * a[None, :]) % S) / S
        mt[b, :128], mt[b, 128:] = np.cos(ang), -np.sin(ang)
    return _pack_rows(split(gf)), _pack_rows(split(gi)), _pack_rows(mt)


def _attn_fill():
    head = np.concatenate([np.zeros(32), np.ones(32), np.zeros(8), np.ones(8)]).astype(int)
    pos32 = np.concatenate([np.arange(8), np.arange(16, 40)])
    pos = np.concatenate([pos32, pos32, np.arange(8, 16), np.arange(8, 16)])
    ok = (pos[:, None] < M) | (pos[:, None] >= pos[None, :])
    fill = np.where(ok, 0.0, -1e9)
    fill = np.where(head[:, None] == head[None, :], fill, -np.inf)
    return fill.astype(np.float32)


def _kernel(x_hbm, mem_hbm, wq_hbm, wk_hbm, wv_hbm, wo_hbm, bx_hbm, wr_hbm, wi_hbm,
            gf_hbm, gi_hbm, mt_hbm, fill_hbm, out_hbm,
            wraw, w0, w1, w2, w3, w4, w5, wo, xbuf, x8, x8c, pre, odef, outbuf, fill_ref,
            xb, wt, wl, gf, gi, mt, xd, yb, sems):
    def start(src, dst, i):
        c = pltpu.make_async_copy(src, dst, sems.at[i])
        c.start()
        return c

    def wait_all(cs):
        for c in cs:
            c.wait()

    dot = functools.partial(jnp.dot, preferred_element_type=f32)
    dot_nt = lambda a, b: lax.dot_general(a, b, (((1,), (1,)), ((), ())), preferred_element_type=f32)
    as_bf16 = lambda w: pltpu.bitcast(w, bf16)
    lo_f32 = lambda w: pltpu.bitcast(w << 16, f32)
    hi_f32 = lambda w: pltpu.bitcast(w & u32(0xFFFF0000), f32)
    out3 = out_hbm.reshape(NSEG, SEG, 2 * D)
    w_hbm = (wq_hbm, wk_hbm, wv_hbm)
    w32 = (w0, w1, w2, w3, w4, w5)

    def start_unit(u):
        return start(w_hbm[u // 2].at[:, :, u % 2], wraw.at[u % NRAW], 4 + u)

    c_b1 = [start(bx_hbm.at[:, pl.ds(128 * j, 128)], xb.at[j], 0) for j in range(8)]
    c_b1 += [start(gf_hbm, gf, 1), start(mt_hbm, mt, 2)]
    c_x8 = start(x_hbm.at[:, pl.ds(0, M), :], x8, 3)
    c_w = [start_unit(u) for u in range(3)]
    c_flt = []
    for t, w in enumerate((wr_hbm, wi_hbm)):
        for d in range(16):
            c_flt.append(start(w.at[pl.ds(0, 512), pl.ds(128 * d, 128)], wt.at[t, d], 10))
        c_flt.append(start(w.at[pl.ds(512, 1), :], wl.at[t], 11 + t))
    c_w.append(start_unit(3))

    wraw32 = wraw.bitcast(u32)
    wt32 = wt.bitcast(u32)

    def relayout_tasks(u):
        def make(r0):
            def task(tok):
                lo = (tok >> 16) | u32(0xFFFF)
                hi = (tok << 16) | u32(0xFFFF0000)
                for r in range(r0, r0 + 2):
                    a, b = wraw32[u % NRAW, r, 0], wraw32[u % NRAW, r, 1]
                    w32[u][pl.ds(r, 8, stride=WP), :] = (a & lo) | (b << 16)
                    w32[u][pl.ds(r + 8 * WP, 8, stride=WP), :] = (a >> 16) | (b & hi)
            return task
        return [make(r0) for r0 in range(0, D // 2, 2)]

    def filter_tasks(rows, wfn):
        def make(phase, k):
            slots = [4 * k + j for j in range(4)] if phase == 1 else [4 * j + k for j in range(4)]

            def task(tok):
                ones = ((tok >> 16) | u32(0xFFFF)) | u32(0xFFFF0000)
                z = [(yb[0, b, rows, :], yb[1, b, rows, :]) for b in slots]
                z[0] = tuple(pltpu.bitcast(pltpu.bitcast(v, u32) & ones, f32) for v in z[0])
                if phase == 0:
                    o = _bfly4(z, 1)
                    o = [_twiddle16(o[j], k * j) for j in range(4)]
                elif phase == 1:
                    o = _bfly4(z, 1)
                    y = []
                    for j in range(4):
                        wr, wi = wfn(k + 4 * j)
                        xr, xi = o[j]
                        y.append((xr * wr - xi * wi, xr * wi + xi * wr))
                    o = _bfly4(y, -1)
                    o = [_twiddle16(o[j], -k * j) for j in range(4)]
                else:
                    o = _bfly4(z, -1)
                for b, v in zip(slots, o):
                    yb[0, b, rows, :] = v[0]
                    yb[1, b, rows, :] = v[1]
            return task
        return [make(phase, k) for phase in range(3) for k in range(4)]

    def all_filter_tasks():
        tasks = []
        for i in range(8):
            for g in range(4):
                for q in range(2):
                    r = RES[g][q]
                    un = lo_f32 if r % 2 == 0 else hi_f32
                    wrows = pl.ds(32 * i + r // 2, 8, stride=4)
                    tasks += filter_tasks(pl.ds(128 * g + 64 * q + 8 * i, 8),
                                          lambda d, un=un, wrows=wrows: [un(wt32[t, d, wrows, :]) for t in range(2)])
        tasks += filter_tasks(pl.ds(512, 8), lambda d: [wl[t, :, pl.ds(128 * d, 128)].astype(f32) for t in range(2)])
        return tasks

    def merge(a, b):
        keyed = [(n / len(a), 0, n) for n in range(len(a))] + [(n / len(b), 1, n) for n in range(len(b))]
        return [(a, b)[w][n] for _, w, n in sorted(keyed)]

    xb32 = xb.bitcast(u32)

    def b_dfwd(b):
        un = lo_f32 if b % 2 == 0 else hi_f32
        z = _fwd8([un(xb32[j, pl.ds(b // 2, 128, stride=8), :]) for j in range(8)])
        ts = []
        for g in range(4):
            rows = 136 if g == 0 else 128
            t = (dot_nt(as_bf16(gf[g, 0, 0:rows]), z[2 * g].astype(bf16))
                 + dot_nt(as_bf16(gf[g, 1, 0:rows]), z[2 * g + 1].astype(bf16)))
            ts.append(t.astype(bf16))
        return ts

    def b_sfwd(b, ts, pacer=None):
        mr, mi = as_bf16(mt[b, 0:64]), as_bf16(mt[b, 64:128])
        for g in range(4):
            pa, pb = dot(ts[g], mr), dot(ts[g], mi)
            yb[0, b, pl.ds(128 * g, 128), :] = pa[0:128] - pb[128:256]
            yb[1, b, pl.ds(128 * g, 128), :] = pb[0:128] + pa[128:256]
            if g == 0:
                yb[0, b, pl.ds(512, 8), :] = pa[256:264]
                yb[1, b, pl.ds(512, 8), :] = pb[256:264]
            if pacer is not None:
                pacer.feed(pa[0:256])

    def b_stage1(b0, b1, pacer=None):
        prev = None
        for b in range(b0, b1):
            ts = b_dfwd(b)
            if prev is not None:
                b_sfwd(b - 1, prev, pacer)
            prev = ts
        b_sfwd(b1 - 1, prev, None)

    wait_all(c_b1)
    b_stage1(0, B1_SPLIT)
    c_x8.wait()
    c_w[0].wait()
    x8v = x8[...].reshape(NSEG * M, D)
    for k in range(8):
        x8c[k] = pltpu.bitcast(x8v[:, 128 * k:128 * k + 128], u32)
    pacer = _Pacer(relayout_tasks(0), (15 - B1_SPLIT) * 128)
    b_stage1(B1_SPLIT, 16, pacer)
    pacer.done()

    def gated(w, toks):
        if not toks:
            return w
        bits = functools.reduce(
            jnp.bitwise_or, [pltpu.bitcast(jnp.broadcast_to(t, (8, 128)), u32) for t in toks])
        ones = ((bits >> 16) | u32(0xFFFF)) | u32(0xFFFF0000)
        return jnp.concatenate([w[0:8] & ones, w[8:]], axis=0)

    def wqkv(i, p, second, toks=(), k0=0, k1=D):
        rows = pl.ds((p % 8 + 8 * second) * WP + k0 // 2, (k1 - k0) // 2)
        return as_bf16(gated(w32[2 * i + p // 8][rows, :], toks))

    def batch_unit(u, tasks):
        pacer = _Pacer(tasks, 7 * 128 + 64) if tasks else None
        for p in range(8 * (u % 2), 8 * (u % 2) + 8):
            for c in range(NSEG * M // BM):
                lhs = jnp.concatenate([as_bf16(x8c[k, pl.ds(c * BM // 2, BM // 2), :]) for k in range(8)], axis=1)
                r1 = dot(lhs, wqkv(u // 2, p, 0))
                r2 = dot(lhs, wqkv(u // 2, p, 1))
                st = jnp.concatenate([r1.reshape(BM // M, M, E), r2.reshape(BM // M, M, E)], axis=1)
                pre[u // 2, p, pl.ds(c * BM, BM), :] = pltpu.bitcast(st.reshape(2 * BM, E).astype(bf16), u32)
                if pacer is not None and pacer.pos < pacer.ntokens:
                    pacer.feed(r1)
                    pacer.feed(r2)
        if pacer is not None:
            pacer.done()

    c_w[1].wait()
    c_w.append(start_unit(4))
    batch_unit(0, relayout_tasks(1))
    c_w[2].wait()
    c_w.append(start_unit(5))
    c_gi = start(gi_hbm, gi, 13)
    c_x = [start(x_hbm.at[:, pl.ds(M, SEG - M), :], xbuf.at[:, pl.ds(M, SEG - M), :], 14),
           start(mem_hbm, xbuf.at[0, pl.ds(0, M), :], 15), start(fill_hbm, fill_ref, 16)]
    c_wo = [start(wo_hbm.at[:, pl.ds(128 * j, 128)], wo.at[j], 17) for j in range(8)]
    batch_unit(1, relayout_tasks(2))
    c_w[3].wait()
    wait_all(c_flt)
    flt = all_filter_tasks()
    third = 12 * 22
    batch_unit(2, merge(relayout_tasks(3), flt[:third]))
    c_w[4].wait()
    c_w[5].wait()
    c_gi.wait()
    batch_unit(3, merge(relayout_tasks(4), flt[third:2 * third]))
    batch_unit(4, merge(relayout_tasks(5), flt[2 * third:]))

    row0 = lax.broadcasted_iota(jnp.int32, (8, 128), 0) == 0
    for b in range(16):
        m = as_bf16(mt[b])
        for g in range(4):
            yr, yi = yb[0, b, pl.ds(128 * g, 128), :], yb[1, b, pl.ds(128 * g, 128), :]
            if g == 0:
                v2 = jnp.concatenate([jnp.where(row0, yb[0, b, pl.ds(512, 8), :], yi[0:8]), yi[8:]], axis=0)
                u2 = jnp.concatenate([jnp.where(row0, -yb[1, b, pl.ds(512, 8), :], yr[0:8]), yr[8:]], axis=0)
                tr = dot_nt(m[:128], yr.astype(bf16)) + dot_nt(m[128:], yi.astype(bf16))
                ti = dot_nt(m[:128], v2.astype(bf16)) - dot_nt(m[128:], u2.astype(bf16))
            else:
                pa, pb = dot_nt(m, yr.astype(bf16)), dot_nt(m, yi.astype(bf16))
                tr = pa[:128] + pb[128:]
                ti = pb[:128] - pa[128:]
            xd[2 * g, pl.ds(XP * b, 128), :] = tr
            xd[2 * g + 1, pl.ds(XP * b, 128), :] = ti
    for t in range(16):
        z = []
        for g in range(4):
            zz = jnp.concatenate(
                [jnp.concatenate([xd[2 * g + h, pl.ds(8 * t + u, 16, stride=XP), :] for u in range(8)], axis=0)
                 for h in range(2)], axis=1).astype(bf16)
            z += [dot(zz, as_bf16(gi[g, 0])), dot(zz, as_bf16(gi[g, 1]))]
        y = _inv8(z)
        for j in range(8):
            xb32[j, pl.ds(64 * t, 64), :] = pltpu.bitcast(y[j].astype(bf16), u32)

    batch_unit(5, None)
    c_out = [start(xb.at[j], out_hbm.at[:, pl.ds(D + 128 * j, 128)], 18) for j in range(8)]
    wait_all(c_x)
    wait_all(c_wo)

    wo32 = wo.bitcast(u32)
    scale = E ** -0.5

    def step(s, mem, early):
        rows = jnp.concatenate([mem, xbuf[s, pl.ds(M, SEG - M), :].astype(f32)], axis=0)
        lhs = rows.astype(bf16)
        head_start = {}
        if early:
            lo, hi = rows[:, :D // 2].astype(bf16), rows[:, D // 2:].astype(bf16)
            for key in early:
                head_start[key] = dot(lo, wqkv(*key, k1=D // 2))
        r8 = pl.multiple_of(M * s, M)
        fill = fill_ref[...]
        heads = [None] * H
        rs = []

        def proj(i, p, toks=()):
            a, b = [
                dot(hi, wqkv(i, p, t, k0=D // 2)) + head_start[i, p, t] if (i, p, t) in head_start
                else dot(lhs, wqkv(i, p, t, toks[t * len(toks) // 2:(t + 1) * len(toks) // 2]))
                for t in range(2)]
            c = as_bf16(pre[i, p, pl.ds(r8, M), :]).astype(f32)
            return jnp.concatenate([a, b, c], axis=0).astype(bf16)

        def probs(q, k):
            sc = dot_nt(q, k) * scale
            sc = jnp.where(fill == 0.0, sc, fill)
            e = jnp.exp(sc - jnp.max(sc, axis=1, keepdims=True))
            l = jnp.sum(e, axis=1, keepdims=True)
            r = pl.reciprocal(l, approx=True)
            r = r * (2.0 - l * r)
            rs.append([r[8 * n:8 * n + 8] for n in range(10)])
            return (e * r).astype(bf16)

        def pv(p, pr, v):
            o = dot(pr, v)
            heads[2 * p] = o[0:32]
            heads[2 * p + 1] = o[32:64]
            odef[2 * p, pl.ds(r8, M), :] = o[64:72].astype(bf16)
            odef[2 * p + 1, pl.ds(r8, M), :] = o[72:80].astype(bf16)

        pend = []
        for g in range(4):
            ps = range(4 * g, 4 * g + 4)
            qk = [(proj(0, p), proj(1, p)) for p in ps]
            vs = [proj(2, p, rs[p - 4] if g else ()) for p in ps]
            for a in pend:
                pv(*a)
            pend = [(p, probs(*qk[t]), vs[t]) for t, p in enumerate(ps)]

        def wo_part(oc, j, h0, h1, toks=()):
            return dot(oc, as_bf16(gated(wo32[j, pl.ds(64 * h0, 64 * (h1 - h0)), :], toks)))

        acc = []
        oc = jnp.concatenate(heads[0:24], axis=1).astype(bf16)
        for j in range(8):
            acc.append(wo_part(oc, j, 0, 24, {3: rs[12] + rs[13], 4: rs[14] + rs[15]}.get(j, ())))
            if j == 4:
                for a in pend:
                    pv(*a)
        oc = jnp.concatenate(heads[24:32], axis=1).astype(bf16)
        nxt = []
        for j in range(8):
            r = wo_part(oc, j, 24, 32) + acc[j]
            outbuf[s, pl.ds(M, SEG - M), pl.ds(128 * j, 128)] = r[M:].astype(bf16)
            nxt.append(r[0:M])
        return jnp.concatenate(nxt, axis=1)

    def steps(n, mem):
        for u in range(UNROLL):
            mem = step(UNROLL * n + u, mem, EARLY if u else ())
        return mem
    lax.fori_loop(0, NSEG // UNROLL, steps, xbuf[0, pl.ds(0, M), :].astype(f32))
    c_out.append(start(outbuf.at[:, pl.ds(M, SEG - M), :], out3.at[:, pl.ds(M, SEG - M), pl.ds(0, D)], 19))

    for t in range(4):
        lhs = jnp.concatenate([odef[h, pl.ds(128 * t, 128), :] for h in range(H)], axis=1)
        for j in range(8):
            r = dot(lhs, as_bf16(wo32[j]))
            outbuf[pl.ds(16 * t, 16), pl.ds(0, M), pl.ds(128 * j, 128)] = r.reshape(16, M, 128).astype(bf16)
        c_out.append(start(outbuf.at[pl.ds(16 * t, 16), pl.ds(0, M), :],
                           out3.at[pl.ds(16 * t, 16), pl.ds(0, M), pl.ds(0, D)], 20 + t))
    wait_all(c_out)


@functools.partial(jax.jit, static_argnames=("A_seg_len",))
def pallas_concat_heads__memory_aug_recurrent_mem_tr__spectral_gfnet__prompt_kernel(
    A_x: jax.Array,
    A_mem0: jax.Array,
    A_Wq: jax.Array,
    A_Wk: jax.Array,
    A_Wv: jax.Array,
    A_Wo: jax.Array,
    A_seg_len,
    B_x: jax.Array,
    B_w_r: jax.Array,
    B_w_i: jax.Array,
):
    assert A_seg_len == SEG
    assert A_x.shape == (1, S, D) and A_mem0.shape == (1, M, D) and B_x.shape == (1, S, D)
    assert A_Wq.shape == (D, H, E) and A_Wo.shape == (H, E, D) and B_w_r.shape == (S, D // 2 + 1)
    gf, gi, mt = _dft_constants()
    fill = _attn_fill()
    hbm = pl.BlockSpec(memory_space=pltpu.HBM)
    wshape = (D // 2, 2, 2, 16, E)
    out = pl.pallas_call(
        _kernel,
        out_shape=jax.ShapeDtypeStruct((S, 2 * D), bf16),
        in_specs=[hbm] * 13,
        out_specs=hbm,
        scratch_shapes=[
            pltpu.VMEM((NRAW, D // 2, 2, 16, E), bf16),
            *[pltpu.VMEM((16 * WP, E), u32)] * 6,
            pltpu.VMEM((8, H * E, 128), bf16),
            pltpu.VMEM((NSEG, SEG, D), bf16),
            pltpu.VMEM((NSEG, M, D), bf16),
            pltpu.VMEM((8, NSEG * M // 2, 128), u32),
            pltpu.VMEM((3, 16, NSEG * M, E), u32),
            pltpu.VMEM((H, NSEG * M, E), bf16),
            pltpu.VMEM((NSEG, SEG, D), bf16),
            pltpu.VMEM(fill.shape, f32),
            pltpu.VMEM((8, S, 128), bf16),
            pltpu.VMEM((2, 16, 512, 128), bf16),
            pltpu.VMEM((2, 1, S), bf16),
            pltpu.VMEM(gf.shape, u32),
            pltpu.VMEM(gi.shape, u32),
            pltpu.VMEM(mt.shape, u32),
            pltpu.VMEM((8, 16 * XP, 128), f32),
            pltpu.VMEM((2, 16, YR, 128), f32),
            pltpu.SemaphoreType.DMA((24,)),
        ],
        compiler_params=pltpu.CompilerParams(vmem_limit_bytes=120 * 1024 * 1024),
    )(A_x.reshape(NSEG, SEG, D), A_mem0.reshape(M, D),
      A_Wq.reshape(wshape), A_Wk.reshape(wshape), A_Wv.reshape(wshape),
      A_Wo.reshape(H * E, D), B_x.reshape(S, D), B_w_r.T, B_w_i.T, gf, gi, mt, fill)
    return out.reshape(1, S, 2 * D)
```

```python
import functools

import jax
import jax.numpy as jnp
import numpy as np
from jax import lax
from jax.experimental import pallas as pl
from jax.experimental.pallas import tpu as pltpu

S, D, H, E, M, SEG = 2048, 1024, 32, 128, 8, 32
NSEG = S // SEG
WP = 516
XP = 132
YR = 520
NRAW = 4
BM = 128
UNROLL = 4
EARLY = ((0, 0, 0), (0, 0, 1), (1, 0, 0), (1, 0, 1), (0, 1, 0), (0, 1, 1))
bf16, f32, u32 = jnp.bfloat16, jnp.float32, jnp.uint32
RES = ((0, 4), (2, 6), (1, 7), (3, 5))
RC = float(np.sqrt(0.5))


def _fwd8(x):
    s04, d04 = x[0] + x[4], x[0] - x[4]
    s26, d26 = x[2] + x[6], x[2] - x[6]
    s15, d15 = x[1] + x[5], x[1] - x[5]
    s37, d37 = x[3] + x[7], x[3] - x[7]
    t1, t2 = (d15 - d37) * RC, (d15 + d37) * RC
    return [s04 + s26, s15 + s37, s04 - s26, s15 - s37, d04 + t1, d26 + t2, d04 - t1, d26 - t2]


def _inv8(z):
    e0, o0, e1, o1, r1, i1, r3, i3 = z
    s04, s26, s15, s37 = e0 + e1, e0 - e1, o0 + o1, o0 - o1
    d04, d26 = r1 + r3, i1 + i3
    t1, t2 = (r1 - r3) * RC, (i1 - i3) * RC
    d15, d37 = t1 + t2, t2 - t1
    return [s04 + d04, s15 + d15, s26 + d26, s37 + d37, s04 - d04, s15 - d15, s26 - d26, s37 - d37]


def _twiddle16(z, k):
    re, im = z
    k = k % 16
    if k == 0:
        return z
    if k == 4:
        return (im, -re)
    if k == 12:
        return (-im, re)
    if k == 2:
        return ((re + im) * RC, (im - re) * RC)
    if k == 14:
        return ((re - im) * RC, (re + im) * RC)
    if k == 6:
        return ((im - re) * RC, (re + im) * -RC)
    if k == 10:
        return ((re + im) * -RC, (re - im) * RC)
    c, s = float(np.cos(2 * np.pi * k / 16)), float(-np.sin(2 * np.pi * k / 16))
    return (re * c - im * s, re * s + im * c)


def _bfly4(z, sign):
    (ar, ai), (br, bi), (cr, ci), (dr, di) = z
    sr, si, tr, ti = ar + cr, ai + ci, ar - cr, ai - ci
    ur, ui, vr, vi = br + dr, bi + di, br - dr, bi - di
    o0, o2 = (sr + ur, si + ui), (sr - ur, si - ui)
    p, q = (tr + vi, ti - vr), (tr - vi, ti + vr)
    return [o0, p, o2, q] if sign > 0 else [o0, q, o2, p]


class _Pacer:
    def __init__(self, tasks, ntokens):
        self.slots = {}
        for n, task in enumerate(tasks):
            self.slots.setdefault(n * ntokens // len(tasks), []).append(task)
        self.pos = 0
        self.ntokens = ntokens

    def feed(self, r):
        for j in range(r.shape[0] // 8):
            for task in self.slots.pop(self.pos, []):
                task(pltpu.bitcast(r[8 * j:8 * j + 8], u32))
            self.pos += 1

    def done(self):
        assert not self.slots and self.pos == self.ntokens


def _pack_rows(m):
    b = np.asarray(m, np.float32).astype(jnp.bfloat16).view(np.uint16).astype(np.uint32)
    return b[..., 0::2, :] | (b[..., 1::2, :] << 16)


@functools.lru_cache(maxsize=None)
def _dft_constants():
    b8 = np.array(_fwd8(list(np.eye(8)))).T
    n = np.arange(D)
    fw = np.zeros((D, D))
    bw = np.zeros((D, D))
    for g in range(4):
        k = np.concatenate([8 * np.arange(64) + r for r in RES[g]])
        ang = 2 * np.pi * ((n[:, None] * k[None, :]) % D) / D
        wgt = np.where(k == 0, 1.0, 2.0) / (D * S)
        fw[:, 256 * g:256 * g + 128] = np.cos(ang)
        fw[:, 256 * g + 128:256 * g + 256] = -np.sin(ang)
        bw[256 * g:256 * g + 128] = (np.cos(ang) * wgt).T
        bw[256 * g + 128:256 * g + 256] = (-np.sin(ang) * wgt).T
    bw[128, :] = (-1.0) ** n / (D * S)
    binv = np.kron(np.linalg.inv(b8), np.eye(128))
    gall = binv @ fw
    giall = bw @ binv.T
    gf = np.zeros((4, 272, 256))
    gi = np.zeros((4, 256, 256))
    for g in range(4):
        sl = slice(256 * g, 256 * g + 256)
        gf[g, :256] = gall[sl, sl].T
        gi[g] = giall[sl, sl]
    gf[0, 256] = (-1.0) ** np.arange(256)
    split = lambda m: np.stack([m[..., :128], m[..., 128:]], axis=1)
    a = np.arange(128)
    mt = np.zeros((16, 256, 128))
    for b in range(16):
        ang = 2 * np.pi * (((16 * a[:, None] + b) * a[None, :]) % S) / S
        mt[b, :128], mt[b, 128:] = np.cos(ang), -np.sin(ang)
    return _pack_rows(split(gf)), _pack_rows(split(gi)), _pack_rows(mt)


def _attn_fill():
    head = np.concatenate([np.zeros(32), np.ones(32), np.zeros(8), np.ones(8)]).astype(int)
    pos32 = np.concatenate([np.arange(8), np.arange(16, 40)])
    pos = np.concatenate([pos32, pos32, np.arange(8, 16), np.arange(8, 16)])
    ok = (pos[:, None] < M) | (pos[:, None] >= pos[None, :])
    fill = np.where(ok, 0.0, -1e9)
    fill = np.where(head[:, None] == head[None, :], fill, -np.inf)
    return fill.astype(np.float32)


def _kernel(x_hbm, mem_hbm, wq_hbm, wk_hbm, wv_hbm, wo_hbm, bx_hbm, wr_hbm, wi_hbm,
            gf_hbm, gi_hbm, mt_hbm, fill_hbm, out_hbm,
            wraw, w0, w1, w2, w3, w4, w5, wo, xbuf, x8, x8c, pre, odef, outbuf, fill_ref,
            xb, wt, wl, gf, gi, mt, xd, yb, sems):
    def start(src, dst, i):
        c = pltpu.make_async_copy(src, dst, sems.at[i])
        c.start()
        return c

    def wait_all(cs):
        for c in cs:
            c.wait()

    dot = functools.partial(jnp.dot, preferred_element_type=f32)
    dot_nt = lambda a, b: lax.dot_general(a, b, (((1,), (1,)), ((), ())), preferred_element_type=f32)
    as_bf16 = lambda w: pltpu.bitcast(w, bf16)
    lo_f32 = lambda w: pltpu.bitcast(w << 16, f32)
    hi_f32 = lambda w: pltpu.bitcast(w & u32(0xFFFF0000), f32)
    out3 = out_hbm.reshape(NSEG, SEG, 2 * D)
    w_hbm = (wq_hbm, wk_hbm, wv_hbm)
    w32 = (w0, w1, w2, w3, w4, w5)

    def start_unit(u):
        return start(w_hbm[u // 2].at[:, :, u % 2], wraw.at[u % NRAW], 4 + u)

    c_a = []
    for n in range(4):
        cols, rows = pl.ds(256 * n, 256), pl.ds(128 * n, 128)
        c_a.append([start(x_hbm.at[:, pl.ds(0, M), cols], x8.at[:, :, cols], 24 + n),
                    start(wq_hbm.at[rows, :, 0], wraw.at[0, rows], 28 + n)])

    wraw32 = wraw.bitcast(u32)
    wt32 = wt.bitcast(u32)

    def relayout_row(u, dst, r, off, lo, hi):
        a, b = wraw32[u % NRAW, r, 0], wraw32[u % NRAW, r, 1]
        dst[pl.ds(off, 8, stride=WP), :] = (a & lo) | (b << 16)
        dst[pl.ds(off + 8 * WP, 8, stride=WP), :] = (a >> 16) | (b & hi)

    def relayout_tasks(u, r0=0, r1=D // 2):
        def make(r):
            def task(tok):
                lo = (tok >> 16) | u32(0xFFFF)
                hi = (tok << 16) | u32(0xFFFF0000)
                relayout_row(u, w32[u], r, r, lo, hi)
                relayout_row(u, w32[u], r + 1, r + 1, lo, hi)
            return task
        return [make(r) for r in range(r0, r1, 2)]

    def filter_tasks(rows, wfn):
        def make(phase, k):
            slots = [4 * k + j for j in range(4)] if phase == 1 else [4 * j + k for j in range(4)]

            def task(tok):
                ones = ((tok >> 16) | u32(0xFFFF)) | u32(0xFFFF0000)
                z = [(yb[0, b, rows, :], yb[1, b, rows, :]) for b in slots]
                z[0] = tuple(pltpu.bitcast(pltpu.bitcast(v, u32) & ones, f32) for v in z[0])
                if phase == 0:
                    o = _bfly4(z, 1)
                    o = [_twiddle16(o[j], k * j) for j in range(4)]
                elif phase == 1:
                    o = _bfly4(z, 1)
                    y = []
                    for j in range(4):
                        wr, wi = wfn(k + 4 * j)
                        xr, xi = o[j]
                        y.append((xr * wr - xi * wi, xr * wi + xi * wr))
                    o = _bfly4(y, -1)
                    o = [_twiddle16(o[j], -k * j) for j in range(4)]
                else:
                    o = _bfly4(z, -1)
                for b, v in zip(slots, o):
                    yb[0, b, rows, :] = v[0]
                    yb[1, b, rows, :] = v[1]
            return task
        return [make(phase, k) for phase in range(3) for k in range(4)]

    def all_filter_tasks():
        tasks = []
        for i in range(8):
            for g in range(4):
                for q in range(2):
                    r = RES[g][q]
                    un = lo_f32 if r % 2 == 0 else hi_f32
                    wrows = pl.ds(32 * i + r // 2, 8, stride=4)
                    tasks += filter_tasks(pl.ds(128 * g + 64 * q + 8 * i, 8),
                                          lambda d, un=un, wrows=wrows: [un(wt32[t, d, wrows, :]) for t in range(2)])
        tasks += filter_tasks(pl.ds(512, 8), lambda d: [wl[t, :, pl.ds(128 * d, 128)].astype(f32) for t in range(2)])
        return tasks

    def merge(a, b):
        keyed = [(n / len(a), 0, n) for n in range(len(a))] + [(n / len(b), 1, n) for n in range(len(b))]
        return [(a, b)[w][n] for _, w, n in sorted(keyed)]

    xb32 = xb.bitcast(u32)

    def b_dfwd(b):
        un = lo_f32 if b % 2 == 0 else hi_f32
        z = _fwd8([un(xb32[j, pl.ds(b // 2, 128, stride=8), :]) for j in range(8)])
        ts = []
        for g in range(4):
            rows = 136 if g == 0 else 128
            t = (dot_nt(as_bf16(gf[g, 0, 0:rows]), z[2 * g].astype(bf16))
                 + dot_nt(as_bf16(gf[g, 1, 0:rows]), z[2 * g + 1].astype(bf16)))
            ts.append(t.astype(bf16))
        return ts

    def b_sfwd(b, ts):
        mr, mi = as_bf16(mt[b, 0:64]), as_bf16(mt[b, 64:128])
        for g in range(4):
            pa, pb = dot(ts[g], mr), dot(ts[g], mi)
            yb[0, b, pl.ds(128 * g, 128), :] = pa[0:128] - pb[128:256]
            yb[1, b, pl.ds(128 * g, 128), :] = pb[0:128] + pa[128:256]
            if g == 0:
                yb[0, b, pl.ds(512, 8), :] = pa[256:264]
                yb[1, b, pl.ds(512, 8), :] = pb[256:264]

    def b_stage1():
        prev = None
        for b in range(16):
            ts = b_dfwd(b)
            if prev is not None:
                b_sfwd(b - 1, prev)
            prev = ts
        b_sfwd(15, prev)

    def gated(w, toks):
        if not toks:
            return w
        bits = functools.reduce(
            jnp.bitwise_or, [pltpu.bitcast(jnp.broadcast_to(t, (8, 128)), u32) for t in toks])
        ones = ((bits >> 16) | u32(0xFFFF)) | u32(0xFFFF0000)
        return jnp.concatenate([w[0:8] & ones, w[8:]], axis=0)

    def wqkv(i, p, second, toks=(), k0=0, k1=D):
        rows = pl.ds((p % 8 + 8 * second) * WP + k0 // 2, (k1 - k0) // 2)
        return as_bf16(gated(w32[2 * i + p // 8][rows, :], toks))

    def batch(n0, n1, tasks=None, k0=0, k1=D):
        pacer = _Pacer(tasks, (n1 - n0 - 1) * BM // 4) if tasks else None
        for n in range(n0, n1):
            i, p, c = n // 64, n % 64 // 4, n % 4
            rows = pl.ds(c * BM, BM)
            lhs = jnp.concatenate([as_bf16(x8c[k, pl.ds(c * BM // 2, BM // 2), :])
                                   for k in range(k0 // 128, k1 // 128)], axis=1)
            rs = [dot(lhs, wqkv(i, p, t, k0=k0, k1=k1)) for t in range(2)]
            if k0 > 0:
                rs = [rs[t] + yb[t, p, rows, :] for t in range(2)]
            if k1 < D:
                for t in range(2):
                    yb[t, p, rows, :] = rs[t]
            else:
                st = jnp.concatenate([r.reshape(BM // M, M, E) for r in rs], axis=1)
                pre[i, p, rows, :] = pltpu.bitcast(st.reshape(2 * BM, E).astype(bf16), u32)
            if pacer is not None and n < n1 - 1:
                pacer.feed(rs[0])
                pacer.feed(rs[1])
        if pacer is not None:
            pacer.done()

    def pack_x8(n):
        x8v = x8[:, :, pl.ds(256 * n, 256)].reshape(NSEG * M, 256)
        for k in range(2):
            x8c[2 * n + k] = pltpu.bitcast(x8v[:, 128 * k:128 * k + 128], u32)

    def relayout_quarter(n):
        def body(t, c):
            off = pl.multiple_of(128 * n + 16 * t, 16)
            for r in range(16):
                relayout_row(0, w0.at[pl.ds(off, 15 * WP + 20)], off + r, r, u32(0xFFFF), u32(0xFFFF0000))
            return c
        lax.fori_loop(0, 8, body, 0)

    c_w = {}
    wait_all(c_a[0])
    relayout_quarter(0)
    pack_x8(0)
    batch(0, 32, None, 0, 256)
    wait_all(c_a[1])
    c_h = [start(wq_hbm.at[pl.ds(256 * n, 256), :, 1], wraw.at[1, pl.ds(256 * n, 256)], 4 + n) for n in range(2)]
    relayout_quarter(1)
    pack_x8(1)
    batch(0, 32, None, 256, 512)
    wait_all(c_a[2])
    relayout_quarter(2)
    wait_all(c_a[3])
    relayout_quarter(3)
    pack_x8(2)
    pack_x8(3)
    batch(0, 24, None, 512, D)
    c_h[0].wait()
    c_w[2] = start_unit(2)
    batch(24, 32, relayout_tasks(1, 0, 256), 512, D)
    batch(32, 52, None, 0, 512)
    c_h[1].wait()
    c_w[3] = start_unit(3)
    batch(52, 64, relayout_tasks(1, 256, 512), 0, 512)
    batch(32, 52, None, 512, D)
    c_w[2].wait()
    c_b1 = [start(bx_hbm.at[:, pl.ds(128 * j, 128)], xb.at[j], 0) for j in range(8)]
    c_b1 += [start(gf_hbm, gf, 1), start(mt_hbm, mt, 2)]
    c_w[4] = start_unit(4)
    batch(52, 64, relayout_tasks(2), 512, D)
    batch(64, 84)
    c_w[3].wait()
    c_flt = []
    for t, w in enumerate((wr_hbm, wi_hbm)):
        for d in range(16):
            c_flt.append(start(w.at[pl.ds(0, 512), pl.ds(128 * d, 128)], wt.at[t, d], 10))
        c_flt.append(start(w.at[pl.ds(512, 1), :], wl.at[t], 11 + t))
    c_w[5] = start_unit(5)
    c_gi = start(gi_hbm, gi, 13)
    batch(84, 96, relayout_tasks(3))
    batch(96, 120)
    wait_all(c_b1)
    c_w[4].wait()
    batch(120, 128, relayout_tasks(4))
    b_stage1()
    wait_all(c_flt)
    c_w[5].wait()
    c_gi.wait()
    c_x = [start(x_hbm.at[:, pl.ds(M, SEG - M), :], xbuf.at[:, pl.ds(M, SEG - M), :], 14),
           start(mem_hbm, xbuf.at[0, pl.ds(0, M), :], 15), start(fill_hbm, fill_ref, 16)]
    c_wo = [start(wo_hbm.at[:, pl.ds(128 * j, 128)], wo.at[j], 17) for j in range(8)]
    flt = all_filter_tasks()
    f1 = 12 * 30
    batch(128, 160, merge(relayout_tasks(5), flt[:f1]))
    batch(160, 192, flt[f1:])

    row0 = lax.broadcasted_iota(jnp.int32, (8, 128), 0) == 0
    for b in range(16):
        m = as_bf16(mt[b])
        for g in range(4):
            yr, yi = yb[0, b, pl.ds(128 * g, 128), :], yb[1, b, pl.ds(128 * g, 128), :]
            if g == 0:
                v2 = jnp.concatenate([jnp.where(row0, yb[0, b, pl.ds(512, 8), :], yi[0:8]), yi[8:]], axis=0)
                u2 = jnp.concatenate([jnp.where(row0, -yb[1, b, pl.ds(512, 8), :], yr[0:8]), yr[8:]], axis=0)
                tr = dot_nt(m[:128], yr.astype(bf16)) + dot_nt(m[128:], yi.astype(bf16))
                ti = dot_nt(m[:128], v2.astype(bf16)) - dot_nt(m[128:], u2.astype(bf16))
            else:
                pa, pb = dot_nt(m, yr.astype(bf16)), dot_nt(m, yi.astype(bf16))
                tr = pa[:128] + pb[128:]
                ti = pb[:128] - pa[128:]
            xd[2 * g, pl.ds(XP * b, 128), :] = tr
            xd[2 * g + 1, pl.ds(XP * b, 128), :] = ti
    for t in range(16):
        z = []
        for g in range(4):
            zz = jnp.concatenate(
                [jnp.concatenate([xd[2 * g + h, pl.ds(8 * t + u, 16, stride=XP), :] for u in range(8)], axis=0)
                 for h in range(2)], axis=1).astype(bf16)
            z += [dot(zz, as_bf16(gi[g, 0])), dot(zz, as_bf16(gi[g, 1]))]
        y = _inv8(z)
        for j in range(8):
            xb32[j, pl.ds(64 * t, 64), :] = pltpu.bitcast(y[j].astype(bf16), u32)

    c_out = [start(xb.at[j], out_hbm.at[:, pl.ds(D + 128 * j, 128)], 18) for j in range(8)]
    wait_all(c_x)
    wait_all(c_wo)

    wo32 = wo.bitcast(u32)
    scale = E ** -0.5

    def step(s, mem, early):
        rows = jnp.concatenate([mem, xbuf[s, pl.ds(M, SEG - M), :].astype(f32)], axis=0)
        lhs = rows.astype(bf16)
        head_start = {}
        if early:
            lo, hi = rows[:, :D // 2].astype(bf16), rows[:, D // 2:].astype(bf16)
            for key in early:
                head_start[key] = dot(lo, wqkv(*key, k1=D // 2))
        r8 = pl.multiple_of(M * s, M)
        fill = fill_ref[...]
        heads = [None] * H
        rs = []

        def proj(i, p, toks=()):
            a, b = [
                dot(hi, wqkv(i, p, t, k0=D // 2)) + head_start[i, p, t] if (i, p, t) in head_start
                else dot(lhs, wqkv(i, p, t, toks[t * len(toks) // 2:(t + 1) * len(toks) // 2]))
                for t in range(2)]
            c = as_bf16(pre[i, p, pl.ds(r8, M), :]).astype(f32)
            return jnp.concatenate([a, b, c], axis=0).astype(bf16)

        def probs(q, k):
            sc = dot_nt(q, k) * scale
            sc = jnp.where(fill == 0.0, sc, fill)
            e = jnp.exp(sc - jnp.max(sc, axis=1, keepdims=True))
            l = jnp.sum(e, axis=1, keepdims=True)
            r = pl.reciprocal(l, approx=True)
            r = r * (2.0 - l * r)
            rs.append([r[8 * n:8 * n + 8] for n in range(10)])
            return (e * r).astype(bf16)

        def pv(p, pr, v):
            o = dot(pr, v)
            heads[2 * p] = o[0:32]
            heads[2 * p + 1] = o[32:64]
            odef[2 * p, pl.ds(r8, M), :] = o[64:72].astype(bf16)
            odef[2 * p + 1, pl.ds(r8, M), :] = o[72:80].astype(bf16)

        pend = []
        for g in range(4):
            ps = range(4 * g, 4 * g + 4)
            qk = [(proj(0, p), proj(1, p)) for p in ps]
            vs = [proj(2, p, rs[p - 4] if g else ()) for p in ps]
            for a in pend:
                pv(*a)
            pend = [(p, probs(*qk[t]), vs[t]) for t, p in enumerate(ps)]

        def wo_part(oc, j, h0, h1, toks=()):
            return dot(oc, as_bf16(gated(wo32[j, pl.ds(64 * h0, 64 * (h1 - h0)), :], toks)))

        acc = []
        oc = jnp.concatenate(heads[0:24], axis=1).astype(bf16)
        for j in range(8):
            acc.append(wo_part(oc, j, 0, 24, {3: rs[12] + rs[13], 4: rs[14] + rs[15]}.get(j, ())))
            if j == 4:
                for a in pend:
                    pv(*a)
        oc = jnp.concatenate(heads[24:32], axis=1).astype(bf16)
        nxt = []
        for j in range(8):
            r = wo_part(oc, j, 24, 32) + acc[j]
            outbuf[s, pl.ds(M, SEG - M), pl.ds(128 * j, 128)] = r[M:].astype(bf16)
            nxt.append(r[0:M])
        return jnp.concatenate(nxt, axis=1)

    def steps(n, mem):
        for u in range(UNROLL):
            mem = step(UNROLL * n + u, mem, EARLY if u else ())
        return mem
    lax.fori_loop(0, NSEG // UNROLL, steps, xbuf[0, pl.ds(0, M), :].astype(f32))
    c_out.append(start(outbuf.at[:, pl.ds(M, SEG - M), :], out3.at[:, pl.ds(M, SEG - M), pl.ds(0, D)], 19))

    for t in range(4):
        lhs = jnp.concatenate([odef[h, pl.ds(128 * t, 128), :] for h in range(H)], axis=1)
        for j in range(8):
            r = dot(lhs, as_bf16(wo32[j]))
            outbuf[pl.ds(16 * t, 16), pl.ds(0, M), pl.ds(128 * j, 128)] = r.reshape(16, M, 128).astype(bf16)
        c_out.append(start(outbuf.at[pl.ds(16 * t, 16), pl.ds(0, M), :],
                           out3.at[pl.ds(16 * t, 16), pl.ds(0, M), pl.ds(0, D)], 20 + t))
    wait_all(c_out)


@functools.partial(jax.jit, static_argnames=("A_seg_len",))
def pallas_concat_heads__memory_aug_recurrent_mem_tr__spectral_gfnet__prompt_kernel(
    A_x: jax.Array,
    A_mem0: jax.Array,
    A_Wq: jax.Array,
    A_Wk: jax.Array,
    A_Wv: jax.Array,
    A_Wo: jax.Array,
    A_seg_len,
    B_x: jax.Array,
    B_w_r: jax.Array,
    B_w_i: jax.Array,
):
    assert A_seg_len == SEG
    assert A_x.shape == (1, S, D) and A_mem0.shape == (1, M, D) and B_x.shape == (1, S, D)
    assert A_Wq.shape == (D, H, E) and A_Wo.shape == (H, E, D) and B_w_r.shape == (S, D // 2 + 1)
    gf, gi, mt = _dft_constants()
    fill = _attn_fill()
    hbm = pl.BlockSpec(memory_space=pltpu.HBM)
    wshape = (D // 2, 2, 2, 16, E)
    out = pl.pallas_call(
        _kernel,
        out_shape=jax.ShapeDtypeStruct((S, 2 * D), bf16),
        in_specs=[hbm] * 13,
        out_specs=hbm,
        scratch_shapes=[
            pltpu.VMEM((NRAW, D // 2, 2, 16, E), bf16),
            *[pltpu.VMEM((16 * WP, E), u32)] * 6,
            pltpu.VMEM((8, H * E, 128), bf16),
            pltpu.VMEM((NSEG, SEG, D), bf16),
            pltpu.VMEM((NSEG, M, D), bf16),
            pltpu.VMEM((8, NSEG * M // 2, 128), u32),
            pltpu.VMEM((3, 16, NSEG * M, E), u32),
            pltpu.VMEM((H, NSEG * M, E), bf16),
            pltpu.VMEM((NSEG, SEG, D), bf16),
            pltpu.VMEM(fill.shape, f32),
            pltpu.VMEM((8, S, 128), bf16),
            pltpu.VMEM((2, 16, 512, 128), bf16),
            pltpu.VMEM((2, 1, S), bf16),
            pltpu.VMEM(gf.shape, u32),
            pltpu.VMEM(gi.shape, u32),
            pltpu.VMEM(mt.shape, u32),
            pltpu.VMEM((8, 16 * XP, 128), f32),
            pltpu.VMEM((2, 16, YR, 128), f32),
            pltpu.SemaphoreType.DMA((32,)),
        ],
        compiler_params=pltpu.CompilerParams(vmem_limit_bytes=120 * 1024 * 1024),
    )(A_x.reshape(NSEG, SEG, D), A_mem0.reshape(M, D),
      A_Wq.reshape(wshape), A_Wk.reshape(wshape), A_Wv.reshape(wshape),
      A_Wo.reshape(H * E, D), B_x.reshape(S, D), B_w_r.T, B_w_i.T, gf, gi, mt, fill)
    return out.reshape(1, S, 2 * D)
```

```python
import functools

import jax
import jax.numpy as jnp
import numpy as np
from jax import lax
from jax.experimental import pallas as pl
from jax.experimental.pallas import tpu as pltpu

S, D, H, E, M, SEG = 2048, 1024, 32, 128, 8, 32
NSEG = S // SEG
WP = 516
XP = 132
ZP = 68
YR = 520
NRAW = 4
BM = 128
UNROLL = 4
EARLY = ((0, 0, 0), (0, 0, 1), (1, 0, 0), (1, 0, 1), (0, 1, 0), (0, 1, 1))
bf16, f32, u32 = jnp.bfloat16, jnp.float32, jnp.uint32
RES = ((0, 4), (2, 6), (1, 7), (3, 5))
RC = float(np.sqrt(0.5))


def _fwd8(x):
    s04, d04 = x[0] + x[4], x[0] - x[4]
    s26, d26 = x[2] + x[6], x[2] - x[6]
    s15, d15 = x[1] + x[5], x[1] - x[5]
    s37, d37 = x[3] + x[7], x[3] - x[7]
    t1, t2 = (d15 - d37) * RC, (d15 + d37) * RC
    e0, o0 = s04 + s26, s15 + s37
    return [e0 + o0, e0 - o0, s04 - s26, s15 - s37, d04 + t1, d26 + t2, d04 - t1, d26 - t2]


def _inv8(z):
    z0, z4, e1, o1, r1, i1, r3, i3 = z
    e0, o0 = z0 + z4, z0 - z4
    s04, s26, s15, s37 = e0 + e1, e0 - e1, o0 + o1, o0 - o1
    d04, d26 = r1 + r3, i1 + i3
    t1, t2 = (r1 - r3) * RC, (i1 - i3) * RC
    d15, d37 = t1 + t2, t2 - t1
    return [s04 + d04, s15 + d15, s26 + d26, s37 + d37, s04 - d04, s15 - d15, s26 - d26, s37 - d37]


def _twiddle16(z, k):
    re, im = z
    k = k % 16
    if k == 0:
        return z
    if k == 4:
        return (im, -re)
    if k == 12:
        return (-im, re)
    if k == 2:
        return ((re + im) * RC, (im - re) * RC)
    if k == 14:
        return ((re - im) * RC, (re + im) * RC)
    if k == 6:
        return ((im - re) * RC, (re + im) * -RC)
    if k == 10:
        return ((re + im) * -RC, (re - im) * RC)
    c, s = float(np.cos(2 * np.pi * k / 16)), float(-np.sin(2 * np.pi * k / 16))
    return (re * c - im * s, re * s + im * c)


def _bfly4(z, sign):
    (ar, ai), (br, bi), (cr, ci), (dr, di) = z
    sr, si, tr, ti = ar + cr, ai + ci, ar - cr, ai - ci
    ur, ui, vr, vi = br + dr, bi + di, br - dr, bi - di
    o0, o2 = (sr + ur, si + ui), (sr - ur, si - ui)
    p, q = (tr + vi, ti - vr), (tr - vi, ti + vr)
    return [o0, p, o2, q] if sign > 0 else [o0, q, o2, p]


class _Pacer:
    def __init__(self, tasks, ntokens):
        self.slots = {}
        for n, task in enumerate(tasks):
            self.slots.setdefault(n * ntokens // len(tasks), []).append(task)
        self.pos = 0
        self.ntokens = ntokens

    def feed(self, r):
        for j in range(r.shape[0] // 8):
            for task in self.slots.pop(self.pos, []):
                task(pltpu.bitcast(r[8 * j:8 * j + 8], u32))
            self.pos += 1

    def done(self):
        assert not self.slots and self.pos == self.ntokens


def _pack_rows(m):
    b = np.asarray(m, np.float32).astype(jnp.bfloat16).view(np.uint16).astype(np.uint32)
    return b[..., 0::2, :] | (b[..., 1::2, :] << 16)


@functools.lru_cache(maxsize=None)
def _dft_constants():
    b8 = np.array(_fwd8(list(np.eye(8)))).T
    n = np.arange(D)
    fw = np.zeros((D, D))
    bw = np.zeros((D, D))
    for g in range(4):
        k = np.concatenate([8 * np.arange(64) + r for r in RES[g]])
        ang = 2 * np.pi * ((n[:, None] * k[None, :]) % D) / D
        wgt = np.where(k == 0, 1.0, 2.0) / (D * S)
        fw[:, 256 * g:256 * g + 128] = np.cos(ang)
        fw[:, 256 * g + 128:256 * g + 256] = -np.sin(ang)
        bw[256 * g:256 * g + 128] = (np.cos(ang) * wgt).T
        bw[256 * g + 128:256 * g + 256] = (-np.sin(ang) * wgt).T
    bw[128, :] = (-1.0) ** n / (D * S)
    binv = np.kron(np.linalg.inv(b8), np.eye(128))
    gall = binv @ fw
    giall = bw @ binv.T
    gf = np.zeros((11, 144, 128))
    gi = np.zeros((11, 128, 128))
    sign = []
    half = lambda m, q: np.concatenate([m[64 * q:64 * q + 64], m[128 + 64 * q:192 + 64 * q]])
    for g in range(4):
        sl = slice(256 * g, 256 * g + 256)
        f, b = gall[sl, sl].T, giall[sl, sl]
        if g == 0:
            for q in range(2):
                gf[q, :128] = half(f, q)[:, 128 * q:128 * q + 128]
                gi[q] = half(b, q)[:, 128 * q:128 * q + 128]
            gf[0, 128] = (-1.0) ** np.arange(128)
            continue
        sg = np.sign(f[:128, 0] * f[128:, 128])[:, None]
        sign.append((int(sg[0, 0]), int(sg[64, 0])))
        p, q, r = f[:128, :128], f[:128, 128:], f[128:, :128]
        gf[3 * g - 1:3 * g + 2, :128] = p, q - p, r - sg * p
        p, q, r = b[:128, :128], b[:128, 128:], b[128:, :128]
        gi[3 * g - 1:3 * g + 2] = p, r - sg * p, q - p
    a = np.arange(128)
    mt = np.zeros((16, 4, 128, 128))
    for b in range(16):
        ang = 2 * np.pi * (((16 * a[:, None] + b) * a[None, :]) % S) / S
        c, sn = np.cos(ang), -np.sin(ang)
        mt[b] = c, c + sn, sn - c, sn
    return _pack_rows(gf), _pack_rows(gi), _pack_rows(mt), tuple(sign)


def _attn_fill():
    pos32 = np.concatenate([np.arange(8), np.arange(16, 40)])
    last = np.arange(16)
    qhead = np.concatenate([np.arange(64) // 32, last // 8])
    khead = np.concatenate([np.arange(64) // 32, last % 2])
    qpos = np.concatenate([pos32, pos32, 8 + last % 8])
    kpos = np.concatenate([pos32, pos32, 8 + last // 2])
    ok = (qpos[:, None] < M) | (qpos[:, None] >= kpos[None, :])
    fill = np.where(ok, 0.0, -1e9)
    fill = np.where(qhead[:, None] == khead[None, :], fill, -np.inf)
    return fill.astype(np.float32)


def _kernel(x_hbm, mem_hbm, wq_hbm, wk_hbm, wv_hbm, wo_hbm, bx_hbm, wr_hbm, wi_hbm,
            gf_hbm, gi_hbm, mt_hbm, fill_hbm, out_hbm,
            wraw, w0, w1, w2, w3, w4, w5, wo, xbuf, x8, x8c, pre, odef, outbuf, fill_ref,
            xb, wt, wl, gf, gi, mt, xd, yb, sems):
    def start(src, dst, i, priority=0):
        c = pltpu.make_async_copy(src, dst, sems.at[i])
        c.start(priority=priority)
        return c

    def wait_all(cs):
        for c in cs:
            c.wait()

    dot = functools.partial(jnp.dot, preferred_element_type=f32)
    dot_nt = lambda a, b: lax.dot_general(a, b, (((1,), (1,)), ((), ())), preferred_element_type=f32)
    as_bf16 = lambda w: pltpu.bitcast(w, bf16)
    lo_f32 = lambda w: pltpu.bitcast(w << 16, f32)
    hi_f32 = lambda w: pltpu.bitcast(w & u32(0xFFFF0000), f32)
    out3 = out_hbm.reshape(NSEG, SEG, 2 * D)
    w_hbm = (wq_hbm, wk_hbm, wv_hbm)
    w32 = (w0, w1, w2, w3, w4, w5)

    def start_unit(u):
        return start(w_hbm[u // 2].at[:, :, u % 2], wraw.at[u % NRAW], 4 + u)

    c_a = []
    for n in range(4):
        cols, rows = pl.ds(256 * n, 256), pl.ds(128 * n, 128)
        c_a.append([start(x_hbm.at[:, pl.ds(0, M), cols], x8.at[:, :, cols], 24 + n),
                    start(wq_hbm.at[rows, :, 0], wraw.at[0, rows], 28 + n)])

    c_x = [start(x_hbm.at[:, pl.ds(M, SEG - M), :], xbuf.at[:, pl.ds(M, SEG - M), :], 14, 1),
           start(mem_hbm, xbuf.at[0, pl.ds(0, M), :], 15, 1), start(fill_hbm, fill_ref, 16, 1)]
    c_wo = [start(wo_hbm.at[:, pl.ds(128 * j, 128)], wo.at[j], 17, 1) for j in range(8)]

    wraw32 = wraw.bitcast(u32)
    wt32 = wt.bitcast(u32)

    def relayout_row(u, dst, r, off, lo, hi):
        a, b = wraw32[u % NRAW, r, 0], wraw32[u % NRAW, r, 1]
        dst[pl.ds(off, 8, stride=WP), :] = (a & lo) | (b << 16)
        dst[pl.ds(off + 8 * WP, 8, stride=WP), :] = (a >> 16) | (b & hi)

    def relayout_tasks(u, r0=0, r1=D // 2):
        def make(r):
            def task(tok):
                lo = (tok >> 16) | u32(0xFFFF)
                hi = (tok << 16) | u32(0xFFFF0000)
                relayout_row(u, w32[u], r, r, lo, hi)
                relayout_row(u, w32[u], r + 1, r + 1, lo, hi)
            return task
        return [make(r) for r in range(r0, r1, 2)]

    def filter_tasks(rows, wfn):
        def make(phase, k):
            slots = [4 * k + j for j in range(4)] if phase == 1 else [4 * j + k for j in range(4)]

            def task(tok):
                ones = ((tok >> 16) | u32(0xFFFF)) | u32(0xFFFF0000)
                z = [(yb[0, b, rows, :], yb[1, b, rows, :]) for b in slots]
                z[0] = tuple(pltpu.bitcast(pltpu.bitcast(v, u32) & ones, f32) for v in z[0])
                if phase == 0:
                    o = _bfly4(z, 1)
                    o = [_twiddle16(o[j], k * j) for j in range(4)]
                elif phase == 1:
                    o = _bfly4(z, 1)
                    y = []
                    for j in range(4):
                        wr, wi = wfn(k + 4 * j)
                        xr, xi = o[j]
                        y.append((xr * wr - xi * wi, xr * wi + xi * wr))
                    o = _bfly4(y, -1)
                    o = [_twiddle16(o[j], -k * j) for j in range(4)]
                else:
                    o = _bfly4(z, -1)
                for b, v in zip(slots, o):
                    yb[0, b, rows, :] = v[0]
                    yb[1, b, rows, :] = v[1]
            return task
        return [make(phase, k) for phase in range(3) for k in range(4)]

    def all_filter_tasks():
        tasks = []
        for i in range(8):
            for g in range(4):
                for q in range(2):
                    r = RES[g][q]
                    un = lo_f32 if r % 2 == 0 else hi_f32
                    wrows = pl.ds(32 * i + r // 2, 8, stride=4)
                    tasks += filter_tasks(pl.ds(128 * g + 64 * q + 8 * i, 8),
                                          lambda d, un=un, wrows=wrows: [un(wt32[t, d, wrows, :]) for t in range(2)])
        tasks += filter_tasks(pl.ds(512, 8), lambda d: [wl[t, :, pl.ds(128 * d, 128)].astype(f32) for t in range(2)])
        return tasks

    def merge(a, b):
        keyed = [(n / len(a), 0, n) for n in range(len(a))] + [(n / len(b), 1, n) for n in range(len(b))]
        return [(a, b)[w][n] for _, w, n in sorted(keyed)]

    xb32 = xb.bitcast(u32)

    sign = _dft_constants()[3]
    cat = lambda *xs: jnp.concatenate(xs, axis=0)

    pack2 = lambda a, b: pltpu.pack_elementwise([a, b], packed_dtype=bf16)

    def z_region(n, par):
        return (2 * n + par) // 3, (2 * n + par) % 3 * 8 * ZP

    def butterfly_tasks():
        def make(a2, par):
            def task(tok):
                zs = []
                for a in (2 * a2, 2 * a2 + 1):
                    w = [xb32[j, pl.ds(8 * a, 8), :] for j in range(8)]
                    if par:
                        hi = (tok << 16) | u32(0xFFFF0000)
                        z = _fwd8([pltpu.bitcast(v & hi, f32) for v in w])
                    else:
                        sh = (tok >> 31) | u32(1)
                        z = _fwd8([pltpu.bitcast(v << (sh << 4), f32) for v in w])
                    zs.append(z[0:2] + [v for g in range(1, 4)
                                        for v in (z[2 * g] + z[2 * g + 1], z[2 * g + 1], z[2 * g])])
                for n in range(11):
                    plane, row = z_region(n, par)
                    xd[plane, pl.ds(row + a2, 8, stride=ZP), :] = pltpu.bitcast(pack2(zs[0][n], zs[1][n]), f32)
            return task
        return [make(a2, par) for a2 in range(64) for par in range(2)]

    def b_dfwd(b):
        def z(n):
            plane, row = z_region(n, b % 2)
            return as_bf16(xd[plane, pl.ds(row + b // 2 * ZP, 64), :])
        t0 = dot_nt(as_bf16(gf[0]), z(0))
        t4 = dot_nt(as_bf16(gf[1, 0:64]), z(1))
        tr, ti = cat(t0[0:64], t4[0:64]), cat(t0[64:128], t4[64:128])
        ts = [(cat(tr + ti, t0[128:144]).astype(bf16), ti.astype(bf16), cat(tr, t0[128:144]).astype(bf16))]
        for g in range(1, 4):
            k1, k2, k3 = [dot_nt(as_bf16(gf[n, 0:64]), z(n)) for n in range(3 * g - 1, 3 * g + 2)]
            tr = k1 + k2
            ti = cat(*[k3[64 * q:64 * q + 64] + k1[64 * q:64 * q + 64] if sign[g - 1][q] > 0
                       else k3[64 * q:64 * q + 64] - k1[64 * q:64 * q + 64] for q in range(2)])
            ts.append(((tr + ti).astype(bf16), ti.astype(bf16), tr.astype(bf16)))
        return ts

    def b_sfwd(b, ts):
        for g in range(4):
            k1, k2, k3 = [dot(ts[g][n], as_bf16(mt[b, n])) for n in range(3)]
            yi = k1 + k3
            yb[0, b, pl.ds(128 * g, 128), :] = k1[0:128] - k2
            yb[1, b, pl.ds(128 * g, 128), :] = yi[0:128]
            if g == 0:
                yb[0, b, pl.ds(512, 8), :] = k1[128:136]
                yb[1, b, pl.ds(512, 8), :] = yi[128:136]

    def b_stage1():
        prev = None
        for b in range(16):
            ts = b_dfwd(b)
            if prev is not None:
                b_sfwd(b - 1, prev)
            prev = ts
        b_sfwd(15, prev)

    def b_stage3():
        row0 = lax.broadcasted_iota(jnp.int32, (8, 128), 0) == 0
        low = lax.broadcasted_iota(jnp.int32, (1, 128), 1) < 64
        for b in range(16):
            m = [as_bf16(mt[b, n]) for n in range(4)]
            for g in range(4):
                yr, yi = yb[0, b, pl.ds(128 * g, 128), :], yb[1, b, pl.ds(128 * g, 128), :]
                if g == 0:
                    nr = -yr
                    u0 = cat(yr[0:64], jnp.where(row0, yb[0, b, pl.ds(512, 8), :], yi[0:8]), yi[8:64])
                    v0 = cat(yi[0:64], jnp.where(row0, yb[1, b, pl.ds(512, 8), :], nr[0:8]), nr[8:64])
                    u4, v4 = cat(yr[64:128], yi[64:128]), cat(yi[64:128], nr[64:128])
                    t1 = dot_nt(m[0], u0.astype(bf16)) + dot_nt(m[3], v0.astype(bf16))
                    t2 = dot_nt(m[0], u4.astype(bf16)) + dot_nt(m[3], v4.astype(bf16))
                else:
                    k1, k2, k3 = [dot_nt(m[n], v.astype(bf16)) for n, v in enumerate((yr + yi, yr, yi))]
                    t1, t2 = k1 + k3, k1 - k2
                slot = b // 2 + 8 * (b % 2)
                xd[2 * g, pl.ds(XP * slot, 128), :] = t1
                xd[2 * g + 1, pl.ds(XP * slot, 128), :] = t2
        for t in range(16):
            rows = lambda j: cat(*[xd[j, pl.ds(8 * t + u, 16, stride=XP), :] for u in range(8)])
            z = [dot(rows(q).astype(bf16), as_bf16(gi[q])) for q in range(2)]
            for g in range(1, 4):
                tr, ti = rows(2 * g), rows(2 * g + 1)
                sg = jnp.where(low, float(sign[g - 1][0]), float(sign[g - 1][1]))
                k1, k2, k3 = [dot(v.astype(bf16), as_bf16(gi[3 * g - 1 + n]))
                              for n, v in enumerate((tr + sg * ti, ti, tr))]
                z += [k1 + k2, k1 + k3]
            y = _inv8(z)
            for j in range(8):
                even = cat(*[y[j][16 * u:16 * u + 8] for u in range(8)])
                odd = cat(*[y[j][16 * u + 8:16 * u + 16] for u in range(8)])
                xb32[j, pl.ds(64 * t, 64), :] = pack2(even, odd)

    def gated(w, toks):
        if not toks:
            return w
        bits = functools.reduce(
            jnp.bitwise_or, [pltpu.bitcast(jnp.broadcast_to(t, (8, 128)), u32) for t in toks])
        ones = ((bits >> 16) | u32(0xFFFF)) | u32(0xFFFF0000)
        return jnp.concatenate([w[0:8] & ones, w[8:]], axis=0)

    def wqkv(i, p, second, toks=(), k0=0, k1=D):
        rows = pl.ds((p % 8 + 8 * second) * WP + k0 // 2, (k1 - k0) // 2)
        return as_bf16(gated(w32[2 * i + p // 8][rows, :], toks))

    def batch(n0, n1, tasks=None, k0=0, k1=D):
        pacer = _Pacer(tasks, (n1 - n0 - 1) * BM // 4) if tasks else None
        for n in range(n0, n1):
            i, p, c = n // 64, n % 64 // 4, n % 4
            rows = pl.ds(c * BM, BM)
            lhs = jnp.concatenate([as_bf16(x8c[k, pl.ds(c * BM // 2, BM // 2), :])
                                   for k in range(k0 // 128, k1 // 128)], axis=1)
            rs = [dot(lhs, wqkv(i, p, t, k0=k0, k1=k1)) for t in range(2)]
            if k0 > 0:
                rs = [rs[t] + yb[t, p, rows, :] for t in range(2)]
            if k1 < D:
                for t in range(2):
                    yb[t, p, rows, :] = rs[t]
            elif i > 0:
                pre[i, p, rows, :] = pack2(rs[0], rs[1])
            else:
                st = jnp.concatenate([r.reshape(BM // M, M, E) for r in rs], axis=1)
                pre[i, p, rows, :] = pltpu.bitcast(st.reshape(2 * BM, E).astype(bf16), u32)
            if pacer is not None and n < n1 - 1:
                pacer.feed(rs[0])
                pacer.feed(rs[1])
        if pacer is not None:
            pacer.done()

    def pack_x8(n):
        x8v = x8[:, :, pl.ds(256 * n, 256)].reshape(NSEG * M, 256)
        for k in range(2):
            x8c[2 * n + k] = pltpu.bitcast(x8v[:, 128 * k:128 * k + 128], u32)

    def relayout_quarter(n):
        def body(t, c):
            off = pl.multiple_of(128 * n + 16 * t, 16)
            for r in range(16):
                relayout_row(0, w0.at[pl.ds(off, 15 * WP + 20)], off + r, r, u32(0xFFFF), u32(0xFFFF0000))
            return c
        lax.fori_loop(0, 8, body, 0)

    c_w = {}
    wait_all(c_a[0])
    relayout_quarter(0)
    pack_x8(0)
    batch(0, 32, None, 0, 256)
    wait_all(c_a[1])
    c_h = [start(wq_hbm.at[pl.ds(256 * n, 256), :, 1], wraw.at[1, pl.ds(256 * n, 256)], 4 + n) for n in range(2)]
    relayout_quarter(1)
    pack_x8(1)
    batch(0, 32, None, 256, 512)
    wait_all(c_a[2])
    relayout_quarter(2)
    wait_all(c_a[3])
    relayout_quarter(3)
    pack_x8(2)
    pack_x8(3)
    batch(0, 24, None, 512, D)
    c_h[0].wait()
    c_w[2] = start_unit(2)
    batch(24, 32, relayout_tasks(1, 0, 256), 512, D)
    batch(32, 52, None, 0, 512)
    c_h[1].wait()
    c_w[3] = start_unit(3)
    batch(52, 64, relayout_tasks(1, 256, 512), 0, 512)
    batch(32, 52, None, 512, D)
    c_w[2].wait()
    c_bx = [start(bx_hbm.at[:, pl.ds(128 * j, 128)], xb.at[j], 0) for j in range(8)]
    c_w[4] = start_unit(4)
    c_b1 = [start(gf_hbm, gf, 1), start(mt_hbm, mt, 2)]
    batch(52, 64, relayout_tasks(2), 512, D)
    batch(64, 88)
    c_w[3].wait()
    wait_all(c_bx)
    c_flt = []
    for t, w in enumerate((wr_hbm, wi_hbm)):
        for d in range(16):
            c_flt.append(start(w.at[pl.ds(0, 512), pl.ds(128 * d, 128)], wt.at[t, d], 10))
        c_flt.append(start(w.at[pl.ds(512, 1), :], wl.at[t], 11 + t))
    c_w[5] = start_unit(5)
    c_gi = start(gi_hbm, gi, 13)
    batch(88, 96, relayout_tasks(3))
    batch(96, 120, butterfly_tasks())
    wait_all(c_b1)
    c_w[4].wait()
    batch(120, 128, relayout_tasks(4))
    b_stage1()
    wait_all(c_flt)
    c_w[5].wait()
    c_gi.wait()
    flt = all_filter_tasks()
    f1 = 12 * 30
    batch(128, 160, merge(relayout_tasks(5), flt[:f1]))
    batch(160, 192, flt[f1:])

    wait_all(c_x)
    wait_all(c_wo)

    wo32 = wo.bitcast(u32)
    scale = E ** -0.5

    def step(s, mem, early):
        rows = jnp.concatenate([mem, xbuf[s, pl.ds(M, SEG - M), :].astype(f32)], axis=0)
        lhs = rows.astype(bf16)
        head_start = {}
        if early:
            lo, hi = rows[:, :D // 2].astype(bf16), rows[:, D // 2:].astype(bf16)
            for key in early:
                head_start[key] = dot(lo, wqkv(*key, k1=D // 2))
        r8 = pl.multiple_of(M * s, M)
        fill = fill_ref[...]
        heads = [None] * H
        rs = []

        def proj(i, p, toks=()):
            a, b = [
                dot(hi, wqkv(i, p, t, k0=D // 2)) + head_start[i, p, t] if (i, p, t) in head_start
                else dot(lhs, wqkv(i, p, t, toks[t * len(toks) // 2:(t + 1) * len(toks) // 2]))
                for t in range(2)]
            c = as_bf16(pre[i, p, pl.ds(r8, M), :]).astype(f32)
            return jnp.concatenate([a, b, c], axis=0).astype(bf16)

        def probs(q, k):
            sc = dot_nt(q, k) * scale
            sc = jnp.where(fill == 0.0, sc, fill)
            e = jnp.exp(sc - jnp.max(sc, axis=1, keepdims=True))
            l = jnp.sum(e, axis=1, keepdims=True)
            r = pl.reciprocal(l, approx=True)
            r = r * (2.0 - l * r)
            rs.append([r[8 * n:8 * n + 8] for n in range(10)])
            return (e * r).astype(bf16)

        def pv(p, pr, v):
            o = dot(pr, v)
            heads[2 * p] = o[0:32]
            heads[2 * p + 1] = o[32:64]
            odef[2 * p, pl.ds(r8, M), :] = o[64:72].astype(bf16)
            odef[2 * p + 1, pl.ds(r8, M), :] = o[72:80].astype(bf16)

        pend = []
        for g in range(4):
            ps = range(4 * g, 4 * g + 4)
            qk = [(proj(0, p), proj(1, p)) for p in ps]
            vs = [proj(2, p, rs[p - 4] if g else ()) for p in ps]
            for a in pend:
                pv(*a)
            pend = [(p, probs(*qk[t]), vs[t]) for t, p in enumerate(ps)]

        def wo_part(oc, j, h0, h1, toks=()):
            return dot(oc, as_bf16(gated(wo32[j, pl.ds(64 * h0, 64 * (h1 - h0)), :], toks)))

        acc = []
        oc = jnp.concatenate(heads[0:24], axis=1).astype(bf16)
        for j in range(8):
            acc.append(wo_part(oc, j, 0, 24, {3: rs[12] + rs[13], 4: rs[14] + rs[15]}.get(j, ())))
            if j == 4:
                for a in pend:
                    pv(*a)
        oc = jnp.concatenate(heads[24:32], axis=1).astype(bf16)
        nxt = []
        for j in range(8):
            r = wo_part(oc, j, 24, 32) + acc[j]
            outbuf[s, pl.ds(M, SEG - M), pl.ds(128 * j, 128)] = r[M:].astype(bf16)
            nxt.append(r[0:M])
        return jnp.concatenate(nxt, axis=1)

    def steps(n, mem):
        for u in range(UNROLL):
            mem = step(UNROLL * n + u, mem, EARLY if u else ())
        return mem
    lax.fori_loop(0, NSEG // UNROLL, steps, xbuf[0, pl.ds(0, M), :].astype(f32))
    c_out = [start(outbuf.at[:, pl.ds(M, SEG - M), :], out3.at[:, pl.ds(M, SEG - M), pl.ds(0, D)], 19)]
    b_stage3()
    c_out += [start(xb.at[j], out_hbm.at[:, pl.ds(D + 128 * j, 128)], 18) for j in range(8)]

    for t in range(4):
        lhs = jnp.concatenate([odef[h, pl.ds(128 * t, 128), :] for h in range(H)], axis=1)
        for j in range(8):
            r = dot(lhs, as_bf16(wo32[j]))
            outbuf[pl.ds(16 * t, 16), pl.ds(0, M), pl.ds(128 * j, 128)] = r.reshape(16, M, 128).astype(bf16)
        c_out.append(start(outbuf.at[pl.ds(16 * t, 16), pl.ds(0, M), :],
                           out3.at[pl.ds(16 * t, 16), pl.ds(0, M), pl.ds(0, D)], 20 + t))
    wait_all(c_out)


@functools.partial(jax.jit, static_argnames=("A_seg_len",))
def pallas_concat_heads__memory_aug_recurrent_mem_tr__spectral_gfnet__prompt_kernel(
    A_x: jax.Array,
    A_mem0: jax.Array,
    A_Wq: jax.Array,
    A_Wk: jax.Array,
    A_Wv: jax.Array,
    A_Wo: jax.Array,
    A_seg_len,
    B_x: jax.Array,
    B_w_r: jax.Array,
    B_w_i: jax.Array,
):
    assert A_seg_len == SEG
    assert A_x.shape == (1, S, D) and A_mem0.shape == (1, M, D) and B_x.shape == (1, S, D)
    assert A_Wq.shape == (D, H, E) and A_Wo.shape == (H, E, D) and B_w_r.shape == (S, D // 2 + 1)
    gf, gi, mt, _ = _dft_constants()
    fill = _attn_fill()
    hbm = pl.BlockSpec(memory_space=pltpu.HBM)
    wshape = (D // 2, 2, 2, 16, E)
    out = pl.pallas_call(
        _kernel,
        out_shape=jax.ShapeDtypeStruct((S, 2 * D), bf16),
        in_specs=[hbm] * 13,
        out_specs=hbm,
        scratch_shapes=[
            pltpu.VMEM((NRAW, D // 2, 2, 16, E), bf16),
            *[pltpu.VMEM((16 * WP, E), u32)] * 6,
            pltpu.VMEM((8, H * E, 128), bf16),
            pltpu.VMEM((NSEG, SEG, D), bf16),
            pltpu.VMEM((NSEG, M, D), bf16),
            pltpu.VMEM((8, NSEG * M // 2, 128), u32),
            pltpu.VMEM((3, 16, NSEG * M, E), u32),
            pltpu.VMEM((H, NSEG * M, E), bf16),
            pltpu.VMEM((NSEG, SEG, D), bf16),
            pltpu.VMEM(fill.shape, f32),
            pltpu.VMEM((8, S, 128), bf16),
            pltpu.VMEM((2, 16, 512, 128), bf16),
            pltpu.VMEM((2, 1, S), bf16),
            pltpu.VMEM(gf.shape, u32),
            pltpu.VMEM(gi.shape, u32),
            pltpu.VMEM(mt.shape, u32),
            pltpu.VMEM((8, 16 * XP, 128), f32),
            pltpu.VMEM((2, 16, YR, 128), f32),
            pltpu.SemaphoreType.DMA((32,)),
        ],
        compiler_params=pltpu.CompilerParams(vmem_limit_bytes=120 * 1024 * 1024),
    )(A_x.reshape(NSEG, SEG, D), A_mem0.reshape(M, D),
      A_Wq.reshape(wshape), A_Wk.reshape(wshape), A_Wv.reshape(wshape),
      A_Wo.reshape(H * E, D), B_x.reshape(S, D), B_w_r.T, B_w_i.T, gf, gi, mt, fill)
    return out.reshape(1, S, 2 * D)
```

```python
import functools

import jax
import jax.numpy as jnp
import numpy as np
from jax import lax
from jax.experimental import pallas as pl
from jax.experimental.pallas import tpu as pltpu

S, D, H, E, M, SEG = 2048, 1024, 32, 128, 8, 32
NSEG = S // SEG
WP = 516
XP = 132
ZP = 68
YR = 520
NRAW = 4
UNROLL = 4
FTOK = 60
EARLY = ((0, 0, 0), (0, 0, 1), (1, 0, 0), (1, 0, 1), (0, 1, 0), (0, 1, 1))
bf16, f32, u32 = jnp.bfloat16, jnp.float32, jnp.uint32
RES = ((0, 4), (2, 6), (1, 7), (3, 5))
RC = float(np.sqrt(0.5))


def _fwd8(x):
    s04, d04 = x[0] + x[4], x[0] - x[4]
    s26, d26 = x[2] + x[6], x[2] - x[6]
    s15, d15 = x[1] + x[5], x[1] - x[5]
    s37, d37 = x[3] + x[7], x[3] - x[7]
    t1, t2 = (d15 - d37) * RC, (d15 + d37) * RC
    e0, o0 = s04 + s26, s15 + s37
    return [e0 + o0, e0 - o0, s04 - s26, s15 - s37, d04 + t1, d26 + t2, d04 - t1, d26 - t2]


def _inv8(z):
    z0, z4, e1, o1, r1, i1, r3, i3 = z
    e0, o0 = z0 + z4, z0 - z4
    s04, s26, s15, s37 = e0 + e1, e0 - e1, o0 + o1, o0 - o1
    d04, d26 = r1 + r3, i1 + i3
    t1, t2 = (r1 - r3) * RC, (i1 - i3) * RC
    d15, d37 = t1 + t2, t2 - t1
    return [s04 + d04, s15 + d15, s26 + d26, s37 + d37, s04 - d04, s15 - d15, s26 - d26, s37 - d37]


def _twiddle16(z, k):
    re, im = z
    k = k % 16
    if k == 0:
        return z
    if k == 4:
        return (im, -re)
    if k == 12:
        return (-im, re)
    if k == 2:
        return ((re + im) * RC, (im - re) * RC)
    if k == 14:
        return ((re - im) * RC, (re + im) * RC)
    if k == 6:
        return ((im - re) * RC, (re + im) * -RC)
    if k == 10:
        return ((re + im) * -RC, (re - im) * RC)
    c, s = float(np.cos(2 * np.pi * k / 16)), float(-np.sin(2 * np.pi * k / 16))
    return (re * c - im * s, re * s + im * c)


def _bfly4(z, sign):
    (ar, ai), (br, bi), (cr, ci), (dr, di) = z
    sr, si, tr, ti = ar + cr, ai + ci, ar - cr, ai - ci
    ur, ui, vr, vi = br + dr, bi + di, br - dr, bi - di
    o0, o2 = (sr + ur, si + ui), (sr - ur, si - ui)
    p, q = (tr + vi, ti - vr), (tr - vi, ti + vr)
    return [o0, p, o2, q] if sign > 0 else [o0, q, o2, p]


class _Pacer:
    def __init__(self, tasks, ntokens):
        self.slots = {}
        for n, task in enumerate(tasks):
            self.slots.setdefault(n * ntokens // len(tasks), []).append(task)
        self.pos = 0

    def feed(self, r):
        for j in range(r.shape[0] // 8):
            for task in self.slots.pop(self.pos, []):
                task(pltpu.bitcast(r[8 * j:8 * j + 8], u32))
            self.pos += 1

    def done(self):
        assert not self.slots


def _pack_rows(m):
    b = np.asarray(m, np.float32).astype(jnp.bfloat16).view(np.uint16).astype(np.uint32)
    return b[..., 0::2, :] | (b[..., 1::2, :] << 16)


@functools.lru_cache(maxsize=None)
def _dft_constants():
    b8 = np.array(_fwd8(list(np.eye(8)))).T
    n = np.arange(D)
    fw = np.zeros((D, D))
    bw = np.zeros((D, D))
    for g in range(4):
        k = np.concatenate([8 * np.arange(64) + r for r in RES[g]])
        ang = 2 * np.pi * ((n[:, None] * k[None, :]) % D) / D
        wgt = np.where(k == 0, 1.0, 2.0) / (D * S)
        fw[:, 256 * g:256 * g + 128] = np.cos(ang)
        fw[:, 256 * g + 128:256 * g + 256] = -np.sin(ang)
        bw[256 * g:256 * g + 128] = (np.cos(ang) * wgt).T
        bw[256 * g + 128:256 * g + 256] = (-np.sin(ang) * wgt).T
    bw[128, :] = (-1.0) ** n / (D * S)
    binv = np.kron(np.linalg.inv(b8), np.eye(128))
    gall = binv @ fw
    giall = bw @ binv.T
    gf = np.zeros((11, 144, 128))
    gi = np.zeros((11, 128, 128))
    sign = []
    half = lambda m, q: np.concatenate([m[64 * q:64 * q + 64], m[128 + 64 * q:192 + 64 * q]])
    for g in range(4):
        sl = slice(256 * g, 256 * g + 256)
        f, b = gall[sl, sl].T, giall[sl, sl]
        if g == 0:
            for q in range(2):
                gf[q, :128] = half(f, q)[:, 128 * q:128 * q + 128]
                gi[q] = half(b, q)[:, 128 * q:128 * q + 128]
            gf[0, 128] = (-1.0) ** np.arange(128)
            continue
        sg = np.sign(f[:128, 0] * f[128:, 128])[:, None]
        sign.append((int(sg[0, 0]), int(sg[64, 0])))
        p, q, r = f[:128, :128], f[:128, 128:], f[128:, :128]
        gf[3 * g - 1:3 * g + 2, :128] = p, q - p, r - sg * p
        p, q, r = b[:128, :128], b[:128, 128:], b[128:, :128]
        gi[3 * g - 1:3 * g + 2] = p, r - sg * p, q - p
    a = np.arange(128)
    mt = np.zeros((4, 16, 128, 128))
    for b in range(16):
        ang = 2 * np.pi * (((16 * a[:, None] + b) * a[None, :]) % S) / S
        c, sn = np.cos(ang), -np.sin(ang)
        mt[:, b] = c, c + sn, sn - c, sn
    return _pack_rows(gf), _pack_rows(gi), _pack_rows(mt), tuple(sign)


def _attn_fill():
    pos32 = np.concatenate([np.arange(8), np.arange(16, 40)])
    last = np.arange(16)
    qhead = np.concatenate([np.arange(64) // 32, last // 8])
    khead = np.concatenate([np.arange(64) // 32, last % 2])
    qpos = np.concatenate([pos32, pos32, 8 + last % 8])
    kpos = np.concatenate([pos32, pos32, 8 + last // 2])
    ok = (qpos[:, None] < M) | (qpos[:, None] >= kpos[None, :])
    fill = np.where(ok, 0.0, -1e9)
    fill = np.where(qhead[:, None] == khead[None, :], fill, -np.inf)
    return fill.astype(np.float32)


def _strassen(prod, b11, b12, b21, b22, add, sub, emit):
    m1 = prod(0, add(b11(), b22()))
    m2 = prod(1, b11())
    m3 = prod(2, sub(b12(), b22()))
    c22 = prod(5, add(b11(), b12())) + ((m1 - m2) + m3)
    m4 = prod(3, sub(b21(), b11()))
    emit(1, m2 + m4, c22)
    m5 = prod(4, b22())
    emit(0, prod(6, add(b21(), b22())) + ((m1 + m4) - m5), m3 + m5)


def _strassen_left(a11, a12, a21, a22):
    return [a11 + a22, a21 + a22, a11, a22, a11 + a12, a21 - a11, a12 - a22]


def _kernel(x_hbm, mem_hbm, wq_hbm, wk_hbm, wv_hbm, wo_hbm, bx_hbm, wr_hbm, wi_hbm,
            gf_hbm, gi_hbm, mt_hbm, fill_hbm, out_hbm,
            wraw, wall, wo, xbuf, mem0, x8, xs, pre, osum, outbuf, fill_ref,
            xb, wt, wl, gf, gi, mt, xd, yb, sems, wsems, xsems):
    def start(src, dst, sem, priority=0):
        c = pltpu.make_async_copy(src, dst, sems.at[sem] if isinstance(sem, int) else sem)
        c.start(priority=priority)
        return c

    def wait_all(cs):
        for c in cs:
            c.wait()

    dot = functools.partial(jnp.dot, preferred_element_type=f32)
    dot_nt = lambda a, b: lax.dot_general(a, b, (((1,), (1,)), ((), ())), preferred_element_type=f32)
    cat = lambda *vs: jnp.concatenate(vs, axis=0)
    as_bf16 = lambda w: pltpu.bitcast(w, bf16)
    lo_f32 = lambda w: pltpu.bitcast(w << 16, f32)
    hi_f32 = lambda w: pltpu.bitcast(w & u32(0xFFFF0000), f32)
    pack2 = lambda a, b: pltpu.pack_elementwise([a, b], packed_dtype=bf16)
    add2 = lambda a, b: pack2(lo_f32(a) + lo_f32(b), hi_f32(a) + hi_f32(b))
    sub2 = lambda a, b: pack2(lo_f32(a) - lo_f32(b), hi_f32(a) - hi_f32(b))
    out4 = out_hbm.reshape(NSEG // 2, 2, SEG, 2 * D)
    w_hbm = (wq_hbm, wk_hbm, wv_hbm)

    def start_unit(u):
        return start(w_hbm[u // 2].at[:, :, u % 2], wraw.at[u % NRAW], wsems.at[u])

    def x_chunk(n):
        segs, rows = pl.ds(UNROLL * n, UNROLL), pl.ds(M, SEG - M)
        return pltpu.make_async_copy(x_hbm.at[segs, rows, :], xbuf.at[segs, rows, :], xsems.at[n])

    c_a = []
    for n in range(4):
        cols, rows = pl.ds(256 * n, 256), pl.ds(128 * n, 128)
        c_a.append([start(x_hbm.at[:, pl.ds(0, M), cols], x8.at[:, :, cols], n),
                    start(wq_hbm.at[rows, :, 0], wraw.at[0, rows], 4 + n)])
    x_chunk(0).start(priority=1)
    c_loop = [start(mem_hbm, mem0, 10, 1), start(fill_hbm, fill_ref, 11, 1)]
    c_loop += [start(wo_hbm.at[:, pl.ds(128 * j, 128)], wo.at[j], 12, 1) for j in range(8)]

    wraw32 = wraw.bitcast(u32)
    wt32 = wt.bitcast(u32)
    xb32 = xb.bitcast(u32)

    def relayout_row(src, dst, r, off, lo, hi):
        a, b = src[r, 0], src[r, 1]
        dst[pl.ds(off, 8, stride=WP), :] = (a & lo) | (b << 16)
        dst[pl.ds(off + 8 * WP, 8, stride=WP), :] = (a >> 16) | (b & hi)

    def relayout_tasks(u, r0=0, r1=D // 2):
        src, dst = wraw32.at[u % NRAW], wall.at[u]

        def make(r):
            def task(tok):
                lo = (tok >> 16) | u32(0xFFFF)
                hi = (tok << 16) | u32(0xFFFF0000)
                relayout_row(src, dst, r, r, lo, hi)
                relayout_row(src, dst, r + 1, r + 1, lo, hi)
            return task
        return [make(r) for r in range(r0, r1, 2)]

    def filter_tasks(rows, wfn):
        def make(phase, k):
            slots = [4 * k + j for j in range(4)] if phase == 1 else [4 * j + k for j in range(4)]

            def task(tok):
                ones = ((tok >> 16) | u32(0xFFFF)) | u32(0xFFFF0000)
                z = [(yb[0, b, rows, :], yb[1, b, rows, :]) for b in slots]
                z[0] = tuple(pltpu.bitcast(pltpu.bitcast(v, u32) & ones, f32) for v in z[0])
                if phase == 0:
                    o = _bfly4(z, 1)
                    o = [_twiddle16(o[j], k * j) for j in range(4)]
                elif phase == 1:
                    o = _bfly4(z, 1)
                    y = []
                    for j in range(4):
                        wr, wi = wfn(k + 4 * j)
                        xr, xi = o[j]
                        y.append((xr * wr - xi * wi, xr * wi + xi * wr))
                    o = _bfly4(y, -1)
                    o = [_twiddle16(o[j], -k * j) for j in range(4)]
                else:
                    o = _bfly4(z, -1)
                for b, v in zip(slots, o):
                    yb[0, b, rows, :] = v[0]
                    yb[1, b, rows, :] = v[1]
            return task
        return [make(phase, k) for phase in range(3) for k in range(4)]

    def z_region(n, par):
        return (2 * n + par) // 3, (2 * n + par) % 3 * 8 * ZP

    def butterfly_tasks(par):
        def make(a2):
            def task(tok):
                zs = []
                for a in (2 * a2, 2 * a2 + 1):
                    w = [xb32[j, pl.ds(8 * a, 8), :] for j in range(8)]
                    if par:
                        hi = (tok << 16) | u32(0xFFFF0000)
                        z = _fwd8([pltpu.bitcast(v & hi, f32) for v in w])
                    else:
                        sixteen = ((tok >> 31) | u32(1)) << 4
                        z = _fwd8([pltpu.bitcast(v << sixteen, f32) for v in w])
                    zs.append(z[0:2] + [v for g in range(1, 4)
                                        for v in (z[2 * g] + z[2 * g + 1], z[2 * g + 1], z[2 * g])])
                for n in range(11):
                    plane, row = z_region(n, par)
                    xd[plane, pl.ds(row + a2, 8, stride=ZP), :] = pltpu.bitcast(pack2(zs[0][n], zs[1][n]), f32)
            return task
        return [make(a2) for a2 in range(64)]

    sign = _dft_constants()[3]

    def b_dfwd(b, pacer):
        def z(n):
            plane, row = z_region(n, b % 2)
            return as_bf16(xd[plane, pl.ds(row + b // 2 * ZP, 64), :])
        t0 = dot_nt(as_bf16(gf[0]), z(0))
        t4 = dot_nt(as_bf16(gf[1, 0:64]), z(1))
        tr, ti = cat(t0[0:64], t4[0:64]), cat(t0[64:128], t4[64:128])
        ts = [(cat(tr + ti, t0[128:144]).astype(bf16), ti.astype(bf16), cat(tr, t0[128:144]).astype(bf16))]
        for g in range(1, 4):
            k1, k2, k3 = [dot_nt(as_bf16(gf[n, 0:64]), z(n)) for n in range(3 * g - 1, 3 * g + 2)]
            pacer.feed(k1)
            tr = k1 + k2
            ti = cat(*[k3[64 * q:64 * q + 64] + k1[64 * q:64 * q + 64] if sign[g - 1][q] > 0
                       else k3[64 * q:64 * q + 64] - k1[64 * q:64 * q + 64] for q in range(2)])
            ts.append(((tr + ti).astype(bf16), ti.astype(bf16), tr.astype(bf16)))
        return ts

    def b_sfwd(b, ts, pacer):
        for g in range(4):
            k1, k2, k3 = [dot(ts[g][n], as_bf16(mt[n, b])) for n in range(3)]
            if g:
                pacer.feed(k2)
            yi = k1 + k3
            yb[0, b, pl.ds(128 * g, 128), :] = k1[0:128] - k2
            yb[1, b, pl.ds(128 * g, 128), :] = yi[0:128]
            if g == 0:
                yb[0, b, pl.ds(512, 8), :] = k1[128:136]
                yb[1, b, pl.ds(512, 8), :] = yi[128:136]

    def b_stage1():
        pacer = _Pacer(butterfly_tasks(1), 14 * 48)
        prev = None
        for b in list(range(0, 16, 2)) + list(range(1, 16, 2)):
            ts = b_dfwd(b, pacer)
            if prev is not None:
                b_sfwd(*prev, pacer)
            prev = (b, ts)
        b_sfwd(*prev, pacer)
        pacer.done()

    def b_stage3():
        row0 = lax.broadcasted_iota(jnp.int32, (8, 128), 0) == 0
        low = lax.broadcasted_iota(jnp.int32, (1, 128), 1) < 64
        for b in range(16):
            m = [as_bf16(mt[n, b]) for n in range(4)]
            for g in (1, 2, 3, 0):
                yr, yi = yb[0, b, pl.ds(128 * g, 128), :], yb[1, b, pl.ds(128 * g, 128), :]
                if g == 0:
                    nr = -yr
                    u0 = cat(yr[0:64], jnp.where(row0, yb[0, b, pl.ds(512, 8), :], yi[0:8]), yi[8:64])
                    v0 = cat(yi[0:64], jnp.where(row0, yb[1, b, pl.ds(512, 8), :], nr[0:8]), nr[8:64])
                    u4, v4 = cat(yr[64:128], yi[64:128]), cat(yi[64:128], nr[64:128])
                    t1 = dot_nt(m[0], u0.astype(bf16)) + dot_nt(m[3], v0.astype(bf16))
                    t2 = dot_nt(m[0], u4.astype(bf16)) + dot_nt(m[3], v4.astype(bf16))
                else:
                    k1, k2, k3 = [dot_nt(m[n], v.astype(bf16)) for n, v in enumerate((yr + yi, yr, yi))]
                    t1, t2 = k1 + k3, k1 - k2
                slot = b // 2 + 8 * (b % 2)
                xd[2 * g, pl.ds(XP * slot, 128), :] = t1
                xd[2 * g + 1, pl.ds(XP * slot, 128), :] = t2
        for t in range(16):
            rows = lambda j: cat(*[xd[j, pl.ds(8 * t + u, 16, stride=XP), :] for u in range(8)])
            z = [dot(rows(q).astype(bf16), as_bf16(gi[q])) for q in range(2)]
            for g in range(1, 4):
                tr, ti = rows(2 * g), rows(2 * g + 1)
                sg = jnp.where(low, float(sign[g - 1][0]), float(sign[g - 1][1]))
                k1, k2, k3 = [dot(v.astype(bf16), as_bf16(gi[3 * g - 1 + n]))
                              for n, v in enumerate((tr + sg * ti, ti, tr))]
                z += [k1 + k2, k1 + k3]
            y = _inv8(z)
            for j in range(8):
                even = cat(*[y[j][16 * u:16 * u + 8] for u in range(8)])
                odd = cat(*[y[j][16 * u + 8:16 * u + 16] for u in range(8)])
                xb32[j, pl.ds(64 * t, 64), :] = pack2(even, odd)

    HALF = NSEG * M // 2

    def batch(u, p0, p1, tasks=(), t0=0, t1=4, query=False):
        pacer = _Pacer(tasks, (7 * (p1 - p0) - 2) * HALF // 8)
        w = wall.at[u]
        for p in range(p0, p1):
            def blk(head, par):
                return lambda: cat(*[w[pl.ds((p + 8 * head) * WP + 64 * (2 * t + par), 64), :]
                                     for t in range(t0, t1)])

            def prod(i, b):
                lhs = jnp.concatenate([as_bf16(xs[i, t]) for t in range(t0, t1)], axis=1)
                r = dot(lhs, as_bf16(b))
                pacer.feed(r)
                return r

            def emit(half, *cs):
                rows = pl.ds(half * HALF, HALF)
                if t0 > 0:
                    cs = [c + yb[t, p, rows, :] for t, c in enumerate(cs)]
                if t1 < 4:
                    for t, c in enumerate(cs):
                        yb[t, p, rows, :] = c
                elif query:
                    st = jnp.concatenate([c.reshape(HALF // M, M, E) for c in cs], axis=1)
                    pre[8 * u + p, rows, :] = pltpu.bitcast(st.reshape(2 * HALF, E).astype(bf16), u32)
                else:
                    pre[8 * u + p, rows, :] = pack2(*cs)
            _strassen(prod, blk(0, 0), blk(1, 0), blk(0, 1), blk(1, 1), add2, sub2, emit)
        pacer.done()

    def prepare_quarter(n):
        def body(t, c):
            off = pl.multiple_of(128 * n + 16 * t, 16)
            dst = wall.at[0, pl.ds(off, 15 * WP + 20)]
            for r in range(16):
                relayout_row(wraw32.at[0], dst, off + r, r, u32(0xFFFF), u32(0xFFFF0000))
            return c
        lax.fori_loop(0, 8, body, 0)
        v = pltpu.bitcast(x8[:, :, pl.ds(256 * n, 256)].reshape(2 * HALF, 256), u32)
        blocks = [v[HALF // 2 * h:HALF // 2 * (h + 1), 128 * k:128 * (k + 1)] for h in range(2) for k in range(2)]
        lo, hi = [_strassen_left(*[un(b) for b in blocks]) for un in (lo_f32, hi_f32)]
        for i in range(7):
            xs[i, n] = pack2(lo[i], hi[i])

    wait_all(c_a[0])
    prepare_quarter(0)
    batch(0, 0, 8, (), 0, 1)
    wait_all(c_a[1])
    c_h = [start(wq_hbm.at[pl.ds(256 * n, 256), :, 1], wraw.at[1, pl.ds(256 * n, 256)], 8 + n) for n in range(2)]
    prepare_quarter(1)
    batch(0, 0, 8, (), 1, 2)
    wait_all(c_a[2])
    prepare_quarter(2)
    wait_all(c_a[3])
    prepare_quarter(3)
    batch(0, 0, 6, (), 2, 4, query=True)
    c_h[0].wait()
    c_w2 = start_unit(2)
    batch(0, 6, 8, relayout_tasks(1, 0, 256), 2, 4, query=True)
    batch(1, 0, 5, (), 0, 2)
    c_h[1].wait()
    start_unit(3)
    batch(1, 5, 8, relayout_tasks(1, 256, 512), 0, 2)
    batch(1, 0, 5, (), 2, 4, query=True)
    c_w2.wait()
    start_unit(4)
    start_unit(5)
    c_b1 = [start(bx_hbm.at[:, pl.ds(128 * j, 128)], xb.at[j], 18) for j in range(8)]
    c_b1 += [start(gf_hbm, gf, 19), start(mt_hbm.at[pl.ds(0, 3)], mt.at[pl.ds(0, 3)], 20)]
    c_loop += [start(w.at[pl.ds(0, 512), pl.ds(128 * d, 128)], wt.at[t, d], 13, 1)
               for t, w in enumerate((wr_hbm, wi_hbm)) for d in range(16)]
    batch(1, 5, 8, relayout_tasks(2), 2, 4, query=True)
    batch(2, 0, 4)

    def unit_body(u, c):
        slot = wraw.at[(u + 1) % NRAW]
        pltpu.make_async_copy(slot, slot, wsems.at[u + 1]).wait()
        batch(u, 4, 8, relayout_tasks(u + 1))
        batch(u + 1, 0, 4)
        return c
    lax.fori_loop(2, 5, unit_body, 0)
    wait_all(c_b1)
    batch(5, 4, 8, butterfly_tasks(0))
    b_stage1()
    wait_all(c_loop)
    for n in range(1, NSEG // UNROLL):
        x_chunk(n).start()
    c_b3 = [start(w.at[pl.ds(512, 1), :], wl.at[t], 14 + t) for t, w in enumerate((wr_hbm, wi_hbm))]
    c_b3 += [start(gi_hbm, gi, 16), start(mt_hbm.at[3], mt.at[3], 17)]

    wo32 = wo.bitcast(u32)
    scale = E ** -0.5

    def gated(w, toks):
        if not toks:
            return w
        bits = functools.reduce(
            jnp.bitwise_or, [pltpu.bitcast(jnp.broadcast_to(t, (8, 128)), u32) for t in toks])
        ones = ((bits >> 16) | u32(0xFFFF)) | u32(0xFFFF0000)
        return cat(w[0:8] & ones, w[8:])

    def wqkv(i, p, second, toks=(), k0=0, k1=D):
        rows = pl.ds((p % 8 + 8 * second) * WP + k0 // 2, (k1 - k0) // 2)
        return as_bf16(gated(wall[2 * i + p // 8, rows, :], toks))

    def step(n, u, mem, held):
        s = UNROLL * n + u
        rows = cat(mem, xbuf[s, pl.ds(M, SEG - M), :].astype(f32))
        lhs = rows.astype(bf16)
        head_start = {}
        if u:
            lo, hi = rows[:, :D // 2].astype(bf16), rows[:, D // 2:].astype(bf16)
            for key in EARLY:
                head_start[key] = dot(lo, wqkv(*key, k1=D // 2))
        r8 = pl.multiple_of(M * s, M)
        fill = fill_ref[...]
        heads = [None] * H
        rs = []

        i8, par = n // 2, n % 2
        base = [128 * g + 64 * q for r in (2 * u, 2 * u + 1) for g in range(4) for q in range(2) if RES[g][q] == r]
        shift = jnp.full((8, 128), 16 - 16 * par, jnp.int32).astype(u32)
        wblk = pl.ds(pl.multiple_of(32 * i8, 32), 32)
        pacer = _Pacer(filter_tasks(
            pl.ds(pl.multiple_of(base[0] + par * (base[1] - base[0]) + 8 * i8, 8), 8),
            lambda d: [hi_f32(wt32.at[t, d, wblk][pl.ds(u, 8, stride=4), :] << shift) for t in range(2)]), FTOK)

        def proj(i, p, toks=()):
            a, b = [
                dot(hi, wqkv(i, p, t, k0=D // 2)) + head_start[i, p, t] if (i, p, t) in head_start
                else dot(lhs, wqkv(i, p, t, toks[t * len(toks) // 2:(t + 1) * len(toks) // 2]))
                for t in range(2)]
            pacer.feed(a)
            pacer.feed(b)
            c = as_bf16(pre[16 * i + p, pl.ds(r8, M), :]).astype(f32)
            return cat(a, b, c).astype(bf16)

        def probs(q, k):
            sc = dot_nt(q, k) * scale
            sc = jnp.where(fill == 0.0, sc, fill)
            e = jnp.exp(sc - jnp.max(sc, axis=1, keepdims=True))
            l = jnp.sum(e, axis=1, keepdims=True)
            r = pl.reciprocal(l, approx=True)
            r = r * (2.0 - l * r)
            rs.append([r[8 * j:8 * j + 8] for j in range(10)])
            return (e * r).astype(bf16)

        def pv(p, pr, v):
            o = dot(pr, v)
            heads[2 * p] = o[0:32]
            heads[2 * p + 1] = o[32:64]
            held[u % 2, p] = (o[64:72], o[72:80])

        def left_task(p):
            def task(tok):
                ones = ((tok >> 16) | u32(0xFFFF)) | u32(0xFFFF0000)
                a11, a12, a21, a22 = held[0, p] + held[1, p]
                a11, a22 = [pltpu.bitcast(pltpu.bitcast(a, u32) & ones, f32) for a in (a11, a22)]
                dst = pl.ds(pl.multiple_of(M * (UNROLL // 2 * n + u // 2), M), M)
                for i, a in enumerate(_strassen_left(a11, a12, a21, a22)):
                    osum[i, p, dst, :] = a.astype(bf16)
            return task

        pend = []
        for g in range(4):
            ps = range(4 * g, 4 * g + 4)
            qk = [(proj(0, p), proj(1, p)) for p in ps]
            vs = [proj(2, p, rs[p - 4] if g else ()) for p in ps]
            for a in pend:
                pv(*a)
            pend = [(p, probs(*qk[t]), vs[t]) for t, p in enumerate(ps)]
        pacer.done()

        def wo_part(oc, j, h0, h1, toks=()):
            return dot(oc, as_bf16(gated(wo32[j, pl.ds(64 * h0, 64 * (h1 - h0)), :], toks)))

        acc = []
        pacer = _Pacer([left_task(p) for p in range(16)] if u % 2 else (), 4 * 10)
        oc = jnp.concatenate(heads[0:24], axis=1).astype(bf16)
        for j in range(8):
            acc.append(wo_part(oc, j, 0, 24, {3: rs[12] + rs[13], 4: rs[14] + rs[15]}.get(j, ())))
            if j == 4:
                for a in pend:
                    pv(*a)
            if j > 5:
                pacer.feed(acc[j])
        oc = jnp.concatenate(heads[24:32], axis=1).astype(bf16)
        nxt = []
        for j in range(8):
            r = wo_part(oc, j, 24, 32) + acc[j]
            outbuf[UNROLL // 2 * n + u // 2, u % 2, pl.ds(M, SEG - M), pl.ds(128 * j, 128)] = r[M:].astype(bf16)
            nxt.append(r[0:M])
            pacer.feed(r)
        pacer.done()
        return jnp.concatenate(nxt, axis=1)

    def steps(n, mem):
        x_chunk(n).wait()
        held = {}
        for u in range(UNROLL):
            mem = step(n, u, mem, held)
        return mem
    lax.fori_loop(0, NSEG // UNROLL, steps, mem0[...].astype(f32))
    tok_rows = pl.ds(M, SEG - M)
    c_out = [start(outbuf.at[:, :, tok_rows, :], out4.at[:, :, tok_rows, pl.ds(0, D)], 21)]

    wait_all(c_b3)
    for task in filter_tasks(pl.ds(512, 8), lambda d: [wl[t, :, pl.ds(128 * d, 128)].astype(f32) for t in range(2)]):
        task(jnp.zeros((8, 128), u32))
    b_stage3()
    c_out += [start(xb.at[j], out_hbm.at[:, pl.ds(D + 128 * j, 128)], 22) for j in range(8)]

    osum32 = osum.bitcast(u32)
    for jp in range(4):
        def blk(col, par):
            return lambda: cat(*[wo32[2 * jp + col, pl.ds(64 * (2 * p + par), 64), :] for p in range(16)])

        def prod(i, b):
            return dot(jnp.concatenate([as_bf16(osum32[i, p]) for p in range(16)], axis=1), as_bf16(b))

        def emit(half, *cs):
            for t, c in enumerate(cs):
                outbuf[:, half, pl.ds(0, M), pl.ds(128 * (2 * jp + t), 128)] = (
                    c.reshape(NSEG // 2, M, 128).astype(bf16))
            cols = pl.ds(256 * jp, 256)
            c_out.append(start(outbuf.at[:, half, pl.ds(0, M), cols], out4.at[:, half, pl.ds(0, M), cols],
                               23 + 2 * jp + half))
        _strassen(prod, blk(0, 0), blk(1, 0), blk(0, 1), blk(1, 1), add2, sub2, emit)
    wait_all(c_out)


@functools.partial(jax.jit, static_argnames=("A_seg_len",))
def pallas_concat_heads__memory_aug_recurrent_mem_tr__spectral_gfnet__prompt_kernel(
    A_x: jax.Array,
    A_mem0: jax.Array,
    A_Wq: jax.Array,
    A_Wk: jax.Array,
    A_Wv: jax.Array,
    A_Wo: jax.Array,
    A_seg_len,
    B_x: jax.Array,
    B_w_r: jax.Array,
    B_w_i: jax.Array,
):
    assert A_seg_len == SEG
    assert A_x.shape == (1, S, D) and A_mem0.shape == (1, M, D) and B_x.shape == (1, S, D)
    assert A_Wq.shape == (D, H, E) and A_Wo.shape == (H, E, D) and B_w_r.shape == (S, D // 2 + 1)
    gf, gi, mt, _ = _dft_constants()
    fill = _attn_fill()
    hbm = pl.BlockSpec(memory_space=pltpu.HBM)
    wshape = (D // 2, 2, 2, 16, E)
    out = pl.pallas_call(
        _kernel,
        out_shape=jax.ShapeDtypeStruct((S, 2 * D), bf16),
        in_specs=[hbm] * 13,
        out_specs=hbm,
        scratch_shapes=[
            pltpu.VMEM((NRAW, D // 2, 2, 16, E), bf16),
            pltpu.VMEM((6, 16 * WP, E), u32),
            pltpu.VMEM((8, H * E, 128), bf16),
            pltpu.VMEM((NSEG, SEG, D), bf16),
            pltpu.VMEM((M, D), bf16),
            pltpu.VMEM((NSEG, M, D), bf16),
            pltpu.VMEM((7, 4, 128, 128), u32),
            pltpu.VMEM((48, NSEG * M, E), u32),
            pltpu.VMEM((7, 16, NSEG * M // 2, E), bf16),
            pltpu.VMEM((NSEG // 2, 2, SEG, D), bf16),
            pltpu.VMEM(fill.shape, f32),
            pltpu.VMEM((8, S, 128), bf16),
            pltpu.VMEM((2, 16, 512, 128), bf16),
            pltpu.VMEM((2, 1, S), bf16),
            pltpu.VMEM(gf.shape, u32),
            pltpu.VMEM(gi.shape, u32),
            pltpu.VMEM(mt.shape, u32),
            pltpu.VMEM((8, 16 * XP, 128), f32),
            pltpu.VMEM((2, 16, YR, 128), f32),
            pltpu.SemaphoreType.DMA((32,)),
            pltpu.SemaphoreType.DMA((6,)),
            pltpu.SemaphoreType.DMA((NSEG // UNROLL,)),
        ],
        compiler_params=pltpu.CompilerParams(vmem_limit_bytes=120 * 1024 * 1024),
    )(A_x.reshape(NSEG, SEG, D), A_mem0.reshape(M, D),
      A_Wq.reshape(wshape), A_Wk.reshape(wshape), A_Wv.reshape(wshape),
      A_Wo.reshape(H * E, D), B_x.reshape(S, D), B_w_r.T, B_w_i.T, gf, gi, mt, fill)
    return out.reshape(1, S, 2 * D)
```

```python
import functools

import jax
import jax.numpy as jnp
import numpy as np
from jax import lax
from jax.experimental import pallas as pl
from jax.experimental.pallas import tpu as pltpu

S, D, H, E, M, SEG = 2048, 1024, 32, 128, 8, 32
NSEG = S // SEG
WP = 516
XP = 132
ZP = 68
NRAW = 4
UNROLL = 4
MCT = 1
MARGIN = 8
EARLY = ((0, 0, 0), (0, 0, 1), (1, 0, 0), (1, 0, 1), (0, 1, 0), (0, 1, 1))
bf16, f32, u32 = jnp.bfloat16, jnp.float32, jnp.uint32
RES = ((0, 4), (2, 6), (1, 7), (3, 5))
RC = float(np.sqrt(0.5))


def _fwd8(x):
    s04, d04 = x[0] + x[4], x[0] - x[4]
    s26, d26 = x[2] + x[6], x[2] - x[6]
    s15, d15 = x[1] + x[5], x[1] - x[5]
    s37, d37 = x[3] + x[7], x[3] - x[7]
    t1, t2 = (d15 - d37) * RC, (d15 + d37) * RC
    e0, o0 = s04 + s26, s15 + s37
    return [e0 + o0, e0 - o0, s04 - s26, s15 - s37, d04 + t1, d26 + t2, d04 - t1, d26 - t2]


def _inv8(z):
    z0, z4, e1, o1, r1, i1, r3, i3 = z
    e0, o0 = z0 + z4, z0 - z4
    s04, s26, s15, s37 = e0 + e1, e0 - e1, o0 + o1, o0 - o1
    d04, d26 = r1 + r3, i1 + i3
    t1, t2 = (r1 - r3) * RC, (i1 - i3) * RC
    d15, d37 = t1 + t2, t2 - t1
    return [s04 + d04, s15 + d15, s26 + d26, s37 + d37, s04 - d04, s15 - d15, s26 - d26, s37 - d37]


def _twiddle16(z, k):
    re, im = z
    k = k % 16
    if k == 0:
        return z
    if k == 4:
        return (im, -re)
    if k == 12:
        return (-im, re)
    if k == 2:
        return ((re + im) * RC, (im - re) * RC)
    if k == 14:
        return ((re - im) * RC, (re + im) * RC)
    if k == 6:
        return ((im - re) * RC, (re + im) * -RC)
    if k == 10:
        return ((re + im) * -RC, (re - im) * RC)
    c, s = float(np.cos(2 * np.pi * k / 16)), float(-np.sin(2 * np.pi * k / 16))
    return (re * c - im * s, re * s + im * c)


def _bfly4(z, sign):
    (ar, ai), (br, bi), (cr, ci), (dr, di) = z
    sr, si, tr, ti = ar + cr, ai + ci, ar - cr, ai - ci
    ur, ui, vr, vi = br + dr, bi + di, br - dr, bi - di
    o0, o2 = (sr + ur, si + ui), (sr - ur, si - ui)
    p, q = (tr + vi, ti - vr), (tr - vi, ti + vr)
    return [o0, p, o2, q] if sign > 0 else [o0, q, o2, p]


class _Pacer:
    def __init__(self, tasks, ntokens):
        self.slots = {}
        for n, task in enumerate(tasks):
            self.slots.setdefault(n * ntokens // len(tasks), []).append(task)
        self.pos = 0

    def feed(self, r):
        for j in range(r.shape[0] // 8):
            for task in self.slots.pop(self.pos, []):
                task(pltpu.bitcast(r[8 * j:8 * j + 8], u32))
            self.pos += 1

    def done(self):
        assert not self.slots


def _pack_rows(m):
    b = np.asarray(m, np.float32).astype(jnp.bfloat16).view(np.uint16).astype(np.uint32)
    return b[..., 0::2, :] | (b[..., 1::2, :] << 16)


@functools.lru_cache(maxsize=None)
def _dft_constants():
    b8 = np.array(_fwd8(list(np.eye(8)))).T
    n = np.arange(D)
    fw = np.zeros((D, D))
    bw = np.zeros((D, D))
    for g in range(4):
        k = np.concatenate([8 * np.arange(64) + r for r in RES[g]])
        ang = 2 * np.pi * ((n[:, None] * k[None, :]) % D) / D
        wgt = np.where(k == 0, 1.0, 2.0) / (D * S)
        fw[:, 256 * g:256 * g + 128] = np.cos(ang)
        fw[:, 256 * g + 128:256 * g + 256] = -np.sin(ang)
        bw[256 * g:256 * g + 128] = (np.cos(ang) * wgt).T
        bw[256 * g + 128:256 * g + 256] = (-np.sin(ang) * wgt).T
    bw[128, :] = (-1.0) ** n / (D * S)
    binv = np.kron(np.linalg.inv(b8), np.eye(128))
    gall = binv @ fw
    giall = bw @ binv.T
    gf = np.zeros((11, 144, 128))
    gi = np.zeros((11, 128, 128))
    sign = []
    half = lambda m, q: np.concatenate([m[64 * q:64 * q + 64], m[128 + 64 * q:192 + 64 * q]])
    for g in range(4):
        sl = slice(256 * g, 256 * g + 256)
        f, b = gall[sl, sl].T, giall[sl, sl]
        if g == 0:
            for q in range(2):
                gf[q, :128] = half(f, q)[:, 128 * q:128 * q + 128]
                gi[q] = half(b, q)[:, 128 * q:128 * q + 128]
            gf[0, 128] = (-1.0) ** np.arange(128)
            continue
        sg = np.sign(f[:128, 0] * f[128:, 128])[:, None]
        sign.append((int(sg[0, 0]), int(sg[64, 0])))
        p, q, r = f[:128, :128], f[:128, 128:], f[128:, :128]
        gf[3 * g - 1:3 * g + 2, :128] = p, q - p, r - sg * p
        p, q, r = b[:128, :128], b[:128, 128:], b[128:, :128]
        gi[3 * g - 1:3 * g + 2] = p, r - sg * p, q - p
    a = np.arange(128)
    mt = np.zeros((4, 16, 128, 128))
    for b in range(16):
        ang = 2 * np.pi * (((16 * a[:, None] + b) * a[None, :]) % S) / S
        c, sn = np.cos(ang), -np.sin(ang)
        mt[:, b] = c, c + sn, sn - c, sn
    return _pack_rows(gf), _pack_rows(gi), _pack_rows(mt), tuple(sign)


def _attn_fill():
    pos32 = np.concatenate([np.arange(8), np.arange(16, 40)])
    last = np.arange(16)
    qhead = np.concatenate([np.arange(64) // 32, last // 8])
    khead = np.concatenate([np.arange(64) // 32, last % 2])
    qpos = np.concatenate([pos32, pos32, 8 + last % 8])
    kpos = np.concatenate([pos32, pos32, 8 + last // 2])
    ok = (qpos[:, None] < M) | (qpos[:, None] >= kpos[None, :])
    fill = np.where(ok, 0.0, -1e9)
    fill = np.where(qhead[:, None] == khead[None, :], fill, -np.inf)
    return fill.astype(np.float32)


def _strassen(prod, b11, b12, b21, b22, add, sub, emit):
    m2 = prod(1, b11())
    m1 = prod(0, add(b11(), b22()))
    m3 = prod(2, sub(b12(), b22()))
    c22 = prod(5, add(b11(), b12())) + ((m1 - m2) + m3)
    m4 = prod(3, sub(b21(), b11()))
    emit(1, m2 + m4, c22)
    m5 = prod(4, b22())
    emit(0, prod(6, add(b21(), b22())) + ((m1 + m4) - m5), m3 + m5)


def _strassen_left(a11, a12, a21, a22):
    return [a11 + a22, a21 + a22, a11, a22, a11 + a12, a21 - a11, a12 - a22]


def _kernel(x_hbm, mem_hbm, wq_hbm, wk_hbm, wv_hbm, wo_hbm, bx_hbm, wr_hbm, wi_hbm,
            gf_hbm, gi_hbm, mt_hbm, fill_hbm, out_hbm,
            wraw, wall, wo, xbuf, mem0, x8, xs, pre, osum, outbuf, fill_ref,
            xb, wt, wl, gf, gi, mt, xd, yb, sems):
    def start(src, dst, sem, priority=0):
        c = pltpu.make_async_copy(src, dst, sems.at[sem])
        c.start(priority=priority)
        return c

    def wait_all(cs):
        for c in cs:
            c.wait()

    dot = functools.partial(jnp.dot, preferred_element_type=f32)
    dot_nt = lambda a, b: lax.dot_general(a, b, (((1,), (1,)), ((), ())), preferred_element_type=f32)
    cat = lambda *vs: jnp.concatenate(vs, axis=0)
    as_bf16 = lambda w: pltpu.bitcast(w, bf16)
    lo_f32 = lambda w: pltpu.bitcast(w << 16, f32)
    hi_f32 = lambda w: pltpu.bitcast(w & u32(0xFFFF0000), f32)
    pack2 = lambda a, b: pltpu.pack_elementwise([a, b], packed_dtype=bf16)
    add2 = lambda a, b: pack2(lo_f32(a) + lo_f32(b), hi_f32(a) + hi_f32(b))
    sub2 = lambda a, b: pack2(lo_f32(a) - lo_f32(b), hi_f32(a) - hi_f32(b))
    out4 = out_hbm.reshape(NSEG // 2, 2, SEG, 2 * D)
    w_hbm = (wq_hbm, wk_hbm, wv_hbm)

    def start_unit(u):
        return start(w_hbm[u // 2].at[:, :, u % 2], wraw.at[u % NRAW], u % NRAW)

    def start_x(seg0, nseg, sem, priority=0):
        segs, rows = pl.ds(seg0, nseg), pl.ds(M, SEG - M)
        return start(x_hbm.at[segs, rows, :], xbuf.at[segs, rows, :], sem, priority)

    c_a = []
    for n in range(4):
        cols, rows = pl.ds(256 * n, 256), pl.ds(128 * n, 128)
        c_a.append([start(x_hbm.at[:, pl.ds(0, M), cols], x8.at[:, :, cols], n),
                    start(wq_hbm.at[rows, :, 0], wraw.at[0, rows], n)])
    c_loop = [start_x(0, UNROLL, 4, 1), start(mem_hbm, mem0, 4, 1), start(fill_hbm, fill_ref, 4, 1)]
    c_loop += [start(wo_hbm.at[:, pl.ds(128 * j, 128)], wo.at[j], 4, 1) for j in range(8)]

    wraw32 = wraw.bitcast(u32)
    wt32 = wt.bitcast(u32)
    xb32 = xb.bitcast(u32)

    def relayout_row(src, dst, r, lo, hi):
        a, b = src[r, 0], src[r, 1]
        dst[pl.ds(r, 8, stride=WP), :] = (a & lo) | (b << 16)
        dst[pl.ds(r + 8 * WP, 8, stride=WP), :] = (a >> 16) | (b & hi)

    def relayout_tasks(u, r0=0, r1=D // 2):
        src, dst = wraw32.at[u % NRAW], wall.at[u]

        def make(r):
            def task(tok):
                lo = (tok >> 16) | u32(0xFFFF)
                hi = (tok << 16) | u32(0xFFFF0000)
                relayout_row(src, dst, r, lo, hi)
                relayout_row(src, dst, r + 1, lo, hi)
            return task
        return [make(r) for r in range(r0, r1, 2)]

    def y_blocks(r):
        return pl.ds(4 * (r % 2) + r // 2, 8, stride=8)

    def filter_tasks(blk, wfn):
        def make(phase, k):
            slots = [4 * k + j for j in range(4)] if phase == 1 else [4 * j + k for j in range(4)]

            def task(tok):
                ones = ((tok >> 16) | u32(0xFFFF)) | u32(0xFFFF0000)
                z = [(yb[0, b, blk], yb[1, b, blk]) for b in slots]
                z[0] = tuple(pltpu.bitcast(pltpu.bitcast(v, u32) & ones, f32) for v in z[0])
                if phase == 0:
                    o = _bfly4(z, 1)
                    o = [_twiddle16(o[j], k * j) for j in range(4)]
                elif phase == 1:
                    o = _bfly4(z, 1)
                    y = []
                    for j in range(4):
                        wr, wi = wfn(k + 4 * j)
                        xr, xi = o[j]
                        y.append((xr * wr - xi * wi, xr * wi + xi * wr))
                    o = _bfly4(y, -1)
                    o = [_twiddle16(o[j], -k * j) for j in range(4)]
                else:
                    o = _bfly4(z, -1)
                for b, v in zip(slots, o):
                    yb[0, b, blk] = v[0]
                    yb[1, b, blk] = v[1]
            return task
        return [make(phase, k) for phase in range(3) for k in range(4)]

    def z_region(n, par):
        return (2 * n + par) // 3, (2 * n + par) % 3 * 8 * ZP

    def butterfly_tasks(par):
        def make(a2):
            def task(tok):
                zs = []
                for a in (2 * a2, 2 * a2 + 1):
                    w = [xb32[j, pl.ds(8 * a, 8), :] for j in range(8)]
                    if par:
                        hi = (tok << 16) | u32(0xFFFF0000)
                        z = _fwd8([pltpu.bitcast(v & hi, f32) for v in w])
                    else:
                        sixteen = ((tok >> 31) | u32(1)) << 4
                        z = _fwd8([pltpu.bitcast(v << sixteen, f32) for v in w])
                    zs.append(z[0:2] + [v for g in range(1, 4)
                                        for v in (z[2 * g] + z[2 * g + 1], z[2 * g + 1], z[2 * g])])
                for n in range(11):
                    plane, row = z_region(n, par)
                    xd[plane, pl.ds(row + a2, 8, stride=ZP), :] = pltpu.bitcast(pack2(zs[0][n], zs[1][n]), f32)
            return task
        return [make(a2) for a2 in range(64)]

    sign = _dft_constants()[3]

    def b_dfwd(b, pacer):
        def z(n):
            plane, row = z_region(n, b % 2)
            return as_bf16(xd[plane, pl.ds(row + b // 2 * ZP, 64), :])
        t0 = dot_nt(as_bf16(gf[0]), z(0))
        t4 = dot_nt(as_bf16(gf[1, 0:64]), z(1))
        tr, ti = cat(t0[0:64], t4[0:64]), cat(t0[64:128], t4[64:128])
        ts = [(cat(tr + ti, t0[128:144]).astype(bf16), ti.astype(bf16), cat(tr, t0[128:144]).astype(bf16))]
        for g in range(1, 4):
            k1, k2, k3 = [dot_nt(as_bf16(gf[n, 0:64]), z(n)) for n in range(3 * g - 1, 3 * g + 2)]
            pacer.feed(k1)
            tr = k1 + k2
            ti = cat(*[k3[64 * q:64 * q + 64] + k1[64 * q:64 * q + 64] if sign[g - 1][q] > 0
                       else k3[64 * q:64 * q + 64] - k1[64 * q:64 * q + 64] for q in range(2)])
            ts.append(((tr + ti).astype(bf16), ti.astype(bf16), tr.astype(bf16)))
        return ts

    def b_sfwd(b, ts, pacer):
        for g in range(4):
            k1, k2, k3 = [dot(ts[g][n], as_bf16(mt[n, b])) for n in range(3)]
            if g:
                pacer.feed(k2)
            yr, yi = k1[0:128] - k2, k1 + k3
            for q in range(2):
                yb[0, b, y_blocks(RES[g][q])] = yr[64 * q:64 * q + 64].reshape(8, 8, 128)
                yb[1, b, y_blocks(RES[g][q])] = yi[64 * q:64 * q + 64].reshape(8, 8, 128)
            if g == 0:
                yb[0, b, 64] = k1[128:136]
                yb[1, b, 64] = yi[128:136]

    def b_stage1():
        pacer = _Pacer(butterfly_tasks(1), 14 * 48)
        prev = None
        for b in list(range(0, 16, 2)) + list(range(1, 16, 2)):
            ts = b_dfwd(b, pacer)
            if prev is not None:
                b_sfwd(*prev, pacer)
            prev = (b, ts)
        b_sfwd(*prev, pacer)
        pacer.done()

    def b_stage3():
        row0 = lax.broadcasted_iota(jnp.int32, (8, 128), 0) == 0
        low = lax.broadcasted_iota(jnp.int32, (1, 128), 1) < 64
        for b in range(16):
            m = [as_bf16(mt[n, b]) for n in range(4)]
            for g in (1, 2, 3, 0):
                yr, yi = [cat(*[yb[c, b, y_blocks(r)].reshape(64, 128) for r in RES[g]]) for c in range(2)]
                if g == 0:
                    nr = -yr
                    u0 = cat(yr[0:64], jnp.where(row0, yb[0, b, 64], yi[0:8]), yi[8:64])
                    v0 = cat(yi[0:64], jnp.where(row0, yb[1, b, 64], nr[0:8]), nr[8:64])
                    u4, v4 = cat(yr[64:128], yi[64:128]), cat(yi[64:128], nr[64:128])
                    t1 = dot_nt(m[0], u0.astype(bf16)) + dot_nt(m[3], v0.astype(bf16))
                    t2 = dot_nt(m[0], u4.astype(bf16)) + dot_nt(m[3], v4.astype(bf16))
                else:
                    k1, k2, k3 = [dot_nt(m[n], v.astype(bf16)) for n, v in enumerate((yr + yi, yr, yi))]
                    t1, t2 = k1 + k3, k1 - k2
                slot = b // 2 + 8 * (b % 2)
                xd[2 * g, pl.ds(XP * slot, 128), :] = t1
                xd[2 * g + 1, pl.ds(XP * slot, 128), :] = t2
        for t in range(16):
            rows = lambda j: cat(*[xd[j, pl.ds(8 * t + u, 16, stride=XP), :] for u in range(8)])
            z = [dot(rows(q).astype(bf16), as_bf16(gi[q])) for q in range(2)]
            for g in range(1, 4):
                tr, ti = rows(2 * g), rows(2 * g + 1)
                sg = jnp.where(low, float(sign[g - 1][0]), float(sign[g - 1][1]))
                k1, k2, k3 = [dot(v.astype(bf16), as_bf16(gi[3 * g - 1 + n]))
                              for n, v in enumerate((tr + sg * ti, ti, tr))]
                z += [k1 + k2, k1 + k3]
            y = _inv8(z)
            for j in range(8):
                even = cat(*[y[j][16 * u:16 * u + 8] for u in range(8)])
                odd = cat(*[y[j][16 * u + 8:16 * u + 16] for u in range(8)])
                xb32[j, pl.ds(64 * t, 64), :] = pack2(even, odd)

    HALF = NSEG * M // 2

    def batch(u, p0, p1, tasks=(), t0=0, t1=4, query=False):
        mc = HALF // 2 if t1 - t0 <= MCT else HALF
        pacer = _Pacer(tasks, (7 * (p1 - p0) - MARGIN // (t1 - t0)) * HALF // 8)
        w = wall.at[u]
        for p in range(p0, p1):
            for r0 in range(0, HALF, mc):
                def blk(head, par):
                    return lambda: cat(*[w[pl.ds((p + 8 * head) * WP + 64 * (2 * t + par), 64), :]
                                         for t in range(t0, t1)])

                def prod(i, b):
                    lhs = jnp.concatenate([as_bf16(xs[i, t, pl.ds(r0 // 2, mc // 2), :])
                                           for t in range(t0, t1)], axis=1)
                    r = dot(lhs, as_bf16(b))
                    pacer.feed(r)
                    return r

                def emit(half, *cs):
                    rows = pl.ds(half * HALF + r0, mc)
                    park = pl.ds((half * HALF + r0) // 8, mc // 8)
                    if t0 > 0:
                        cs = [c + yb[t, p, park].reshape(mc, E) for t, c in enumerate(cs)]
                    if t1 < 4:
                        for t, c in enumerate(cs):
                            yb[t, p, park] = c.reshape(mc // 8, 8, E)
                    elif query:
                        st = jnp.concatenate([c.reshape(mc // M, M, E) for c in cs], axis=1)
                        pre[8 * u + p, rows, :] = pltpu.bitcast(st.reshape(2 * mc, E).astype(bf16), u32)
                    else:
                        pre[8 * u + p, rows, :] = pack2(*cs)
                _strassen(prod, blk(0, 0), blk(1, 0), blk(0, 1), blk(1, 1), add2, sub2, emit)
        pacer.done()

    def prepare_left(n):
        v = pltpu.bitcast(x8[:, :, pl.ds(256 * n, 256)].reshape(2 * HALF, 256), u32)
        blocks = [v[HALF // 2 * h:HALF // 2 * (h + 1), 128 * k:128 * (k + 1)] for h in range(2) for k in range(2)]
        lo, hi = [_strassen_left(*[un(b) for b in blocks]) for un in (lo_f32, hi_f32)]
        for i in range(7):
            xs[i, n] = pack2(lo[i], hi[i])

    wait_all(c_a[0])
    for task in relayout_tasks(0, 0, 128):
        task(jnp.zeros((8, 128), u32))
    prepare_left(0)
    batch(0, 0, 6, (), 0, 1)
    wait_all(c_a[1])
    c_h = [start(wq_hbm.at[pl.ds(256 * n, 256), :, 1], wraw.at[1, pl.ds(256 * n, 256)], n) for n in range(2)]
    prepare_left(1)
    batch(0, 6, 8, relayout_tasks(0, 128, 256), 0, 1)
    batch(0, 0, 6, (), 1, 2)
    wait_all(c_a[2])
    prepare_left(2)
    batch(0, 6, 8, relayout_tasks(0, 256, 384), 1, 2)
    batch(0, 0, 6, (), 2, 3)
    wait_all(c_a[3])
    c_w2 = start_unit(2)
    prepare_left(3)
    batch(0, 6, 8, relayout_tasks(0, 384, 512), 2, 3)
    batch(0, 0, 5, (), 3, 4, query=True)
    c_h[0].wait()
    batch(0, 5, 8, relayout_tasks(1, 0, 256), 3, 4, query=True)
    batch(1, 0, 5, (), 0, 2)
    c_h[1].wait()
    start_unit(3)
    batch(1, 5, 8, relayout_tasks(1, 256, 512), 0, 2)
    batch(1, 0, 4, (), 2, 4, query=True)
    c_w2.wait()
    start_unit(4)
    start_unit(5)
    c_b1 = [start(bx_hbm.at[:, pl.ds(128 * j, 128)], xb.at[j], 5) for j in range(8)]
    c_b1 += [start(gf_hbm, gf, 5), start(mt_hbm.at[pl.ds(0, 3)], mt.at[pl.ds(0, 3)], 5)]
    c_loop += [start(w.at[pl.ds(0, 512), pl.ds(128 * d, 128)], wt.at[t, d], 4, 1)
               for t, w in enumerate((wr_hbm, wi_hbm)) for d in range(16)]
    batch(1, 4, 8, relayout_tasks(2), 2, 4, query=True)
    batch(2, 0, 4)

    def unit_body(u, c):
        slot = (u + 1) % NRAW
        pltpu.make_async_copy(wraw.at[slot], wraw.at[slot], sems.at[slot]).wait()
        batch(u, 4, 8, relayout_tasks(u + 1))
        batch(u + 1, 0, 4)
        return c
    lax.fori_loop(2, 5, unit_body, 0)
    wait_all(c_b1)
    batch(5, 4, 8, butterfly_tasks(0))
    b_stage1()
    wait_all(c_loop)
    c_rest = start_x(UNROLL, NSEG - UNROLL, 6)
    c_b3 = [start(w.at[pl.ds(512, 1), :], wl.at[t], 5) for t, w in enumerate((wr_hbm, wi_hbm))]
    c_b3 += [start(gi_hbm, gi, 5), start(mt_hbm.at[3], mt.at[3], 5)]

    wo32 = wo.bitcast(u32)
    scale = E ** -0.5

    def gated(w, toks):
        if not toks:
            return w
        bits = functools.reduce(
            jnp.bitwise_or, [pltpu.bitcast(jnp.broadcast_to(t, (8, 128)), u32) for t in toks])
        ones = ((bits >> 16) | u32(0xFFFF)) | u32(0xFFFF0000)
        return cat(w[0:8] & ones, w[8:])

    def wqkv(i, p, second, toks=(), k0=0, k1=D):
        rows = pl.ds((p % 8 + 8 * second) * WP + k0 // 2, (k1 - k0) // 2)
        return as_bf16(gated(wall[2 * i + p // 8, rows, :], toks))

    def step(n, u, mem, held):
        s = UNROLL * n + u
        rows = cat(mem, xbuf[s, pl.ds(M, SEG - M), :].astype(f32))
        lhs = rows.astype(bf16)
        head_start = {}
        if u:
            lo, hi = rows[:, :D // 2].astype(bf16), rows[:, D // 2:].astype(bf16)
            for key in EARLY:
                head_start[key] = dot(lo, wqkv(*key, k1=D // 2))
        r8 = pl.multiple_of(M * s, M)
        fill = fill_ref[...]
        heads = [None] * H
        rs = []

        shift = jnp.full((8, 128), 16 - 16 * (n % 2), jnp.int32).astype(u32)
        wblk = pl.ds(pl.multiple_of(32 * (n // 2), 32), 32)
        flt = filter_tasks(
            s, lambda d: [hi_f32(wt32.at[t, d, wblk][pl.ds(u, 8, stride=4), :] << shift) for t in range(2)])
        pacer = _Pacer(flt, 48)

        def proj(i, p, toks=()):
            a, b = [
                dot(hi, wqkv(i, p, t, k0=D // 2)) + head_start[i, p, t] if (i, p, t) in head_start
                else dot(lhs, wqkv(i, p, t, toks[t * len(toks) // 2:(t + 1) * len(toks) // 2]))
                for t in range(2)]
            pacer.feed(a)
            pacer.feed(b)
            c = as_bf16(pre[16 * i + p, pl.ds(r8, M), :]).astype(f32)
            return cat(a, b, c).astype(bf16)

        def probs(q, k):
            sc = dot_nt(q, k) * scale
            sc = jnp.where(fill == 0.0, sc, fill)
            e = jnp.exp(sc - jnp.max(sc, axis=1, keepdims=True))
            l = jnp.sum(e, axis=1, keepdims=True)
            r = pl.reciprocal(l, approx=True)
            r = r * (2.0 - l * r)
            rs.append([r[8 * j:8 * j + 8] for j in range(10)])
            return (e * r).astype(bf16)

        def pv(p, pr, v):
            o = dot(pr, v)
            heads[2 * p] = o[0:32]
            heads[2 * p + 1] = o[32:64]
            held[u % 2, p] = (o[64:72], o[72:80])

        def left_task(p):
            def task(tok):
                ones = ((tok >> 16) | u32(0xFFFF)) | u32(0xFFFF0000)
                a11, a12, a21, a22 = held[0, p] + held[1, p]
                a11, a22 = [pltpu.bitcast(pltpu.bitcast(a, u32) & ones, f32) for a in (a11, a22)]
                dst = pl.ds(pl.multiple_of(M * (UNROLL // 2 * n + u // 2), M), M)
                for i, a in enumerate(_strassen_left(a11, a12, a21, a22)):
                    osum[i, p, dst, :] = a.astype(bf16)
            return task

        pend = []
        for g in range(4):
            ps = range(4 * g, 4 * g + 4)
            qk = [(proj(0, p), proj(1, p)) for p in ps]
            vs = [proj(2, p, rs[p - 4] if g else ()) for p in ps]
            for a in pend:
                pv(*a)
            pend = [(p, probs(*qk[t]), vs[t]) for t, p in enumerate(ps)]
        pacer.done()

        def wo_part(oc, j, h0, h1, toks=()):
            return dot(oc, as_bf16(gated(wo32[j, pl.ds(64 * h0, 64 * (h1 - h0)), :], toks)))

        acc = []
        pacer = _Pacer([left_task(p) for p in range(16)] if u % 2 else (), 4 * 10)
        oc = jnp.concatenate(heads[0:24], axis=1).astype(bf16)
        for j in range(8):
            acc.append(wo_part(oc, j, 0, 24, {3: rs[12] + rs[13], 4: rs[14] + rs[15]}.get(j, ())))
            if j == 4:
                for a in pend:
                    pv(*a)
            if j > 5:
                pacer.feed(acc[j])
        oc = jnp.concatenate(heads[24:32], axis=1).astype(bf16)
        nxt = []
        for j in range(8):
            r = wo_part(oc, j, 24, 32) + acc[j]
            outbuf[UNROLL // 2 * n + u // 2, u % 2, pl.ds(M, SEG - M), pl.ds(128 * j, 128)] = r[M:].astype(bf16)
            nxt.append(r[0:M])
            pacer.feed(r)
        pacer.done()
        return jnp.concatenate(nxt, axis=1)

    def steps(n, mem):
        pl.when(n == 1)(c_rest.wait)
        held = {}
        for u in range(UNROLL):
            mem = step(n, u, mem, held)
        return mem
    lax.fori_loop(0, NSEG // UNROLL, steps, mem0[...].astype(f32))
    tok_rows = pl.ds(M, SEG - M)
    c_out = [start(outbuf.at[:, :, tok_rows, :], out4.at[:, :, tok_rows, pl.ds(0, D)], 0)]

    wait_all(c_b3)
    for task in filter_tasks(64, lambda d: [wl[t, :, pl.ds(128 * d, 128)].astype(f32) for t in range(2)]):
        task(jnp.zeros((8, 128), u32))
    b_stage3()
    c_out += [start(xb.at[j], out_hbm.at[:, pl.ds(D + 128 * j, 128)], 0) for j in range(8)]

    osum32 = osum.bitcast(u32)
    for jp in range(4):
        def blk(col, par):
            return lambda: cat(*[wo32[2 * jp + col, pl.ds(64 * (2 * p + par), 64), :] for p in range(16)])

        def prod(i, b):
            return dot(jnp.concatenate([as_bf16(osum32[i, p]) for p in range(16)], axis=1), as_bf16(b))

        def emit(half, *cs):
            for t, c in enumerate(cs):
                outbuf[:, half, pl.ds(0, M), pl.ds(128 * (2 * jp + t), 128)] = (
                    c.reshape(NSEG // 2, M, 128).astype(bf16))
            cols = pl.ds(256 * jp, 256)
            c_out.append(start(outbuf.at[:, half, pl.ds(0, M), cols], out4.at[:, half, pl.ds(0, M), cols], 0))
        _strassen(prod, blk(0, 0), blk(1, 0), blk(0, 1), blk(1, 1), add2, sub2, emit)
    wait_all(c_out)


@functools.partial(jax.jit, static_argnames=("A_seg_len",))
def pallas_concat_heads__memory_aug_recurrent_mem_tr__spectral_gfnet__prompt_kernel(
    A_x: jax.Array,
    A_mem0: jax.Array,
    A_Wq: jax.Array,
    A_Wk: jax.Array,
    A_Wv: jax.Array,
    A_Wo: jax.Array,
    A_seg_len,
    B_x: jax.Array,
    B_w_r: jax.Array,
    B_w_i: jax.Array,
):
    assert A_seg_len == SEG
    assert A_x.shape == (1, S, D) and A_mem0.shape == (1, M, D) and B_x.shape == (1, S, D)
    assert A_Wq.shape == (D, H, E) and A_Wo.shape == (H, E, D) and B_w_r.shape == (S, D // 2 + 1)
    gf, gi, mt, _ = _dft_constants()
    fill = _attn_fill()
    hbm = pl.BlockSpec(memory_space=pltpu.HBM)
    wshape = (D // 2, 2, 2, 16, E)
    out = pl.pallas_call(
        _kernel,
        out_shape=jax.ShapeDtypeStruct((S, 2 * D), bf16),
        in_specs=[hbm] * 13,
        out_specs=hbm,
        scratch_shapes=[
            pltpu.VMEM((NRAW, D // 2, 2, 16, E), bf16),
            pltpu.VMEM((6, 16 * WP, E), u32),
            pltpu.VMEM((8, H * E, 128), bf16),
            pltpu.VMEM((NSEG, SEG, D), bf16),
            pltpu.VMEM((M, D), bf16),
            pltpu.VMEM((NSEG, M, D), bf16),
            pltpu.VMEM((7, 4, 128, 128), u32),
            pltpu.VMEM((48, NSEG * M, E), u32),
            pltpu.VMEM((7, 16, NSEG * M // 2, E), bf16),
            pltpu.VMEM((NSEG // 2, 2, SEG, D), bf16),
            pltpu.VMEM(fill.shape, f32),
            pltpu.VMEM((8, S, 128), bf16),
            pltpu.VMEM((2, 16, 512, 128), bf16),
            pltpu.VMEM((2, 1, S), bf16),
            pltpu.VMEM(gf.shape, u32),
            pltpu.VMEM(gi.shape, u32),
            pltpu.VMEM(mt.shape, u32),
            pltpu.VMEM((8, 16 * XP, 128), f32),
            pltpu.VMEM((2, 16, 65, 8, 128), f32),
            pltpu.SemaphoreType.DMA((7,)),
        ],
        compiler_params=pltpu.CompilerParams(vmem_limit_bytes=120 * 1024 * 1024),
    )(A_x.reshape(NSEG, SEG, D), A_mem0.reshape(M, D),
      A_Wq.reshape(wshape), A_Wk.reshape(wshape), A_Wv.reshape(wshape),
      A_Wo.reshape(H * E, D), B_x.reshape(S, D), B_w_r.T, B_w_i.T, gf, gi, mt, fill)
    return out.reshape(1, S, 2 * D)
```

```python
import functools

import jax
import jax.numpy as jnp
import numpy as np
from jax import lax
from jax.experimental import pallas as pl
from jax.experimental.pallas import tpu as pltpu

S, D, H, E, M, SEG = 2048, 1024, 32, 128, 8, 32
NSEG = S // SEG
WP = 516
XP = 132
ZP = 68
NRAW = 4
UNROLL = 4
MCT = 1
MARGIN = 8
EARLY = ((0, 0, 0), (0, 0, 1), (1, 0, 0), (1, 0, 1), (0, 1, 0), (0, 1, 1))
bf16, f32, u32 = jnp.bfloat16, jnp.float32, jnp.uint32
RES = ((0, 4), (2, 6), (1, 7), (3, 5))
RC = float(np.sqrt(0.5))


def _fwd8(x):
    s04, d04 = x[0] + x[4], x[0] - x[4]
    s26, d26 = x[2] + x[6], x[2] - x[6]
    s15, d15 = x[1] + x[5], x[1] - x[5]
    s37, d37 = x[3] + x[7], x[3] - x[7]
    t1, t2 = (d15 - d37) * RC, (d15 + d37) * RC
    e0, o0 = s04 + s26, s15 + s37
    return [e0 + o0, e0 - o0, s04 - s26, s15 - s37, d04 + t1, d26 + t2, d04 - t1, d26 - t2]


def _inv8(z):
    z0, z4, e1, o1, r1, i1, r3, i3 = z
    e0, o0 = z0 + z4, z0 - z4
    s04, s26, s15, s37 = e0 + e1, e0 - e1, o0 + o1, o0 - o1
    d04, d26 = r1 + r3, i1 + i3
    t1, t2 = (r1 - r3) * RC, (i1 - i3) * RC
    d15, d37 = t1 + t2, t2 - t1
    return [s04 + d04, s15 + d15, s26 + d26, s37 + d37, s04 - d04, s15 - d15, s26 - d26, s37 - d37]


def _twiddle16(z, k):
    re, im = z
    k = k % 16
    if k == 0:
        return z
    if k == 4:
        return (im, -re)
    if k == 12:
        return (-im, re)
    if k == 2:
        return ((re + im) * RC, (im - re) * RC)
    if k == 14:
        return ((re - im) * RC, (re + im) * RC)
    if k == 6:
        return ((im - re) * RC, (re + im) * -RC)
    if k == 10:
        return ((re + im) * -RC, (re - im) * RC)
    c, s = float(np.cos(2 * np.pi * k / 16)), float(-np.sin(2 * np.pi * k / 16))
    return (re * c - im * s, re * s + im * c)


def _bfly4(z, sign):
    (ar, ai), (br, bi), (cr, ci), (dr, di) = z
    sr, si, tr, ti = ar + cr, ai + ci, ar - cr, ai - ci
    ur, ui, vr, vi = br + dr, bi + di, br - dr, bi - di
    o0, o2 = (sr + ur, si + ui), (sr - ur, si - ui)
    p, q = (tr + vi, ti - vr), (tr - vi, ti + vr)
    return [o0, p, o2, q] if sign > 0 else [o0, q, o2, p]


class _Pacer:
    def __init__(self, tasks, ntokens):
        self.slots = {}
        for n, task in enumerate(tasks):
            self.slots.setdefault(n * ntokens // len(tasks), []).append(task)
        self.pos = 0

    def feed(self, r):
        for j in range(r.shape[0] // 8):
            for task in self.slots.pop(self.pos, []):
                task(pltpu.bitcast(r[8 * j:8 * j + 8], u32))
            self.pos += 1

    def done(self):
        assert not self.slots


def _pack_rows(m):
    b = np.asarray(m, np.float32).astype(jnp.bfloat16).view(np.uint16).astype(np.uint32)
    return b[..., 0::2, :] | (b[..., 1::2, :] << 16)


@functools.lru_cache(maxsize=None)
def _dft_constants():
    b8 = np.array(_fwd8(list(np.eye(8)))).T
    n = np.arange(D)
    fw = np.zeros((D, D))
    bw = np.zeros((D, D))
    for g in range(4):
        k = np.concatenate([8 * np.arange(64) + r for r in RES[g]])
        ang = 2 * np.pi * ((n[:, None] * k[None, :]) % D) / D
        wgt = np.where(k == 0, 1.0, 2.0) / (D * S)
        fw[:, 256 * g:256 * g + 128] = np.cos(ang)
        fw[:, 256 * g + 128:256 * g + 256] = -np.sin(ang)
        bw[256 * g:256 * g + 128] = (np.cos(ang) * wgt).T
        bw[256 * g + 128:256 * g + 256] = (-np.sin(ang) * wgt).T
    bw[128, :] = (-1.0) ** n / (D * S)
    binv = np.kron(np.linalg.inv(b8), np.eye(128))
    gall = binv @ fw
    giall = bw @ binv.T
    gf = np.zeros((11, 144, 128))
    gi = np.zeros((11, 128, 128))
    sign = []
    half = lambda m, q: np.concatenate([m[64 * q:64 * q + 64], m[128 + 64 * q:192 + 64 * q]])
    for g in range(4):
        sl = slice(256 * g, 256 * g + 256)
        f, b = gall[sl, sl].T, giall[sl, sl]
        if g == 0:
            for q in range(2):
                gf[q, :128] = half(f, q)[:, 128 * q:128 * q + 128]
                gi[q] = half(b, q)[:, 128 * q:128 * q + 128]
            gf[0, 128] = (-1.0) ** np.arange(128)
            continue
        sg = np.sign(f[:128, 0] * f[128:, 128])[:, None]
        sign.append((int(sg[0, 0]), int(sg[64, 0])))
        p, q, r = f[:128, :128], f[:128, 128:], f[128:, :128]
        gf[3 * g - 1:3 * g + 2, :128] = p, q - p, r - sg * p
        p, q, r = b[:128, :128], b[:128, 128:], b[128:, :128]
        gi[3 * g - 1:3 * g + 2] = p, r - sg * p, q - p
    a = np.arange(128)
    mt = np.zeros((4, 16, 128, 128))
    for b in range(16):
        ang = 2 * np.pi * (((16 * a[:, None] + b) * a[None, :]) % S) / S
        c, sn = np.cos(ang), -np.sin(ang)
        mt[:, b] = c, c + sn, sn - c, sn
    return _pack_rows(gf), _pack_rows(gi), _pack_rows(mt), tuple(sign)


def _attn_fill():
    pos32 = np.concatenate([np.arange(8), np.arange(16, 40)])
    last = np.arange(16)
    qhead = np.concatenate([np.arange(64) // 32, last // 8])
    khead = np.concatenate([np.arange(64) // 32, last % 2])
    qpos = np.concatenate([pos32, pos32, 8 + last % 8])
    kpos = np.concatenate([pos32, pos32, 8 + last // 2])
    ok = (qpos[:, None] < M) | (qpos[:, None] >= kpos[None, :])
    fill = np.where(ok, 0.0, -1e9)
    fill = np.where(qhead[:, None] == khead[None, :], fill, -np.inf)
    return fill.astype(np.float32)


def _strassen(prod, b11, b12, b21, b22, add, sub, emit):
    m2 = prod(1, b11())
    m1 = prod(0, add(b11(), b22()))
    m3 = prod(2, sub(b12(), b22()))
    c22 = prod(5, add(b11(), b12())) + ((m1 - m2) + m3)
    m4 = prod(3, sub(b21(), b11()))
    emit(1, m2 + m4, c22)
    m5 = prod(4, b22())
    emit(0, prod(6, add(b21(), b22())) + ((m1 + m4) - m5), m3 + m5)


def _strassen_left(a11, a12, a21, a22):
    return [a11 + a22, a21 + a22, a11, a22, a11 + a12, a21 - a11, a12 - a22]


def _kernel(x_hbm, mem_hbm, wq_hbm, wk_hbm, wv_hbm, wo_hbm, bx_hbm, wr_hbm, wi_hbm,
            gf_hbm, gi_hbm, mt_hbm, fill_hbm, out_hbm,
            wraw, wall, wo, xbuf, mem0, x8, xs, pre, osum, outbuf, fill_ref,
            xb, wt, wl, gf, gi, mt, xd, yb, sems):
    def start(src, dst, sem, priority=0):
        c = pltpu.make_async_copy(src, dst, sems.at[sem])
        c.start(priority=priority)
        return c

    def wait_all(cs):
        for c in cs:
            c.wait()

    dot = functools.partial(jnp.dot, preferred_element_type=f32)
    dot_nt = lambda a, b: lax.dot_general(a, b, (((1,), (1,)), ((), ())), preferred_element_type=f32)
    cat = lambda *vs: jnp.concatenate(vs, axis=0)
    as_bf16 = lambda w: pltpu.bitcast(w, bf16)
    lo_f32 = lambda w: pltpu.bitcast(w << 16, f32)
    hi_f32 = lambda w: pltpu.bitcast(w & u32(0xFFFF0000), f32)
    pack2 = lambda a, b: pltpu.pack_elementwise([a, b], packed_dtype=bf16)
    add2 = lambda a, b: pack2(lo_f32(a) + lo_f32(b), hi_f32(a) + hi_f32(b))
    sub2 = lambda a, b: pack2(lo_f32(a) - lo_f32(b), hi_f32(a) - hi_f32(b))
    out4 = out_hbm.reshape(NSEG // 2, 2, SEG, 2 * D)
    w_hbm = (wq_hbm, wk_hbm, wv_hbm)

    def start_unit(u):
        return start(w_hbm[u // 2].at[:, :, u % 2], wraw.at[u % NRAW], u % NRAW)

    def start_x(seg0, nseg, sem, priority=0):
        segs, rows = pl.ds(seg0, nseg), pl.ds(M, SEG - M)
        return start(x_hbm.at[segs, rows, :], xbuf.at[segs, rows, :], sem, priority)

    c_a = []
    for n in range(4):
        cols, rows = pl.ds(256 * n, 256), pl.ds(128 * n, 128)
        c_a.append([start(x_hbm.at[:, pl.ds(0, M), cols], x8.at[:, :, cols], n),
                    start(wq_hbm.at[rows, :, 0], wraw.at[0, rows], n)])
    c_loop = [start_x(0, UNROLL, 4, 1), start(mem_hbm, mem0, 4, 1), start(fill_hbm, fill_ref.at[pl.ds(0, 80)], 4, 1)]
    c_loop += [start(wo_hbm.at[:, pl.ds(128 * j, 128)], wo.at[j], 4, 1) for j in range(8)]

    wraw32 = wraw.bitcast(u32)
    wt32 = wt.bitcast(u32)
    xb32 = xb.bitcast(u32)

    def relayout_row(src, dst, r, lo, hi):
        a, b = src[r, 0], src[r, 1]
        dst[pl.ds(r, 8, stride=WP), :] = (a & lo) | (b << 16)
        dst[pl.ds(r + 8 * WP, 8, stride=WP), :] = (a >> 16) | (b & hi)

    def relayout_tasks(u, r0=0, r1=D // 2):
        src, dst = wraw32.at[u % NRAW], wall.at[u]

        def make(r):
            def task(tok):
                lo = (tok >> 16) | u32(0xFFFF)
                hi = (tok << 16) | u32(0xFFFF0000)
                relayout_row(src, dst, r, lo, hi)
                relayout_row(src, dst, r + 1, lo, hi)
            return task
        return [make(r) for r in range(r0, r1, 2)]

    def y_blocks(r):
        return pl.ds(4 * (r % 2) + r // 2, 8, stride=8)

    def filter_tasks(blk, wfn):
        def make(phase, k):
            slots = [4 * k + j for j in range(4)] if phase == 1 else [4 * j + k for j in range(4)]

            def task(tok):
                ones = ((tok >> 16) | u32(0xFFFF)) | u32(0xFFFF0000)
                z = [(yb[0, b, blk], yb[1, b, blk]) for b in slots]
                z[0] = tuple(pltpu.bitcast(pltpu.bitcast(v, u32) & ones, f32) for v in z[0])
                if phase == 0:
                    o = _bfly4(z, 1)
                    o = [_twiddle16(o[j], k * j) for j in range(4)]
                elif phase == 1:
                    o = _bfly4(z, 1)
                    y = []
                    for j in range(4):
                        wr, wi = wfn(k + 4 * j)
                        xr, xi = o[j]
                        y.append((xr * wr - xi * wi, xr * wi + xi * wr))
                    o = _bfly4(y, -1)
                    o = [_twiddle16(o[j], -k * j) for j in range(4)]
                else:
                    o = _bfly4(z, -1)
                for b, v in zip(slots, o):
                    yb[0, b, blk] = v[0]
                    yb[1, b, blk] = v[1]
            return task
        return [make(phase, k) for phase in range(3) for k in range(4)]

    def z_region(n, par):
        return (2 * n + par) // 3, (2 * n + par) % 3 * 8 * ZP

    def butterfly_tasks(par):
        def make(a2):
            def task(tok):
                zs = []
                for a in (2 * a2, 2 * a2 + 1):
                    w = [xb32[j, pl.ds(8 * a, 8), :] for j in range(8)]
                    if par:
                        hi = (tok << 16) | u32(0xFFFF0000)
                        z = _fwd8([pltpu.bitcast(v & hi, f32) for v in w])
                    else:
                        sixteen = ((tok >> 31) | u32(1)) << 4
                        z = _fwd8([pltpu.bitcast(v << sixteen, f32) for v in w])
                    zs.append(z[0:2] + [v for g in range(1, 4)
                                        for v in (z[2 * g] + z[2 * g + 1], z[2 * g + 1], z[2 * g])])
                for n in range(11):
                    plane, row = z_region(n, par)
                    xd[plane, pl.ds(row + a2, 8, stride=ZP), :] = pltpu.bitcast(pack2(zs[0][n], zs[1][n]), f32)
            return task
        return [make(a2) for a2 in range(64)]

    sign = _dft_constants()[3]

    def b_dfwd(b, pacer):
        def z(n):
            plane, row = z_region(n, b % 2)
            return as_bf16(xd[plane, pl.ds(row + b // 2 * ZP, 64), :])
        t0 = dot_nt(as_bf16(gf[0]), z(0))
        t4 = dot_nt(as_bf16(gf[1, 0:64]), z(1))
        tr, ti = cat(t0[0:64], t4[0:64]), cat(t0[64:128], t4[64:128])
        ts = [(cat(tr + ti, t0[128:144]).astype(bf16), ti.astype(bf16), cat(tr, t0[128:144]).astype(bf16))]
        for g in range(1, 4):
            k1, k2, k3 = [dot_nt(as_bf16(gf[n, 0:64]), z(n)) for n in range(3 * g - 1, 3 * g + 2)]
            pacer.feed(k1)
            tr = k1 + k2
            ti = cat(*[k3[64 * q:64 * q + 64] + k1[64 * q:64 * q + 64] if sign[g - 1][q] > 0
                       else k3[64 * q:64 * q + 64] - k1[64 * q:64 * q + 64] for q in range(2)])
            ts.append(((tr + ti).astype(bf16), ti.astype(bf16), tr.astype(bf16)))
        return ts

    def b_sfwd(b, ts, pacer):
        for g in range(4):
            k1, k2, k3 = [dot(ts[g][n], as_bf16(mt[n, b])) for n in range(3)]
            if g:
                pacer.feed(k2)
            yr, yi = k1[0:128] - k2, k1 + k3
            for q in range(2):
                yb[0, b, y_blocks(RES[g][q])] = yr[64 * q:64 * q + 64].reshape(8, 8, 128)
                yb[1, b, y_blocks(RES[g][q])] = yi[64 * q:64 * q + 64].reshape(8, 8, 128)
            if g == 0:
                yb[0, b, 64] = k1[128:136]
                yb[1, b, 64] = yi[128:136]

    def b_stage1():
        pacer = _Pacer(butterfly_tasks(1), 14 * 48)
        prev = None
        for b in list(range(0, 16, 2)) + list(range(1, 16, 2)):
            ts = b_dfwd(b, pacer)
            if prev is not None:
                b_sfwd(*prev, pacer)
            prev = (b, ts)
        b_sfwd(*prev, pacer)
        pacer.done()

    def b_stage3():
        row0 = lax.broadcasted_iota(jnp.int32, (8, 128), 0) == 0
        low = lax.broadcasted_iota(jnp.int32, (1, 128), 1) < 64
        for b in range(16):
            m = [as_bf16(mt[n, b]) for n in range(4)]
            for g in (1, 2, 3, 0):
                yr, yi = [cat(*[yb[c, b, y_blocks(r)].reshape(64, 128) for r in RES[g]]) for c in range(2)]
                if g == 0:
                    nr = -yr
                    u0 = cat(yr[0:64], jnp.where(row0, yb[0, b, 64], yi[0:8]), yi[8:64])
                    v0 = cat(yi[0:64], jnp.where(row0, yb[1, b, 64], nr[0:8]), nr[8:64])
                    u4, v4 = cat(yr[64:128], yi[64:128]), cat(yi[64:128], nr[64:128])
                    t1 = dot_nt(m[0], u0.astype(bf16)) + dot_nt(m[3], v0.astype(bf16))
                    t2 = dot_nt(m[0], u4.astype(bf16)) + dot_nt(m[3], v4.astype(bf16))
                else:
                    k1, k2, k3 = [dot_nt(m[n], v.astype(bf16)) for n, v in enumerate((yr + yi, yr, yi))]
                    t1, t2 = k1 + k3, k1 - k2
                slot = b // 2 + 8 * (b % 2)
                xd[2 * g, pl.ds(XP * slot, 128), :] = t1
                xd[2 * g + 1, pl.ds(XP * slot, 128), :] = t2
        for t in range(16):
            rows = lambda j: cat(*[xd[j, pl.ds(8 * t + u, 16, stride=XP), :] for u in range(8)])
            z = [dot(rows(q).astype(bf16), as_bf16(gi[q])) for q in range(2)]
            for g in range(1, 4):
                tr, ti = rows(2 * g), rows(2 * g + 1)
                sg = jnp.where(low, float(sign[g - 1][0]), float(sign[g - 1][1]))
                k1, k2, k3 = [dot(v.astype(bf16), as_bf16(gi[3 * g - 1 + n]))
                              for n, v in enumerate((tr + sg * ti, ti, tr))]
                z += [k1 + k2, k1 + k3]
            y = _inv8(z)
            for j in range(8):
                even = cat(*[y[j][16 * u:16 * u + 8] for u in range(8)])
                odd = cat(*[y[j][16 * u + 8:16 * u + 16] for u in range(8)])
                xb32[j, pl.ds(64 * t, 64), :] = pack2(even, odd)

    HALF = NSEG * M // 2

    def batch(u, p0, p1, tasks=(), t0=0, t1=4, query=False):
        mc = HALF // 2 if t1 - t0 <= MCT else HALF
        pacer = _Pacer(tasks, (7 * (p1 - p0) - MARGIN // (t1 - t0)) * HALF // 8)
        w = wall.at[u]
        for p in range(p0, p1):
            for r0 in range(0, HALF, mc):
                def blk(head, par):
                    return lambda: cat(*[w[pl.ds((p + 8 * head) * WP + 64 * (2 * t + par), 64), :]
                                         for t in range(t0, t1)])

                def prod(i, b):
                    lhs = jnp.concatenate([as_bf16(xs[i, t, pl.ds(r0 // 2, mc // 2), :])
                                           for t in range(t0, t1)], axis=1)
                    r = dot(lhs, as_bf16(b))
                    pacer.feed(r)
                    return r

                def emit(half, *cs):
                    rows = pl.ds(half * HALF + r0, mc)
                    park = pl.ds((half * HALF + r0) // 8, mc // 8)
                    if t0 > 0:
                        cs = [c + yb[t, p, park].reshape(mc, E) for t, c in enumerate(cs)]
                    if t1 < 4:
                        for t, c in enumerate(cs):
                            yb[t, p, park] = c.reshape(mc // 8, 8, E)
                    elif query:
                        st = jnp.concatenate([c.reshape(mc // M, M, E) for c in cs], axis=1)
                        pre[8 * u + p, rows, :] = pltpu.bitcast(st.reshape(2 * mc, E).astype(bf16), u32)
                    else:
                        pre[8 * u + p, rows, :] = pack2(*cs)
                _strassen(prod, blk(0, 0), blk(1, 0), blk(0, 1), blk(1, 1), add2, sub2, emit)
        pacer.done()

    def prepare_left(n):
        v = pltpu.bitcast(x8[:, :, pl.ds(256 * n, 256)].reshape(2 * HALF, 256), u32)
        blocks = [v[HALF // 2 * h:HALF // 2 * (h + 1), 128 * k:128 * (k + 1)] for h in range(2) for k in range(2)]
        lo, hi = [_strassen_left(*[un(b) for b in blocks]) for un in (lo_f32, hi_f32)]
        for i in range(7):
            xs[i, n] = pack2(lo[i], hi[i])

    wait_all(c_a[0])
    for task in relayout_tasks(0, 0, 128):
        task(jnp.zeros((8, 128), u32))
    prepare_left(0)
    batch(0, 0, 6, (), 0, 1)
    wait_all(c_a[1])
    c_h = [start(wq_hbm.at[pl.ds(256 * n, 256), :, 1], wraw.at[1, pl.ds(256 * n, 256)], n) for n in range(2)]
    prepare_left(1)
    batch(0, 6, 8, relayout_tasks(0, 128, 256), 0, 1)
    batch(0, 0, 6, (), 1, 2)
    wait_all(c_a[2])
    prepare_left(2)
    batch(0, 6, 8, relayout_tasks(0, 256, 384), 1, 2)
    batch(0, 0, 6, (), 2, 3)
    wait_all(c_a[3])
    c_w2 = start_unit(2)
    prepare_left(3)
    batch(0, 6, 8, relayout_tasks(0, 384, 512), 2, 3)
    batch(0, 0, 5, (), 3, 4, query=True)
    c_h[0].wait()
    batch(0, 5, 8, relayout_tasks(1, 0, 256), 3, 4, query=True)
    batch(1, 0, 5, (), 0, 2)
    c_h[1].wait()
    start_unit(3)
    batch(1, 5, 8, relayout_tasks(1, 256, 512), 0, 2)
    batch(1, 0, 4, (), 2, 4, query=True)
    c_w2.wait()
    start_unit(4)
    start_unit(5)
    c_b1 = [start(bx_hbm.at[:, pl.ds(128 * j, 128)], xb.at[j], 5) for j in range(8)]
    c_b1 += [start(gf_hbm, gf.at[pl.ds(0, 11)], 5), start(mt_hbm.at[pl.ds(0, 3)], mt.at[pl.ds(0, 3)], 5)]
    c_loop += [start(w.at[pl.ds(0, 512), pl.ds(128 * d, 128)], wt.at[t, d], 4, 1)
               for t, w in enumerate((wr_hbm, wi_hbm)) for d in range(16)]
    batch(1, 4, 8, relayout_tasks(2), 2, 4, query=True)
    batch(2, 0, 4)

    def unit_body(u, c):
        slot = (u + 1) % NRAW
        pltpu.make_async_copy(wraw.at[slot], wraw.at[slot], sems.at[slot]).wait()
        batch(u, 4, 8, relayout_tasks(u + 1))
        batch(u + 1, 0, 4)
        return c
    lax.fori_loop(2, 5, unit_body, 0)
    wait_all(c_b1)
    batch(5, 4, 8, butterfly_tasks(0))
    b_stage1()
    wait_all(c_loop)
    c_rest = start_x(UNROLL, NSEG - UNROLL, 6)
    c_b3 = [start(w.at[pl.ds(512, 1), :], wl.at[t], 5) for t, w in enumerate((wr_hbm, wi_hbm))]
    c_b3 += [start(gi_hbm, gi, 5), start(mt_hbm.at[3], mt.at[3], 5)]

    wo32 = wo.bitcast(u32)
    scale = E ** -0.5

    def gated(w, toks):
        if not toks:
            return w
        bits = functools.reduce(
            jnp.bitwise_or, [pltpu.bitcast(jnp.broadcast_to(t, (8, 128)), u32) for t in toks])
        ones = ((bits >> 16) | u32(0xFFFF)) | u32(0xFFFF0000)
        return cat(w[0:8] & ones, w[8:])

    def wqkv(i, p, second, toks=(), k0=0, k1=D):
        rows = pl.ds((p % 8 + 8 * second) * WP + k0 // 2, (k1 - k0) // 2)
        return as_bf16(gated(wall[2 * i + p // 8, rows, :], toks))

    def step(n, u, mem, held):
        s = UNROLL * n + u
        rows = cat(mem, xbuf[s, pl.ds(M, SEG - M), :].astype(f32))
        lhs = rows.astype(bf16)
        head_start = {}
        if u:
            lo, hi = rows[:, :D // 2].astype(bf16), rows[:, D // 2:].astype(bf16)
            for key in EARLY:
                head_start[key] = dot(lo, wqkv(*key, k1=D // 2))
        r8 = pl.multiple_of(M * s, M)
        fill = fill_ref[pl.ds(0, 80), :]
        heads = [None] * H
        rs = []

        shift = jnp.full((8, 128), 16 - 16 * (n % 2), jnp.int32).astype(u32)
        wblk = pl.ds(pl.multiple_of(32 * (n // 2), 32), 32)
        flt = filter_tasks(
            s, lambda d: [hi_f32(wt32.at[t, d, wblk][pl.ds(u, 8, stride=4), :] << shift) for t in range(2)])
        pacer = _Pacer(flt, 48)

        def proj(i, p, toks=()):
            a, b = [
                dot(hi, wqkv(i, p, t, k0=D // 2)) + head_start[i, p, t] if (i, p, t) in head_start
                else dot(lhs, wqkv(i, p, t, toks[t * len(toks) // 2:(t + 1) * len(toks) // 2]))
                for t in range(2)]
            pacer.feed(a)
            pacer.feed(b)
            c = as_bf16(pre[16 * i + p, pl.ds(r8, M), :]).astype(f32)
            return cat(a, b, c).astype(bf16)

        def probs(q, k):
            sc = dot_nt(q, k) * scale
            sc = jnp.where(fill == 0.0, sc, fill)
            e = jnp.exp(sc - jnp.max(sc, axis=1, keepdims=True))
            l = jnp.sum(e, axis=1, keepdims=True)
            r = pl.reciprocal(l, approx=True)
            r = r * (2.0 - l * r)
            rs.append([r[8 * j:8 * j + 8] for j in range(10)])
            return (e * r).astype(bf16)

        def pv(p, pr, v):
            o = dot(pr, v)
            heads[2 * p] = o[0:32]
            heads[2 * p + 1] = o[32:64]
            held[u % 2, p] = (o[64:72], o[72:80])

        def left_task(p):
            def task(tok):
                ones = ((tok >> 16) | u32(0xFFFF)) | u32(0xFFFF0000)
                a11, a12, a21, a22 = held[0, p] + held[1, p]
                a11, a22 = [pltpu.bitcast(pltpu.bitcast(a, u32) & ones, f32) for a in (a11, a22)]
                dst = pl.ds(pl.multiple_of(M * (UNROLL // 2 * n + u // 2), M), M)
                for i, a in enumerate(_strassen_left(a11, a12, a21, a22)):
                    osum[i, p, dst, :] = a.astype(bf16)
            return task

        pend = []
        for g in range(4):
            ps = range(4 * g, 4 * g + 4)
            qk = [(proj(0, p), proj(1, p)) for p in ps]
            vs = [proj(2, p, rs[p - 4] if g else ()) for p in ps]
            for a in pend:
                pv(*a)
            pend = [(p, probs(*qk[t]), vs[t]) for t, p in enumerate(ps)]
        pacer.done()

        def wo_part(oc, j, h0, h1, toks=()):
            return dot(oc, as_bf16(gated(wo32[j, pl.ds(64 * h0, 64 * (h1 - h0)), :], toks)))

        acc = []
        pacer = _Pacer([left_task(p) for p in range(16)] if u % 2 else (), 4 * 10)
        oc = jnp.concatenate(heads[0:24], axis=1).astype(bf16)
        for j in range(8):
            acc.append(wo_part(oc, j, 0, 24, {3: rs[12] + rs[13], 4: rs[14] + rs[15]}.get(j, ())))
            if j == 4:
                for a in pend:
                    pv(*a)
            if j > 5:
                pacer.feed(acc[j])
        oc = jnp.concatenate(heads[24:32], axis=1).astype(bf16)
        nxt = []
        for j in range(8):
            r = wo_part(oc, j, 24, 32) + acc[j]
            outbuf[UNROLL // 2 * n + u // 2, u % 2, pl.ds(M, SEG - M), pl.ds(128 * j, 128)] = r[M:].astype(bf16)
            nxt.append(r[0:M])
            pacer.feed(r)
        pacer.done()
        return jnp.concatenate(nxt, axis=1)

    def steps(n, mem):
        pl.when(n == 1)(c_rest.wait)
        held = {}
        for u in range(UNROLL):
            mem = step(n, u, mem, held)
        return mem
    lax.fori_loop(0, NSEG // UNROLL, steps, mem0[...].astype(f32))
    tok_rows = pl.ds(M, SEG - M)
    c_out = [start(outbuf.at[:, :, tok_rows, :], out4.at[:, :, tok_rows, pl.ds(0, D)], 0)]

    wait_all(c_b3)
    for task in filter_tasks(64, lambda d: [wl[t, :, pl.ds(128 * d, 128)].astype(f32) for t in range(2)]):
        task(jnp.zeros((8, 128), u32))
    b_stage3()
    c_out += [start(xb.at[j], out_hbm.at[:, pl.ds(D + 128 * j, 128)], 0) for j in range(8)]

    osum32 = osum.bitcast(u32)
    for jp in range(4):
        def blk(col, par):
            return lambda: cat(*[wo32[2 * jp + col, pl.ds(64 * (2 * p + par), 64), :] for p in range(16)])

        def prod(i, b):
            return dot(jnp.concatenate([as_bf16(osum32[i, p]) for p in range(16)], axis=1), as_bf16(b))

        def emit(half, *cs):
            for t, c in enumerate(cs):
                outbuf[:, half, pl.ds(0, M), pl.ds(128 * (2 * jp + t), 128)] = (
                    c.reshape(NSEG // 2, M, 128).astype(bf16))
            cols = pl.ds(256 * jp, 256)
            c_out.append(start(outbuf.at[:, half, pl.ds(0, M), cols], out4.at[:, half, pl.ds(0, M), cols], 0))
        _strassen(prod, blk(0, 0), blk(1, 0), blk(0, 1), blk(1, 1), add2, sub2, emit)
    wait_all(c_out)


@functools.partial(jax.jit, static_argnames=("A_seg_len",))
def pallas_concat_heads__memory_aug_recurrent_mem_tr__spectral_gfnet__prompt_kernel(
    A_x: jax.Array,
    A_mem0: jax.Array,
    A_Wq: jax.Array,
    A_Wk: jax.Array,
    A_Wv: jax.Array,
    A_Wo: jax.Array,
    A_seg_len,
    B_x: jax.Array,
    B_w_r: jax.Array,
    B_w_i: jax.Array,
):
    assert A_seg_len == SEG
    assert A_x.shape == (1, S, D) and A_mem0.shape == (1, M, D) and B_x.shape == (1, S, D)
    assert A_Wq.shape == (D, H, E) and A_Wo.shape == (H, E, D) and B_w_r.shape == (S, D // 2 + 1)
    gf, gi, mt, _ = _dft_constants()
    fill = _attn_fill()
    hbm = pl.BlockSpec(memory_space=pltpu.HBM)
    wshape = (D // 2, 2, 2, 16, E)
    out = pl.pallas_call(
        _kernel,
        out_shape=jax.ShapeDtypeStruct((S, 2 * D), bf16),
        in_specs=[hbm] * 13,
        out_specs=hbm,
        scratch_shapes=[
            pltpu.VMEM((NRAW, D // 2, 2, 16, E), bf16),
            pltpu.VMEM((6, 16 * WP, E), u32),
            pltpu.VMEM((8, H * E, 128), bf16),
            pltpu.VMEM((NSEG, SEG, D), bf16),
            pltpu.VMEM((M, D), bf16),
            pltpu.VMEM((NSEG, M, D), bf16),
            pltpu.VMEM((7, 4, 128, 128), u32),
            pltpu.VMEM((48, NSEG * M, E), u32),
            pltpu.VMEM((7, 16, NSEG * M // 2, E), bf16),
            pltpu.VMEM((NSEG // 2, 2, SEG, D), bf16),
            pltpu.VMEM((96, 80), f32),
            pltpu.VMEM((8, S, 128), bf16),
            pltpu.VMEM((2, 16, 512, 128), bf16),
            pltpu.VMEM((2, 1, S), bf16),
            pltpu.VMEM((12,) + gf.shape[1:], u32),
            pltpu.VMEM(gi.shape, u32),
            pltpu.VMEM(mt.shape, u32),
            pltpu.VMEM((8, 16 * XP, 128), f32),
            pltpu.VMEM((2, 16, 65, 8, 128), f32),
            pltpu.SemaphoreType.DMA((7,)),
        ],
        compiler_params=pltpu.CompilerParams(vmem_limit_bytes=120 * 1024 * 1024),
    )(A_x.reshape(NSEG, SEG, D), A_mem0.reshape(M, D),
      A_Wq.reshape(wshape), A_Wk.reshape(wshape), A_Wv.reshape(wshape),
      A_Wo.reshape(H * E, D), B_x.reshape(S, D), B_w_r.T, B_w_i.T, gf, gi, mt, fill)
    return out.reshape(1, S, 2 * D)
```

```python
import functools

import jax
import jax.numpy as jnp
import numpy as np
from jax import lax
from jax.experimental import pallas as pl
from jax.experimental.pallas import tpu as pltpu

S, D, H, E, M, SEG = 2048, 1024, 32, 128, 8, 32
NSEG = S // SEG
WP = 516
XP = 132
ZP = 68
NRAW = 4
UNROLL = 4
MCT = 1
LAG = 8
NB0 = 64
NBT = 13
MARGIN = 8
EARLY = ((0, 0, 0), (0, 0, 1), (1, 0, 0), (1, 0, 1), (0, 1, 0), (0, 1, 1))
bf16, f32, u32 = jnp.bfloat16, jnp.float32, jnp.uint32
RES = ((0, 4), (2, 6), (1, 7), (3, 5))
RC = float(np.sqrt(0.5))


def _fwd8(x):
    s04, d04 = x[0] + x[4], x[0] - x[4]
    s26, d26 = x[2] + x[6], x[2] - x[6]
    s15, d15 = x[1] + x[5], x[1] - x[5]
    s37, d37 = x[3] + x[7], x[3] - x[7]
    t1, t2 = (d15 - d37) * RC, (d15 + d37) * RC
    e0, o0 = s04 + s26, s15 + s37
    return [e0 + o0, e0 - o0, s04 - s26, s15 - s37, d04 + t1, d26 + t2, d04 - t1, d26 - t2]


def _inv8(z):
    z0, z4, e1, o1, r1, i1, r3, i3 = z
    e0, o0 = z0 + z4, z0 - z4
    s04, s26, s15, s37 = e0 + e1, e0 - e1, o0 + o1, o0 - o1
    d04, d26 = r1 + r3, i1 + i3
    t1, t2 = (r1 - r3) * RC, (i1 - i3) * RC
    d15, d37 = t1 + t2, t2 - t1
    return [s04 + d04, s15 + d15, s26 + d26, s37 + d37, s04 - d04, s15 - d15, s26 - d26, s37 - d37]


def _twiddle16(z, k):
    re, im = z
    k = k % 16
    if k == 0:
        return z
    if k == 4:
        return (im, -re)
    if k == 12:
        return (-im, re)
    if k == 2:
        return ((re + im) * RC, (im - re) * RC)
    if k == 14:
        return ((re - im) * RC, (re + im) * RC)
    if k == 6:
        return ((im - re) * RC, (re + im) * -RC)
    if k == 10:
        return ((re + im) * -RC, (re - im) * RC)
    c, s = float(np.cos(2 * np.pi * k / 16)), float(-np.sin(2 * np.pi * k / 16))
    return (re * c - im * s, re * s + im * c)


def _bfly4(z, sign):
    (ar, ai), (br, bi), (cr, ci), (dr, di) = z
    sr, si, tr, ti = ar + cr, ai + ci, ar - cr, ai - ci
    ur, ui, vr, vi = br + dr, bi + di, br - dr, bi - di
    o0, o2 = (sr + ur, si + ui), (sr - ur, si - ui)
    p, q = (tr + vi, ti - vr), (tr - vi, ti + vr)
    return [o0, p, o2, q] if sign > 0 else [o0, q, o2, p]


class _Pacer:
    def __init__(self, tasks, ntokens):
        self.slots = {}
        for n, task in enumerate(tasks):
            self.slots.setdefault(n * ntokens // len(tasks), []).append(task)
        self.pos = 0

    def feed(self, r):
        for j in range(r.shape[0] // 8):
            for task in self.slots.pop(self.pos, []):
                task(pltpu.bitcast(r[8 * j:8 * j + 8], u32))
            self.pos += 1

    def done(self):
        assert not self.slots


def _pack_rows(m):
    b = np.asarray(m, np.float32).astype(jnp.bfloat16).view(np.uint16).astype(np.uint32)
    return b[..., 0::2, :] | (b[..., 1::2, :] << 16)


@functools.lru_cache(maxsize=None)
def _dft_constants():
    b8 = np.array(_fwd8(list(np.eye(8)))).T
    n = np.arange(D)
    fw = np.zeros((D, D))
    bw = np.zeros((D, D))
    for g in range(4):
        k = np.concatenate([8 * np.arange(64) + r for r in RES[g]])
        ang = 2 * np.pi * ((n[:, None] * k[None, :]) % D) / D
        wgt = np.where(k == 0, 1.0, 2.0) / (D * S)
        fw[:, 256 * g:256 * g + 128] = np.cos(ang)
        fw[:, 256 * g + 128:256 * g + 256] = -np.sin(ang)
        bw[256 * g:256 * g + 128] = (np.cos(ang) * wgt).T
        bw[256 * g + 128:256 * g + 256] = (-np.sin(ang) * wgt).T
    bw[128, :] = (-1.0) ** n / (D * S)
    binv = np.kron(np.linalg.inv(b8), np.eye(128))
    gall = binv @ fw
    giall = bw @ binv.T
    gf = np.zeros((11, 144, 128))
    gi = np.zeros((11, 128, 128))
    sign = []
    half = lambda m, q: np.concatenate([m[64 * q:64 * q + 64], m[128 + 64 * q:192 + 64 * q]])
    for g in range(4):
        sl = slice(256 * g, 256 * g + 256)
        f, b = gall[sl, sl].T, giall[sl, sl]
        if g == 0:
            for q in range(2):
                gf[q, :128] = half(f, q)[:, 128 * q:128 * q + 128]
                gi[q] = half(b, q)[:, 128 * q:128 * q + 128]
            gf[0, 128] = (-1.0) ** np.arange(128)
            continue
        sg = np.sign(f[:128, 0] * f[128:, 128])[:, None]
        sign.append((int(sg[0, 0]), int(sg[64, 0])))
        p, q, r = f[:128, :128], f[:128, 128:], f[128:, :128]
        gf[3 * g - 1:3 * g + 2, :128] = p, q - p, r - sg * p
        p, q, r = b[:128, :128], b[:128, 128:], b[128:, :128]
        gi[3 * g - 1:3 * g + 2] = p, r - sg * p, q - p
    a = np.arange(128)
    mt = np.zeros((4, 16, 128, 128))
    for b in range(16):
        ang = 2 * np.pi * (((16 * a[:, None] + b) * a[None, :]) % S) / S
        c, sn = np.cos(ang), -np.sin(ang)
        mt[:, b] = c, c + sn, sn - c, sn
    return _pack_rows(gf), _pack_rows(gi), _pack_rows(mt), tuple(sign)


def _attn_fill():
    pos32 = np.arange(32)
    last = np.arange(16)
    qhead = np.concatenate([np.arange(64) // 32, last // 8])
    khead = np.concatenate([np.arange(64) // 32, last % 2])
    qpos = np.concatenate([pos32, pos32, 32 + last % 8])
    kpos = np.concatenate([pos32, pos32, 32 + last // 2])
    ok = (qpos[:, None] < M) | (qpos[:, None] >= kpos[None, :])
    fill = np.where(ok, 0.0, -1e9)
    fill = np.where(qhead[:, None] == khead[None, :], fill, -np.inf)
    return fill.astype(np.float32)


def _strassen(prod, b11, b12, b21, b22, add, sub, emit):
    m2 = prod(1, b11())
    m1 = prod(0, add(b11(), b22()))
    m3 = prod(2, sub(b12(), b22()))
    c22 = prod(5, add(b11(), b12())) + ((m1 - m2) + m3)
    m4 = prod(3, sub(b21(), b11()))
    emit(1, m2 + m4, c22)
    m5 = prod(4, b22())
    emit(0, prod(6, add(b21(), b22())) + ((m1 + m4) - m5), m3 + m5)


class _Blocks(list):
    def __add__(self, other):
        return _Blocks(a + b for a, b in zip(self, other))

    def __sub__(self, other):
        return _Blocks(a - b for a, b in zip(self, other))


def _strassen_left(a11, a12, a21, a22):
    return [a11 + a22, a21 + a22, a11, a22, a11 + a12, a21 - a11, a12 - a22]


def _kernel(x_hbm, mem_hbm, wq_hbm, wk_hbm, wv_hbm, wo_hbm, bx_hbm, wr_hbm, wi_hbm,
            gf_hbm, gi_hbm, mt_hbm, fill_hbm, out_hbm,
            wraw, wall, wo, xbuf, mem0, x8, xs, xs2, pre, osum, outbuf, fill_ref,
            xb, wt, wl, gf, gi, mt, xd, yb, sems):
    def start(src, dst, sem, priority=0):
        c = pltpu.make_async_copy(src, dst, sems.at[sem])
        c.start(priority=priority)
        return c

    def wait_all(cs):
        for c in cs:
            c.wait()

    dot = functools.partial(jnp.dot, preferred_element_type=f32)
    dot_nt = lambda a, b: lax.dot_general(a, b, (((1,), (1,)), ((), ())), preferred_element_type=f32)
    cat = lambda *vs: jnp.concatenate(vs, axis=0)
    as_bf16 = lambda w: pltpu.bitcast(w, bf16)
    lo_f32 = lambda w: pltpu.bitcast(w << 16, f32)
    hi_f32 = lambda w: pltpu.bitcast(w & u32(0xFFFF0000), f32)
    pack2 = lambda a, b: pltpu.pack_elementwise([a, b], packed_dtype=bf16)
    add2 = lambda a, b: pack2(lo_f32(a) + lo_f32(b), hi_f32(a) + hi_f32(b))
    sub2 = lambda a, b: pack2(lo_f32(a) - lo_f32(b), hi_f32(a) - hi_f32(b))
    out4 = out_hbm.reshape(NSEG // 2, 2, SEG, 2 * D)
    w_hbm = (wq_hbm, wk_hbm, wv_hbm)

    def start_unit(u):
        return start(w_hbm[u // 2].at[:, :, u % 2], wraw.at[u % NRAW], u % NRAW)

    def start_x(seg0, nseg, sem, priority=0):
        segs, rows = pl.ds(seg0, nseg), pl.ds(0, SEG - M)
        return start(x_hbm.at[segs, rows, :], xbuf.at[segs, rows, :], sem, priority)

    def start_filter(row0, nrows, sem, priority=0):
        rows = pl.ds(row0, nrows)
        return [start(w.at[rows, pl.ds(128 * d, 128)], wt.at[t, d, rows], sem, priority)
                for t, w in enumerate((wr_hbm, wi_hbm)) for d in range(16)]

    c_a = []
    for n in range(4):
        cols, rows = pl.ds(256 * n, 256), pl.ds(128 * n, 128)
        c_a.append([start(x_hbm.at[:, pl.ds(SEG - M, M), cols], x8.at[:, :, cols], n),
                    start(wq_hbm.at[rows, :, 0], wraw.at[0, rows], n)])
    c_loop = [start_x(0, UNROLL, 4, 1), start(mem_hbm, mem0, 4, 1), start(fill_hbm, fill_ref.at[pl.ds(0, 80)], 4, 1)]
    c_loop += [start(wo_hbm.at[:, pl.ds(128 * j, 128)], wo.at[j], 4, 1) for j in range(8)]

    wraw32 = wraw.bitcast(u32)
    wt32 = wt.bitcast(u32)
    xb32 = xb.bitcast(u32)

    def relayout_row(src, dst, r, lo, hi):
        a, b = src[r, 0], src[r, 1]
        dst[pl.ds(r, 8, stride=WP), :] = (a & lo) | (b << 16)
        dst[pl.ds(r + 8 * WP, 8, stride=WP), :] = (a >> 16) | (b & hi)

    def relayout_tasks(u, r0=0, r1=D // 2):
        src, dst = wraw32.at[u % NRAW], wall.at[u]

        def make(r):
            def task(tok):
                lo = (tok >> 16) | u32(0xFFFF)
                hi = (tok << 16) | u32(0xFFFF0000)
                relayout_row(src, dst, r, lo, hi)
                relayout_row(src, dst, r + 1, lo, hi)
            return task
        return [make(r) for r in range(r0, r1, 2)]

    def y_blocks(r):
        return pl.ds(4 * (r % 2) + r // 2, 8, stride=8)

    def filter_tasks(blk, wfn):
        def make(phase, k):
            slots = [4 * k + j for j in range(4)] if phase == 1 else [4 * j + k for j in range(4)]

            def task(tok):
                ones = ((tok >> 16) | u32(0xFFFF)) | u32(0xFFFF0000)
                z = [(yb[0, b, blk], yb[1, b, blk]) for b in slots]
                z[0] = tuple(pltpu.bitcast(pltpu.bitcast(v, u32) & ones, f32) for v in z[0])
                if phase == 0:
                    o = _bfly4(z, 1)
                    o = [_twiddle16(o[j], k * j) for j in range(4)]
                elif phase == 1:
                    o = _bfly4(z, 1)
                    y = []
                    for j in range(4):
                        wr, wi = wfn(k + 4 * j)
                        xr, xi = o[j]
                        y.append((xr * wr - xi * wi, xr * wi + xi * wr))
                    o = _bfly4(y, -1)
                    o = [_twiddle16(o[j], -k * j) for j in range(4)]
                else:
                    o = _bfly4(z, -1)
                for b, v in zip(slots, o):
                    yb[0, b, blk] = v[0]
                    yb[1, b, blk] = v[1]
            return task
        return [make(phase, k) for phase in range(3) for k in range(4)]

    def z_region(n, par):
        return (2 * n + par) // 3, (2 * n + par) % 3 * 8 * ZP

    def butterfly_tasks(par):
        def make(a2):
            def task(tok):
                zs = []
                for a in (2 * a2, 2 * a2 + 1):
                    w = [xb32[j, pl.ds(8 * a, 8), :] for j in range(8)]
                    if par:
                        hi = (tok << 16) | u32(0xFFFF0000)
                        z = _fwd8([pltpu.bitcast(v & hi, f32) for v in w])
                    else:
                        sixteen = ((tok >> 31) | u32(1)) << 4
                        z = _fwd8([pltpu.bitcast(v << sixteen, f32) for v in w])
                    zs.append(z[0:2] + [v for g in range(1, 4)
                                        for v in (z[2 * g] + z[2 * g + 1], z[2 * g + 1], z[2 * g])])
                for n in range(11):
                    plane, row = z_region(n, par)
                    xd[plane, pl.ds(row + a2, 8, stride=ZP), :] = pltpu.bitcast(pack2(zs[0][n], zs[1][n]), f32)
            return task
        return [make(a2) for a2 in range(64)]

    sign = _dft_constants()[3]

    def b_dfwd(b, pacer):
        def z(n):
            plane, row = z_region(n, b % 2)
            return as_bf16(xd[plane, pl.ds(row + b // 2 * ZP, 64), :])
        t0 = dot_nt(as_bf16(gf[0]), z(0))
        t4 = dot_nt(as_bf16(gf[1, 0:64]), z(1))
        tr, ti = cat(t0[0:64], t4[0:64]), cat(t0[64:128], t4[64:128])
        ts = [(cat(tr + ti, t0[128:144]).astype(bf16), ti.astype(bf16), cat(tr, t0[128:144]).astype(bf16))]
        for g in range(1, 4):
            k1, k2, k3 = [dot_nt(as_bf16(gf[n, 0:64]), z(n)) for n in range(3 * g - 1, 3 * g + 2)]
            pacer.feed(k1)
            tr = k1 + k2
            ti = cat(*[k3[64 * q:64 * q + 64] + k1[64 * q:64 * q + 64] if sign[g - 1][q] > 0
                       else k3[64 * q:64 * q + 64] - k1[64 * q:64 * q + 64] for q in range(2)])
            ts.append(((tr + ti).astype(bf16), ti.astype(bf16), tr.astype(bf16)))
        return ts

    def b_sfwd(b, ts, pacer):
        for g in range(4):
            k1, k2, k3 = [dot(ts[g][n], as_bf16(mt[n, b])) for n in range(3)]
            if g:
                pacer.feed(k2)
            yr, yi = k1[0:128] - k2, k1 + k3
            for q in range(2):
                yb[0, b, y_blocks(RES[g][q])] = yr[64 * q:64 * q + 64].reshape(8, 8, 128)
                yb[1, b, y_blocks(RES[g][q])] = yi[64 * q:64 * q + 64].reshape(8, 8, 128)
            if g == 0:
                yb[0, b, 64] = k1[128:136]
                yb[1, b, 64] = yi[128:136]

    def b_stage1(tasks):
        pacer = _Pacer(tasks, NBT * 48)
        prev = None
        for b in list(range(0, 16, 2)) + list(range(1, 16, 2)):
            ts = b_dfwd(b, pacer)
            if prev is not None:
                b_sfwd(*prev, pacer)
            prev = (b, ts)
        b_sfwd(*prev, pacer)
        pacer.done()

    def b_stage3():
        row0 = lax.broadcasted_iota(jnp.int32, (8, 128), 0) == 0
        low = lax.broadcasted_iota(jnp.int32, (1, 128), 1) < 64
        for b in range(16):
            m = [as_bf16(mt[n, b]) for n in range(4)]
            for g in (1, 2, 3, 0):
                yr, yi = [cat(*[yb[c, b, y_blocks(r)].reshape(64, 128) for r in RES[g]]) for c in range(2)]
                if g == 0:
                    nr = -yr
                    u0 = cat(yr[0:64], jnp.where(row0, yb[0, b, 64], yi[0:8]), yi[8:64])
                    v0 = cat(yi[0:64], jnp.where(row0, yb[1, b, 64], nr[0:8]), nr[8:64])
                    u4, v4 = cat(yr[64:128], yi[64:128]), cat(yi[64:128], nr[64:128])
                    t1 = dot_nt(m[0], u0.astype(bf16)) + dot_nt(m[3], v0.astype(bf16))
                    t2 = dot_nt(m[0], u4.astype(bf16)) + dot_nt(m[3], v4.astype(bf16))
                else:
                    k1, k2, k3 = [dot_nt(m[n], v.astype(bf16)) for n, v in enumerate((yr + yi, yr, yi))]
                    t1, t2 = k1 + k3, k1 - k2
                slot = b // 2 + 8 * (b % 2)
                xd[2 * g, pl.ds(XP * slot, 128), :] = t1
                xd[2 * g + 1, pl.ds(XP * slot, 128), :] = t2
        for t in range(16):
            rows = lambda j: cat(*[xd[j, pl.ds(8 * t + u, 16, stride=XP), :] for u in range(8)])
            z = [dot(rows(q).astype(bf16), as_bf16(gi[q])) for q in range(2)]
            for g in range(1, 4):
                tr, ti = rows(2 * g), rows(2 * g + 1)
                sg = jnp.where(low, float(sign[g - 1][0]), float(sign[g - 1][1]))
                k1, k2, k3 = [dot(v.astype(bf16), as_bf16(gi[3 * g - 1 + n]))
                              for n, v in enumerate((tr + sg * ti, ti, tr))]
                z += [k1 + k2, k1 + k3]
            y = _inv8(z)
            for j in range(8):
                even = cat(*[y[j][16 * u:16 * u + 8] for u in range(8)])
                odd = cat(*[y[j][16 * u + 8:16 * u + 16] for u in range(8)])
                xb32[j, pl.ds(64 * t, 64), :] = pack2(even, odd)

    HALF = NSEG * M // 2

    def batch(u, p0, p1, tasks=(), t0=0, t1=4):
        mc = HALF // 2 if t1 - t0 <= MCT else HALF
        pacer = _Pacer(tasks, (7 * (p1 - p0) - MARGIN // (t1 - t0)) * HALF // 8)
        w = wall.at[u]
        for p in range(p0, p1):
            for r0 in range(0, HALF, mc):
                def blk(head, par):
                    return lambda: cat(*[w[pl.ds((p + 8 * head) * WP + 64 * (2 * t + par), 64), :]
                                         for t in range(t0, t1)])

                def prod(i, b):
                    lhs = jnp.concatenate([as_bf16(xs[i, t, pl.ds(r0 // 2, mc // 2), :])
                                           for t in range(t0, t1)], axis=1)
                    r = dot(lhs, as_bf16(b))
                    pacer.feed(r)
                    return r

                def emit(half, *cs):
                    rows = pl.ds(half * HALF + r0, mc)
                    park = pl.ds((half * HALF + r0) // 8, mc // 8)
                    if t0 > 0:
                        cs = [c + yb[t, p, park].reshape(mc, E) for t, c in enumerate(cs)]
                    if t1 < 4:
                        for t, c in enumerate(cs):
                            yb[t, p, park] = c.reshape(mc // 8, 8, E)
                    elif u >= 2:
                        pre[8 * u + p, rows, :] = pack2(*cs)
                    else:
                        st = jnp.concatenate([c.reshape(mc // M, M, E) for c in cs], axis=1)
                        pre[8 * u + p, rows, :] = pltpu.bitcast(st.reshape(2 * mc, E).astype(bf16), u32)
                _strassen(prod, blk(0, 0), blk(1, 0), blk(0, 1), blk(1, 1), add2, sub2, emit)
        pacer.done()

    QUART = HALF // 2

    def unpack_after(w, tok):
        reps = (w.shape[0] // 8, 1)
        hi = jnp.tile((tok << 16) | u32(0xFFFF0000), reps)
        sixteen = jnp.tile(((tok >> 31) | u32(1)) << 4, reps)
        return _Blocks([pltpu.bitcast(w << sixteen, f32), pltpu.bitcast(w & hi, f32)])

    def batch2(u, q0, q1, done, tasks=()):
        pacer = _Pacer(tasks, (49 * (q1 - q0) - MARGIN) * QUART // 8)
        w = wall.at[u]

        def unpack(b):
            if isinstance(b, _Blocks):
                return b
            if len(done) < LAG:
                return _Blocks([lo_f32(b), hi_f32(b)])
            return unpack_after(b, done[-LAG])
        add4 = lambda a, b: unpack(a) + unpack(b)
        sub4 = lambda a, b: unpack(a) - unpack(b)
        for q in range(q0, q1):
            def outer_blk(pair, kh):
                return lambda: [cat(*[w[pl.ds((2 * q + pair + 8 * head) * WP + 64 * (2 * kh + kl + 4 * t), 64), :]
                                      for t in range(2)]) for kl in range(2) for head in range(2)]

            def outer_prod(i, bs):
                def prod(j, b):
                    lhs = jnp.concatenate([as_bf16(xs2[7 * i + j, t]) for t in range(2)], axis=1)
                    r = dot(lhs, as_bf16(pack2(*b) if isinstance(b, _Blocks) else b))
                    pacer.feed(r)
                    done.append(pltpu.bitcast(r[0:8], u32))
                    return r
                cs = {}
                _strassen(prod, *[(lambda b=b: b) for b in bs], add4, sub4,
                          lambda half, *c: cs.update({half: c}))
                return _Blocks(cs[0] + cs[1])

            def emit(half, *cs):
                for pair, c in enumerate(cs):
                    for a in range(2):
                        rows = pl.ds(half * HALF + a * QUART, QUART)
                        pre[8 * u + 2 * q + pair, rows, :] = pack2(c[2 * a], c[2 * a + 1])
            _strassen(outer_prod, outer_blk(0, 0), outer_blk(1, 0), outer_blk(0, 1), outer_blk(1, 1),
                      lambda x, y: [add4(a, b) for a, b in zip(x, y)],
                      lambda x, y: [sub4(a, b) for a, b in zip(x, y)], emit)
        pacer.done()

    def left2_tasks():
        def make(i, t, r):
            def task(tok):
                def blk(rh, kh):
                    ws = [pltpu.bitcast(x8[pl.ds(32 * rh + 16 * rl + 2 * r, 2), :,
                                           pl.ds(128 * (2 * kh + kl + 4 * t), 128)].reshape(16, 128), u32)
                          for rl in range(2) for kl in range(2)]
                    return _Blocks(unpack_after(v, tok) for v in ws)
                terms = ((0, 3, 1), (2, 3, 1), (0,), (3,), (0, 1, 1), (2, 0, -1), (1, 3, -1))[i]
                a = blk(*divmod(terms[0], 2))
                if len(terms) > 1:
                    b = blk(*divmod(terms[1], 2))
                    a = a + b if terms[2] > 0 else a - b
                for j, v in enumerate(_strassen_left(*a)):
                    xs2[7 * i + j, t, pl.ds(8 * r, 8), :] = pack2(*v)
            return task
        return [make(i, t, r) for i in range(7) for t in range(2) for r in range(8)]

    def prepare_left(n):
        v = pltpu.bitcast(x8[:, :, pl.ds(256 * n, 256)].reshape(2 * HALF, 256), u32)
        blocks = [v[HALF // 2 * h:HALF // 2 * (h + 1), 128 * k:128 * (k + 1)] for h in range(2) for k in range(2)]
        lo, hi = [_strassen_left(*[un(b) for b in blocks]) for un in (lo_f32, hi_f32)]
        for i in range(7):
            xs[i, n] = pack2(lo[i], hi[i])

    wait_all(c_a[0])
    for task in relayout_tasks(0, 0, 128):
        task(jnp.zeros((8, 128), u32))
    prepare_left(0)
    batch(0, 0, 6, (), 0, 1)
    wait_all(c_a[1])
    c_h = [start(wq_hbm.at[pl.ds(256 * n, 256), :, 1], wraw.at[1, pl.ds(256 * n, 256)], n) for n in range(2)]
    prepare_left(1)
    batch(0, 6, 8, relayout_tasks(0, 128, 256), 0, 1)
    batch(0, 0, 6, (), 1, 2)
    wait_all(c_a[2])
    prepare_left(2)
    batch(0, 6, 8, relayout_tasks(0, 256, 384), 1, 2)
    batch(0, 0, 6, (), 2, 3)
    wait_all(c_a[3])
    c_w2 = start_unit(2)
    prepare_left(3)
    batch(0, 6, 8, relayout_tasks(0, 384, 512), 2, 3)
    batch(0, 0, 5, (), 3, 4)
    c_h[0].wait()
    batch(0, 5, 8, relayout_tasks(1, 0, 256), 3, 4)
    left2 = left2_tasks()
    batch(1, 0, 5, left2[:64], 0, 2)
    c_h[1].wait()
    start_unit(3)
    batch(1, 5, 8, relayout_tasks(1, 256, 512), 0, 2)
    batch(1, 0, 4, left2[64:], 2, 4)
    c_w2.wait()
    start_unit(4)
    start_unit(5)
    c_b1 = [start(bx_hbm.at[:, pl.ds(128 * j, 128)], xb.at[j], 5) for j in range(8)]
    c_b1 += [start(gf_hbm, gf.at[pl.ds(0, 11)], 5), start(mt_hbm.at[pl.ds(0, 3)], mt.at[pl.ds(0, 3)], 5)]
    c_loop += start_filter(0, 64, 4, 1)
    batch(1, 4, 8, relayout_tasks(2), 2, 4)
    batch2(2, 0, 2, [])

    def unit_body(u, c):
        slot = (u + 1) % NRAW
        pltpu.make_async_copy(wraw.at[slot], wraw.at[slot], sems.at[slot]).wait()
        done = []
        batch2(u, 2, 4, done, relayout_tasks(u + 1))
        batch2(u + 1, 0, 2, done)
        return c
    lax.fori_loop(2, 5, unit_body, 0)
    wait_all(c_b1)
    bfly = butterfly_tasks(0) + butterfly_tasks(1)
    batch(5, 6, 8, bfly[:NB0])
    batch2(5, 2, 3, [])
    b_stage1(bfly[NB0:])
    wait_all(c_loop)
    c_rest = [start_x(UNROLL, NSEG - UNROLL, 6)] + start_filter(64, 448, 6)
    c_b3 = [start(w.at[pl.ds(512, 1), :], wl.at[t], 5) for t, w in enumerate((wr_hbm, wi_hbm))]
    c_b3 += [start(gi_hbm, gi, 5), start(mt_hbm.at[3], mt.at[3], 5)]

    wo32 = wo.bitcast(u32)
    scale = E ** -0.5

    def gated(w, toks):
        if not toks:
            return w
        bits = functools.reduce(
            jnp.bitwise_or, [pltpu.bitcast(jnp.broadcast_to(t, (8, 128)), u32) for t in toks])
        ones = ((bits >> 16) | u32(0xFFFF)) | u32(0xFFFF0000)
        return cat(w[0:8] & ones, w[8:])

    def wqkv(i, p, second, toks=(), k0=0, k1=D):
        rows = pl.ds((p % 8 + 8 * second) * WP + k0 // 2, (k1 - k0) // 2)
        return as_bf16(gated(wall[2 * i + p // 8, rows, :], toks))

    def step(n, u, mem, held):
        s = UNROLL * n + u
        rows = cat(mem, xbuf[s, pl.ds(0, SEG - M), :].astype(f32))
        lhs = rows.astype(bf16)
        head_start = {}
        if u:
            lo, hi = rows[:, :D // 2].astype(bf16), rows[:, D // 2:].astype(bf16)
            for key in EARLY:
                head_start[key] = dot(lo, wqkv(*key, k1=D // 2))
        r8 = pl.multiple_of(M * s, M)
        fill = fill_ref[pl.ds(0, 80), :]
        heads = [None] * H
        rs = []

        shift = jnp.full((8, 128), 16 - 16 * (n % 2), jnp.int32).astype(u32)
        wblk = pl.ds(pl.multiple_of(32 * (n // 2), 32), 32)
        flt = filter_tasks(
            s, lambda d: [hi_f32(wt32.at[t, d, wblk][pl.ds(u, 8, stride=4), :] << shift) for t in range(2)])
        pacer = _Pacer(flt, 48)

        def proj(i, p, toks=()):
            a, b = [
                dot(hi, wqkv(i, p, t, k0=D // 2)) + head_start[i, p, t] if (i, p, t) in head_start
                else dot(lhs, wqkv(i, p, t, toks[t * len(toks) // 2:(t + 1) * len(toks) // 2]))
                for t in range(2)]
            pacer.feed(a)
            pacer.feed(b)
            c = as_bf16(pre[16 * i + p, pl.ds(r8, M), :]).astype(f32)
            return cat(a, b, c).astype(bf16)

        def probs(q, k):
            sc = dot_nt(q, k) * scale
            sc = jnp.where(fill == 0.0, sc, fill)
            e = jnp.exp(sc - jnp.max(sc, axis=1, keepdims=True))
            l = jnp.sum(e, axis=1, keepdims=True)
            r = pl.reciprocal(l, approx=True)
            r = r * (2.0 - l * r)
            rs.append([r[8 * j:8 * j + 8] for j in range(10)])
            return (e * r).astype(bf16)

        def pv(p, pr, v):
            o = dot(pr, v)
            heads[2 * p] = cat(o[0:8], o[16:32], o[64:72])
            heads[2 * p + 1] = cat(o[32:40], o[48:64], o[72:80])
            held[u % 2, p] = (o[8:16], o[40:48])

        def left_task(p):
            def task(tok):
                ones = ((tok >> 16) | u32(0xFFFF)) | u32(0xFFFF0000)
                a11, a12, a21, a22 = held[0, p] + held[1, p]
                a11, a22 = [pltpu.bitcast(pltpu.bitcast(a, u32) & ones, f32) for a in (a11, a22)]
                dst = pl.ds(pl.multiple_of(M * (UNROLL // 2 * n + u // 2), M), M)
                for i, a in enumerate(_strassen_left(a11, a12, a21, a22)):
                    osum[i, p, dst, :] = a.astype(bf16)
            return task

        pend = []
        for g in range(4):
            ps = range(4 * g, 4 * g + 4)
            qk = [(proj(0, p), proj(1, p)) for p in ps]
            vs = [proj(2, p, rs[p - 4] if g else ()) for p in ps]
            for a in pend:
                pv(*a)
            pend = [(p, probs(*qk[t]), vs[t]) for t, p in enumerate(ps)]
        pacer.done()

        def wo_part(oc, j, h0, h1, toks=()):
            return dot(oc, as_bf16(gated(wo32[j, pl.ds(64 * h0, 64 * (h1 - h0)), :], toks)))

        acc = []
        pacer = _Pacer([left_task(p) for p in range(16)] if u % 2 else (), 4 * 10)
        oc = jnp.concatenate(heads[0:24], axis=1).astype(bf16)
        for j in range(8):
            acc.append(wo_part(oc, j, 0, 24, {3: rs[12] + rs[13], 4: rs[14] + rs[15]}.get(j, ())))
            if j == 4:
                for a in pend:
                    pv(*a)
            if j > 5:
                pacer.feed(acc[j])
        oc = jnp.concatenate(heads[24:32], axis=1).astype(bf16)
        nxt = []
        for j in range(8):
            r = wo_part(oc, j, 24, 32) + acc[j]
            outbuf[UNROLL // 2 * n + u // 2, u % 2, pl.ds(M, SEG - M), pl.ds(128 * j, 128)] = r[M:].astype(bf16)
            nxt.append(r[0:M])
            pacer.feed(r)
        pacer.done()
        return jnp.concatenate(nxt, axis=1)

    def steps(n, mem):
        pl.when(n == 1)(functools.partial(wait_all, c_rest))
        held = {}
        for u in range(UNROLL):
            mem = step(n, u, mem, held)
        return mem
    lax.fori_loop(0, NSEG // UNROLL, steps, mem0[...].astype(f32))
    tok_rows = pl.ds(M, SEG - M)
    c_out = [start(outbuf.at[:, :, tok_rows, :], out4.at[:, :, tok_rows, pl.ds(0, D)], 0)]

    wait_all(c_b3)
    for task in filter_tasks(64, lambda d: [wl[t, :, pl.ds(128 * d, 128)].astype(f32) for t in range(2)]):
        task(jnp.zeros((8, 128), u32))
    b_stage3()
    c_out += [start(xb.at[j], out_hbm.at[:, pl.ds(D + 128 * j, 128)], 0) for j in range(8)]

    osum32 = osum.bitcast(u32)
    for jp in range(4):
        def blk(col, par):
            return lambda: cat(*[wo32[2 * jp + col, pl.ds(64 * (2 * p + par), 64), :] for p in range(16)])

        def prod(i, b):
            return dot(jnp.concatenate([as_bf16(osum32[i, p]) for p in range(16)], axis=1), as_bf16(b))

        def emit(half, *cs):
            for t, c in enumerate(cs):
                outbuf[:, half, pl.ds(0, M), pl.ds(128 * (2 * jp + t), 128)] = (
                    c.reshape(NSEG // 2, M, 128).astype(bf16))
            cols = pl.ds(256 * jp, 256)
            c_out.append(start(outbuf.at[:, half, pl.ds(0, M), cols], out4.at[:, half, pl.ds(0, M), cols], 0))
        _strassen(prod, blk(0, 0), blk(1, 0), blk(0, 1), blk(1, 1), add2, sub2, emit)
    wait_all(c_out)


@functools.partial(jax.jit, static_argnames=("A_seg_len",))
def pallas_concat_heads__memory_aug_recurrent_mem_tr__spectral_gfnet__prompt_kernel(
    A_x: jax.Array,
    A_mem0: jax.Array,
    A_Wq: jax.Array,
    A_Wk: jax.Array,
    A_Wv: jax.Array,
    A_Wo: jax.Array,
    A_seg_len,
    B_x: jax.Array,
    B_w_r: jax.Array,
    B_w_i: jax.Array,
):
    assert A_seg_len == SEG
    assert A_x.shape == (1, S, D) and A_mem0.shape == (1, M, D) and B_x.shape == (1, S, D)
    assert A_Wq.shape == (D, H, E) and A_Wo.shape == (H, E, D) and B_w_r.shape == (S, D // 2 + 1)
    gf, gi, mt, _ = _dft_constants()
    fill = _attn_fill()
    hbm = pl.BlockSpec(memory_space=pltpu.HBM)
    wshape = (D // 2, 2, 2, 16, E)
    out = pl.pallas_call(
        _kernel,
        out_shape=jax.ShapeDtypeStruct((S, 2 * D), bf16),
        in_specs=[hbm] * 13,
        out_specs=hbm,
        scratch_shapes=[
            pltpu.VMEM((NRAW, D // 2, 2, 16, E), bf16),
            pltpu.VMEM((6, 16 * WP, E), u32),
            pltpu.VMEM((8, H * E, 128), bf16),
            pltpu.VMEM((NSEG, SEG, D), bf16),
            pltpu.VMEM((M, D), bf16),
            pltpu.VMEM((NSEG, M, D), bf16),
            pltpu.VMEM((7, 4, 128, 128), u32),
            pltpu.VMEM((49, 2, 64, 128), u32),
            pltpu.VMEM((48, NSEG * M, E), u32),
            pltpu.VMEM((7, 16, NSEG * M // 2, E), bf16),
            pltpu.VMEM((NSEG // 2, 2, SEG, D), bf16),
            pltpu.VMEM((96, 80), f32),
            pltpu.VMEM((8, S, 128), bf16),
            pltpu.VMEM((2, 16, 512, 128), bf16),
            pltpu.VMEM((2, 1, S), bf16),
            pltpu.VMEM((12,) + gf.shape[1:], u32),
            pltpu.VMEM(gi.shape, u32),
            pltpu.VMEM(mt.shape, u32),
            pltpu.VMEM((8, 16 * XP, 128), f32),
            pltpu.VMEM((2, 16, 65, 8, 128), f32),
            pltpu.SemaphoreType.DMA((7,)),
        ],
        compiler_params=pltpu.CompilerParams(vmem_limit_bytes=120 * 1024 * 1024),
    )(A_x.reshape(NSEG, SEG, D), A_mem0.reshape(M, D),
      A_Wq.reshape(wshape), A_Wk.reshape(wshape), A_Wv.reshape(wshape),
      A_Wo.reshape(H * E, D), B_x.reshape(S, D), B_w_r.T, B_w_i.T, gf, gi, mt, fill)
    return out.reshape(1, S, 2 * D)
```

```python
import functools

import jax
import jax.numpy as jnp
import numpy as np
from jax import lax
from jax.experimental import pallas as pl
from jax.experimental.pallas import tpu as pltpu

S, D, H, E, M, SEG = 2048, 1024, 32, 128, 8, 32
NSEG = S // SEG
WP = 516
XP = 132
ZP = 68
NRAW = 4
UNROLL = 4
MCT = 1
LAG = 8
NB0 = 64
NBT = 13
MARGIN = 8
EARLY = ((0, 0, 0), (0, 0, 1), (1, 0, 0), (1, 0, 1), (0, 1, 0), (0, 1, 1))
bf16, f32, u32 = jnp.bfloat16, jnp.float32, jnp.uint32
RES = ((0, 4), (2, 6), (1, 7), (3, 5))
RC = float(np.sqrt(0.5))


def _fwd8(x):
    s04, d04 = x[0] + x[4], x[0] - x[4]
    s26, d26 = x[2] + x[6], x[2] - x[6]
    s15, d15 = x[1] + x[5], x[1] - x[5]
    s37, d37 = x[3] + x[7], x[3] - x[7]
    t1, t2 = (d15 - d37) * RC, (d15 + d37) * RC
    e0, o0 = s04 + s26, s15 + s37
    return [e0 + o0, e0 - o0, s04 - s26, s15 - s37, d04 + t1, d26 + t2, d04 - t1, d26 - t2]


def _inv8(z):
    z0, z4, e1, o1, r1, i1, r3, i3 = z
    e0, o0 = z0 + z4, z0 - z4
    s04, s26, s15, s37 = e0 + e1, e0 - e1, o0 + o1, o0 - o1
    d04, d26 = r1 + r3, i1 + i3
    t1, t2 = (r1 - r3) * RC, (i1 - i3) * RC
    d15, d37 = t1 + t2, t2 - t1
    return [s04 + d04, s15 + d15, s26 + d26, s37 + d37, s04 - d04, s15 - d15, s26 - d26, s37 - d37]


def _twiddle16(z, k):
    re, im = z
    k = k % 16
    if k == 0:
        return z
    if k == 4:
        return (im, -re)
    if k == 12:
        return (-im, re)
    if k == 2:
        return ((re + im) * RC, (im - re) * RC)
    if k == 14:
        return ((re - im) * RC, (re + im) * RC)
    if k == 6:
        return ((im - re) * RC, (re + im) * -RC)
    if k == 10:
        return ((re + im) * -RC, (re - im) * RC)
    c, s = float(np.cos(2 * np.pi * k / 16)), float(-np.sin(2 * np.pi * k / 16))
    return (re * c - im * s, re * s + im * c)


def _bfly4(z, sign):
    (ar, ai), (br, bi), (cr, ci), (dr, di) = z
    sr, si, tr, ti = ar + cr, ai + ci, ar - cr, ai - ci
    ur, ui, vr, vi = br + dr, bi + di, br - dr, bi - di
    o0, o2 = (sr + ur, si + ui), (sr - ur, si - ui)
    p, q = (tr + vi, ti - vr), (tr - vi, ti + vr)
    return [o0, p, o2, q] if sign > 0 else [o0, q, o2, p]


class _Pacer:
    def __init__(self, tasks, ntokens):
        self.slots = {}
        for n, task in enumerate(tasks):
            self.slots.setdefault(n * ntokens // len(tasks), []).append(task)
        self.pos = 0

    def feed(self, r):
        for j in range(r.shape[0] // 8):
            for task in self.slots.pop(self.pos, []):
                task(pltpu.bitcast(r[8 * j:8 * j + 8], u32))
            self.pos += 1

    def done(self):
        assert not self.slots


def _pack_rows(m):
    b = np.asarray(m, np.float32).astype(jnp.bfloat16).view(np.uint16).astype(np.uint32)
    return b[..., 0::2, :] | (b[..., 1::2, :] << 16)


@functools.lru_cache(maxsize=None)
def _dft_constants():
    b8 = np.array(_fwd8(list(np.eye(8)))).T
    n = np.arange(D)
    fw = np.zeros((D, D))
    bw = np.zeros((D, D))
    for g in range(4):
        k = np.concatenate([8 * np.arange(64) + r for r in RES[g]])
        ang = 2 * np.pi * ((n[:, None] * k[None, :]) % D) / D
        wgt = np.where(k == 0, 1.0, 2.0) / (D * S)
        fw[:, 256 * g:256 * g + 128] = np.cos(ang)
        fw[:, 256 * g + 128:256 * g + 256] = -np.sin(ang)
        bw[256 * g:256 * g + 128] = (np.cos(ang) * wgt).T
        bw[256 * g + 128:256 * g + 256] = (-np.sin(ang) * wgt).T
    bw[128, :] = (-1.0) ** n / (D * S)
    binv = np.kron(np.linalg.inv(b8), np.eye(128))
    gall = binv @ fw
    giall = bw @ binv.T
    gf = np.zeros((11, 144, 128))
    gi = np.zeros((11, 128, 128))
    sign = []
    half = lambda m, q: np.concatenate([m[64 * q:64 * q + 64], m[128 + 64 * q:192 + 64 * q]])
    for g in range(4):
        sl = slice(256 * g, 256 * g + 256)
        f, b = gall[sl, sl].T, giall[sl, sl]
        if g == 0:
            for q in range(2):
                gf[q, :128] = half(f, q)[:, 128 * q:128 * q + 128]
                gi[q] = half(b, q)[:, 128 * q:128 * q + 128]
            gf[0, 128] = (-1.0) ** np.arange(128)
            continue
        sg = np.sign(f[:128, 0] * f[128:, 128])[:, None]
        sign.append((int(sg[0, 0]), int(sg[64, 0])))
        p, q, r = f[:128, :128], f[:128, 128:], f[128:, :128]
        gf[3 * g - 1:3 * g + 2, :128] = p, q - p, r - sg * p
        p, q, r = b[:128, :128], b[:128, 128:], b[128:, :128]
        gi[3 * g - 1:3 * g + 2] = p, r - sg * p, q - p
    a = np.arange(128)
    mt = np.zeros((4, 16, 128, 128))
    for b in range(16):
        ang = 2 * np.pi * (((16 * a[:, None] + b) * a[None, :]) % S) / S
        c, sn = np.cos(ang), -np.sin(ang)
        mt[:, b] = c, c + sn, sn - c, sn
    return _pack_rows(gf), _pack_rows(gi), _pack_rows(mt), tuple(sign)


def _attn_fill():
    pos32 = np.arange(32)
    last = np.arange(16)
    qhead = np.concatenate([np.arange(64) // 32, last // 8])
    khead = np.concatenate([np.arange(64) // 32, last % 2])
    qpos = np.concatenate([pos32, pos32, 32 + last % 8])
    kpos = np.concatenate([pos32, pos32, 32 + last // 2])
    ok = (qpos[:, None] < M) | (qpos[:, None] >= kpos[None, :])
    fill = np.where(ok, 0.0, -1e9)
    fill = np.where(qhead[:, None] == khead[None, :], fill, -np.inf)
    return fill.astype(np.float32)


def _strassen(prod, b11, b12, b21, b22, add, sub, emit):
    m2 = prod(1, b11())
    m1 = prod(0, add(b11(), b22()))
    m3 = prod(2, sub(b12(), b22()))
    c22 = prod(5, add(b11(), b12())) + ((m1 - m2) + m3)
    m4 = prod(3, sub(b21(), b11()))
    emit(1, m2 + m4, c22)
    m5 = prod(4, b22())
    emit(0, prod(6, add(b21(), b22())) + ((m1 + m4) - m5), m3 + m5)


class _Blocks(list):
    def __add__(self, other):
        return _Blocks(a + b for a, b in zip(self, other))

    def __sub__(self, other):
        return _Blocks(a - b for a, b in zip(self, other))


def _strassen_left(a11, a12, a21, a22):
    return [a11 + a22, a21 + a22, a11, a22, a11 + a12, a21 - a11, a12 - a22]


def _kernel(x_hbm, mem_hbm, wq_hbm, wk_hbm, wv_hbm, wo_hbm, bx_hbm, wr_hbm, wi_hbm,
            gf_hbm, gi_hbm, mt_hbm, fill_hbm, out_hbm,
            wraw, wall, wo, xbuf, mem0, x8, xs, xs2, pre, osum, outbuf, fill_ref,
            xb, wt, wl, gf, gi, mt, xd, yb, sems):
    def start(src, dst, sem, priority=0):
        c = pltpu.make_async_copy(src, dst, sems.at[sem])
        c.start(priority=priority)
        return c

    def wait_all(cs):
        for c in cs:
            c.wait()

    dot = functools.partial(jnp.dot, preferred_element_type=f32)
    dot_nt = lambda a, b: lax.dot_general(a, b, (((1,), (1,)), ((), ())), preferred_element_type=f32)
    cat = lambda *vs: jnp.concatenate(vs, axis=0)
    as_bf16 = lambda w: pltpu.bitcast(w, bf16)
    lo_f32 = lambda w: pltpu.bitcast(w << 16, f32)
    hi_f32 = lambda w: pltpu.bitcast(w & u32(0xFFFF0000), f32)
    pack2 = lambda a, b: pltpu.pack_elementwise([a, b], packed_dtype=bf16)
    add2 = lambda a, b: pack2(lo_f32(a) + lo_f32(b), hi_f32(a) + hi_f32(b))
    sub2 = lambda a, b: pack2(lo_f32(a) - lo_f32(b), hi_f32(a) - hi_f32(b))
    w_hbm = (wq_hbm, wk_hbm, wv_hbm)

    def start_unit(u):
        return start(w_hbm[u // 2].at[:, :, u % 2], wraw.at[u % NRAW], u % NRAW)

    def start_x(seg0, nseg, sem, priority=0):
        segs, rows = pl.ds(seg0, nseg), pl.ds(0, SEG - M)
        return start(x_hbm.at[segs, rows, :], xbuf.at[segs, rows, :], sem, priority)

    def start_filter(row0, nrows, sem, priority=0):
        rows = pl.ds(row0, nrows)
        return [start(w.at[rows, pl.ds(128 * d, 128)], wt.at[t, d, rows], sem, priority)
                for t, w in enumerate((wr_hbm, wi_hbm)) for d in range(16)]

    c_a = []
    for n in range(4):
        cols, rows = pl.ds(256 * n, 256), pl.ds(128 * n, 128)
        c_a.append([start(x_hbm.at[:, pl.ds(SEG - M, M), cols], x8.at[:, :, cols], n),
                    start(wq_hbm.at[rows, :, 0], wraw.at[0, rows], n)])
    c_loop = [start_x(0, UNROLL, 4, 1), start(mem_hbm, mem0, 4, 1), start(fill_hbm, fill_ref.at[pl.ds(0, 80)], 4, 1)]
    c_loop += [start(wo_hbm.at[:, pl.ds(128 * j, 128)], wo.at[j], 4, 1) for j in range(8)]

    xb32 = xb.bitcast(u32)

    def relayout_row(src, dst, r, lo, hi):
        a, b = src.at[r].bitcast(u32)[...]
        dst[pl.ds(r, 8, stride=WP), :] = (a & lo) | (b << 16)
        dst[pl.ds(r + 8 * WP, 8, stride=WP), :] = (a >> 16) | (b & hi)

    def relayout_tasks(u, r0=0, r1=D // 2):
        src, dst = wraw.at[u % NRAW], wall.at[u]

        def make(r):
            def task(tok):
                lo = (tok >> 16) | u32(0xFFFF)
                hi = (tok << 16) | u32(0xFFFF0000)
                relayout_row(src, dst, r, lo, hi)
                relayout_row(src, dst, r + 1, lo, hi)
            return task
        return [make(r) for r in range(r0, r1, 2)]

    def y_blocks(r):
        return pl.ds(4 * (r % 2) + r // 2, 8, stride=8)

    def filter_tasks(blk, wfn):
        def make(phase, k):
            slots = [4 * k + j for j in range(4)] if phase == 1 else [4 * j + k for j in range(4)]

            def task(tok):
                ones = ((tok >> 16) | u32(0xFFFF)) | u32(0xFFFF0000)
                z = [(yb[0, b, blk], yb[1, b, blk]) for b in slots]
                z[0] = tuple(pltpu.bitcast(pltpu.bitcast(v, u32) & ones, f32) for v in z[0])
                if phase == 0:
                    o = _bfly4(z, 1)
                    o = [_twiddle16(o[j], k * j) for j in range(4)]
                elif phase == 1:
                    o = _bfly4(z, 1)
                    y = []
                    for j in range(4):
                        wr, wi = wfn(k + 4 * j)
                        xr, xi = o[j]
                        y.append((xr * wr - xi * wi, xr * wi + xi * wr))
                    o = _bfly4(y, -1)
                    o = [_twiddle16(o[j], -k * j) for j in range(4)]
                else:
                    o = _bfly4(z, -1)
                for b, v in zip(slots, o):
                    yb[0, b, blk] = v[0]
                    yb[1, b, blk] = v[1]
            return task
        return [make(phase, k) for phase in range(3) for k in range(4)]

    def z_region(n, par):
        return (2 * n + par) // 3, (2 * n + par) % 3 * 8 * ZP

    def butterfly_tasks(par):
        def make(a2):
            def task(tok):
                zs = []
                for a in (2 * a2, 2 * a2 + 1):
                    w = [xb32[j, a // 4, a // 2 % 2, pl.ds(8 * (a % 2), 8), :] for j in range(8)]
                    if par:
                        hi = (tok << 16) | u32(0xFFFF0000)
                        z = _fwd8([pltpu.bitcast(v & hi, f32) for v in w])
                    else:
                        sixteen = ((tok >> 31) | u32(1)) << 4
                        z = _fwd8([pltpu.bitcast(v << sixteen, f32) for v in w])
                    zs.append(z[0:2] + [v for g in range(1, 4)
                                        for v in (z[2 * g] + z[2 * g + 1], z[2 * g + 1], z[2 * g])])
                for n in range(11):
                    plane, row = z_region(n, par)
                    xd[plane, pl.ds(row + a2, 8, stride=ZP), :] = pltpu.bitcast(pack2(zs[0][n], zs[1][n]), f32)
            return task
        return [make(a2) for a2 in range(64)]

    sign = _dft_constants()[3]

    def b_dfwd(b, pacer):
        def z(n):
            plane, row = z_region(n, b % 2)
            return as_bf16(xd[plane, pl.ds(row + b // 2 * ZP, 64), :])
        t0 = dot_nt(as_bf16(gf[0]), z(0))
        t4 = dot_nt(as_bf16(gf[1, 0:64]), z(1))
        tr, ti = cat(t0[0:64], t4[0:64]), cat(t0[64:128], t4[64:128])
        ts = [(cat(tr + ti, t0[128:144]).astype(bf16), ti.astype(bf16), cat(tr, t0[128:144]).astype(bf16))]
        for g in range(1, 4):
            k1, k2, k3 = [dot_nt(as_bf16(gf[n, 0:64]), z(n)) for n in range(3 * g - 1, 3 * g + 2)]
            pacer.feed(k1)
            tr = k1 + k2
            ti = cat(*[k3[64 * q:64 * q + 64] + k1[64 * q:64 * q + 64] if sign[g - 1][q] > 0
                       else k3[64 * q:64 * q + 64] - k1[64 * q:64 * q + 64] for q in range(2)])
            ts.append(((tr + ti).astype(bf16), ti.astype(bf16), tr.astype(bf16)))
        return ts

    def b_sfwd(b, ts, pacer):
        for g in range(4):
            k1, k2, k3 = [dot(ts[g][n], as_bf16(mt[n, b])) for n in range(3)]
            if g:
                pacer.feed(k2)
            yr, yi = k1[0:128] - k2, k1 + k3
            for q in range(2):
                yb[0, b, y_blocks(RES[g][q])] = yr[64 * q:64 * q + 64].reshape(8, 8, 128)
                yb[1, b, y_blocks(RES[g][q])] = yi[64 * q:64 * q + 64].reshape(8, 8, 128)
            if g == 0:
                yb[0, b, 64] = k1[128:136]
                yb[1, b, 64] = yi[128:136]

    def b_stage1(tasks):
        pacer = _Pacer(tasks, NBT * 48)
        prev = None
        for b in list(range(0, 16, 2)) + list(range(1, 16, 2)):
            ts = b_dfwd(b, pacer)
            if prev is not None:
                b_sfwd(*prev, pacer)
            prev = (b, ts)
        b_sfwd(*prev, pacer)
        pacer.done()

    def b_stage3():
        row0 = lax.broadcasted_iota(jnp.int32, (8, 128), 0) == 0
        low = lax.broadcasted_iota(jnp.int32, (1, 128), 1) < 64
        for b in range(16):
            m = [as_bf16(mt[n, b]) for n in range(4)]
            for g in (1, 2, 3, 0):
                yr, yi = [cat(*[yb[c, b, y_blocks(r)].reshape(64, 128) for r in RES[g]]) for c in range(2)]
                if g == 0:
                    nr = -yr
                    u0 = cat(yr[0:64], jnp.where(row0, yb[0, b, 64], yi[0:8]), yi[8:64])
                    v0 = cat(yi[0:64], jnp.where(row0, yb[1, b, 64], nr[0:8]), nr[8:64])
                    u4, v4 = cat(yr[64:128], yi[64:128]), cat(yi[64:128], nr[64:128])
                    t1 = dot_nt(m[0], u0.astype(bf16)) + dot_nt(m[3], v0.astype(bf16))
                    t2 = dot_nt(m[0], u4.astype(bf16)) + dot_nt(m[3], v4.astype(bf16))
                else:
                    k1, k2, k3 = [dot_nt(m[n], v.astype(bf16)) for n, v in enumerate((yr + yi, yr, yi))]
                    t1, t2 = k1 + k3, k1 - k2
                slot = b // 2 + 8 * (b % 2)
                xd[2 * g, pl.ds(XP * slot, 128), :] = t1
                xd[2 * g + 1, pl.ds(XP * slot, 128), :] = t2
        for t in range(16):
            rows = lambda j: cat(*[xd[j, pl.ds(8 * t + u, 16, stride=XP), :] for u in range(8)])
            z = [dot(rows(q).astype(bf16), as_bf16(gi[q])) for q in range(2)]
            for g in range(1, 4):
                tr, ti = rows(2 * g), rows(2 * g + 1)
                sg = jnp.where(low, float(sign[g - 1][0]), float(sign[g - 1][1]))
                k1, k2, k3 = [dot(v.astype(bf16), as_bf16(gi[3 * g - 1 + n]))
                              for n, v in enumerate((tr + sg * ti, ti, tr))]
                z += [k1 + k2, k1 + k3]
            y = _inv8(z)
            for j in range(8):
                even = cat(*[y[j][16 * u:16 * u + 8] for u in range(8)])
                odd = cat(*[y[j][16 * u + 8:16 * u + 16] for u in range(8)])
                xb32[j, pl.ds(2 * t, 2)] = pack2(even, odd).reshape(2, 2, 16, 128)

    HALF = NSEG * M // 2

    def batch(u, p0, p1, tasks=(), t0=0, t1=4):
        mc = HALF // 2 if t1 - t0 <= MCT else HALF
        pacer = _Pacer(tasks, (7 * (p1 - p0) - MARGIN // (t1 - t0)) * HALF // 8)
        w = wall.at[u]
        for p in range(p0, p1):
            for r0 in range(0, HALF, mc):
                def blk(head, par):
                    return lambda: cat(*[w[pl.ds((p + 8 * head) * WP + 64 * (2 * t + par), 64), :]
                                         for t in range(t0, t1)])

                def prod(i, b):
                    lhs = jnp.concatenate([as_bf16(xs[i, t, pl.ds(r0 // 2, mc // 2), :])
                                           for t in range(t0, t1)], axis=1)
                    r = dot(lhs, as_bf16(b))
                    pacer.feed(r)
                    return r

                def emit(half, *cs):
                    rows = pl.ds(half * HALF + r0, mc)
                    park = pl.ds((half * HALF + r0) // 8, mc // 8)
                    if t0 > 0:
                        cs = [c + yb[t, p, park].reshape(mc, E) for t, c in enumerate(cs)]
                    if t1 < 4:
                        for t, c in enumerate(cs):
                            yb[t, p, park] = c.reshape(mc // 8, 8, E)
                    elif u >= 2:
                        pre[8 * u + p, rows, :] = pack2(*cs)
                    else:
                        st = jnp.concatenate([c.reshape(mc // M, M, E) for c in cs], axis=1)
                        pre[8 * u + p, rows, :] = pltpu.bitcast(st.reshape(2 * mc, E).astype(bf16), u32)
                _strassen(prod, blk(0, 0), blk(1, 0), blk(0, 1), blk(1, 1), add2, sub2, emit)
        pacer.done()

    QUART = HALF // 2

    def unpack_after(w, tok):
        reps = (w.shape[0] // 8, 1)
        hi = jnp.tile((tok << 16) | u32(0xFFFF0000), reps)
        sixteen = jnp.tile(((tok >> 31) | u32(1)) << 4, reps)
        return _Blocks([pltpu.bitcast(w << sixteen, f32), pltpu.bitcast(w & hi, f32)])

    def batch2(u, q0, q1, done, tasks=()):
        pacer = _Pacer(tasks, (49 * (q1 - q0) - MARGIN) * QUART // 8)
        w = wall.at[u]

        def unpack(b):
            if isinstance(b, _Blocks):
                return b
            if len(done) < LAG:
                return _Blocks([lo_f32(b), hi_f32(b)])
            return unpack_after(b, done[-LAG])
        add4 = lambda a, b: unpack(a) + unpack(b)
        sub4 = lambda a, b: unpack(a) - unpack(b)
        for q in range(q0, q1):
            def outer_blk(pair, kh):
                return lambda: [cat(*[w[pl.ds((2 * q + pair + 8 * head) * WP + 64 * (2 * kh + kl + 4 * t), 64), :]
                                      for t in range(2)]) for kl in range(2) for head in range(2)]

            def outer_prod(i, bs):
                def prod(j, b):
                    lhs = jnp.concatenate([as_bf16(xs2[7 * i + j, t]) for t in range(2)], axis=1)
                    r = dot(lhs, as_bf16(pack2(*b) if isinstance(b, _Blocks) else b))
                    pacer.feed(r)
                    done.append(pltpu.bitcast(r[0:8], u32))
                    return r
                cs = {}
                _strassen(prod, *[(lambda b=b: b) for b in bs], add4, sub4,
                          lambda half, *c: cs.update({half: c}))
                return _Blocks(cs[0] + cs[1])

            def emit(half, *cs):
                for pair, c in enumerate(cs):
                    for a in range(2):
                        rows = pl.ds(half * HALF + a * QUART, QUART)
                        pre[8 * u + 2 * q + pair, rows, :] = pack2(c[2 * a], c[2 * a + 1])
            _strassen(outer_prod, outer_blk(0, 0), outer_blk(1, 0), outer_blk(0, 1), outer_blk(1, 1),
                      lambda x, y: [add4(a, b) for a, b in zip(x, y)],
                      lambda x, y: [sub4(a, b) for a, b in zip(x, y)], emit)
        pacer.done()

    def left2_tasks():
        def make(i, t, r):
            def task(tok):
                def blk(rh, kh):
                    ws = [pltpu.bitcast(x8[pl.ds(32 * rh + 16 * rl + 2 * r, 2), :,
                                           pl.ds(128 * (2 * kh + kl + 4 * t), 128)].reshape(16, 128), u32)
                          for rl in range(2) for kl in range(2)]
                    return _Blocks(unpack_after(v, tok) for v in ws)
                terms = ((0, 3, 1), (2, 3, 1), (0,), (3,), (0, 1, 1), (2, 0, -1), (1, 3, -1))[i]
                a = blk(*divmod(terms[0], 2))
                if len(terms) > 1:
                    b = blk(*divmod(terms[1], 2))
                    a = a + b if terms[2] > 0 else a - b
                for j, v in enumerate(_strassen_left(*a)):
                    xs2[7 * i + j, t, pl.ds(8 * r, 8), :] = pack2(*v)
            return task
        return [make(i, t, r) for i in range(7) for t in range(2) for r in range(8)]

    def prepare_left(n):
        v = pltpu.bitcast(x8[:, :, pl.ds(256 * n, 256)].reshape(2 * HALF, 256), u32)
        blocks = [v[HALF // 2 * h:HALF // 2 * (h + 1), 128 * k:128 * (k + 1)] for h in range(2) for k in range(2)]
        lo, hi = [_strassen_left(*[un(b) for b in blocks]) for un in (lo_f32, hi_f32)]
        for i in range(7):
            xs[i, n] = pack2(lo[i], hi[i])

    wait_all(c_a[0])
    for task in relayout_tasks(0, 0, 128):
        task(jnp.zeros((8, 128), u32))
    prepare_left(0)
    batch(0, 0, 6, (), 0, 1)
    wait_all(c_a[1])
    c_h = [start(wq_hbm.at[pl.ds(256 * n, 256), :, 1], wraw.at[1, pl.ds(256 * n, 256)], n) for n in range(2)]
    prepare_left(1)
    batch(0, 6, 8, relayout_tasks(0, 128, 256), 0, 1)
    batch(0, 0, 6, (), 1, 2)
    wait_all(c_a[2])
    prepare_left(2)
    batch(0, 6, 8, relayout_tasks(0, 256, 384), 1, 2)
    batch(0, 0, 6, (), 2, 3)
    wait_all(c_a[3])
    c_w2 = start_unit(2)
    prepare_left(3)
    batch(0, 6, 8, relayout_tasks(0, 384, 512), 2, 3)
    batch(0, 0, 5, (), 3, 4)
    c_h[0].wait()
    batch(0, 5, 8, relayout_tasks(1, 0, 256), 3, 4)
    left2 = left2_tasks()
    batch(1, 0, 5, left2[:64], 0, 2)
    c_h[1].wait()
    start_unit(3)
    batch(1, 5, 8, relayout_tasks(1, 256, 512), 0, 2)
    batch(1, 0, 4, left2[64:], 2, 4)
    c_w2.wait()
    start_unit(4)
    start_unit(5)
    c_b1 = [start(bx_hbm.at[:, :, :, pl.ds(128 * j, 128)], xb.at[j], 5) for j in range(8)]
    c_b1 += [start(gf_hbm, gf.at[pl.ds(0, 11)], 5), start(mt_hbm.at[pl.ds(0, 3)], mt.at[pl.ds(0, 3)], 5)]
    c_loop += start_filter(0, 64, 4, 1)
    batch(1, 4, 8, relayout_tasks(2), 2, 4)
    batch2(2, 0, 2, [])

    def unit_body(u, c):
        slot = (u + 1) % NRAW
        pltpu.make_async_copy(wraw.at[slot], wraw.at[slot], sems.at[slot]).wait()
        done = []
        batch2(u, 2, 4, done, relayout_tasks(u + 1))
        batch2(u + 1, 0, 2, done)
        return c
    lax.fori_loop(2, 5, unit_body, 0)
    wait_all(c_b1)
    bfly = butterfly_tasks(0) + butterfly_tasks(1)
    batch(5, 6, 8, bfly[:NB0])
    batch2(5, 2, 3, [])
    b_stage1(bfly[NB0:])
    wait_all(c_loop)
    c_rest = [start_x(UNROLL, NSEG - UNROLL, 6)] + start_filter(64, 448, 6)
    c_b3 = [start(w.at[pl.ds(512, 1), :], wl.at[t], 5) for t, w in enumerate((wr_hbm, wi_hbm))]
    c_b3 += [start(gi_hbm, gi, 5), start(mt_hbm.at[3], mt.at[3], 5)]

    wo32 = wo.bitcast(u32)
    scale = E ** -0.5

    def gated(w, toks):
        if not toks:
            return w
        bits = functools.reduce(
            jnp.bitwise_or, [pltpu.bitcast(jnp.broadcast_to(t, (8, 128)), u32) for t in toks])
        ones = ((bits >> 16) | u32(0xFFFF)) | u32(0xFFFF0000)
        return cat(w[0:8] & ones, w[8:])

    def wqkv(i, p, second, toks=(), k0=0, k1=D):
        rows = pl.ds((p % 8 + 8 * second) * WP + k0 // 2, (k1 - k0) // 2)
        return as_bf16(gated(wall[2 * i + p // 8, rows, :], toks))

    def step(n, u, mem, held):
        s = UNROLL * n + u
        rows = cat(mem, xbuf[s, pl.ds(0, SEG - M), :].astype(f32))
        lhs = rows.astype(bf16)
        head_start = {}
        if u:
            lo, hi = rows[:, :D // 2].astype(bf16), rows[:, D // 2:].astype(bf16)
            for key in EARLY:
                head_start[key] = dot(lo, wqkv(*key, k1=D // 2))
        r8 = pl.multiple_of(M * s, M)
        fill = fill_ref[pl.ds(0, 80), :]
        heads = [None] * H
        rs = []

        shift = jnp.full((8, 128), 16 - 16 * (n % 2), jnp.int32).astype(u32)
        wblk = pl.ds(pl.multiple_of(64 * (n // 2), 64), 64)
        flt = filter_tasks(
            s, lambda d: [hi_f32(wt.at[t, d, wblk].bitcast(u32)[pl.ds(u, 8, stride=4), :] << shift) for t in range(2)])
        pacer = _Pacer(flt, 48)

        def proj(i, p, toks=()):
            a, b = [
                dot(hi, wqkv(i, p, t, k0=D // 2)) + head_start[i, p, t] if (i, p, t) in head_start
                else dot(lhs, wqkv(i, p, t, toks[t * len(toks) // 2:(t + 1) * len(toks) // 2]))
                for t in range(2)]
            pacer.feed(a)
            pacer.feed(b)
            c = as_bf16(pre[16 * i + p, pl.ds(r8, M), :]).astype(f32)
            return cat(a, b, c).astype(bf16)

        def probs(q, k):
            sc = dot_nt(q, k) * scale
            sc = jnp.where(fill == 0.0, sc, fill)
            e = jnp.exp(sc - jnp.max(sc, axis=1, keepdims=True))
            l = jnp.sum(e, axis=1, keepdims=True)
            r = pl.reciprocal(l, approx=True)
            r = r * (2.0 - l * r)
            rs.append([r[8 * j:8 * j + 8] for j in range(10)])
            return (e * r).astype(bf16)

        def pv(p, pr, v):
            o = dot(pr, v)
            heads[2 * p] = cat(o[0:8], o[16:32], o[64:72])
            heads[2 * p + 1] = cat(o[32:40], o[48:64], o[72:80])
            held[u % 2, p] = (o[8:16], o[40:48])

        def left_task(p):
            def task(tok):
                ones = ((tok >> 16) | u32(0xFFFF)) | u32(0xFFFF0000)
                a11, a12, a21, a22 = held[0, p] + held[1, p]
                a11, a22 = [pltpu.bitcast(pltpu.bitcast(a, u32) & ones, f32) for a in (a11, a22)]
                dst = pl.ds(pl.multiple_of(M * (UNROLL // 2 * n + u // 2), M), M)
                for i, a in enumerate(_strassen_left(a11, a12, a21, a22)):
                    osum[i, p, dst, :] = a.astype(bf16)
            return task

        pend = []
        for g in range(4):
            ps = range(4 * g, 4 * g + 4)
            qk = [(proj(0, p), proj(1, p)) for p in ps]
            vs = [proj(2, p, rs[p - 4] if g else ()) for p in ps]
            for a in pend:
                pv(*a)
            pend = [(p, probs(*qk[t]), vs[t]) for t, p in enumerate(ps)]
        pacer.done()

        def wo_part(oc, j, h0, h1, toks=()):
            return dot(oc, as_bf16(gated(wo32[j, pl.ds(64 * h0, 64 * (h1 - h0)), :], toks)))

        acc = []
        pacer = _Pacer([left_task(p) for p in range(16)] if u % 2 else (), 4 * 10)
        oc = jnp.concatenate(heads[0:24], axis=1).astype(bf16)
        for j in range(8):
            acc.append(wo_part(oc, j, 0, 24, {3: rs[12] + rs[13], 4: rs[14] + rs[15]}.get(j, ())))
            if j == 4:
                for a in pend:
                    pv(*a)
            if j > 5:
                pacer.feed(acc[j])
        oc = jnp.concatenate(heads[24:32], axis=1).astype(bf16)
        nxt = []
        for j in range(8):
            r = wo_part(oc, j, 24, 32) + acc[j]
            outbuf[UNROLL // 2 * n + u // 2, u % 2, pl.ds(M, SEG - M), pl.ds(128 * j, 128)] = r[M:].astype(bf16)
            nxt.append(r[0:M])
            pacer.feed(r)
        pacer.done()
        return jnp.concatenate(nxt, axis=1)

    def steps(n, mem):
        pl.when(n == 1)(functools.partial(wait_all, c_rest))
        held = {}
        for u in range(UNROLL):
            mem = step(n, u, mem, held)
        return mem
    lax.fori_loop(0, NSEG // UNROLL, steps, mem0[...].astype(f32))
    tok_rows = pl.ds(M, SEG - M)
    c_out = [start(outbuf.at[:, :, tok_rows, :], out_hbm.at[:, :, tok_rows, pl.ds(0, D)], 0)]

    wait_all(c_b3)
    for task in filter_tasks(64, lambda d: [wl[t, :, pl.ds(128 * d, 128)].astype(f32) for t in range(2)]):
        task(jnp.zeros((8, 128), u32))
    b_stage3()
    c_out += [start(xb.at[j], out_hbm.at[:, :, :, pl.ds(D + 128 * j, 128)], 0) for j in range(8)]

    osum32 = osum.bitcast(u32)
    for jp in range(4):
        def blk(col, par):
            return lambda: cat(*[wo32[2 * jp + col, pl.ds(64 * (2 * p + par), 64), :] for p in range(16)])

        def prod(i, b):
            return dot(jnp.concatenate([as_bf16(osum32[i, p]) for p in range(16)], axis=1), as_bf16(b))

        def emit(half, *cs):
            for t, c in enumerate(cs):
                outbuf[:, half, pl.ds(0, M), pl.ds(128 * (2 * jp + t), 128)] = (
                    c.reshape(NSEG // 2, M, 128).astype(bf16))
            cols = pl.ds(256 * jp, 256)
            c_out.append(start(outbuf.at[:, half, pl.ds(0, M), cols], out_hbm.at[:, half, pl.ds(0, M), cols], 0))
        _strassen(prod, blk(0, 0), blk(1, 0), blk(0, 1), blk(1, 1), add2, sub2, emit)
    wait_all(c_out)


@jax.jit
def pallas_concat_heads__memory_aug_recurrent_mem_tr__spectral_gfnet__prompt_kernel(
    A_x: jax.Array,
    A_mem0: jax.Array,
    A_Wq: jax.Array,
    A_Wk: jax.Array,
    A_Wv: jax.Array,
    A_Wo: jax.Array,
    A_seg_len: jax.Array,
    B_x: jax.Array,
    B_w_r: jax.Array,
    B_w_i: jax.Array,
):
    del A_seg_len
    assert A_x.shape == (1, S, D) and A_mem0.shape == (1, M, D) and B_x.shape == (1, S, D)
    assert A_Wq.shape == (D, H, E) and A_Wo.shape == (H, E, D) and B_w_r.shape == (S, D // 2 + 1)
    gf, gi, mt, _ = _dft_constants()
    fill = _attn_fill()
    hbm = pl.BlockSpec(memory_space=pltpu.HBM)
    wshape = (D // 2, 2, 2, 16, E)
    out = pl.pallas_call(
        _kernel,
        out_shape=jax.ShapeDtypeStruct((NSEG // 2, 2, SEG, 2 * D), bf16),
        in_specs=[hbm] * 13,
        out_specs=hbm,
        scratch_shapes=[
            pltpu.VMEM((NRAW, D // 2, 2, 16, E), bf16),
            pltpu.VMEM((6, 16 * WP, E), u32),
            pltpu.VMEM((8, H * E, 128), bf16),
            pltpu.VMEM((NSEG, SEG, D), bf16),
            pltpu.VMEM((M, D), bf16),
            pltpu.VMEM((NSEG, M, D), bf16),
            pltpu.VMEM((7, 4, 128, 128), u32),
            pltpu.VMEM((49, 2, 64, 128), u32),
            pltpu.VMEM((48, NSEG * M, E), u32),
            pltpu.VMEM((7, 16, NSEG * M // 2, E), bf16),
            pltpu.VMEM((NSEG // 2, 2, SEG, D), bf16),
            pltpu.VMEM((96, 80), f32),
            pltpu.VMEM((8, NSEG // 2, 2, SEG, 128), bf16),
            pltpu.VMEM((2, 16, 512, 128), bf16),
            pltpu.VMEM((2, 1, S), bf16),
            pltpu.VMEM((12,) + gf.shape[1:], u32),
            pltpu.VMEM(gi.shape, u32),
            pltpu.VMEM(mt.shape, u32),
            pltpu.VMEM((8, 16 * XP, 128), f32),
            pltpu.VMEM((2, 16, 65, 8, 128), f32),
            pltpu.SemaphoreType.DMA((7,)),
        ],
        compiler_params=pltpu.CompilerParams(vmem_limit_bytes=120 * 1024 * 1024),
    )(A_x.reshape(NSEG, SEG, D), A_mem0.reshape(M, D),
      A_Wq.reshape(wshape), A_Wk.reshape(wshape), A_Wv.reshape(wshape),
      A_Wo.reshape(H * E, D), B_x.reshape(NSEG // 2, 2, SEG, D), B_w_r.T, B_w_i.T, gf, gi, mt, fill)
    return out.reshape(1, S, 2 * D)
```

```python
import functools

import jax
import jax.numpy as jnp
import numpy as np
from jax import lax
from jax.experimental import pallas as pl
from jax.experimental.pallas import tpu as pltpu

S, D, H, E, M, SEG = 2048, 1024, 32, 128, 8, 32
NSEG = S // SEG
WP = 516
XP = 132
ZP = 68
NRAW = 4
UNROLL = 4
MCT = 1
LAG = 8
DLAG = 100
LSTART = 5
LEFT_AT = ((), (2,), (4,), (0, 1, 3, 5, 6))
NB0 = 64
NBT = 13
MARGIN = 8
EARLY = ((0, 0, 0), (0, 0, 1), (1, 0, 0), (1, 0, 1), (0, 1, 0), (0, 1, 1))
bf16, f32, u32 = jnp.bfloat16, jnp.float32, jnp.uint32
RES = ((0, 4), (2, 6), (1, 7), (3, 5))
RC = float(np.sqrt(0.5))


def _fwd8(x):
    s04, d04 = x[0] + x[4], x[0] - x[4]
    s26, d26 = x[2] + x[6], x[2] - x[6]
    s15, d15 = x[1] + x[5], x[1] - x[5]
    s37, d37 = x[3] + x[7], x[3] - x[7]
    t1, t2 = (d15 - d37) * RC, (d15 + d37) * RC
    e0, o0 = s04 + s26, s15 + s37
    return [e0 + o0, e0 - o0, s04 - s26, s15 - s37, d04 + t1, d26 + t2, d04 - t1, d26 - t2]


def _inv8(z):
    z0, z4, e1, o1, r1, i1, r3, i3 = z
    e0, o0 = z0 + z4, z0 - z4
    s04, s26, s15, s37 = e0 + e1, e0 - e1, o0 + o1, o0 - o1
    d04, d26 = r1 + r3, i1 + i3
    t1, t2 = (r1 - r3) * RC, (i1 - i3) * RC
    d15, d37 = t1 + t2, t2 - t1
    return [s04 + d04, s15 + d15, s26 + d26, s37 + d37, s04 - d04, s15 - d15, s26 - d26, s37 - d37]


def _twiddle16(z, k):
    re, im = z
    k = k % 16
    if k == 0:
        return z
    if k == 4:
        return (im, -re)
    if k == 12:
        return (-im, re)
    if k == 2:
        return ((re + im) * RC, (im - re) * RC)
    if k == 14:
        return ((re - im) * RC, (re + im) * RC)
    if k == 6:
        return ((im - re) * RC, (re + im) * -RC)
    if k == 10:
        return ((re + im) * -RC, (re - im) * RC)
    c, s = float(np.cos(2 * np.pi * k / 16)), float(-np.sin(2 * np.pi * k / 16))
    return (re * c - im * s, re * s + im * c)


def _bfly4(z, sign):
    (ar, ai), (br, bi), (cr, ci), (dr, di) = z
    sr, si, tr, ti = ar + cr, ai + ci, ar - cr, ai - ci
    ur, ui, vr, vi = br + dr, bi + di, br - dr, bi - di
    o0, o2 = (sr + ur, si + ui), (sr - ur, si - ui)
    p, q = (tr + vi, ti - vr), (tr - vi, ti + vr)
    return [o0, p, o2, q] if sign > 0 else [o0, q, o2, p]


class _Pacer:
    def __init__(self, tasks, ntokens):
        self.slots = {}
        for n, task in enumerate(tasks):
            self.slots.setdefault(n * ntokens // len(tasks), []).append(task)
        self.pos = 0

    def feed(self, r):
        for j in range(r.shape[0] // 8):
            for task in self.slots.pop(self.pos, []):
                task(pltpu.bitcast(r[8 * j:8 * j + 8], u32))
            self.pos += 1

    def done(self):
        assert not self.slots


def _pack_rows(m):
    b = np.asarray(m, np.float32).astype(jnp.bfloat16).view(np.uint16).astype(np.uint32)
    return b[..., 0::2, :] | (b[..., 1::2, :] << 16)


@functools.lru_cache(maxsize=None)
def _dft_constants():
    b8 = np.array(_fwd8(list(np.eye(8)))).T
    n = np.arange(D)
    fw = np.zeros((D, D))
    bw = np.zeros((D, D))
    for g in range(4):
        k = np.concatenate([8 * np.arange(64) + r for r in RES[g]])
        ang = 2 * np.pi * ((n[:, None] * k[None, :]) % D) / D
        wgt = np.where(k == 0, 1.0, 2.0) / (D * S)
        fw[:, 256 * g:256 * g + 128] = np.cos(ang)
        fw[:, 256 * g + 128:256 * g + 256] = -np.sin(ang)
        bw[256 * g:256 * g + 128] = (np.cos(ang) * wgt).T
        bw[256 * g + 128:256 * g + 256] = (-np.sin(ang) * wgt).T
    bw[128, :] = (-1.0) ** n / (D * S)
    binv = np.kron(np.linalg.inv(b8), np.eye(128))
    gall = binv @ fw
    giall = bw @ binv.T
    gf = np.zeros((11, 144, 128))
    gi = np.zeros((11, 128, 128))
    sign = []
    half = lambda m, q: np.concatenate([m[64 * q:64 * q + 64], m[128 + 64 * q:192 + 64 * q]])
    for g in range(4):
        sl = slice(256 * g, 256 * g + 256)
        f, b = gall[sl, sl].T, giall[sl, sl]
        if g == 0:
            for q in range(2):
                gf[q, :128] = half(f, q)[:, 128 * q:128 * q + 128]
                gi[q] = half(b, q)[:, 128 * q:128 * q + 128]
            gf[0, 128] = (-1.0) ** np.arange(128)
            continue
        sg = np.sign(f[:128, 0] * f[128:, 128])[:, None]
        sign.append((int(sg[0, 0]), int(sg[64, 0])))
        p, q, r = f[:128, :128], f[:128, 128:], f[128:, :128]
        gf[3 * g - 1:3 * g + 2, :128] = p, q - p, r - sg * p
        p, q, r = b[:128, :128], b[:128, 128:], b[128:, :128]
        gi[3 * g - 1:3 * g + 2] = p, r - sg * p, q - p
    a = np.arange(128)
    mt = np.zeros((4, 16, 128, 128))
    for b in range(16):
        ang = 2 * np.pi * (((16 * a[:, None] + b) * a[None, :]) % S) / S
        c, sn = np.cos(ang), -np.sin(ang)
        mt[:, b] = c, c + sn, sn - c, sn
    return _pack_rows(gf), _pack_rows(gi), _pack_rows(mt), tuple(sign)


def _attn_fill():
    pos32 = np.arange(32)
    last = np.arange(16)
    qhead = np.concatenate([np.arange(64) // 32, last // 8])
    khead = np.concatenate([np.arange(64) // 32, last % 2])
    qpos = np.concatenate([pos32, pos32, 32 + last % 8])
    kpos = np.concatenate([pos32, pos32, 32 + last // 2])
    ok = (qpos[:, None] < M) | (qpos[:, None] >= kpos[None, :])
    fill = np.where(ok, 0.0, -1e9)
    fill = np.where(qhead[:, None] == khead[None, :], fill, -np.inf)
    return fill.astype(np.float32)


def _strassen(prod, b11, b12, b21, b22, add, sub, emit):
    m2 = prod(1, b11())
    m1 = prod(0, add(b11(), b22()))
    m3 = prod(2, sub(b12(), b22()))
    c22 = prod(5, add(b11(), b12())) + ((m1 - m2) + m3)
    m4 = prod(3, sub(b21(), b11()))
    emit(1, m2 + m4, c22)
    m5 = prod(4, b22())
    emit(0, prod(6, add(b21(), b22())) + ((m1 + m4) - m5), m3 + m5)


class _Blocks(list):
    def __add__(self, other):
        return _Blocks(a + b for a, b in zip(self, other))

    def __sub__(self, other):
        return _Blocks(a - b for a, b in zip(self, other))


def _strassen_left(a11, a12, a21, a22):
    return [a11 + a22, a21 + a22, a11, a22, a11 + a12, a21 - a11, a12 - a22]


def _strassen_left_one(i, blk):
    terms = ((0, 3, 1), (2, 3, 1), (0,), (3,), (0, 1, 1), (2, 0, -1), (1, 3, -1))[i]
    a = blk(*divmod(terms[0], 2))
    if len(terms) == 1:
        return a
    b = blk(*divmod(terms[1], 2))
    return a + b if terms[2] > 0 else a - b


def _kernel(x_hbm, mem_hbm, wq_hbm, wk_hbm, wv_hbm, wo_hbm, bx_hbm, wr_hbm, wi_hbm,
            gf_hbm, gi_hbm, mt_hbm, fill_hbm, out_hbm,
            wraw, wall, wo, xbuf, mem0, x8, xs, xs2, pre, osum, outbuf, fill_ref,
            xb, wt, wl, gf, gi, mt, xd, yb, sems):
    def start(src, dst, sem, priority=0):
        c = pltpu.make_async_copy(src, dst, sems.at[sem])
        c.start(priority=priority)
        return c

    def wait_all(cs):
        for c in cs:
            c.wait()

    dot = functools.partial(jnp.dot, preferred_element_type=f32)
    dot_nt = lambda a, b: lax.dot_general(a, b, (((1,), (1,)), ((), ())), preferred_element_type=f32)
    cat = lambda *vs: jnp.concatenate(vs, axis=0)
    as_bf16 = lambda w: pltpu.bitcast(w, bf16)
    lo_f32 = lambda w: pltpu.bitcast(w << 16, f32)
    hi_f32 = lambda w: pltpu.bitcast(w & u32(0xFFFF0000), f32)
    pack2 = lambda a, b: pltpu.pack_elementwise([a, b], packed_dtype=bf16)
    add2 = lambda a, b: pack2(lo_f32(a) + lo_f32(b), hi_f32(a) + hi_f32(b))
    sub2 = lambda a, b: pack2(lo_f32(a) - lo_f32(b), hi_f32(a) - hi_f32(b))
    w_hbm = (wq_hbm, wk_hbm, wv_hbm)

    def start_unit(u):
        return start(w_hbm[u // 2].at[:, :, u % 2], wraw.at[u % NRAW], u % NRAW)

    def start_x(seg0, nseg, sem, priority=0):
        segs, rows = pl.ds(seg0, nseg), pl.ds(0, SEG - M)
        return start(x_hbm.at[segs, rows, :], xbuf.at[segs], sem, priority)

    def start_filter(row0, nrows, sem, priority=0):
        rows = pl.ds(row0, nrows)
        return [start(w.at[rows, pl.ds(128 * d, 128)], wt.at[t, d, rows], sem, priority)
                for t, w in enumerate((wr_hbm, wi_hbm)) for d in range(16)]

    c_a = []
    for n in range(4):
        cols, rows = pl.ds(256 * n, 256), pl.ds(128 * n, 128)
        c_a.append([start(x_hbm.at[:, pl.ds(SEG - M, M), cols], x8.at[:, :, cols], n),
                    start(wq_hbm.at[rows, :, 0], wraw.at[0, rows], n)])
    c_loop = [start_x(0, UNROLL, 4, 1), start(mem_hbm, mem0, 4, 1), start(fill_hbm, fill_ref.at[pl.ds(0, 80)], 4, 1)]
    c_loop += [start(wo_hbm.at[:, pl.ds(128 * j, 128)], wo.at[j], 4, 1) for j in range(8)]

    xb32 = xb.bitcast(u32)

    def relayout_row(src, dst, r, lo, hi):
        a, b = src.at[r].bitcast(u32)[...]
        dst[pl.ds(r, 8, stride=WP), :] = (a & lo) | (b << 16)
        dst[pl.ds(r + 8 * WP, 8, stride=WP), :] = (a >> 16) | (b & hi)

    def relayout_tasks(u, r0=0, r1=D // 2):
        src, dst = wraw.at[u % NRAW], wall.at[u]

        def make(r):
            def task(tok):
                lo = (tok >> 16) | u32(0xFFFF)
                hi = (tok << 16) | u32(0xFFFF0000)
                relayout_row(src, dst, r, lo, hi)
                relayout_row(src, dst, r + 1, lo, hi)
            return task
        return [make(r) for r in range(r0, r1, 2)]

    def y_blocks(r):
        return pl.ds(4 * (r % 2) + r // 2, 8, stride=8)

    def filter_tasks(blk, wfn):
        def make(phase, k):
            slots = [4 * k + j for j in range(4)] if phase == 1 else [4 * j + k for j in range(4)]

            def task(tok):
                ones = ((tok >> 16) | u32(0xFFFF)) | u32(0xFFFF0000)
                z = [(yb[0, b, blk], yb[1, b, blk]) for b in slots]
                z[0] = tuple(pltpu.bitcast(pltpu.bitcast(v, u32) & ones, f32) for v in z[0])
                if phase == 0:
                    o = _bfly4(z, 1)
                    o = [_twiddle16(o[j], k * j) for j in range(4)]
                elif phase == 1:
                    o = _bfly4(z, 1)
                    y = []
                    for j in range(4):
                        wr, wi = wfn(k + 4 * j)
                        xr, xi = o[j]
                        y.append((xr * wr - xi * wi, xr * wi + xi * wr))
                    o = _bfly4(y, -1)
                    o = [_twiddle16(o[j], -k * j) for j in range(4)]
                else:
                    o = _bfly4(z, -1)
                for b, v in zip(slots, o):
                    yb[0, b, blk] = v[0]
                    yb[1, b, blk] = v[1]
            return task
        return [make(phase, k) for phase in range(3) for k in range(4)]

    def z_region(n, par):
        return (2 * n + par) // 3, (2 * n + par) % 3 * 8 * ZP

    def butterfly_tasks(par):
        def make(a2):
            def task(tok):
                zs = []
                for a in (2 * a2, 2 * a2 + 1):
                    w = [xb32[j, a // 8, a // 2 % 4, pl.ds(8 * (a % 2), 8), :] for j in range(8)]
                    if par:
                        hi = (tok << 16) | u32(0xFFFF0000)
                        z = _fwd8([pltpu.bitcast(v & hi, f32) for v in w])
                    else:
                        sixteen = ((tok >> 31) | u32(1)) << 4
                        z = _fwd8([pltpu.bitcast(v << sixteen, f32) for v in w])
                    zs.append(z[0:2] + [v for g in range(1, 4)
                                        for v in (z[2 * g] + z[2 * g + 1], z[2 * g + 1], z[2 * g])])
                for n in range(11):
                    plane, row = z_region(n, par)
                    xd[plane, pl.ds(row + a2, 8, stride=ZP), :] = pltpu.bitcast(pack2(zs[0][n], zs[1][n]), f32)
            return task
        return [make(a2) for a2 in range(64)]

    sign = _dft_constants()[3]

    def b_dfwd(b, pacer):
        def z(n):
            plane, row = z_region(n, b % 2)
            return as_bf16(xd[plane, pl.ds(row + b // 2 * ZP, 64), :])
        t0 = dot_nt(as_bf16(gf[0]), z(0))
        t4 = dot_nt(as_bf16(gf[1, 0:64]), z(1))
        tr, ti = cat(t0[0:64], t4[0:64]), cat(t0[64:128], t4[64:128])
        ts = [(cat(tr + ti, t0[128:144]).astype(bf16), ti.astype(bf16), cat(tr, t0[128:144]).astype(bf16))]
        for g in range(1, 4):
            k1, k2, k3 = [dot_nt(as_bf16(gf[n, 0:64]), z(n)) for n in range(3 * g - 1, 3 * g + 2)]
            pacer.feed(k1)
            tr = k1 + k2
            ti = cat(*[k3[64 * q:64 * q + 64] + k1[64 * q:64 * q + 64] if sign[g - 1][q] > 0
                       else k3[64 * q:64 * q + 64] - k1[64 * q:64 * q + 64] for q in range(2)])
            ts.append(((tr + ti).astype(bf16), ti.astype(bf16), tr.astype(bf16)))
        return ts

    def b_sfwd(b, ts, pacer):
        for g in range(4):
            k1, k2, k3 = [dot(ts[g][n], as_bf16(mt[n, b])) for n in range(3)]
            if g:
                pacer.feed(k2)
            yr, yi = k1[0:128] - k2, k1 + k3
            for q in range(2):
                yb[0, b, y_blocks(RES[g][q])] = yr[64 * q:64 * q + 64].reshape(8, 8, 128)
                yb[1, b, y_blocks(RES[g][q])] = yi[64 * q:64 * q + 64].reshape(8, 8, 128)
            if g == 0:
                yb[0, b, 64] = k1[128:136]
                yb[1, b, 64] = yi[128:136]

    def b_stage1(tasks):
        pacer = _Pacer(tasks, NBT * 48)
        prev = None
        for b in list(range(0, 16, 2)) + list(range(1, 16, 2)):
            ts = b_dfwd(b, pacer)
            if prev is not None:
                b_sfwd(*prev, pacer)
            prev = (b, ts)
        b_sfwd(*prev, pacer)
        pacer.done()

    def b_stage3():
        row0 = lax.broadcasted_iota(jnp.int32, (8, 128), 0) == 0
        low = lax.broadcasted_iota(jnp.int32, (1, 128), 1) < 64
        for b in range(16):
            m = [as_bf16(mt[n, b]) for n in range(4)]
            for g in (1, 2, 3, 0):
                yr, yi = [cat(*[yb[c, b, y_blocks(r)].reshape(64, 128) for r in RES[g]]) for c in range(2)]
                if g == 0:
                    nr = -yr
                    u0 = cat(yr[0:64], jnp.where(row0, yb[0, b, 64], yi[0:8]), yi[8:64])
                    v0 = cat(yi[0:64], jnp.where(row0, yb[1, b, 64], nr[0:8]), nr[8:64])
                    u4, v4 = cat(yr[64:128], yi[64:128]), cat(yi[64:128], nr[64:128])
                    t1 = dot_nt(m[0], u0.astype(bf16)) + dot_nt(m[3], v0.astype(bf16))
                    t2 = dot_nt(m[0], u4.astype(bf16)) + dot_nt(m[3], v4.astype(bf16))
                else:
                    k1, k2, k3 = [dot_nt(m[n], v.astype(bf16)) for n, v in enumerate((yr + yi, yr, yi))]
                    t1, t2 = k1 + k3, k1 - k2
                slot = b // 2 + 8 * (b % 2)
                xd[2 * g, pl.ds(XP * slot, 128), :] = t1
                xd[2 * g + 1, pl.ds(XP * slot, 128), :] = t2
        for t in range(16):
            rows = lambda j: cat(*[xd[j, pl.ds(8 * t + u, 16, stride=XP), :] for u in range(8)])
            z = [dot(rows(q).astype(bf16), as_bf16(gi[q])) for q in range(2)]
            for g in range(1, 4):
                tr, ti = rows(2 * g), rows(2 * g + 1)
                sg = jnp.where(low, float(sign[g - 1][0]), float(sign[g - 1][1]))
                k1, k2, k3 = [dot(v.astype(bf16), as_bf16(gi[3 * g - 1 + n]))
                              for n, v in enumerate((tr + sg * ti, ti, tr))]
                z += [k1 + k2, k1 + k3]
            y = _inv8(z)
            for j in range(8):
                even = cat(*[y[j][16 * u:16 * u + 8] for u in range(8)])
                odd = cat(*[y[j][16 * u + 8:16 * u + 16] for u in range(8)])
                xb32[j, t] = pack2(even, odd).reshape(4, 16, 128)

    HALF = NSEG * M // 2

    def batch(u, p0, p1, tasks=(), t0=0, t1=4):
        mc = HALF // 2 if t1 - t0 <= MCT else HALF
        pacer = _Pacer(tasks, (7 * (p1 - p0) - MARGIN // (t1 - t0)) * HALF // 8)
        w = wall.at[u]
        for p in range(p0, p1):
            for r0 in range(0, HALF, mc):
                def blk(head, par):
                    return lambda: cat(*[w[pl.ds((p + 8 * head) * WP + 64 * (2 * t + par), 64), :]
                                         for t in range(t0, t1)])

                def prod(i, b):
                    lhs = jnp.concatenate([as_bf16(xs[i, t, pl.ds(r0 // 2, mc // 2), :])
                                           for t in range(t0, t1)], axis=1)
                    r = dot(lhs, as_bf16(b))
                    pacer.feed(r)
                    return r

                def emit(half, *cs):
                    rows = pl.ds(half * HALF + r0, mc)
                    park = pl.ds((half * HALF + r0) // 8, mc // 8)
                    if t0 > 0:
                        cs = [c + yb[t, p, park].reshape(mc, E) for t, c in enumerate(cs)]
                    if t1 < 4:
                        for t, c in enumerate(cs):
                            yb[t, p, park] = c.reshape(mc // 8, 8, E)
                    elif u >= 2:
                        pre[8 * u + p, rows, :] = pack2(*cs)
                    else:
                        st = jnp.concatenate([c.reshape(mc // M, M, E) for c in cs], axis=1)
                        pre[8 * u + p, rows, :] = pltpu.bitcast(st.reshape(2 * mc, E).astype(bf16), u32)
                _strassen(prod, blk(0, 0), blk(1, 0), blk(0, 1), blk(1, 1), add2, sub2, emit)
        pacer.done()

    QUART = HALF // 2

    def unpack_after(w, tok):
        reps = (w.shape[0] // 8, 1)
        hi = jnp.tile((tok << 16) | u32(0xFFFF0000), reps)
        sixteen = jnp.tile(((tok >> 31) | u32(1)) << 4, reps)
        return _Blocks([pltpu.bitcast(w << sixteen, f32), pltpu.bitcast(w & hi, f32)])

    def strassen2(right, left, emit, done, pacer, lag=LAG):
        def unpack(b):
            if isinstance(b, _Blocks):
                return b
            if len(done) < lag:
                return _Blocks([lo_f32(b), hi_f32(b)])
            return unpack_after(b, done[-lag])
        add = lambda a, b: unpack(a) + unpack(b)
        sub = lambda a, b: unpack(a) - unpack(b)

        def outer_prod(i, bs):
            def prod(j, b):
                r = dot(left(7 * i + j), as_bf16(pack2(*b) if isinstance(b, _Blocks) else b))
                pacer.feed(r)
                done.append(pltpu.bitcast(r[0:8], u32))
                return r
            order = (1, 0, 3, 2) if i in (1, 4, 5, 6) else (0, 1, 2, 3)
            cs = {}
            _strassen(prod, *[(lambda b=bs[k]: b) for k in order], add, sub, lambda half, *c: cs.update({half: c}))
            return _Blocks((cs[0] + cs[1])[k] for k in order)

        def outer_emit(half, *cs):
            for col in (1, 0):
                for a in range(2):
                    emit(2 * half + a, 2 * col, cs[col][2 * a], cs[col][2 * a + 1])
        outer = lambda k, c: lambda: [right(2 * k + k2, 2 * c + c2) for k2 in range(2) for c2 in range(2)]
        _strassen(outer_prod, outer(0, 0), outer(0, 1), outer(1, 0), outer(1, 1),
                  lambda x, y: [add(a, b) for a, b in zip(x, y)],
                  lambda x, y: [sub(a, b) for a, b in zip(x, y)], outer_emit)

    def batch2(u, q0, q1, done, tasks=()):
        pacer = _Pacer(tasks, (49 * (q1 - q0) - MARGIN) * QUART // 8)
        w = wall.at[u]
        for q in range(q0, q1):
            def emit(row, col, c0, c1):
                pre[8 * u + 2 * q + col // 2, pl.ds(row * QUART, QUART), :] = pack2(c0, c1)
            strassen2(lambda k, c: cat(*[w[pl.ds((2 * q + c // 2 + 8 * (c % 2)) * WP + 64 * (k + 4 * t), 64), :]
                                         for t in range(2)]),
                      lambda i: jnp.concatenate([as_bf16(xs2[i, t]) for t in range(2)], axis=1),
                      emit, done, pacer)
        pacer.done()

    def left2_tasks():
        def make(i, t, r):
            def task(tok):
                def blk(rh, kh):
                    ws = [pltpu.bitcast(x8[pl.ds(32 * rh + 16 * rl + 2 * r, 2), :,
                                           pl.ds(128 * (2 * kh + kl + 4 * t), 128)].reshape(16, 128), u32)
                          for rl in range(2) for kl in range(2)]
                    return _Blocks(unpack_after(v, tok) for v in ws)
                for j, v in enumerate(_strassen_left(*_strassen_left_one(i, blk))):
                    xs2[7 * i + j, t, pl.ds(8 * r, 8), :] = pack2(*v)
            return task
        return [make(i, t, r) for i in range(7) for t in range(2) for r in range(8)]

    def prepare_left(n):
        v = pltpu.bitcast(x8[:, :, pl.ds(256 * n, 256)].reshape(2 * HALF, 256), u32)
        blocks = [v[HALF // 2 * h:HALF // 2 * (h + 1), 128 * k:128 * (k + 1)] for h in range(2) for k in range(2)]
        lo, hi = [_strassen_left(*[un(b) for b in blocks]) for un in (lo_f32, hi_f32)]
        for i in range(7):
            xs[i, n] = pack2(lo[i], hi[i])

    wait_all(c_a[0])
    for task in relayout_tasks(0, 0, 128):
        task(jnp.zeros((8, 128), u32))
    prepare_left(0)
    batch(0, 0, 6, (), 0, 1)
    wait_all(c_a[1])
    c_h = [start(wq_hbm.at[pl.ds(256 * n, 256), :, 1], wraw.at[1, pl.ds(256 * n, 256)], n) for n in range(2)]
    prepare_left(1)
    batch(0, 6, 8, relayout_tasks(0, 128, 256), 0, 1)
    batch(0, 0, 6, (), 1, 2)
    wait_all(c_a[2])
    prepare_left(2)
    batch(0, 6, 8, relayout_tasks(0, 256, 384), 1, 2)
    batch(0, 0, 6, (), 2, 3)
    wait_all(c_a[3])
    c_w2 = start_unit(2)
    prepare_left(3)
    batch(0, 6, 8, relayout_tasks(0, 384, 512), 2, 3)
    batch(0, 0, 5, (), 3, 4)
    c_h[0].wait()
    batch(0, 5, 8, relayout_tasks(1, 0, 256), 3, 4)
    left2 = left2_tasks()
    batch(1, 0, 5, left2[:64], 0, 2)
    c_h[1].wait()
    start_unit(3)
    batch(1, 5, 8, relayout_tasks(1, 256, 512), 0, 2)
    batch(1, 0, 4, left2[64:], 2, 4)
    c_w2.wait()
    start_unit(4)
    start_unit(5)
    c_b1 = [start(bx_hbm.at[:, :, :, pl.ds(128 * j, 128)], xb.at[j], 5) for j in range(8)]
    c_b1 += [start(gf_hbm, gf.at[pl.ds(0, 11)], 5), start(mt_hbm.at[pl.ds(0, 3)], mt.at[pl.ds(0, 3)], 5)]
    c_loop += start_filter(0, 64, 4, 1)
    batch(1, 4, 8, relayout_tasks(2), 2, 4)
    batch2(2, 0, 2, [])

    def unit_body(u, c):
        slot = (u + 1) % NRAW
        pltpu.make_async_copy(wraw.at[slot], wraw.at[slot], sems.at[slot]).wait()
        done = []
        batch2(u, 2, 4, done, relayout_tasks(u + 1))
        batch2(u + 1, 0, 2, done)
        return c
    lax.fori_loop(2, 5, unit_body, 0)
    wait_all(c_b1)
    bfly = butterfly_tasks(0) + butterfly_tasks(1)
    batch(5, 6, 8, bfly[:NB0])
    batch2(5, 2, 3, [])
    b_stage1(bfly[NB0:])
    wait_all(c_loop)
    c_rest = [start_x(UNROLL, NSEG - UNROLL, 6)] + start_filter(64, 448, 6)
    c_b3 = [start(w.at[pl.ds(512, 1), :], wl.at[t], 5) for t, w in enumerate((wr_hbm, wi_hbm))]
    c_b3 += [start(gi_hbm, gi, 5), start(mt_hbm.at[3], mt.at[3], 5)]

    wo32 = wo.bitcast(u32)
    scale = E ** -0.5

    def gated(w, toks):
        if not toks:
            return w
        bits = functools.reduce(
            jnp.bitwise_or, [pltpu.bitcast(jnp.broadcast_to(t, (8, 128)), u32) for t in toks])
        ones = ((bits >> 16) | u32(0xFFFF)) | u32(0xFFFF0000)
        return cat(w[0:8] & ones, w[8:])

    def wqkv(i, p, second, toks=(), k0=0, k1=D):
        rows = pl.ds((p % 8 + 8 * second) * WP + k0 // 2, (k1 - k0) // 2)
        return as_bf16(gated(wall[2 * i + p // 8, rows, :], toks))

    def step(n, u, mem, held):
        s = UNROLL * n + u
        rows = cat(mem, xbuf[s].astype(f32))
        lhs = rows.astype(bf16)
        head_start = {}
        if u:
            lo, hi = rows[:, :D // 2].astype(bf16), rows[:, D // 2:].astype(bf16)
            for key in EARLY:
                head_start[key] = dot(lo, wqkv(*key, k1=D // 2))
        r8 = pl.multiple_of(M * s, M)
        fill = fill_ref[pl.ds(0, 80), :]
        heads = [None] * H
        rs = []

        shift = jnp.full((8, 128), 16 - 16 * (n % 2), jnp.int32).astype(u32)
        wblk = pl.ds(pl.multiple_of(64 * (n // 2), 64), 64)
        flt = filter_tasks(
            s, lambda d: [hi_f32(wt.at[t, d, wblk].bitcast(u32)[pl.ds(u, 8, stride=4), :] << shift) for t in range(2)])
        pacer = _Pacer(flt, 48)

        def proj(i, p, toks=()):
            a, b = [
                dot(hi, wqkv(i, p, t, k0=D // 2)) + head_start[i, p, t] if (i, p, t) in head_start
                else dot(lhs, wqkv(i, p, t, toks[t * len(toks) // 2:(t + 1) * len(toks) // 2]))
                for t in range(2)]
            pacer.feed(a)
            pacer.feed(b)
            c = as_bf16(pre[16 * i + p, pl.ds(r8, M), :]).astype(f32)
            return cat(a, b, c).astype(bf16)

        def probs(q, k):
            sc = dot_nt(q, k) * scale
            sc = jnp.where(fill == 0.0, sc, fill)
            e = jnp.exp(sc - jnp.max(sc, axis=1, keepdims=True))
            l = jnp.sum(e, axis=1, keepdims=True)
            r = pl.reciprocal(l, approx=True)
            r = r * (2.0 - l * r)
            rs.append([r[8 * j:8 * j + 8] for j in range(10)])
            return (e * r).astype(bf16)

        def pv(p, pr, v):
            o = dot(pr, v)
            heads[2 * p] = cat(o[0:8], o[16:32], o[64:72])
            heads[2 * p + 1] = cat(o[32:40], o[48:64], o[72:80])
            held[u, 2 * p], held[u, 2 * p + 1] = o[8:16], o[40:48]

        def left_task(q, i):
            def task(tok):
                ones = ((tok >> 16) | u32(0xFFFF)) | u32(0xFFFF0000)
                a = _strassen_left_one(i, lambda r, k: _Blocks(
                    held[2 * r + r2, 4 * q + 2 * k + k2] for r2 in range(2) for k2 in range(2)))
                for j in (0, 3):
                    a[j] = pltpu.bitcast(pltpu.bitcast(a[j], u32) & ones, f32)
                for j, v in enumerate(_strassen_left(*a)):
                    osum[7 * i + j, q, pl.ds(pl.multiple_of(M * n, M), M), :] = v.astype(bf16)
            return task

        pend = []
        for g in range(4):
            ps = range(4 * g, 4 * g + 4)
            qk = [(proj(0, p), proj(1, p)) for p in ps]
            vs = [proj(2, p, rs[p - 4] if g else ()) for p in ps]
            for a in pend:
                pv(*a)
            pend = [(p, probs(*qk[t]), vs[t]) for t, p in enumerate(ps)]
        pacer.done()

        def wo_part(oc, j, h0, h1, toks=()):
            return dot(oc, as_bf16(gated(wo32[j, pl.ds(64 * h0, 64 * (h1 - h0)), :], toks)))

        acc = []
        pacer = _Pacer([left_task(q, i) for q in range(8) for i in LEFT_AT[u]], 4 * (16 - LSTART) - 6)
        oc = jnp.concatenate(heads[0:24], axis=1).astype(bf16)
        for j in range(8):
            acc.append(wo_part(oc, j, 0, 24, {3: rs[12] + rs[13], 4: rs[14] + rs[15]}.get(j, ())))
            if j == 4:
                for a in pend:
                    pv(*a)
            if j >= LSTART:
                pacer.feed(acc[j])
        oc = jnp.concatenate(heads[24:32], axis=1).astype(bf16)
        nxt = []
        for j in range(8):
            r = wo_part(oc, j, 24, 32) + acc[j]
            outbuf[n, u, pl.ds(M, SEG - M), pl.ds(128 * j, 128)] = r[M:].astype(bf16)
            nxt.append(r[0:M])
            pacer.feed(r)
        pacer.done()
        return jnp.concatenate(nxt, axis=1)

    def steps(n, mem):
        pl.when(n == 1)(functools.partial(wait_all, c_rest))
        held = {}
        for u in range(UNROLL):
            mem = step(n, u, mem, held)
        return mem
    lax.fori_loop(0, NSEG // UNROLL, steps, mem0[...].astype(f32))
    tok_rows = pl.ds(M, SEG - M)
    c_out = [start(outbuf.at[:, :, tok_rows, :], out_hbm.at[:, :, tok_rows, pl.ds(0, D)], 0)]

    wait_all(c_b3)
    for task in filter_tasks(64, lambda d: [wl[t, :, pl.ds(128 * d, 128)].astype(f32) for t in range(2)]):
        task(jnp.zeros((8, 128), u32))
    b_stage3()
    c_out += [start(xb.at[j], out_hbm.at[:, :, :, pl.ds(D + 128 * j, 128)], 0) for j in range(8)]

    osum32 = osum.bitcast(u32)
    done = []
    for cq in range(2):
        def emit(row, col, *cs):
            for t, c in enumerate(cs):
                outbuf[:, row, pl.ds(0, M), pl.ds(128 * (4 * cq + col + t), 128)] = (
                    c.reshape(NSEG // 4, M, 128).astype(bf16))
            idx = (slice(None), row, pl.ds(0, M), pl.ds(128 * (4 * cq + col), 256))
            c_out.append(start(outbuf.at[idx], out_hbm.at[idx], 0))
        strassen2(lambda k, c: cat(*[wo32[4 * cq + c, pl.ds(64 * (4 * q + k), 64), :] for q in range(8)]),
                  lambda i: jnp.concatenate([as_bf16(osum32[i, q]) for q in range(8)], axis=1),
                  emit, done, _Pacer((), 0), DLAG)
    wait_all(c_out)


@jax.jit
def pallas_concat_heads__memory_aug_recurrent_mem_tr__spectral_gfnet__prompt_kernel(
    A_x: jax.Array,
    A_mem0: jax.Array,
    A_Wq: jax.Array,
    A_Wk: jax.Array,
    A_Wv: jax.Array,
    A_Wo: jax.Array,
    A_seg_len: jax.Array,
    B_x: jax.Array,
    B_w_r: jax.Array,
    B_w_i: jax.Array,
):
    del A_seg_len
    assert A_x.shape == (1, S, D) and A_mem0.shape == (1, M, D) and B_x.shape == (1, S, D)
    assert A_Wq.shape == (D, H, E) and A_Wo.shape == (H, E, D) and B_w_r.shape == (S, D // 2 + 1)
    gf, gi, mt, _ = _dft_constants()
    fill = _attn_fill()
    hbm = pl.BlockSpec(memory_space=pltpu.HBM)
    wshape = (D // 2, 2, 2, 16, E)
    out = pl.pallas_call(
        _kernel,
        out_shape=jax.ShapeDtypeStruct((NSEG // 4, 4, SEG, 2 * D), bf16),
        in_specs=[hbm] * 13,
        out_specs=hbm,
        scratch_shapes=[
            pltpu.VMEM((NRAW, D // 2, 2, 16, E), bf16),
            pltpu.VMEM((6, 16 * WP, E), u32),
            pltpu.VMEM((8, H * E, 128), bf16),
            pltpu.VMEM((NSEG, SEG - M, D), bf16),
            pltpu.VMEM((M, D), bf16),
            pltpu.VMEM((NSEG, M, D), bf16),
            pltpu.VMEM((7, 4, 128, 128), u32),
            pltpu.VMEM((49, 2, 64, 128), u32),
            pltpu.VMEM((48, NSEG * M, E), u32),
            pltpu.VMEM((49, 8, NSEG * M // 4, E), bf16),
            pltpu.VMEM((NSEG // 4, 4, SEG, D), bf16),
            pltpu.VMEM((96, 80), f32),
            pltpu.VMEM((8, NSEG // 4, 4, SEG, 128), bf16),
            pltpu.VMEM((2, 16, 512, 128), bf16),
            pltpu.VMEM((2, 1, S), bf16),
            pltpu.VMEM((12,) + gf.shape[1:], u32),
            pltpu.VMEM(gi.shape, u32),
            pltpu.VMEM(mt.shape, u32),
            pltpu.VMEM((8, 16 * XP, 128), f32),
            pltpu.VMEM((2, 16, 65, 8, 128), f32),
            pltpu.SemaphoreType.DMA((7,)),
        ],
        compiler_params=pltpu.CompilerParams(vmem_limit_bytes=120 * 1024 * 1024),
    )(A_x.reshape(NSEG, SEG, D), A_mem0.reshape(M, D),
      A_Wq.reshape(wshape), A_Wk.reshape(wshape), A_Wv.reshape(wshape),
      A_Wo.reshape(H * E, D), B_x.reshape(NSEG // 4, 4, SEG, D), B_w_r.T, B_w_i.T, gf, gi, mt, fill)
    return out.reshape(1, S, 2 * D)
```

```python
import functools

import jax
import jax.numpy as jnp
import numpy as np
from jax import lax
from jax.experimental import pallas as pl
from jax.experimental.pallas import tpu as pltpu

S, D, H, E, M, SEG = 2048, 1024, 32, 128, 8, 32
NSEG = S // SEG
WP = 516
XP = 132
ZP = 68
NRAW = 4
UNROLL = 4
MCT = 1
LAG = 8
DLAG = 100
LSTART = 5
LEFT_AT = ((), (2,), (4,), (0, 1, 3, 5, 6))
NB0 = 64
NBT = 13
MARGIN = 8
EARLY = ((0, 0, 0), (0, 0, 1), (1, 0, 0), (1, 0, 1), (0, 1, 0), (0, 1, 1))
bf16, f32, u32 = jnp.bfloat16, jnp.float32, jnp.uint32
RES = ((0, 4), (2, 6), (1, 7), (3, 5))
RC = float(np.sqrt(0.5))


def _fwd8(x):
    s04, d04 = x[0] + x[4], x[0] - x[4]
    s26, d26 = x[2] + x[6], x[2] - x[6]
    s15, d15 = x[1] + x[5], x[1] - x[5]
    s37, d37 = x[3] + x[7], x[3] - x[7]
    t1, t2 = (d15 - d37) * RC, (d15 + d37) * RC
    e0, o0 = s04 + s26, s15 + s37
    return [e0 + o0, e0 - o0, s04 - s26, s15 - s37, d04 + t1, d26 + t2, d04 - t1, d26 - t2]


def _inv8(z):
    z0, z4, e1, o1, r1, i1, r3, i3 = z
    e0, o0 = z0 + z4, z0 - z4
    s04, s26, s15, s37 = e0 + e1, e0 - e1, o0 + o1, o0 - o1
    d04, d26 = r1 + r3, i1 + i3
    t1, t2 = (r1 - r3) * RC, (i1 - i3) * RC
    d15, d37 = t1 + t2, t2 - t1
    return [s04 + d04, s15 + d15, s26 + d26, s37 + d37, s04 - d04, s15 - d15, s26 - d26, s37 - d37]


def _twiddle16(z, k):
    re, im = z
    k = k % 16
    if k == 0:
        return z
    if k == 4:
        return (im, -re)
    if k == 12:
        return (-im, re)
    if k == 2:
        return ((re + im) * RC, (im - re) * RC)
    if k == 14:
        return ((re - im) * RC, (re + im) * RC)
    if k == 6:
        return ((im - re) * RC, (re + im) * -RC)
    if k == 10:
        return ((re + im) * -RC, (re - im) * RC)
    c, s = float(np.cos(2 * np.pi * k / 16)), float(-np.sin(2 * np.pi * k / 16))
    return (re * c - im * s, re * s + im * c)


def _bfly4(z, sign):
    (ar, ai), (br, bi), (cr, ci), (dr, di) = z
    sr, si, tr, ti = ar + cr, ai + ci, ar - cr, ai - ci
    ur, ui, vr, vi = br + dr, bi + di, br - dr, bi - di
    o0, o2 = (sr + ur, si + ui), (sr - ur, si - ui)
    p, q = (tr + vi, ti - vr), (tr - vi, ti + vr)
    return [o0, p, o2, q] if sign > 0 else [o0, q, o2, p]


class _Pacer:
    def __init__(self, tasks, ntokens):
        self.slots = {}
        for n, task in enumerate(tasks):
            self.slots.setdefault(n * ntokens // len(tasks), []).append(task)
        self.pos = 0

    def feed(self, r):
        for j in range(r.shape[0] // 8):
            for task in self.slots.pop(self.pos, []):
                task(pltpu.bitcast(r[8 * j:8 * j + 8], u32))
            self.pos += 1

    def done(self):
        assert not self.slots


def _pack_rows(m):
    b = np.asarray(m, np.float32).astype(jnp.bfloat16).view(np.uint16).astype(np.uint32)
    return b[..., 0::2, :] | (b[..., 1::2, :] << 16)


@functools.lru_cache(maxsize=None)
def _dft_constants():
    b8 = np.array(_fwd8(list(np.eye(8)))).T
    n = np.arange(D)
    fw = np.zeros((D, D))
    bw = np.zeros((D, D))
    for g in range(4):
        k = np.concatenate([8 * np.arange(64) + r for r in RES[g]])
        ang = 2 * np.pi * ((n[:, None] * k[None, :]) % D) / D
        wgt = np.where(k == 0, 1.0, 2.0) / (D * S)
        fw[:, 256 * g:256 * g + 128] = np.cos(ang)
        fw[:, 256 * g + 128:256 * g + 256] = -np.sin(ang)
        bw[256 * g:256 * g + 128] = (np.cos(ang) * wgt).T
        bw[256 * g + 128:256 * g + 256] = (-np.sin(ang) * wgt).T
    bw[128, :] = (-1.0) ** n / (D * S)
    binv = np.kron(np.linalg.inv(b8), np.eye(128))
    gall = binv @ fw
    giall = bw @ binv.T
    gf = np.zeros((11, 144, 128))
    gi = np.zeros((11, 128, 128))
    sign = []
    half = lambda m, q: np.concatenate([m[64 * q:64 * q + 64], m[128 + 64 * q:192 + 64 * q]])
    for g in range(4):
        sl = slice(256 * g, 256 * g + 256)
        f, b = gall[sl, sl].T, giall[sl, sl]
        if g == 0:
            for q in range(2):
                gf[q, :128] = half(f, q)[:, 128 * q:128 * q + 128]
                gi[q] = half(b, q)[:, 128 * q:128 * q + 128]
            gf[0, 128] = (-1.0) ** np.arange(128)
            continue
        sg = np.sign(f[:128, 0] * f[128:, 128])[:, None]
        sign.append((int(sg[0, 0]), int(sg[64, 0])))
        p, q, r = f[:128, :128], f[:128, 128:], f[128:, :128]
        gf[3 * g - 1:3 * g + 2, :128] = p, q - p, r - sg * p
        p, q, r = b[:128, :128], b[:128, 128:], b[128:, :128]
        gi[3 * g - 1:3 * g + 2] = p, r - sg * p, q - p
    a = np.arange(128)
    mt = np.zeros((4, 16, 128, 128))
    for b in range(16):
        ang = 2 * np.pi * (((16 * a[:, None] + b) * a[None, :]) % S) / S
        c, sn = np.cos(ang), -np.sin(ang)
        mt[:, b] = c, c + sn, sn - c, sn
    return _pack_rows(gf), _pack_rows(gi), _pack_rows(mt), tuple(sign)


def _attn_fill():
    pos32 = np.arange(32)
    last = np.arange(16)
    qhead = np.concatenate([np.arange(64) // 32, last // 8])
    khead = np.concatenate([np.arange(64) // 32, last % 2])
    qpos = np.concatenate([pos32, pos32, 32 + last % 8])
    kpos = np.concatenate([pos32, pos32, 32 + last // 2])
    ok = (qpos[:, None] < M) | (qpos[:, None] >= kpos[None, :])
    fill = np.where(ok, 0.0, -1e9)
    fill = np.where(qhead[:, None] == khead[None, :], fill, -np.inf)
    return fill.astype(np.float32)


def _strassen(prod, b11, b12, b21, b22, add, sub, emit):
    m2 = prod(1, b11())
    m1 = prod(0, add(b11(), b22()))
    m3 = prod(2, sub(b12(), b22()))
    c22 = prod(5, add(b11(), b12())) + ((m1 - m2) + m3)
    m4 = prod(3, sub(b21(), b11()))
    emit(1, m2 + m4, c22)
    m5 = prod(4, b22())
    emit(0, prod(6, add(b21(), b22())) + ((m1 + m4) - m5), m3 + m5)


class _Blocks(list):
    def __add__(self, other):
        return _Blocks(a + b for a, b in zip(self, other))

    def __sub__(self, other):
        return _Blocks(a - b for a, b in zip(self, other))


def _strassen_left(a11, a12, a21, a22):
    return [a11 + a22, a21 + a22, a11, a22, a11 + a12, a21 - a11, a12 - a22]


def _strassen_left_one(i, blk):
    terms = ((0, 3, 1), (2, 3, 1), (0,), (3,), (0, 1, 1), (2, 0, -1), (1, 3, -1))[i]
    a = blk(*divmod(terms[0], 2))
    if len(terms) == 1:
        return a
    b = blk(*divmod(terms[1], 2))
    return a + b if terms[2] > 0 else a - b


def _kernel(x_hbm, mem_hbm, wq_hbm, wk_hbm, wv_hbm, wo_hbm, bx_hbm, wr_hbm, wi_hbm,
            gf_hbm, gi_hbm, mt_hbm, fill_hbm, out_hbm,
            wraw, wall, wo, xbuf, mem0, x8, xs, xs2, pre, osum, outbuf, fill_ref,
            xb, wt, wl, gf, gi, mt, xd, yb, sems):
    def start(src, dst, sem, priority=0):
        c = pltpu.make_async_copy(src, dst, sems.at[sem])
        c.start(priority=priority)
        return c

    def wait_all(cs):
        for c in cs:
            c.wait()

    dot = functools.partial(jnp.dot, preferred_element_type=f32)
    dot_nt = lambda a, b: lax.dot_general(a, b, (((1,), (1,)), ((), ())), preferred_element_type=f32)
    cat = lambda *vs: jnp.concatenate(vs, axis=0)
    as_bf16 = lambda w: pltpu.bitcast(w, bf16)
    lo_f32 = lambda w: pltpu.bitcast(w << 16, f32)
    hi_f32 = lambda w: pltpu.bitcast(w & u32(0xFFFF0000), f32)
    pack2 = lambda a, b: pltpu.pack_elementwise([a, b], packed_dtype=bf16)
    add2 = lambda a, b: pack2(lo_f32(a) + lo_f32(b), hi_f32(a) + hi_f32(b))
    sub2 = lambda a, b: pack2(lo_f32(a) - lo_f32(b), hi_f32(a) - hi_f32(b))
    w_hbm = (wq_hbm, wk_hbm, wv_hbm)

    def start_unit(u):
        return start(w_hbm[u // 2].at[:, :, u % 2], wraw.at[u % NRAW], u % NRAW)

    def start_x(seg0, nseg, sem, priority=0):
        segs, rows = pl.ds(seg0, nseg), pl.ds(0, SEG - M)
        return start(x_hbm.at[segs, rows, :], xbuf.at[segs], sem, priority)

    def start_filter(row0, nrows, sem, priority=0):
        rows = pl.ds(row0, nrows)
        return [start(w.at[rows, pl.ds(128 * d, 128)], wt.at[t, d, rows], sem, priority)
                for t, w in enumerate((wr_hbm, wi_hbm)) for d in range(16)]

    c_a = []
    for n in range(4):
        cols, rows = pl.ds(256 * n, 256), pl.ds(128 * n, 128)
        c_a.append([start(x_hbm.at[:, pl.ds(SEG - M, M), cols], x8.at[:, :, cols], n),
                    start(wq_hbm.at[rows, :, 0], wraw.at[0, rows], n)])
    c_loop = [start_x(0, UNROLL, 4, 1), start(mem_hbm, mem0, 4, 1), start(fill_hbm, fill_ref.at[pl.ds(0, 80)], 4, 1)]
    c_loop += [start(wo_hbm.at[:, pl.ds(128 * j, 128)], wo.at[j], 4, 1) for j in range(8)]

    xb32 = xb.bitcast(u32)

    def relayout_row(src, dst, r, lo, hi):
        a, b = src.at[r].bitcast(u32)[...]
        dst[pl.ds(r, 8, stride=WP), :] = (a & lo) | (b << 16)
        dst[pl.ds(r + 8 * WP, 8, stride=WP), :] = (a >> 16) | (b & hi)

    def relayout_tasks(u, r0=0, r1=D // 2):
        src, dst = wraw.at[u % NRAW], wall.at[u]

        def make(r):
            def task(tok):
                lo = (tok >> 16) | u32(0xFFFF)
                hi = (tok << 16) | u32(0xFFFF0000)
                relayout_row(src, dst, r, lo, hi)
                relayout_row(src, dst, r + 1, lo, hi)
            return task
        return [make(r) for r in range(r0, r1, 2)]

    def y_blocks(r):
        return pl.ds(4 * (r % 2) + r // 2, 8, stride=8)

    def filter_tasks(blk, wfn):
        def make(phase, k):
            slots = [4 * k + j for j in range(4)] if phase == 1 else [4 * j + k for j in range(4)]

            def task(tok):
                ones = ((tok >> 16) | u32(0xFFFF)) | u32(0xFFFF0000)
                z = [(yb[0, b, blk], yb[1, b, blk]) for b in slots]
                z[0] = tuple(pltpu.bitcast(pltpu.bitcast(v, u32) & ones, f32) for v in z[0])
                if phase == 0:
                    o = _bfly4(z, 1)
                    o = [_twiddle16(o[j], k * j) for j in range(4)]
                elif phase == 1:
                    o = _bfly4(z, 1)
                    y = []
                    for j in range(4):
                        wr, wi = wfn(k + 4 * j)
                        xr, xi = o[j]
                        y.append((xr * wr - xi * wi, xr * wi + xi * wr))
                    o = _bfly4(y, -1)
                    o = [_twiddle16(o[j], -k * j) for j in range(4)]
                else:
                    o = _bfly4(z, -1)
                for b, v in zip(slots, o):
                    yb[0, b, blk] = v[0]
                    yb[1, b, blk] = v[1]
            return task
        return [make(phase, k) for phase in range(3) for k in range(4)]

    def z_region(n, par):
        return (2 * n + par) // 3, (2 * n + par) % 3 * 8 * ZP

    def butterfly_tasks(par):
        def make(a2):
            def task(tok):
                zs = []
                for a in (2 * a2, 2 * a2 + 1):
                    w = [xb32[j, a // 8, a // 2 % 4, pl.ds(8 * (a % 2), 8), :] for j in range(8)]
                    if par:
                        hi = (tok << 16) | u32(0xFFFF0000)
                        z = _fwd8([pltpu.bitcast(v & hi, f32) for v in w])
                    else:
                        sixteen = ((tok >> 31) | u32(1)) << 4
                        z = _fwd8([pltpu.bitcast(v << sixteen, f32) for v in w])
                    zs.append(z[0:2] + [v for g in range(1, 4)
                                        for v in (z[2 * g] + z[2 * g + 1], z[2 * g + 1], z[2 * g])])
                for n in range(11):
                    plane, row = z_region(n, par)
                    xd[plane, pl.ds(row + a2, 8, stride=ZP), :] = pltpu.bitcast(pack2(zs[0][n], zs[1][n]), f32)
            return task
        return [make(a2) for a2 in range(64)]

    sign = _dft_constants()[3]

    def b_dfwd(b, pacer):
        def z(n):
            plane, row = z_region(n, b % 2)
            return as_bf16(xd[plane, pl.ds(row + b // 2 * ZP, 64), :])
        t0 = dot_nt(as_bf16(gf[0]), z(0))
        t4 = dot_nt(as_bf16(gf[1, 0:64]), z(1))
        tr, ti = cat(t0[0:64], t4[0:64]), cat(t0[64:128], t4[64:128])
        ts = [(cat(tr + ti, t0[128:144]).astype(bf16), ti.astype(bf16), cat(tr, t0[128:144]).astype(bf16))]
        for g in range(1, 4):
            k1, k2, k3 = [dot_nt(as_bf16(gf[n, 0:64]), z(n)) for n in range(3 * g - 1, 3 * g + 2)]
            pacer.feed(k1)
            tr = k1 + k2
            ti = cat(*[k3[64 * q:64 * q + 64] + k1[64 * q:64 * q + 64] if sign[g - 1][q] > 0
                       else k3[64 * q:64 * q + 64] - k1[64 * q:64 * q + 64] for q in range(2)])
            ts.append(((tr + ti).astype(bf16), ti.astype(bf16), tr.astype(bf16)))
        return ts

    def b_sfwd(b, ts, pacer):
        for g in range(4):
            k1, k2, k3 = [dot(ts[g][n], as_bf16(mt[n, b])) for n in range(3)]
            if g:
                pacer.feed(k2)
            yr, yi = k1[0:128] - k2, k1 + k3
            for q in range(2):
                yb[0, b, y_blocks(RES[g][q])] = yr[64 * q:64 * q + 64].reshape(8, 8, 128)
                yb[1, b, y_blocks(RES[g][q])] = yi[64 * q:64 * q + 64].reshape(8, 8, 128)
            if g == 0:
                yb[0, b, 64] = k1[128:136]
                yb[1, b, 64] = yi[128:136]

    def b_stage1(tasks):
        pacer = _Pacer(tasks, NBT * 48)
        prev = None
        for b in list(range(0, 16, 2)) + list(range(1, 16, 2)):
            ts = b_dfwd(b, pacer)
            if prev is not None:
                b_sfwd(*prev, pacer)
            prev = (b, ts)
        b_sfwd(*prev, pacer)
        pacer.done()

    def b_stage3():
        row0 = lax.broadcasted_iota(jnp.int32, (8, 128), 0) == 0
        low = lax.broadcasted_iota(jnp.int32, (1, 128), 1) < 64
        for b in range(16):
            m = [as_bf16(mt[n, b]) for n in range(4)]
            for g in (1, 2, 3, 0):
                yr, yi = [cat(*[yb[c, b, y_blocks(r)].reshape(64, 128) for r in RES[g]]) for c in range(2)]
                if g == 0:
                    nr = -yr
                    u0 = cat(yr[0:64], jnp.where(row0, yb[0, b, 64], yi[0:8]), yi[8:64])
                    v0 = cat(yi[0:64], jnp.where(row0, yb[1, b, 64], nr[0:8]), nr[8:64])
                    u4, v4 = cat(yr[64:128], yi[64:128]), cat(yi[64:128], nr[64:128])
                    t1 = dot_nt(m[0], u0.astype(bf16)) + dot_nt(m[3], v0.astype(bf16))
                    t2 = dot_nt(m[0], u4.astype(bf16)) + dot_nt(m[3], v4.astype(bf16))
                else:
                    k1, k2, k3 = [dot_nt(m[n], v.astype(bf16)) for n, v in enumerate((yr + yi, yr, yi))]
                    t1, t2 = k1 + k3, k1 - k2
                slot = b // 2 + 8 * (b % 2)
                xd[2 * g, pl.ds(XP * slot, 128), :] = t1
                xd[2 * g + 1, pl.ds(XP * slot, 128), :] = t2
        for t in range(16):
            rows = lambda j: cat(*[xd[j, pl.ds(8 * t + u, 16, stride=XP), :] for u in range(8)])
            z = [dot(rows(q).astype(bf16), as_bf16(gi[q])) for q in range(2)]
            for g in range(1, 4):
                tr, ti = rows(2 * g), rows(2 * g + 1)
                sg = jnp.where(low, float(sign[g - 1][0]), float(sign[g - 1][1]))
                k1, k2, k3 = [dot(v.astype(bf16), as_bf16(gi[3 * g - 1 + n]))
                              for n, v in enumerate((tr + sg * ti, ti, tr))]
                z += [k1 + k2, k1 + k3]
            y = _inv8(z)
            for j in range(8):
                even = cat(*[y[j][16 * u:16 * u + 8] for u in range(8)])
                odd = cat(*[y[j][16 * u + 8:16 * u + 16] for u in range(8)])
                xb32[j, t] = pack2(even, odd).reshape(4, 16, 128)

    HALF = NSEG * M // 2

    def batch(u, p0, p1, tasks=(), t0=0, t1=4):
        mc = HALF // 2 if t1 - t0 <= MCT else HALF
        pacer = _Pacer(tasks, (7 * (p1 - p0) - MARGIN // (t1 - t0)) * HALF // 8)
        w = wall.at[u]
        for p in range(p0, p1):
            for r0 in range(0, HALF, mc):
                def blk(head, par):
                    return lambda: cat(*[w[pl.ds((p + 8 * head) * WP + 64 * (2 * t + par), 64), :]
                                         for t in range(t0, t1)])

                def prod(i, b):
                    lhs = jnp.concatenate([as_bf16(xs[i, t, pl.ds(r0 // 2, mc // 2), :])
                                           for t in range(t0, t1)], axis=1)
                    r = dot(lhs, as_bf16(b))
                    pacer.feed(r)
                    return r

                def emit(half, *cs):
                    rows = pl.ds(half * HALF + r0, mc)
                    park = pl.ds((half * HALF + r0) // 8, mc // 8)
                    if t0 > 0:
                        cs = [c + yb[t, p, park].reshape(mc, E) for t, c in enumerate(cs)]
                    if t1 < 4:
                        for t, c in enumerate(cs):
                            yb[t, p, park] = c.reshape(mc // 8, 8, E)
                    elif u >= 2:
                        pre[8 * u + p, rows, :] = pack2(*cs)
                    else:
                        st = jnp.concatenate([c.reshape(mc // M, M, E) for c in cs], axis=1)
                        pre[8 * u + p, rows, :] = pltpu.bitcast(st.reshape(2 * mc, E).astype(bf16), u32)
                if t0 // (t1 - t0) % 2:
                    _strassen(prod, blk(1, 0), blk(0, 0), blk(1, 1), blk(0, 1), add2, sub2,
                              lambda half, c1, c0: emit(half, c0, c1))
                else:
                    _strassen(prod, blk(0, 0), blk(1, 0), blk(0, 1), blk(1, 1), add2, sub2, emit)
        pacer.done()

    QUART = HALF // 2

    def unpack_after(w, tok):
        reps = (w.shape[0] // 8, 1)
        hi = jnp.tile((tok << 16) | u32(0xFFFF0000), reps)
        sixteen = jnp.tile(((tok >> 31) | u32(1)) << 4, reps)
        return _Blocks([pltpu.bitcast(w << sixteen, f32), pltpu.bitcast(w & hi, f32)])

    def strassen2(right, left, emit, done, pacer, lag=LAG):
        def unpack(b):
            if isinstance(b, _Blocks):
                return b
            if len(done) < lag:
                return _Blocks([lo_f32(b), hi_f32(b)])
            return unpack_after(b, done[-lag])
        add = lambda a, b: unpack(a) + unpack(b)
        sub = lambda a, b: unpack(a) - unpack(b)

        def outer_prod(i, bs):
            def prod(j, b):
                r = dot(left(7 * i + j), as_bf16(pack2(*b) if isinstance(b, _Blocks) else b))
                pacer.feed(r)
                done.append(pltpu.bitcast(r[0:8], u32))
                return r
            order = (1, 0, 3, 2) if i in (1, 4, 5, 6) else (0, 1, 2, 3)
            cs = {}
            _strassen(prod, *[(lambda b=bs[k]: b) for k in order], add, sub, lambda half, *c: cs.update({half: c}))
            return _Blocks((cs[0] + cs[1])[k] for k in order)

        def outer_emit(half, *cs):
            for col in (1, 0):
                for a in range(2):
                    emit(2 * half + a, 2 * col, cs[col][2 * a], cs[col][2 * a + 1])
        outer = lambda k, c: lambda: [right(2 * k + k2, 2 * c + c2) for k2 in range(2) for c2 in range(2)]
        _strassen(outer_prod, outer(0, 0), outer(0, 1), outer(1, 0), outer(1, 1),
                  lambda x, y: [add(a, b) for a, b in zip(x, y)],
                  lambda x, y: [sub(a, b) for a, b in zip(x, y)], outer_emit)

    def batch2(u, q0, q1, done, tasks=()):
        pacer = _Pacer(tasks, (49 * (q1 - q0) - MARGIN) * QUART // 8)
        w = wall.at[u]
        for q in range(q0, q1):
            def emit(row, col, c0, c1):
                pre[8 * u + 2 * q + col // 2, pl.ds(row * QUART, QUART), :] = pack2(c0, c1)
            strassen2(lambda k, c: cat(*[w[pl.ds((2 * q + c // 2 + 8 * (c % 2)) * WP + 64 * (k + 4 * t), 64), :]
                                         for t in range(2)]),
                      lambda i: jnp.concatenate([as_bf16(xs2[i, t]) for t in range(2)], axis=1),
                      emit, done, pacer)
        pacer.done()

    def left2_tasks():
        def make(i, t, r):
            def task(tok):
                def blk(rh, kh):
                    ws = [pltpu.bitcast(x8[pl.ds(32 * rh + 16 * rl + 2 * r, 2), :,
                                           pl.ds(128 * (2 * kh + kl + 4 * t), 128)].reshape(16, 128), u32)
                          for rl in range(2) for kl in range(2)]
                    return _Blocks(unpack_after(v, tok) for v in ws)
                for j, v in enumerate(_strassen_left(*_strassen_left_one(i, blk))):
                    xs2[7 * i + j, t, pl.ds(8 * r, 8), :] = pack2(*v)
            return task
        return [make(i, t, r) for i in range(7) for t in range(2) for r in range(8)]

    def prepare_left(n):
        v = pltpu.bitcast(x8[:, :, pl.ds(256 * n, 256)].reshape(2 * HALF, 256), u32)
        blocks = [v[HALF // 2 * h:HALF // 2 * (h + 1), 128 * k:128 * (k + 1)] for h in range(2) for k in range(2)]
        lo, hi = [_strassen_left(*[un(b) for b in blocks]) for un in (lo_f32, hi_f32)]
        for i in range(7):
            xs[i, n] = pack2(lo[i], hi[i])

    wait_all(c_a[0])
    for task in relayout_tasks(0, 0, 128):
        task(jnp.zeros((8, 128), u32))
    prepare_left(0)
    batch(0, 0, 6, (), 0, 1)
    wait_all(c_a[1])
    c_h = [start(wq_hbm.at[pl.ds(256 * n, 256), :, 1], wraw.at[1, pl.ds(256 * n, 256)], n) for n in range(2)]
    prepare_left(1)
    batch(0, 6, 8, relayout_tasks(0, 128, 256), 0, 1)
    batch(0, 0, 6, (), 1, 2)
    wait_all(c_a[2])
    prepare_left(2)
    batch(0, 6, 8, relayout_tasks(0, 256, 384), 1, 2)
    batch(0, 0, 6, (), 2, 3)
    wait_all(c_a[3])
    c_w2 = start_unit(2)
    prepare_left(3)
    batch(0, 6, 8, relayout_tasks(0, 384, 512), 2, 3)
    batch(0, 0, 5, (), 3, 4)
    c_h[0].wait()
    batch(0, 5, 8, relayout_tasks(1, 0, 256), 3, 4)
    left2 = left2_tasks()
    batch(1, 0, 5, left2[:64], 0, 2)
    c_h[1].wait()
    start_unit(3)
    batch(1, 5, 8, relayout_tasks(1, 256, 512), 0, 2)
    batch(1, 0, 4, left2[64:], 2, 4)
    c_w2.wait()
    start_unit(4)
    start_unit(5)
    c_b1 = [start(bx_hbm.at[:, :, :, pl.ds(128 * j, 128)], xb.at[j], 5) for j in range(8)]
    c_b1 += [start(gf_hbm, gf.at[pl.ds(0, 11)], 5), start(mt_hbm.at[pl.ds(0, 3)], mt.at[pl.ds(0, 3)], 5)]
    c_loop += start_filter(0, 64, 4, 1)
    batch(1, 4, 8, relayout_tasks(2), 2, 4)
    batch2(2, 0, 2, [])

    def unit_body(u, c):
        slot = (u + 1) % NRAW
        pltpu.make_async_copy(wraw.at[slot], wraw.at[slot], sems.at[slot]).wait()
        done = []
        batch2(u, 2, 4, done, relayout_tasks(u + 1))
        batch2(u + 1, 0, 2, done)
        return c
    lax.fori_loop(2, 5, unit_body, 0)
    wait_all(c_b1)
    bfly = butterfly_tasks(0) + butterfly_tasks(1)
    batch(5, 6, 8, bfly[:NB0])
    batch2(5, 2, 3, [])
    b_stage1(bfly[NB0:])
    wait_all(c_loop)
    c_rest = [start_x(UNROLL, NSEG - UNROLL, 6)] + start_filter(64, 448, 6)
    c_b3 = [start(w.at[pl.ds(512, 1), :], wl.at[t], 5) for t, w in enumerate((wr_hbm, wi_hbm))]
    c_b3 += [start(gi_hbm, gi, 5), start(mt_hbm.at[3], mt.at[3], 5)]

    wo32 = wo.bitcast(u32)
    scale = E ** -0.5

    def gated(w, toks):
        if not toks:
            return w
        bits = functools.reduce(
            jnp.bitwise_or, [pltpu.bitcast(jnp.broadcast_to(t, (8, 128)), u32) for t in toks])
        ones = ((bits >> 16) | u32(0xFFFF)) | u32(0xFFFF0000)
        return cat(w[0:8] & ones, w[8:])

    def wqkv(i, p, second, toks=(), k0=0, k1=D):
        rows = pl.ds((p % 8 + 8 * second) * WP + k0 // 2, (k1 - k0) // 2)
        return as_bf16(gated(wall[2 * i + p // 8, rows, :], toks))

    def step(n, u, mem, held):
        s = UNROLL * n + u
        rows = cat(mem, xbuf[s].astype(f32))
        lhs = rows.astype(bf16)
        head_start = {}
        if u:
            lo, hi = rows[:, :D // 2].astype(bf16), rows[:, D // 2:].astype(bf16)
            for key in EARLY:
                head_start[key] = dot(lo, wqkv(*key, k1=D // 2))
        r8 = pl.multiple_of(M * s, M)
        fill = fill_ref[pl.ds(0, 80), :]
        heads = [None] * H
        rs = []

        shift = jnp.full((8, 128), 16 - 16 * (n % 2), jnp.int32).astype(u32)
        wblk = pl.ds(pl.multiple_of(64 * (n // 2), 64), 64)
        flt = filter_tasks(
            s, lambda d: [hi_f32(wt.at[t, d, wblk].bitcast(u32)[pl.ds(u, 8, stride=4), :] << shift) for t in range(2)])
        pacer = _Pacer(flt, 48)

        def proj(i, p, toks=()):
            a, b = [
                dot(hi, wqkv(i, p, t, k0=D // 2)) + head_start[i, p, t] if (i, p, t) in head_start
                else dot(lhs, wqkv(i, p, t, toks[t * len(toks) // 2:(t + 1) * len(toks) // 2]))
                for t in range(2)]
            pacer.feed(a)
            pacer.feed(b)
            c = as_bf16(pre[16 * i + p, pl.ds(r8, M), :]).astype(f32)
            return cat(a, b, c).astype(bf16)

        def probs(q, k):
            sc = dot_nt(q, k) * scale
            sc = jnp.where(fill == 0.0, sc, fill)
            e = jnp.exp(sc - jnp.max(sc, axis=1, keepdims=True))
            l = jnp.sum(e, axis=1, keepdims=True)
            r = pl.reciprocal(l, approx=True)
            r = r * (2.0 - l * r)
            rs.append([r[8 * j:8 * j + 8] for j in range(10)])
            return (e * r).astype(bf16)

        def pv(p, pr, v):
            o = dot(pr, v)
            heads[2 * p] = cat(o[0:8], o[16:32], o[64:72])
            heads[2 * p + 1] = cat(o[32:40], o[48:64], o[72:80])
            held[u, 2 * p], held[u, 2 * p + 1] = o[8:16], o[40:48]

        def left_task(q, i):
            def task(tok):
                ones = ((tok >> 16) | u32(0xFFFF)) | u32(0xFFFF0000)
                a = _strassen_left_one(i, lambda r, k: _Blocks(
                    held[2 * r + r2, 4 * q + 2 * k + k2] for r2 in range(2) for k2 in range(2)))
                for j in (0, 3):
                    a[j] = pltpu.bitcast(pltpu.bitcast(a[j], u32) & ones, f32)
                for j, v in enumerate(_strassen_left(*a)):
                    osum[7 * i + j, q, pl.ds(pl.multiple_of(M * n, M), M), :] = v.astype(bf16)
            return task

        pend = []
        for g in range(4):
            ps = range(4 * g, 4 * g + 4)
            qk = [(proj(0, p), proj(1, p)) for p in ps]
            vs = [proj(2, p, rs[p - 4] if g else ()) for p in ps]
            for a in pend:
                pv(*a)
            pend = [(p, probs(*qk[t]), vs[t]) for t, p in enumerate(ps)]
        pacer.done()

        def wo_part(oc, j, h0, h1, toks=()):
            return dot(oc, as_bf16(gated(wo32[j, pl.ds(64 * h0, 64 * (h1 - h0)), :], toks)))

        acc = []
        pacer = _Pacer([left_task(q, i) for q in range(8) for i in LEFT_AT[u]], 4 * (16 - LSTART) - 6)
        oc = jnp.concatenate(heads[0:24], axis=1).astype(bf16)
        for j in range(8):
            acc.append(wo_part(oc, j, 0, 24, {3: rs[12] + rs[13], 4: rs[14] + rs[15]}.get(j, ())))
            if j == 4:
                for a in pend:
                    pv(*a)
            if j >= LSTART:
                pacer.feed(acc[j])
        oc = jnp.concatenate(heads[24:32], axis=1).astype(bf16)
        nxt = []
        for j in range(8):
            r = wo_part(oc, j, 24, 32) + acc[j]
            outbuf[n, u, pl.ds(M, SEG - M), pl.ds(128 * j, 128)] = r[M:].astype(bf16)
            nxt.append(r[0:M])
            pacer.feed(r)
        pacer.done()
        return jnp.concatenate(nxt, axis=1)

    def steps(n, mem):
        pl.when(n == 1)(functools.partial(wait_all, c_rest))
        held = {}
        for u in range(UNROLL):
            mem = step(n, u, mem, held)
        return mem
    lax.fori_loop(0, NSEG // UNROLL, steps, mem0[...].astype(f32))
    tok_rows = pl.ds(M, SEG - M)
    c_out = [start(outbuf.at[:, :, tok_rows, :], out_hbm.at[:, :, tok_rows, pl.ds(0, D)], 0)]

    wait_all(c_b3)
    for task in filter_tasks(64, lambda d: [wl[t, :, pl.ds(128 * d, 128)].astype(f32) for t in range(2)]):
        task(jnp.zeros((8, 128), u32))
    b_stage3()
    c_out += [start(xb.at[j], out_hbm.at[:, :, :, pl.ds(D + 128 * j, 128)], 0) for j in range(8)]

    osum32 = osum.bitcast(u32)
    done = []
    for cq in range(2):
        def emit(row, col, *cs):
            for t, c in enumerate(cs):
                outbuf[:, row, pl.ds(0, M), pl.ds(128 * (4 * cq + col + t), 128)] = (
                    c.reshape(NSEG // 4, M, 128).astype(bf16))
            idx = (slice(None), row, pl.ds(0, M), pl.ds(128 * (4 * cq + col), 256))
            c_out.append(start(outbuf.at[idx], out_hbm.at[idx], 0))
        strassen2(lambda k, c: cat(*[wo32[4 * cq + c, pl.ds(64 * (4 * q + k), 64), :] for q in range(8)]),
                  lambda i: jnp.concatenate([as_bf16(osum32[i, q]) for q in range(8)], axis=1),
                  emit, done, _Pacer((), 0), DLAG)
    wait_all(c_out)


@jax.jit
def pallas_concat_heads__memory_aug_recurrent_mem_tr__spectral_gfnet__prompt_kernel(
    A_x: jax.Array,
    A_mem0: jax.Array,
    A_Wq: jax.Array,
    A_Wk: jax.Array,
    A_Wv: jax.Array,
    A_Wo: jax.Array,
    A_seg_len: jax.Array,
    B_x: jax.Array,
    B_w_r: jax.Array,
    B_w_i: jax.Array,
):
    del A_seg_len
    assert A_x.shape == (1, S, D) and A_mem0.shape == (1, M, D) and B_x.shape == (1, S, D)
    assert A_Wq.shape == (D, H, E) and A_Wo.shape == (H, E, D) and B_w_r.shape == (S, D // 2 + 1)
    gf, gi, mt, _ = _dft_constants()
    fill = _attn_fill()
    hbm = pl.BlockSpec(memory_space=pltpu.HBM)
    wshape = (D // 2, 2, 2, 16, E)
    out = pl.pallas_call(
        _kernel,
        out_shape=jax.ShapeDtypeStruct((NSEG // 4, 4, SEG, 2 * D), bf16),
        in_specs=[hbm] * 13,
        out_specs=hbm,
        scratch_shapes=[
            pltpu.VMEM((NRAW, D // 2, 2, 16, E), bf16),
            pltpu.VMEM((6, 16 * WP, E), u32),
            pltpu.VMEM((8, H * E, 128), bf16),
            pltpu.VMEM((NSEG, SEG - M, D), bf16),
            pltpu.VMEM((M, D), bf16),
            pltpu.VMEM((NSEG, M, D), bf16),
            pltpu.VMEM((7, 4, 128, 128), u32),
            pltpu.VMEM((49, 2, 64, 128), u32),
            pltpu.VMEM((48, NSEG * M, E), u32),
            pltpu.VMEM((49, 8, NSEG * M // 4, E), bf16),
            pltpu.VMEM((NSEG // 4, 4, SEG, D), bf16),
            pltpu.VMEM((96, 80), f32),
            pltpu.VMEM((8, NSEG // 4, 4, SEG, 128), bf16),
            pltpu.VMEM((2, 16, 512, 128), bf16),
            pltpu.VMEM((2, 1, S), bf16),
            pltpu.VMEM((12,) + gf.shape[1:], u32),
            pltpu.VMEM(gi.shape, u32),
            pltpu.VMEM(mt.shape, u32),
            pltpu.VMEM((8, 16 * XP, 128), f32),
            pltpu.VMEM((2, 16, 65, 8, 128), f32),
            pltpu.SemaphoreType.DMA((7,)),
        ],
        compiler_params=pltpu.CompilerParams(vmem_limit_bytes=120 * 1024 * 1024),
    )(A_x.reshape(NSEG, SEG, D), A_mem0.reshape(M, D),
      A_Wq.reshape(wshape), A_Wk.reshape(wshape), A_Wv.reshape(wshape),
      A_Wo.reshape(H * E, D), B_x.reshape(NSEG // 4, 4, SEG, D), B_w_r.T, B_w_i.T, gf, gi, mt, fill)
    return out.reshape(1, S, 2 * D)
```

```python
import functools

import jax
import jax.numpy as jnp
import numpy as np
from jax import lax
from jax.experimental import pallas as pl
from jax.experimental.pallas import tpu as pltpu

S, D, H, E, M, SEG = 2048, 1024, 32, 128, 8, 32
NSEG = S // SEG
WP = 516
XP = 132
NRAW = 4
UNROLL = 4
MCT = 1
LAG = 8
PM1 = 0
PS = (6, 4, 4, 4)
PM2 = 1
DLAG = 100
LSTART = 5
LEFT_AT = ((), (2,), (4,), (0, 1, 3, 5, 6))
NB0 = 128
NBT = 13
MARGIN = 4
EARLY = ((0, 0, 0), (0, 0, 1), (1, 0, 0), (1, 0, 1), (0, 1, 0), (0, 1, 1))
bf16, f32, u32 = jnp.bfloat16, jnp.float32, jnp.uint32
RES = ((0, 4), (2, 6), (1, 7), (3, 5))
RC = float(np.sqrt(0.5))


def _fwd8(x):
    s04, d04 = x[0] + x[4], x[0] - x[4]
    s26, d26 = x[2] + x[6], x[2] - x[6]
    s15, d15 = x[1] + x[5], x[1] - x[5]
    s37, d37 = x[3] + x[7], x[3] - x[7]
    t1, t2 = (d15 - d37) * RC, (d15 + d37) * RC
    e0, o0 = s04 + s26, s15 + s37
    return [e0 + o0, e0 - o0, s04 - s26, s15 - s37, d04 + t1, d26 + t2, d04 - t1, d26 - t2]


def _inv8(z):
    z0, z4, e1, o1, r1, i1, r3, i3 = z
    e0, o0 = z0 + z4, z0 - z4
    s04, s26, s15, s37 = e0 + e1, e0 - e1, o0 + o1, o0 - o1
    d04, d26 = r1 + r3, i1 + i3
    t1, t2 = (r1 - r3) * RC, (i1 - i3) * RC
    d15, d37 = t1 + t2, t2 - t1
    return [s04 + d04, s15 + d15, s26 + d26, s37 + d37, s04 - d04, s15 - d15, s26 - d26, s37 - d37]


def _twiddle16(z, k):
    re, im = z
    k = k % 16
    if k == 0:
        return z
    if k == 4:
        return (im, -re)
    if k == 12:
        return (-im, re)
    if k == 2:
        return ((re + im) * RC, (im - re) * RC)
    if k == 14:
        return ((re - im) * RC, (re + im) * RC)
    if k == 6:
        return ((im - re) * RC, (re + im) * -RC)
    if k == 10:
        return ((re + im) * -RC, (re - im) * RC)
    c, s = float(np.cos(2 * np.pi * k / 16)), float(-np.sin(2 * np.pi * k / 16))
    return (re * c - im * s, re * s + im * c)


def _bfly4(z, sign):
    (ar, ai), (br, bi), (cr, ci), (dr, di) = z
    sr, si, tr, ti = ar + cr, ai + ci, ar - cr, ai - ci
    ur, ui, vr, vi = br + dr, bi + di, br - dr, bi - di
    o0, o2 = (sr + ur, si + ui), (sr - ur, si - ui)
    p, q = (tr + vi, ti - vr), (tr - vi, ti + vr)
    return [o0, p, o2, q] if sign > 0 else [o0, q, o2, p]


class _Pacer:
    def __init__(self, tasks, ntokens):
        self.slots = {}
        for n, task in enumerate(tasks):
            self.slots.setdefault(n * ntokens // len(tasks), []).append(task)
        self.pos = 0

    def feed(self, r):
        for j in range(r.shape[0] // 8):
            for task in self.slots.pop(self.pos, []):
                task(pltpu.bitcast(r[8 * j:8 * j + 8], u32))
            self.pos += 1

    def done(self):
        assert not self.slots


def _pack_rows(m):
    b = np.asarray(m, np.float32).astype(jnp.bfloat16).view(np.uint16).astype(np.uint32)
    return b[..., 0::2, :] | (b[..., 1::2, :] << 16)


@functools.lru_cache(maxsize=None)
def _dft_constants():
    b8 = np.array(_fwd8(list(np.eye(8)))).T
    n = np.arange(D)
    fw = np.zeros((D, D))
    bw = np.zeros((D, D))
    for g in range(4):
        k = np.concatenate([8 * np.arange(64) + r for r in RES[g]])
        ang = 2 * np.pi * ((n[:, None] * k[None, :]) % D) / D
        wgt = np.where(k == 0, 1.0, 2.0) / (D * S)
        fw[:, 256 * g:256 * g + 128] = np.cos(ang)
        fw[:, 256 * g + 128:256 * g + 256] = -np.sin(ang)
        bw[256 * g:256 * g + 128] = (np.cos(ang) * wgt).T
        bw[256 * g + 128:256 * g + 256] = (-np.sin(ang) * wgt).T
    bw[128, :] = (-1.0) ** n / (D * S)
    binv = np.kron(np.linalg.inv(b8), np.eye(128))
    gall = binv @ fw
    giall = bw @ binv.T
    gf = np.zeros((11, 144, 128))
    gi = np.zeros((11, 128, 128))
    sign = []
    half = lambda m, q: np.concatenate([m[64 * q:64 * q + 64], m[128 + 64 * q:192 + 64 * q]])
    for g in range(4):
        sl = slice(256 * g, 256 * g + 256)
        f, b = gall[sl, sl].T, giall[sl, sl]
        if g == 0:
            for q in range(2):
                gf[q, :128] = half(f, q)[:, 128 * q:128 * q + 128]
                gi[q] = half(b, q)[:, 128 * q:128 * q + 128]
            gf[0, 128] = (-1.0) ** np.arange(128)
            continue
        sg = np.sign(f[:128, 0] * f[128:, 128])[:, None]
        sign.append((int(sg[0, 0]), int(sg[64, 0])))
        p, q, r = f[:128, :128], f[:128, 128:], f[128:, :128]
        gf[3 * g - 1:3 * g + 2, :128] = p, q - p, r - sg * p
        p, q, r = b[:128, :128], b[:128, 128:], b[128:, :128]
        gi[3 * g - 1:3 * g + 2] = p, r - sg * p, q - p
    a = np.arange(128)
    mt = np.zeros((4, 16, 128, 128))
    for b in range(16):
        ang = 2 * np.pi * (((16 * a[:, None] + b) * a[None, :]) % S) / S
        c, sn = np.cos(ang), -np.sin(ang)
        mt[:, b] = c, c + sn, sn - c, sn
    return _pack_rows(gf), _pack_rows(gi), _pack_rows(mt), tuple(sign)


def _attn_fill():
    head = np.concatenate([np.arange(64) // 32, np.arange(16) // 8])
    pos = np.concatenate([np.arange(64) % 32, 32 + np.arange(16) % 8])
    ok = (pos[:, None] < M) | (pos[:, None] >= pos[None, :])
    fill = np.where(ok, 0.0, -1e9)
    fill = np.where(head[:, None] == head[None, :], fill, -np.inf)
    return fill.astype(np.float32)


def _strassen(prod, b11, b12, b21, b22, add, sub, emit):
    m2 = prod(1, b11())
    m1 = prod(0, add(b11(), b22()))
    m3 = prod(2, sub(b12(), b22()))
    c22 = prod(5, add(b11(), b12())) + ((m1 - m2) + m3)
    m4 = prod(3, sub(b21(), b11()))
    emit(1, m2 + m4, c22)
    m5 = prod(4, b22())
    emit(0, prod(6, add(b21(), b22())) + ((m1 + m4) - m5), m3 + m5)


class _Blocks(list):
    def __add__(self, other):
        return _Blocks(a + b for a, b in zip(self, other))

    def __sub__(self, other):
        return _Blocks(a - b for a, b in zip(self, other))


def _strassen_left(a11, a12, a21, a22):
    return [a11 + a22, a21 + a22, a11, a22, a11 + a12, a21 - a11, a12 - a22]


def _strassen_left_one(i, blk):
    terms = ((0, 3, 1), (2, 3, 1), (0,), (3,), (0, 1, 1), (2, 0, -1), (1, 3, -1))[i]
    a = blk(*divmod(terms[0], 2))
    if len(terms) == 1:
        return a
    b = blk(*divmod(terms[1], 2))
    return a + b if terms[2] > 0 else a - b


def _kernel(x_hbm, mem_hbm, wq_hbm, wk_hbm, wv_hbm, wo_hbm, bx_hbm, wr_hbm, wi_hbm,
            gf_hbm, gi_hbm, mt_hbm, fill_hbm, out_hbm,
            wraw, wall, wo, xbuf, mem0, x8, xs, xs2, pre, osum, outbuf, fill_ref,
            xb, wt, wl, gf, gi, mt, xd, yb, sems):
    def start(src, dst, sem, priority=0):
        c = pltpu.make_async_copy(src, dst, sems.at[sem])
        c.start(priority=priority)
        return c

    def wait_all(cs):
        for c in cs:
            c.wait()

    dot = functools.partial(jnp.dot, preferred_element_type=f32)
    dot_nt = lambda a, b: lax.dot_general(a, b, (((1,), (1,)), ((), ())), preferred_element_type=f32)
    cat = lambda *vs: jnp.concatenate(vs, axis=0)
    as_bf16 = lambda w: pltpu.bitcast(w, bf16)
    hi_f32 = lambda w: pltpu.bitcast(w & u32(0xFFFF0000), f32)
    all_ones = lambda tok: ((tok >> 16) | u32(0xFFFF)) | u32(0xFFFF0000)
    after = lambda v, tok: pltpu.bitcast(pltpu.bitcast(v, u32) & all_ones(tok), f32)
    widen = lambda w: as_bf16(w).astype(f32) if w.dtype == u32 else w
    narrow = lambda w: as_bf16(w) if w.dtype == u32 else w.astype(bf16)
    add2 = lambda a, b: widen(a) + widen(b)
    sub2 = lambda a, b: widen(a) - widen(b)
    w_hbm = (wq_hbm, wk_hbm, wv_hbm)

    def start_unit(u):
        return start(w_hbm[u // 2].at[:, :, u % 2], wraw.at[u % NRAW], u % NRAW)

    def start_x(seg0, nseg, sem, priority=0):
        segs, rows = pl.ds(seg0, nseg), pl.ds(0, SEG - M)
        return start(x_hbm.at[segs, rows, :], xbuf.at[segs], sem, priority)

    def start_filter(row0, nrows, sem, priority=0):
        rows = pl.ds(row0, nrows)
        return [start(w.at[rows, pl.ds(128 * d, 128)], wt.at[t, d, rows], sem, priority)
                for t, w in enumerate((wr_hbm, wi_hbm)) for d in range(16)]

    def start_piece(n, xsem, parts):
        cols = pl.ds(256 * n, 256)
        cs = [start(x_hbm.at[:, pl.ds(SEG - M, M), cols], x8.at[:, :, cols], xsem)]
        for k, sem in enumerate(parts):
            rows = pl.ds(128 * n + 128 // len(parts) * k, 128 // len(parts))
            cs.append(start(wq_hbm.at[rows, :, 0], wraw.at[0, rows], sem))
        return cs
    c_a = [start_piece(0, 5, (6, 0))] + [start_piece(n, n, (n,)) for n in range(1, 4)]
    c_loop = [start_x(0, UNROLL, 4, 1), start(mem_hbm, mem0, 4, 1), start(fill_hbm, fill_ref.at[pl.ds(0, 80)], 4, 1)]
    c_loop += [start(wo_hbm.at[:, pl.ds(128 * j, 128)], wo.at[j], 4, 1) for j in range(8)]

    xb32 = xb.bitcast(u32)

    def relayout_row(src, dst, r, lo, hi):
        a, b = src.at[r].bitcast(u32)[...]
        dst[pl.ds(r, 8, stride=WP), :] = (a & lo) | (b << 16)
        dst[pl.ds(r + 8 * WP, 8, stride=WP), :] = (a >> 16) | (b & hi)

    def relayout_tasks(u, r0=0, r1=D // 2):
        src, dst = wraw.at[u % NRAW], wall.at[u]

        def make(r):
            def task(tok):
                lo = (tok >> 16) | u32(0xFFFF)
                hi = (tok << 16) | u32(0xFFFF0000)
                relayout_row(src, dst, r, lo, hi)
                relayout_row(src, dst, r + 1, lo, hi)
            return task
        return [make(r) for r in range(r0, r1, 2)]

    def y_blocks(r):
        return pl.ds(4 * (r % 2) + r // 2, 8, stride=8)

    def filter_tasks(blk, wfn):
        def make(phase, k):
            slots = [4 * k + j for j in range(4)] if phase == 1 else [4 * j + k for j in range(4)]

            def task(tok):
                z = [(yb[0, b, blk], yb[1, b, blk]) for b in slots]
                z[0] = tuple(after(v, tok) for v in z[0])
                if phase == 0:
                    o = _bfly4(z, 1)
                    o = [_twiddle16(o[j], k * j) for j in range(4)]
                elif phase == 1:
                    o = _bfly4(z, 1)
                    y = []
                    for j in range(4):
                        wr, wi = wfn(k + 4 * j)
                        xr, xi = o[j]
                        y.append((xr * wr - xi * wi, xr * wi + xi * wr))
                    o = _bfly4(y, -1)
                    o = [_twiddle16(o[j], -k * j) for j in range(4)]
                else:
                    o = _bfly4(z, -1)
                for b, v in zip(slots, o):
                    yb[0, b, blk] = v[0]
                    yb[1, b, blk] = v[1]
            return task
        return [make(phase, k) for phase in range(3) for k in range(4)]

    def butterfly_tasks(par):
        def make(a):
            def task(tok):
                w = [xb32[j, a // 8, a // 2 % 4, pl.ds(8 * (a % 2), 8), :] for j in range(8)]
                if par:
                    hi = (tok << 16) | u32(0xFFFF0000)
                    z = _fwd8([pltpu.bitcast(v & hi, f32) for v in w])
                else:
                    sixteen = ((tok >> 31) | u32(1)) << 4
                    z = _fwd8([pltpu.bitcast(v << sixteen, f32) for v in w])
                for n in range(8):
                    xd[n, pl.ds(8 * XP * par + a, 8, stride=XP), :] = z[n]
            return task
        return [make(a) for a in range(128)]

    sign = _dft_constants()[3]

    def b_dfwd(b, pacer):
        z = lambda n: xd[n, pl.ds(XP * (b // 2 + 8 * (b % 2)), 128), :]
        t0 = dot_nt(as_bf16(gf[0]), z(0).astype(bf16))
        t4 = dot_nt(as_bf16(gf[1, 0:64]), z(1).astype(bf16))
        tr, ti = cat(t0[0:64], t4[0:64]), cat(t0[64:128], t4[64:128])
        ts = [(cat(tr + ti, t0[128:144]).astype(bf16), ti.astype(bf16), cat(tr, t0[128:144]).astype(bf16))]
        for g in range(1, 4):
            x, y = z(2 * g), z(2 * g + 1)
            k1, k2, k3 = [dot_nt(as_bf16(gf[3 * g - 1 + n, 0:64]), v.astype(bf16))
                          for n, v in enumerate((x + y, y, x))]
            pacer.feed(k1)
            tr = k1 + k2
            ti = cat(*[k3[64 * q:64 * q + 64] + k1[64 * q:64 * q + 64] if sign[g - 1][q] > 0
                       else k3[64 * q:64 * q + 64] - k1[64 * q:64 * q + 64] for q in range(2)])
            ts.append(((tr + ti).astype(bf16), ti.astype(bf16), tr.astype(bf16)))
        return ts

    def b_sfwd(b, ts, pacer):
        for g in range(4):
            k1, k2, k3 = [dot(ts[g][n], as_bf16(mt[n, b])) for n in range(3)]
            if g:
                pacer.feed(k2)
            yr, yi = k1[0:128] - k2, k1 + k3
            for q in range(2):
                yb[0, b, y_blocks(RES[g][q])] = yr[64 * q:64 * q + 64].reshape(8, 8, 128)
                yb[1, b, y_blocks(RES[g][q])] = yi[64 * q:64 * q + 64].reshape(8, 8, 128)
            if g == 0:
                yb[0, b, 64] = k1[128:136]
                yb[1, b, 64] = yi[128:136]

    def b_stage1(tasks):
        pacer = _Pacer(tasks, NBT * 48)
        prev = None
        for b in list(range(0, 16, 2)) + list(range(1, 16, 2)):
            ts = b_dfwd(b, pacer)
            if prev is not None:
                b_sfwd(*prev, pacer)
            prev = (b, ts)
        b_sfwd(*prev, pacer)
        pacer.done()

    def b_stage3():
        row0 = lax.broadcasted_iota(jnp.int32, (8, 128), 0) == 0
        low = lax.broadcasted_iota(jnp.int32, (1, 128), 1) < 64
        for b in range(16):
            m = [as_bf16(mt[n, b]) for n in range(4)]
            for g in (1, 2, 3, 0):
                yr, yi = [cat(*[yb[c, b, y_blocks(r)].reshape(64, 128) for r in RES[g]]) for c in range(2)]
                if g == 0:
                    nr = -yr
                    u0 = cat(yr[0:64], jnp.where(row0, yb[0, b, 64], yi[0:8]), yi[8:64])
                    v0 = cat(yi[0:64], jnp.where(row0, yb[1, b, 64], nr[0:8]), nr[8:64])
                    u4, v4 = cat(yr[64:128], yi[64:128]), cat(yi[64:128], nr[64:128])
                    t1 = dot_nt(m[0], u0.astype(bf16)) + dot_nt(m[3], v0.astype(bf16))
                    t2 = dot_nt(m[0], u4.astype(bf16)) + dot_nt(m[3], v4.astype(bf16))
                else:
                    k1, k2, k3 = [dot_nt(m[n], v.astype(bf16)) for n, v in enumerate((yr + yi, yr, yi))]
                    t1, t2 = k1 + k3, k1 - k2
                xd[2 * g, pl.ds(XP * b, 128), :] = t1
                xd[2 * g + 1, pl.ds(XP * b, 128), :] = t2
        for t in range(16):
            rows = lambda j: cat(*[xd[j, pl.ds(8 * t + u, 16, stride=XP), :] for u in range(8)])
            z = [dot(rows(q).astype(bf16), as_bf16(gi[q])) for q in range(2)]
            for g in range(1, 4):
                tr, ti = rows(2 * g), rows(2 * g + 1)
                sg = jnp.where(low, float(sign[g - 1][0]), float(sign[g - 1][1]))
                k1, k2, k3 = [dot(v.astype(bf16), as_bf16(gi[3 * g - 1 + n]))
                              for n, v in enumerate((tr + sg * ti, ti, tr))]
                z += [k1 + k2, k1 + k3]
            y = _inv8(z)
            for j in range(8):
                xb[j, t] = y[j].reshape(4, SEG, 128).astype(bf16)

    HALF = NSEG * M // 2
    pre32 = pre.bitcast(u32)

    def store_pre(pair, row0, cs, mode):
        n = cs[0].shape[0] // M
        segs = pl.ds(row0 // M, n)
        if mode:
            st = jnp.concatenate([c.reshape(n, M, E) for c in cs], axis=1)
            pre32[pair, segs] = pltpu.bitcast(st.reshape(2 * M * n, E).astype(bf16), u32).reshape(n, M, E)
        else:
            for t, c in enumerate(cs):
                pre[pair, segs, pl.ds(M * t, M), :] = c.reshape(n, M, E).astype(bf16)

    def batch(u, p0, p1, tasks=(), t0=0, t1=4):
        mc = HALF // 2 if t1 - t0 <= MCT else HALF
        pacer = _Pacer(tasks, (7 * (p1 - p0) - MARGIN // (t1 - t0)) * HALF // 8)
        w = wall.at[u]
        for p in range(p0, p1):
            for r0 in range(0, HALF, mc):
                def blk(head, par):
                    return lambda: cat(*[w[pl.ds((p + 8 * head) * WP + 64 * (2 * t + par), 64), :]
                                         for t in range(t0, t1)])

                def prod(i, b):
                    lhs = jnp.concatenate([as_bf16(xs32[i, t, pl.ds(r0 // 2, mc // 2), :])
                                           for t in range(t0, t1)], axis=1)
                    r = dot(lhs, narrow(b))
                    pacer.feed(r)
                    return r

                def emit(half, *cs):
                    park = pl.ds((half * HALF + r0) // 8, mc // 8)
                    if t0 > 0:
                        cs = [c + yb[t, p, park].reshape(mc, E) for t, c in enumerate(cs)]
                    if t1 < 4:
                        for t, c in enumerate(cs):
                            yb[t, p, park] = c.reshape(mc // 8, 8, E)
                    else:
                        store_pre(8 * u + p, half * HALF + r0, cs, PM1)
                if t0 // (t1 - t0) % 2:
                    _strassen(prod, blk(1, 0), blk(0, 0), blk(1, 1), blk(0, 1), add2, sub2,
                              lambda half, c1, c0: emit(half, c0, c1))
                else:
                    _strassen(prod, blk(0, 0), blk(1, 0), blk(0, 1), blk(1, 1), add2, sub2, emit)
        pacer.done()

    QUART = HALF // 2
    xs32, xs2_32 = xs.bitcast(u32), xs2.bitcast(u32)

    def strassen2(right, left, emit, done, pacer, lag):
        def unpack(b):
            if b.dtype == u32 and len(done) >= lag:
                b = b & jnp.tile(all_ones(done[-lag]), (b.shape[0] // 8, 1))
            return widen(b)
        add = lambda a, b: unpack(a) + unpack(b)
        sub = lambda a, b: unpack(a) - unpack(b)

        def outer_prod(i, bs):
            def prod(j, b):
                r = dot(left(7 * i + j), narrow(b))
                pacer.feed(r)
                done.append(pltpu.bitcast(r[0:8], u32))
                return r
            order = (1, 0, 3, 2) if i in (1, 4, 5, 6) else (0, 1, 2, 3)
            cs = {}
            _strassen(prod, *[(lambda b=bs[k]: b) for k in order], add, sub, lambda half, *c: cs.update({half: c}))
            return _Blocks((cs[0] + cs[1])[k] for k in order)

        def outer_emit(half, *cs):
            for col in (1, 0):
                for a in range(2):
                    emit(2 * half + a, 2 * col, cs[col][2 * a], cs[col][2 * a + 1])
        outer = lambda k, c: lambda: [right(2 * k + k2, 2 * c + c2) for k2 in range(2) for c2 in range(2)]
        _strassen(outer_prod, outer(0, 0), outer(0, 1), outer(1, 0), outer(1, 1),
                  lambda x, y: [add(a, b) for a, b in zip(x, y)],
                  lambda x, y: [sub(a, b) for a, b in zip(x, y)], outer_emit)

    def batch2(u, q0, q1, done, tasks=(), lag=LAG):
        pacer = _Pacer(tasks, (49 * (q1 - q0) - 12) * QUART // 8)
        w = wall.at[u]
        for q in range(q0, q1):
            def emit(row, col, *cs):
                store_pre(8 * u + 2 * q + col // 2, row * QUART, cs, PM2)
            strassen2(lambda k, c: cat(*[w[pl.ds((2 * q + c // 2 + 8 * (c % 2)) * WP + 64 * (k + 4 * t), 64), :]
                                         for t in range(2)]),
                      lambda i: jnp.concatenate([as_bf16(xs2_32[i, t]) for t in range(2)], axis=1),
                      emit, done, pacer, lag)
        pacer.done()

    def left2_tasks():
        def make(i, t, r):
            def task(tok):
                a = _strassen_left_one(i, lambda rh, kh: _Blocks(
                    x8[32 * rh + 16 * rl + r, :, pl.ds(128 * (2 * kh + kl + 4 * t), 128)].astype(f32)
                    for rl in range(2) for kl in range(2)))
                a[0], a[3] = after(a[0], tok), after(a[3], tok)
                for j, v in enumerate(_strassen_left(*a)):
                    xs2[7 * i + j, t, pl.ds(M * r, M), :] = v.astype(bf16)
            return task
        return [make(i, t, r) for i in range(7) for t in range(2) for r in range(16)]

    def left_tasks(n):
        def make(r):
            def task(tok):
                a = [x8[NSEG // 2 * h + r, :, pl.ds(256 * n + 128 * k, 128)].astype(f32)
                     for h in range(2) for k in range(2)]
                a[0], a[3] = after(a[0], tok), after(a[3], tok)
                for i, v in enumerate(_strassen_left(*a)):
                    xs[i, n, pl.ds(M * r, M), :] = v.astype(bf16)
            return task
        return [make(r) for r in range(NSEG // 2)]

    def piece_tasks(n):
        rel, left = relayout_tasks(0, 128 * n, 128 * n + 128), left_tasks(n)
        return [t for r in range(32) for t in (rel[2 * r], left[r], rel[2 * r + 1])]

    run_now = lambda tasks: [task(jnp.zeros((8, 128), u32)) for task in tasks]

    c_a[0][0].wait()
    run_now(left_tasks(0))
    c_a[0][1].wait()
    run_now(relayout_tasks(0, 0, 64))
    c_a[0][2].wait()
    run_now(relayout_tasks(0, 64, 128))
    batch(0, 0, PS[0], (), 0, 1)
    wait_all(c_a[1])
    c_h = [start(wq_hbm.at[pl.ds(256 * n, 256), :, 1], wraw.at[1, pl.ds(256 * n, 256)], n) for n in range(2)]
    batch(0, PS[0], 8, piece_tasks(1), 0, 1)
    batch(0, 0, PS[1], (), 1, 2)
    wait_all(c_a[2])
    batch(0, PS[1], 8, piece_tasks(2), 1, 2)
    batch(0, 0, PS[2], (), 2, 3)
    wait_all(c_a[3])
    c_w2 = start_unit(2)
    batch(0, PS[2], 8, piece_tasks(3), 2, 3)
    batch(0, 0, PS[3], (), 3, 4)
    c_h[0].wait()
    batch(0, PS[3], 8, relayout_tasks(1, 0, 256), 3, 4)
    left2 = left2_tasks()
    batch(1, 0, 5, left2[:128], 0, 2)
    c_h[1].wait()
    start_unit(3)
    batch(1, 5, 8, relayout_tasks(1, 256, 512), 0, 2)
    batch(1, 0, 4, left2[128:], 2, 4)
    c_w2.wait()
    start_unit(4)
    start_unit(5)
    c_b1 = [start(bx_hbm.at[:, :, :, pl.ds(128 * j, 128)], xb.at[j], 5) for j in range(8)]
    c_b1 += [start(gf_hbm, gf.at[pl.ds(0, 11)], 5), start(mt_hbm.at[pl.ds(0, 3)], mt.at[pl.ds(0, 3)], 5)]
    c_loop += start_filter(0, 64, 4, 1)
    batch(1, 4, 8, relayout_tasks(2), 2, 4)
    batch2(2, 0, 2, [])

    def unit_body(u, c):
        slot = (u + 1) % NRAW
        pltpu.make_async_copy(wraw.at[slot], wraw.at[slot], sems.at[slot]).wait()
        done = []
        batch2(u, 2, 4, done, relayout_tasks(u + 1))
        batch2(u + 1, 0, 2, done)
        return c
    lax.fori_loop(2, 5, unit_body, 0)
    wait_all(c_b1)
    bfly = butterfly_tasks(0) + butterfly_tasks(1)
    batch(5, 6, 8, bfly[:NB0])
    batch2(5, 2, 3, [], lag=DLAG)
    b_stage1(bfly[NB0:])
    wait_all(c_loop)
    c_rest = [start_x(UNROLL, NSEG - UNROLL, 6)] + start_filter(64, 448, 6)
    c_b3 = [start(w.at[pl.ds(512, 1), :], wl.at[t], 5) for t, w in enumerate((wr_hbm, wi_hbm))]
    c_b3 += [start(gi_hbm, gi, 5), start(mt_hbm.at[3], mt.at[3], 5)]

    wo32 = wo.bitcast(u32)
    scale = E ** -0.5

    def gated(w, toks):
        if not toks:
            return w
        bits = functools.reduce(
            jnp.bitwise_or, [pltpu.bitcast(jnp.broadcast_to(t, (8, 128)), u32) for t in toks])
        return cat(w[0:8] & all_ones(bits), w[8:])

    def wqkv(i, p, second, toks=(), k0=0, k1=D):
        rows = pl.ds((p % 8 + 8 * second) * WP + k0 // 2, (k1 - k0) // 2)
        return as_bf16(gated(wall[2 * i + p // 8, rows, :], toks))

    def step(n, u, mem, held):
        s = UNROLL * n + u
        rows = cat(mem, xbuf[s].astype(f32))
        lhs = rows.astype(bf16)
        head_start = {}
        if u:
            lo, hi = rows[:, :D // 2].astype(bf16), rows[:, D // 2:].astype(bf16)
            for key in EARLY:
                head_start[key] = dot(lo, wqkv(*key, k1=D // 2))
        fill = fill_ref[pl.ds(0, 80), :]
        heads = [None] * H
        rs = []

        shift = jnp.full((8, 128), 16 - 16 * (n % 2), jnp.int32).astype(u32)
        wblk = pl.ds(pl.multiple_of(64 * (n // 2), 64), 64)
        flt = filter_tasks(
            s, lambda d: [hi_f32(wt.at[t, d, wblk].bitcast(u32)[pl.ds(u, 8, stride=4), :] << shift) for t in range(2)])
        pacer = _Pacer(flt, 48)

        def proj(i, p, toks=()):
            a, b = [
                dot(hi, wqkv(i, p, t, k0=D // 2)) + head_start[i, p, t] if (i, p, t) in head_start
                else dot(lhs, wqkv(i, p, t, toks[t * len(toks) // 2:(t + 1) * len(toks) // 2]))
                for t in range(2)]
            pacer.feed(a)
            pacer.feed(b)
            c = widen(pre32[16 * i + p, s])
            return cat(a, b, c).astype(bf16)

        def probs(q, k):
            sc = dot_nt(q, k) * scale
            sc = jnp.where(fill == 0.0, sc, fill)
            e = jnp.exp(sc - jnp.max(sc, axis=1, keepdims=True))
            l = jnp.sum(e, axis=1, keepdims=True)
            r = pl.reciprocal(l, approx=True)
            r = r * (2.0 - l * r)
            rs.append([r[8 * j:8 * j + 8] for j in range(10)])
            return (e * r).astype(bf16)

        def pv(p, pr, v):
            o = dot(pr, v)
            heads[2 * p] = cat(o[0:8], o[16:32], o[64:72])
            heads[2 * p + 1] = cat(o[32:40], o[48:64], o[72:80])
            held[u, 2 * p], held[u, 2 * p + 1] = o[8:16], o[40:48]

        def left_task(q, i):
            def task(tok):
                a = _strassen_left_one(i, lambda r, k: _Blocks(
                    held[2 * r + r2, 4 * q + 2 * k + k2] for r2 in range(2) for k2 in range(2)))
                a[0], a[3] = after(a[0], tok), after(a[3], tok)
                for j, v in enumerate(_strassen_left(*a)):
                    osum[7 * i + j, q, pl.ds(pl.multiple_of(M * n, M), M), :] = v.astype(bf16)
            return task

        pend = []
        for g in range(4):
            ps = range(4 * g, 4 * g + 4)
            qk = [(proj(0, p), proj(1, p)) for p in ps]
            vs = [proj(2, p, rs[p - 4] if g else ()) for p in ps]
            for a in pend:
                pv(*a)
            pend = [(p, probs(*qk[t]), vs[t]) for t, p in enumerate(ps)]
        pacer.done()

        def wo_part(oc, j, h0, h1, toks=()):
            return dot(oc, as_bf16(gated(wo32[j, pl.ds(64 * h0, 64 * (h1 - h0)), :], toks)))

        acc = []
        pacer = _Pacer([left_task(q, i) for q in range(8) for i in LEFT_AT[u]], 4 * (16 - LSTART) - 6)
        oc = jnp.concatenate(heads[0:24], axis=1).astype(bf16)
        for j in range(8):
            acc.append(wo_part(oc, j, 0, 24, {3: rs[12] + rs[13], 4: rs[14] + rs[15]}.get(j, ())))
            if j == 4:
                for a in pend:
                    pv(*a)
            if j >= LSTART:
                pacer.feed(acc[j])
        oc = jnp.concatenate(heads[24:32], axis=1).astype(bf16)
        nxt = []
        for j in range(8):
            r = wo_part(oc, j, 24, 32) + acc[j]
            outbuf[n, u, pl.ds(M, SEG - M), pl.ds(128 * j, 128)] = r[M:].astype(bf16)
            nxt.append(r[0:M])
            pacer.feed(r)
        pacer.done()
        return jnp.concatenate(nxt, axis=1)

    def steps(n, mem):
        pl.when(n == 1)(functools.partial(wait_all, c_rest))
        held = {}
        for u in range(UNROLL):
            mem = step(n, u, mem, held)
        return mem
    lax.fori_loop(0, NSEG // UNROLL, steps, mem0[...].astype(f32))
    tok_rows = pl.ds(M, SEG - M)
    c_out = [start(outbuf.at[:, :, tok_rows, :], out_hbm.at[:, :, tok_rows, pl.ds(0, D)], 0)]

    wait_all(c_b3)
    run_now(filter_tasks(64, lambda d: [wl[t, :, pl.ds(128 * d, 128)].astype(f32) for t in range(2)]))
    b_stage3()
    c_out += [start(xb.at[j], out_hbm.at[:, :, :, pl.ds(D + 128 * j, 128)], 0) for j in range(8)]

    osum32 = osum.bitcast(u32)
    done = []
    for cq in range(2):
        def emit(row, col, *cs):
            for t, c in enumerate(cs):
                outbuf[:, row, pl.ds(0, M), pl.ds(128 * (4 * cq + col + t), 128)] = (
                    c.reshape(NSEG // 4, M, 128).astype(bf16))
            idx = (slice(None), row, pl.ds(0, M), pl.ds(128 * (4 * cq + col), 256))
            c_out.append(start(outbuf.at[idx], out_hbm.at[idx], 0))
        strassen2(lambda k, c: cat(*[wo32[4 * cq + c, pl.ds(64 * (4 * q + k), 64), :] for q in range(8)]),
                  lambda i: jnp.concatenate([as_bf16(osum32[i, q]) for q in range(8)], axis=1),
                  emit, done, _Pacer((), 0), DLAG)
    wait_all(c_out)


@jax.jit
def pallas_concat_heads__memory_aug_recurrent_mem_tr__spectral_gfnet__prompt_kernel(
    A_x: jax.Array,
    A_mem0: jax.Array,
    A_Wq: jax.Array,
    A_Wk: jax.Array,
    A_Wv: jax.Array,
    A_Wo: jax.Array,
    A_seg_len: jax.Array,
    B_x: jax.Array,
    B_w_r: jax.Array,
    B_w_i: jax.Array,
):
    del A_seg_len
    assert A_x.shape == (1, S, D) and A_mem0.shape == (1, M, D) and B_x.shape == (1, S, D)
    assert A_Wq.shape == (D, H, E) and A_Wo.shape == (H, E, D) and B_w_r.shape == (S, D // 2 + 1)
    gf, gi, mt, _ = _dft_constants()
    fill = _attn_fill()
    hbm = pl.BlockSpec(memory_space=pltpu.HBM)
    wshape = (D // 2, 2, 2, 16, E)
    out = pl.pallas_call(
        _kernel,
        out_shape=jax.ShapeDtypeStruct((NSEG // 4, 4, SEG, 2 * D), bf16),
        in_specs=[hbm] * 13,
        out_specs=hbm,
        scratch_shapes=[
            pltpu.VMEM((NRAW, D // 2, 2, 16, E), bf16),
            pltpu.VMEM((6, 16 * WP, E), u32),
            pltpu.VMEM((8, H * E, 128), bf16),
            pltpu.VMEM((NSEG, SEG - M, D), bf16),
            pltpu.VMEM((M, D), bf16),
            pltpu.VMEM((NSEG, M, D), bf16),
            pltpu.VMEM((7, 4, 256, 128), bf16),
            pltpu.VMEM((49, 2, 128, 128), bf16),
            pltpu.VMEM((48, NSEG, 2 * M, E), bf16),
            pltpu.VMEM((49, 8, NSEG * M // 4, E), bf16),
            pltpu.VMEM((NSEG // 4, 4, SEG, D), bf16),
            pltpu.VMEM((96, 80), f32),
            pltpu.VMEM((8, NSEG // 4, 4, SEG, 128), bf16),
            pltpu.VMEM((2, 16, 512, 128), bf16),
            pltpu.VMEM((2, 1, S), bf16),
            pltpu.VMEM((12,) + gf.shape[1:], u32),
            pltpu.VMEM(gi.shape, u32),
            pltpu.VMEM(mt.shape, u32),
            pltpu.VMEM((8, 16 * XP, 128), f32),
            pltpu.VMEM((2, 16, 65, 8, 128), f32),
            pltpu.SemaphoreType.DMA((7,)),
        ],
        compiler_params=pltpu.CompilerParams(vmem_limit_bytes=120 * 1024 * 1024),
    )(A_x.reshape(NSEG, SEG, D), A_mem0.reshape(M, D),
      A_Wq.reshape(wshape), A_Wk.reshape(wshape), A_Wv.reshape(wshape),
      A_Wo.reshape(H * E, D), B_x.reshape(NSEG // 4, 4, SEG, D), B_w_r.T, B_w_i.T, gf, gi, mt, fill)
    return out.reshape(1, S, 2 * D)
```

```python
import functools

import jax
import jax.numpy as jnp
import numpy as np
from jax import lax
from jax.experimental import pallas as pl
from jax.experimental.pallas import tpu as pltpu

S, D, H, E, M, SEG = 2048, 1024, 32, 128, 8, 32
NSEG = S // SEG
WP = 516
XP = 132
NRAW = 4
UNROLL = 4
MCT = 1
LAG = 8
PM1 = 0
PS = (6, 4, 4, 4)
PM2 = 1
DLAG = 100
LSTART = 5
LEFT_AT = ((), (2,), (4,), (0, 1, 3, 5, 6))
NB0 = 128
NBT = 13
MARGIN = 4
EARLY = ((0, 0, 0), (0, 0, 1), (1, 0, 0), (1, 0, 1), (0, 1, 0), (0, 1, 1))
bf16, f32, u32 = jnp.bfloat16, jnp.float32, jnp.uint32
RES = ((0, 4), (2, 6), (1, 7), (3, 5))
RC = float(np.sqrt(0.5))


def _fwd8(x):
    s04, d04 = x[0] + x[4], x[0] - x[4]
    s26, d26 = x[2] + x[6], x[2] - x[6]
    s15, d15 = x[1] + x[5], x[1] - x[5]
    s37, d37 = x[3] + x[7], x[3] - x[7]
    t1, t2 = (d15 - d37) * RC, (d15 + d37) * RC
    e0, o0 = s04 + s26, s15 + s37
    return [e0 + o0, e0 - o0, s04 - s26, s15 - s37, d04 + t1, d26 + t2, d04 - t1, d26 - t2]


def _inv8(z):
    z0, z4, e1, o1, r1, i1, r3, i3 = z
    e0, o0 = z0 + z4, z0 - z4
    s04, s26, s15, s37 = e0 + e1, e0 - e1, o0 + o1, o0 - o1
    d04, d26 = r1 + r3, i1 + i3
    t1, t2 = (r1 - r3) * RC, (i1 - i3) * RC
    d15, d37 = t1 + t2, t2 - t1
    return [s04 + d04, s15 + d15, s26 + d26, s37 + d37, s04 - d04, s15 - d15, s26 - d26, s37 - d37]


def _twiddle16(z, k):
    re, im = z
    k = k % 16
    if k == 0:
        return z
    if k == 4:
        return (im, -re)
    if k == 12:
        return (-im, re)
    if k == 2:
        return ((re + im) * RC, (im - re) * RC)
    if k == 14:
        return ((re - im) * RC, (re + im) * RC)
    if k == 6:
        return ((im - re) * RC, (re + im) * -RC)
    if k == 10:
        return ((re + im) * -RC, (re - im) * RC)
    c, s = float(np.cos(2 * np.pi * k / 16)), float(-np.sin(2 * np.pi * k / 16))
    return (re * c - im * s, re * s + im * c)


def _bfly4(z, sign):
    (ar, ai), (br, bi), (cr, ci), (dr, di) = z
    sr, si, tr, ti = ar + cr, ai + ci, ar - cr, ai - ci
    ur, ui, vr, vi = br + dr, bi + di, br - dr, bi - di
    o0, o2 = (sr + ur, si + ui), (sr - ur, si - ui)
    p, q = (tr + vi, ti - vr), (tr - vi, ti + vr)
    return [o0, p, o2, q] if sign > 0 else [o0, q, o2, p]


class _Pacer:
    def __init__(self, tasks, ntokens):
        self.slots = {}
        for n, task in enumerate(tasks):
            self.slots.setdefault(n * ntokens // len(tasks), []).append(task)
        self.pos = 0

    def feed(self, r):
        for j in range(r.shape[0] // 8):
            for task in self.slots.pop(self.pos, []):
                task(pltpu.bitcast(r[8 * j:8 * j + 8], u32))
            self.pos += 1

    def done(self):
        assert not self.slots


def _pack_rows(m):
    b = np.asarray(m, np.float32).astype(jnp.bfloat16).view(np.uint16).astype(np.uint32)
    return b[..., 0::2, :] | (b[..., 1::2, :] << 16)


@functools.lru_cache(maxsize=None)
def _dft_constants():
    b8 = np.array(_fwd8(list(np.eye(8)))).T
    n = np.arange(D)
    fw = np.zeros((D, D))
    bw = np.zeros((D, D))
    for g in range(4):
        k = np.concatenate([8 * np.arange(64) + r for r in RES[g]])
        ang = 2 * np.pi * ((n[:, None] * k[None, :]) % D) / D
        wgt = np.where(k == 0, 1.0, 2.0) / (D * S)
        fw[:, 256 * g:256 * g + 128] = np.cos(ang)
        fw[:, 256 * g + 128:256 * g + 256] = -np.sin(ang)
        bw[256 * g:256 * g + 128] = (np.cos(ang) * wgt).T
        bw[256 * g + 128:256 * g + 256] = (-np.sin(ang) * wgt).T
    bw[128, :] = (-1.0) ** n / (D * S)
    binv = np.kron(np.linalg.inv(b8), np.eye(128))
    gall = binv @ fw
    giall = bw @ binv.T
    gf = np.zeros((11, 144, 128))
    gi = np.zeros((11, 128, 128))
    sign = []
    half = lambda m, q: np.concatenate([m[64 * q:64 * q + 64], m[128 + 64 * q:192 + 64 * q]])
    for g in range(4):
        sl = slice(256 * g, 256 * g + 256)
        f, b = gall[sl, sl].T, giall[sl, sl]
        if g == 0:
            for q in range(2):
                gf[q, :128] = half(f, q)[:, 128 * q:128 * q + 128]
                gi[q] = half(b, q)[:, 128 * q:128 * q + 128]
            gf[0, 128] = (-1.0) ** np.arange(128)
            continue
        sg = np.sign(f[:128, 0] * f[128:, 128])[:, None]
        sign.append((int(sg[0, 0]), int(sg[64, 0])))
        p, q, r = f[:128, :128], f[:128, 128:], f[128:, :128]
        gf[3 * g - 1:3 * g + 2, :128] = p, q - p, r - sg * p
        p, q, r = b[:128, :128], b[:128, 128:], b[128:, :128]
        gi[3 * g - 1:3 * g + 2] = p, r - sg * p, q - p
    a = np.arange(128)
    mt = np.zeros((4, 16, 128, 128))
    for b in range(16):
        ang = 2 * np.pi * (((16 * a[:, None] + b) * a[None, :]) % S) / S
        c, sn = np.cos(ang), -np.sin(ang)
        mt[:, b] = c, c + sn, sn - c, sn
    return _pack_rows(gf), _pack_rows(gi), _pack_rows(mt), tuple(sign)


def _attn_fill():
    head = np.concatenate([np.arange(64) // 32, np.arange(16) // 8])
    pos = np.concatenate([np.arange(64) % 32, 32 + np.arange(16) % 8])
    ok = (pos[:, None] < M) | (pos[:, None] >= pos[None, :])
    fill = np.where(ok, 0.0, -1e9)
    fill = np.where(head[:, None] == head[None, :], fill, -np.inf)
    return fill.astype(np.float32)


def _strassen(prod, b11, b12, b21, b22, add, sub, emit):
    m2 = prod(1, b11())
    m1 = prod(0, add(b11(), b22()))
    m3 = prod(2, sub(b12(), b22()))
    c22 = prod(5, add(b11(), b12())) + ((m1 - m2) + m3)
    m4 = prod(3, sub(b21(), b11()))
    emit(1, m2 + m4, c22)
    m5 = prod(4, b22())
    emit(0, prod(6, add(b21(), b22())) + ((m1 + m4) - m5), m3 + m5)


class _Blocks(list):
    def __add__(self, other):
        return _Blocks(a + b for a, b in zip(self, other))

    def __sub__(self, other):
        return _Blocks(a - b for a, b in zip(self, other))


def _strassen_left(a11, a12, a21, a22):
    return [a11 + a22, a21 + a22, a11, a22, a11 + a12, a21 - a11, a12 - a22]


def _strassen_left_one(i, blk):
    terms = ((0, 3, 1), (2, 3, 1), (0,), (3,), (0, 1, 1), (2, 0, -1), (1, 3, -1))[i]
    a = blk(*divmod(terms[0], 2))
    if len(terms) == 1:
        return a
    b = blk(*divmod(terms[1], 2))
    return a + b if terms[2] > 0 else a - b


def _kernel(x_hbm, mem_hbm, wq_hbm, wk_hbm, wv_hbm, wo_hbm, bx_hbm, wr_hbm, wi_hbm,
            gf_hbm, gi_hbm, mt_hbm, fill_hbm, out_hbm,
            wraw, wall, wo, xbuf, mem0, x8, xs, xs2, pre, osum, outbuf, fill_ref,
            xb, wt, wl, gf, gi, mt, xd, yb, sems):
    def start(src, dst, sem):
        c = pltpu.make_async_copy(src, dst, sems.at[sem])
        c.start()
        return c

    def wait_all(cs):
        for c in cs:
            c.wait()

    dot = functools.partial(jnp.dot, preferred_element_type=f32)
    dot_nt = lambda a, b: lax.dot_general(a, b, (((1,), (1,)), ((), ())), preferred_element_type=f32)
    cat = lambda *vs: jnp.concatenate(vs, axis=0)
    as_bf16 = lambda w: pltpu.bitcast(w, bf16)
    hi_f32 = lambda w: pltpu.bitcast(w & u32(0xFFFF0000), f32)
    all_ones = lambda tok: ((tok >> 16) | u32(0xFFFF)) | u32(0xFFFF0000)
    after = lambda v, tok: pltpu.bitcast(pltpu.bitcast(v, u32) & all_ones(tok), f32)
    widen = lambda w: as_bf16(w).astype(f32) if w.dtype == u32 else w
    narrow = lambda w: as_bf16(w) if w.dtype == u32 else w.astype(bf16)
    add2 = lambda a, b: widen(a) + widen(b)
    sub2 = lambda a, b: widen(a) - widen(b)
    w_hbm = (wq_hbm, wk_hbm, wv_hbm)

    def start_unit(u):
        return start(w_hbm[u // 2].at[:, :, u % 2], wraw.at[u % NRAW], u % NRAW)

    def start_x(seg0, nseg, sem):
        segs, rows = pl.ds(seg0, nseg), pl.ds(0, SEG - M)
        return start(x_hbm.at[segs, rows, :], xbuf.at[segs], sem)

    def start_filter(row0, nrows, sem):
        rows = pl.ds(row0, nrows)
        return [start(w.at[rows, pl.ds(128 * d, 128)], wt.at[t, d, rows], sem)
                for t, w in enumerate((wr_hbm, wi_hbm)) for d in range(16)]

    def start_piece(n, xsem, parts):
        cols = pl.ds(256 * n, 256)
        cs = [start(x_hbm.at[:, pl.ds(SEG - M, M), cols], x8.at[:, :, cols], xsem)]
        for k, sem in enumerate(parts):
            rows = pl.ds(128 * n + 128 // len(parts) * k, 128 // len(parts))
            cs.append(start(wq_hbm.at[rows, :, 0], wraw.at[0, rows], sem))
        return cs
    c_a = [start_piece(0, 5, (6, 0))] + [start_piece(n, n, (n,)) for n in range(1, 4)]

    xb32 = xb.bitcast(u32)

    def relayout_row(src, dst, r, lo, hi):
        a, b = src.at[r].bitcast(u32)[...]
        dst[pl.ds(r, 8, stride=WP), :] = (a & lo) | (b << 16)
        dst[pl.ds(r + 8 * WP, 8, stride=WP), :] = (a >> 16) | (b & hi)

    def relayout_tasks(u, r0=0, r1=D // 2):
        src, dst = wraw.at[u % NRAW], wall.at[u]

        def make(r):
            def task(tok):
                lo = (tok >> 16) | u32(0xFFFF)
                hi = (tok << 16) | u32(0xFFFF0000)
                relayout_row(src, dst, r, lo, hi)
                relayout_row(src, dst, r + 1, lo, hi)
            return task
        return [make(r) for r in range(r0, r1, 2)]

    def y_blocks(r):
        return pl.ds(4 * (r % 2) + r // 2, 8, stride=8)

    def filter_tasks(blk, wfn):
        def make(phase, k):
            slots = [4 * k + j for j in range(4)] if phase == 1 else [4 * j + k for j in range(4)]

            def task(tok):
                z = [(yb[0, b, blk], yb[1, b, blk]) for b in slots]
                z[0] = tuple(after(v, tok) for v in z[0])
                if phase == 0:
                    o = _bfly4(z, 1)
                    o = [_twiddle16(o[j], k * j) for j in range(4)]
                elif phase == 1:
                    o = _bfly4(z, 1)
                    y = []
                    for j in range(4):
                        wr, wi = wfn(k + 4 * j)
                        xr, xi = o[j]
                        y.append((xr * wr - xi * wi, xr * wi + xi * wr))
                    o = _bfly4(y, -1)
                    o = [_twiddle16(o[j], -k * j) for j in range(4)]
                else:
                    o = _bfly4(z, -1)
                for b, v in zip(slots, o):
                    yb[0, b, blk] = v[0]
                    yb[1, b, blk] = v[1]
            return task
        return [make(phase, k) for phase in range(3) for k in range(4)]

    def butterfly_tasks(par):
        def make(a):
            def task(tok):
                w = [xb32[j, a // 8, a // 2 % 4, pl.ds(8 * (a % 2), 8), :] for j in range(8)]
                if par:
                    hi = (tok << 16) | u32(0xFFFF0000)
                    z = _fwd8([pltpu.bitcast(v & hi, f32) for v in w])
                else:
                    sixteen = ((tok >> 31) | u32(1)) << 4
                    z = _fwd8([pltpu.bitcast(v << sixteen, f32) for v in w])
                for n in range(8):
                    xd[n, pl.ds(8 * XP * par + a, 8, stride=XP), :] = z[n]
            return task
        return [make(a) for a in range(128)]

    sign = _dft_constants()[3]

    def b_dfwd(b, pacer):
        z = lambda n: xd[n, pl.ds(XP * (b // 2 + 8 * (b % 2)), 128), :]
        t0 = dot_nt(as_bf16(gf[0]), z(0).astype(bf16))
        t4 = dot_nt(as_bf16(gf[1, 0:64]), z(1).astype(bf16))
        tr, ti = cat(t0[0:64], t4[0:64]), cat(t0[64:128], t4[64:128])
        ts = [(cat(tr + ti, t0[128:144]).astype(bf16), ti.astype(bf16), cat(tr, t0[128:144]).astype(bf16))]
        for g in range(1, 4):
            x, y = z(2 * g), z(2 * g + 1)
            k1, k2, k3 = [dot_nt(as_bf16(gf[3 * g - 1 + n, 0:64]), v.astype(bf16))
                          for n, v in enumerate((x + y, y, x))]
            pacer.feed(k1)
            tr = k1 + k2
            ti = cat(*[k3[64 * q:64 * q + 64] + k1[64 * q:64 * q + 64] if sign[g - 1][q] > 0
                       else k3[64 * q:64 * q + 64] - k1[64 * q:64 * q + 64] for q in range(2)])
            ts.append(((tr + ti).astype(bf16), ti.astype(bf16), tr.astype(bf16)))
        return ts

    def b_sfwd(b, ts, pacer):
        for g in range(4):
            k1, k2, k3 = [dot(ts[g][n], as_bf16(mt[n, b])) for n in range(3)]
            if g:
                pacer.feed(k2)
            yr, yi = k1[0:128] - k2, k1 + k3
            for q in range(2):
                yb[0, b, y_blocks(RES[g][q])] = yr[64 * q:64 * q + 64].reshape(8, 8, 128)
                yb[1, b, y_blocks(RES[g][q])] = yi[64 * q:64 * q + 64].reshape(8, 8, 128)
            if g == 0:
                yb[0, b, 64] = k1[128:136]
                yb[1, b, 64] = yi[128:136]

    def b_stage1(tasks):
        pacer = _Pacer(tasks, NBT * 48)
        prev = None
        for b in list(range(0, 16, 2)) + list(range(1, 16, 2)):
            ts = b_dfwd(b, pacer)
            if prev is not None:
                b_sfwd(*prev, pacer)
            prev = (b, ts)
        b_sfwd(*prev, pacer)
        pacer.done()

    def b_stage3():
        row0 = lax.broadcasted_iota(jnp.int32, (8, 128), 0) == 0
        low = lax.broadcasted_iota(jnp.int32, (1, 128), 1) < 64
        for b in range(16):
            m = [as_bf16(mt[n, b]) for n in range(4)]
            for g in (1, 2, 3, 0):
                yr, yi = [cat(*[yb[c, b, y_blocks(r)].reshape(64, 128) for r in RES[g]]) for c in range(2)]
                if g == 0:
                    nr = -yr
                    u0 = cat(yr[0:64], jnp.where(row0, yb[0, b, 64], yi[0:8]), yi[8:64])
                    v0 = cat(yi[0:64], jnp.where(row0, yb[1, b, 64], nr[0:8]), nr[8:64])
                    u4, v4 = cat(yr[64:128], yi[64:128]), cat(yi[64:128], nr[64:128])
                    t1 = dot_nt(m[0], u0.astype(bf16)) + dot_nt(m[3], v0.astype(bf16))
                    t2 = dot_nt(m[0], u4.astype(bf16)) + dot_nt(m[3], v4.astype(bf16))
                else:
                    k1, k2, k3 = [dot_nt(m[n], v.astype(bf16)) for n, v in enumerate((yr + yi, yr, yi))]
                    t1, t2 = k1 + k3, k1 - k2
                xd[2 * g, pl.ds(XP * b, 128), :] = t1
                xd[2 * g + 1, pl.ds(XP * b, 128), :] = t2
        for t in range(16):
            rows = lambda j: cat(*[xd[j, pl.ds(8 * t + u, 16, stride=XP), :] for u in range(8)])
            z = [dot(rows(q).astype(bf16), as_bf16(gi[q])) for q in range(2)]
            for g in range(1, 4):
                tr, ti = rows(2 * g), rows(2 * g + 1)
                sg = jnp.where(low, float(sign[g - 1][0]), float(sign[g - 1][1]))
                k1, k2, k3 = [dot(v.astype(bf16), as_bf16(gi[3 * g - 1 + n]))
                              for n, v in enumerate((tr + sg * ti, ti, tr))]
                z += [k1 + k2, k1 + k3]
            y = _inv8(z)
            for j in range(8):
                xb[j, t] = y[j].reshape(4, SEG, 128).astype(bf16)

    HALF = NSEG * M // 2
    pre32 = pre.bitcast(u32)

    def store_pre(pair, row0, cs, mode):
        n = cs[0].shape[0] // M
        segs = pl.ds(row0 // M, n)
        if mode:
            st = jnp.concatenate([c.reshape(n, M, E) for c in cs], axis=1)
            pre32[pair, segs] = pltpu.bitcast(st.reshape(2 * M * n, E).astype(bf16), u32).reshape(n, M, E)
        else:
            for t, c in enumerate(cs):
                pre[pair, segs, pl.ds(M * t, M), :] = c.reshape(n, M, E).astype(bf16)

    def batch(u, p0, p1, tasks=(), t0=0, t1=4):
        mc = HALF // 2 if t1 - t0 <= MCT else HALF
        pacer = _Pacer(tasks, (7 * (p1 - p0) - MARGIN // (t1 - t0)) * HALF // 8)
        w = wall.at[u]
        for p in range(p0, p1):
            for r0 in range(0, HALF, mc):
                def blk(head, par):
                    return lambda: cat(*[w[pl.ds((p + 8 * head) * WP + 64 * (2 * t + par), 64), :]
                                         for t in range(t0, t1)])

                def prod(i, b):
                    lhs = jnp.concatenate([as_bf16(xs32[i, t, pl.ds(r0 // 2, mc // 2), :])
                                           for t in range(t0, t1)], axis=1)
                    r = dot(lhs, narrow(b))
                    pacer.feed(r)
                    return r

                def emit(half, *cs):
                    park = pl.ds((half * HALF + r0) // 8, mc // 8)
                    if t0 > 0:
                        cs = [c + yb[t, p, park].reshape(mc, E) for t, c in enumerate(cs)]
                    if t1 < 4:
                        for t, c in enumerate(cs):
                            yb[t, p, park] = c.reshape(mc // 8, 8, E)
                    else:
                        store_pre(8 * u + p, half * HALF + r0, cs, PM1)
                if t0 // (t1 - t0) % 2:
                    _strassen(prod, blk(1, 0), blk(0, 0), blk(1, 1), blk(0, 1), add2, sub2,
                              lambda half, c1, c0: emit(half, c0, c1))
                else:
                    _strassen(prod, blk(0, 0), blk(1, 0), blk(0, 1), blk(1, 1), add2, sub2, emit)
        pacer.done()

    QUART = HALF // 2
    xs32, xs2_32 = xs.bitcast(u32), xs2.bitcast(u32)

    def strassen2(right, left, emit, done, pacer, lag):
        def unpack(b):
            if b.dtype == u32 and len(done) >= lag:
                b = b & jnp.tile(all_ones(done[-lag]), (b.shape[0] // 8, 1))
            return widen(b)
        add = lambda a, b: unpack(a) + unpack(b)
        sub = lambda a, b: unpack(a) - unpack(b)

        def outer_prod(i, bs):
            def prod(j, b):
                r = dot(left(7 * i + j), narrow(b))
                pacer.feed(r)
                done.append(pltpu.bitcast(r[0:8], u32))
                return r
            order = (1, 0, 3, 2) if i in (1, 4, 5, 6) else (0, 1, 2, 3)
            cs = {}
            _strassen(prod, *[(lambda b=bs[k]: b) for k in order], add, sub, lambda half, *c: cs.update({half: c}))
            return _Blocks((cs[0] + cs[1])[k] for k in order)

        def outer_emit(half, *cs):
            for col in (1, 0):
                for a in range(2):
                    emit(2 * half + a, 2 * col, cs[col][2 * a], cs[col][2 * a + 1])
        outer = lambda k, c: lambda: [right(2 * k + k2, 2 * c + c2) for k2 in range(2) for c2 in range(2)]
        _strassen(outer_prod, outer(0, 0), outer(0, 1), outer(1, 0), outer(1, 1),
                  lambda x, y: [add(a, b) for a, b in zip(x, y)],
                  lambda x, y: [sub(a, b) for a, b in zip(x, y)], outer_emit)

    def batch2(u, q0, q1, done, tasks=(), lag=LAG):
        pacer = _Pacer(tasks, (49 * (q1 - q0) - 12) * QUART // 8)
        w = wall.at[u]
        for q in range(q0, q1):
            def emit(row, col, *cs):
                store_pre(8 * u + 2 * q + col // 2, row * QUART, cs, PM2)
            strassen2(lambda k, c: cat(*[w[pl.ds((2 * q + c // 2 + 8 * (c % 2)) * WP + 64 * (k + 4 * t), 64), :]
                                         for t in range(2)]),
                      lambda i: jnp.concatenate([as_bf16(xs2_32[i, t]) for t in range(2)], axis=1),
                      emit, done, pacer, lag)
        pacer.done()

    def left2_tasks():
        def make(i, t, r):
            def task(tok):
                a = _strassen_left_one(i, lambda rh, kh: _Blocks(
                    x8[32 * rh + 16 * rl + r, :, pl.ds(128 * (2 * kh + kl + 4 * t), 128)].astype(f32)
                    for rl in range(2) for kl in range(2)))
                a[0], a[3] = after(a[0], tok), after(a[3], tok)
                for j, v in enumerate(_strassen_left(*a)):
                    xs2[7 * i + j, t, pl.ds(M * r, M), :] = v.astype(bf16)
            return task
        return [make(i, t, r) for i in range(7) for t in range(2) for r in range(16)]

    def left_tasks(n):
        def make(r):
            def task(tok):
                a = [x8[NSEG // 2 * h + r, :, pl.ds(256 * n + 128 * k, 128)].astype(f32)
                     for h in range(2) for k in range(2)]
                a[0], a[3] = after(a[0], tok), after(a[3], tok)
                for i, v in enumerate(_strassen_left(*a)):
                    xs[i, n, pl.ds(M * r, M), :] = v.astype(bf16)
            return task
        return [make(r) for r in range(NSEG // 2)]

    def piece_tasks(n):
        rel, left = relayout_tasks(0, 128 * n, 128 * n + 128), left_tasks(n)
        return [t for r in range(32) for t in (rel[2 * r], left[r], rel[2 * r + 1])]

    run_now = lambda tasks: [task(jnp.zeros((8, 128), u32)) for task in tasks]

    c_a[0][0].wait()
    run_now(left_tasks(0))
    c_a[0][1].wait()
    run_now(relayout_tasks(0, 0, 64))
    c_a[0][2].wait()
    run_now(relayout_tasks(0, 64, 128))
    batch(0, 0, PS[0], (), 0, 1)
    wait_all(c_a[1])
    c_h = [start(wq_hbm.at[pl.ds(256 * n, 256), :, 1], wraw.at[1, pl.ds(256 * n, 256)], n) for n in range(2)]
    batch(0, PS[0], 8, piece_tasks(1), 0, 1)
    batch(0, 0, PS[1], (), 1, 2)
    wait_all(c_a[2])
    batch(0, PS[1], 8, piece_tasks(2), 1, 2)
    batch(0, 0, PS[2], (), 2, 3)
    wait_all(c_a[3])
    c_w2 = start_unit(2)
    batch(0, PS[2], 8, piece_tasks(3), 2, 3)
    batch(0, 0, PS[3], (), 3, 4)
    c_h[0].wait()
    batch(0, PS[3], 8, relayout_tasks(1, 0, 256), 3, 4)
    left2 = left2_tasks()
    batch(1, 0, 5, left2[:128], 0, 2)
    c_h[1].wait()
    start_unit(3)
    batch(1, 5, 8, relayout_tasks(1, 256, 512), 0, 2)
    batch(1, 0, 4, left2[128:], 2, 4)
    c_w2.wait()
    start_unit(4)
    start_unit(5)
    c_b1 = [start(bx_hbm.at[:, :, :, pl.ds(128 * j, 128)], xb.at[j], 5) for j in range(8)]
    c_b1 += [start(gf_hbm, gf.at[pl.ds(0, 11)], 5), start(mt_hbm.at[pl.ds(0, 3)], mt.at[pl.ds(0, 3)], 5)]
    c_loop = [start(wo_hbm.at[:, pl.ds(128 * j, 128)], wo.at[j], 4) for j in range(8)]
    c_loop += [start_x(0, UNROLL, 4), start(mem_hbm, mem0, 4), start(fill_hbm, fill_ref.at[pl.ds(0, 80)], 4)]
    c_loop += start_filter(0, 64, 4)
    batch(1, 4, 8, relayout_tasks(2), 2, 4)
    batch2(2, 0, 2, [])

    def unit_body(u, c):
        slot = (u + 1) % NRAW
        pltpu.make_async_copy(wraw.at[slot], wraw.at[slot], sems.at[slot]).wait()
        done = []
        batch2(u, 2, 4, done, relayout_tasks(u + 1))
        batch2(u + 1, 0, 2, done)
        return c
    lax.fori_loop(2, 5, unit_body, 0)
    wait_all(c_b1)
    bfly = butterfly_tasks(0) + butterfly_tasks(1)
    batch(5, 6, 8, bfly[:NB0])
    batch2(5, 2, 3, [], lag=DLAG)
    b_stage1(bfly[NB0:])
    wait_all(c_loop)
    c_rest = [start_x(UNROLL, NSEG - UNROLL, 6)] + start_filter(64, 448, 6)
    c_b3 = [start(w.at[pl.ds(512, 1), :], wl.at[t], 5) for t, w in enumerate((wr_hbm, wi_hbm))]
    c_b3 += [start(gi_hbm, gi, 5), start(mt_hbm.at[3], mt.at[3], 5)]

    wo32 = wo.bitcast(u32)
    scale = E ** -0.5

    def gated(w, toks):
        if not toks:
            return w
        bits = functools.reduce(
            jnp.bitwise_or, [pltpu.bitcast(jnp.broadcast_to(t, (8, 128)), u32) for t in toks])
        return cat(w[0:8] & all_ones(bits), w[8:])

    def wqkv(i, p, second, toks=(), k0=0, k1=D):
        rows = pl.ds((p % 8 + 8 * second) * WP + k0 // 2, (k1 - k0) // 2)
        return as_bf16(gated(wall[2 * i + p // 8, rows, :], toks))

    def step(n, u, mem, held):
        s = UNROLL * n + u
        rows = cat(mem, xbuf[s].astype(f32))
        lhs = rows.astype(bf16)
        head_start = {}
        if u:
            lo, hi = rows[:, :D // 2].astype(bf16), rows[:, D // 2:].astype(bf16)
            for key in EARLY:
                head_start[key] = dot(lo, wqkv(*key, k1=D // 2))
        fill = fill_ref[pl.ds(0, 80), :]
        heads = [None] * H
        rs = []

        shift = jnp.full((8, 128), 16 - 16 * (n % 2), jnp.int32).astype(u32)
        wblk = pl.ds(pl.multiple_of(64 * (n // 2), 64), 64)
        flt = filter_tasks(
            s, lambda d: [hi_f32(wt.at[t, d, wblk].bitcast(u32)[pl.ds(u, 8, stride=4), :] << shift) for t in range(2)])
        pacer = _Pacer(flt, 48)

        def proj(i, p, toks=()):
            a, b = [
                dot(hi, wqkv(i, p, t, k0=D // 2)) + head_start[i, p, t] if (i, p, t) in head_start
                else dot(lhs, wqkv(i, p, t, toks[t * len(toks) // 2:(t + 1) * len(toks) // 2]))
                for t in range(2)]
            pacer.feed(a)
            pacer.feed(b)
            c = widen(pre32[16 * i + p, s])
            return cat(a, b, c).astype(bf16)

        def probs(q, k):
            sc = dot_nt(q, k) * scale
            sc = jnp.where(fill == 0.0, sc, fill)
            e = jnp.exp(sc - jnp.max(sc, axis=1, keepdims=True))
            l = jnp.sum(e, axis=1, keepdims=True)
            r = pl.reciprocal(l, approx=True)
            r = r * (2.0 - l * r)
            rs.append([r[8 * j:8 * j + 8] for j in range(10)])
            return (e * r).astype(bf16)

        def pv(p, pr, v):
            o = dot(pr, v)
            heads[2 * p] = cat(o[0:8], o[16:32], o[64:72])
            heads[2 * p + 1] = cat(o[32:40], o[48:64], o[72:80])
            held[u, 2 * p], held[u, 2 * p + 1] = o[8:16], o[40:48]

        def left_task(q, i):
            def task(tok):
                a = _strassen_left_one(i, lambda r, k: _Blocks(
                    held[2 * r + r2, 4 * q + 2 * k + k2] for r2 in range(2) for k2 in range(2)))
                a[0], a[3] = after(a[0], tok), after(a[3], tok)
                for j, v in enumerate(_strassen_left(*a)):
                    osum[7 * i + j, q, pl.ds(pl.multiple_of(M * n, M), M), :] = v.astype(bf16)
            return task

        pend = []
        for g in range(4):
            ps = range(4 * g, 4 * g + 4)
            qk = [(proj(0, p), proj(1, p)) for p in ps]
            vs = [proj(2, p, rs[p - 4] if g else ()) for p in ps]
            for a in pend:
                pv(*a)
            pend = [(p, probs(*qk[t]), vs[t]) for t, p in enumerate(ps)]
        pacer.done()

        def wo_part(oc, j, h0, h1, toks=()):
            return dot(oc, as_bf16(gated(wo32[j, pl.ds(64 * h0, 64 * (h1 - h0)), :], toks)))

        acc = []
        pacer = _Pacer([left_task(q, i) for q in range(8) for i in LEFT_AT[u]], 4 * (16 - LSTART) - 6)
        oc = jnp.concatenate(heads[0:24], axis=1).astype(bf16)
        for j in range(8):
            acc.append(wo_part(oc, j, 0, 24, {3: rs[12] + rs[13], 4: rs[14] + rs[15]}.get(j, ())))
            if j == 4:
                for a in pend:
                    pv(*a)
            if j >= LSTART:
                pacer.feed(acc[j])
        oc = jnp.concatenate(heads[24:32], axis=1).astype(bf16)
        nxt = []
        for j in range(8):
            r = wo_part(oc, j, 24, 32) + acc[j]
            outbuf[n, u, pl.ds(M, SEG - M), pl.ds(128 * j, 128)] = r[M:].astype(bf16)
            nxt.append(r[0:M])
            pacer.feed(r)
        pacer.done()
        return jnp.concatenate(nxt, axis=1)

    def steps(n, mem):
        pl.when(n == 1)(functools.partial(wait_all, c_rest))
        held = {}
        for u in range(UNROLL):
            mem = step(n, u, mem, held)
        return mem
    lax.fori_loop(0, NSEG // UNROLL, steps, mem0[...].astype(f32))
    tok_rows = pl.ds(M, SEG - M)
    c_out = [start(outbuf.at[:, :, tok_rows, :], out_hbm.at[:, :, tok_rows, pl.ds(0, D)], 0)]

    wait_all(c_b3)
    run_now(filter_tasks(64, lambda d: [wl[t, :, pl.ds(128 * d, 128)].astype(f32) for t in range(2)]))
    b_stage3()
    c_out += [start(xb.at[j], out_hbm.at[:, :, :, pl.ds(D + 128 * j, 128)], 0) for j in range(8)]

    osum32 = osum.bitcast(u32)
    done = []
    for cq in range(2):
        def emit(row, col, *cs):
            for t, c in enumerate(cs):
                outbuf[:, row, pl.ds(0, M), pl.ds(128 * (4 * cq + col + t), 128)] = (
                    c.reshape(NSEG // 4, M, 128).astype(bf16))
            idx = (slice(None), row, pl.ds(0, M), pl.ds(128 * (4 * cq + col), 256))
            c_out.append(start(outbuf.at[idx], out_hbm.at[idx], 0))
        strassen2(lambda k, c: cat(*[wo32[4 * cq + c, pl.ds(64 * (4 * q + k), 64), :] for q in range(8)]),
                  lambda i: jnp.concatenate([as_bf16(osum32[i, q]) for q in range(8)], axis=1),
                  emit, done, _Pacer((), 0), DLAG)
    wait_all(c_out)


@jax.jit
def pallas_concat_heads__memory_aug_recurrent_mem_tr__spectral_gfnet__prompt_kernel(
    A_x: jax.Array,
    A_mem0: jax.Array,
    A_Wq: jax.Array,
    A_Wk: jax.Array,
    A_Wv: jax.Array,
    A_Wo: jax.Array,
    A_seg_len: jax.Array,
    B_x: jax.Array,
    B_w_r: jax.Array,
    B_w_i: jax.Array,
):
    del A_seg_len
    assert A_x.shape == (1, S, D) and A_mem0.shape == (1, M, D) and B_x.shape == (1, S, D)
    assert A_Wq.shape == (D, H, E) and A_Wo.shape == (H, E, D) and B_w_r.shape == (S, D // 2 + 1)
    gf, gi, mt, _ = _dft_constants()
    fill = _attn_fill()
    hbm = pl.BlockSpec(memory_space=pltpu.HBM)
    wshape = (D // 2, 2, 2, 16, E)
    out = pl.pallas_call(
        _kernel,
        out_shape=jax.ShapeDtypeStruct((NSEG // 4, 4, SEG, 2 * D), bf16),
        in_specs=[hbm] * 13,
        out_specs=hbm,
        scratch_shapes=[
            pltpu.VMEM((NRAW, D // 2, 2, 16, E), bf16),
            pltpu.VMEM((6, 16 * WP, E), u32),
            pltpu.VMEM((8, H * E, 128), bf16),
            pltpu.VMEM((NSEG, SEG - M, D), bf16),
            pltpu.VMEM((M, D), bf16),
            pltpu.VMEM((NSEG, M, D), bf16),
            pltpu.VMEM((7, 4, 256, 128), bf16),
            pltpu.VMEM((49, 2, 128, 128), bf16),
            pltpu.VMEM((48, NSEG, 2 * M, E), bf16),
            pltpu.VMEM((49, 8, NSEG * M // 4, E), bf16),
            pltpu.VMEM((NSEG // 4, 4, SEG, D), bf16),
            pltpu.VMEM((96, 80), f32),
            pltpu.VMEM((8, NSEG // 4, 4, SEG, 128), bf16),
            pltpu.VMEM((2, 16, 512, 128), bf16),
            pltpu.VMEM((2, 1, S), bf16),
            pltpu.VMEM((12,) + gf.shape[1:], u32),
            pltpu.VMEM(gi.shape, u32),
            pltpu.VMEM(mt.shape, u32),
            pltpu.VMEM((8, 16 * XP, 128), f32),
            pltpu.VMEM((2, 16, 65, 8, 128), f32),
            pltpu.SemaphoreType.DMA((7,)),
        ],
        compiler_params=pltpu.CompilerParams(vmem_limit_bytes=120 * 1024 * 1024),
    )(A_x.reshape(NSEG, SEG, D), A_mem0.reshape(M, D),
      A_Wq.reshape(wshape), A_Wk.reshape(wshape), A_Wv.reshape(wshape),
      A_Wo.reshape(H * E, D), B_x.reshape(NSEG // 4, 4, SEG, D), B_w_r.T, B_w_i.T, gf, gi, mt, fill)
    return out.reshape(1, S, 2 * D)
```

```python
import functools

import jax
import jax.numpy as jnp
import numpy as np
from jax import lax
from jax.experimental import pallas as pl
from jax.experimental.pallas import tpu as pltpu

S, D, H, E, M, SEG = 2048, 1024, 32, 128, 8, 32
NSEG = S // SEG
WP = 516
XP = 132
NRAW = 4
UNROLL = 4
PS = (6, 4, 4, 4)
LAG = 8
LEFT_AT = ((), (2,), (4,), (0, 1, 3, 5, 6))
EARLY = ((0, 0, 0), (0, 0, 1), (1, 0, 0), (1, 0, 1), (0, 1, 0))
bf16, f32, u32 = jnp.bfloat16, jnp.float32, jnp.uint32
RES = ((0, 4), (2, 6), (1, 7), (3, 5))
RC = float(np.sqrt(0.5))


def _fwd8(x):
    s04, d04 = x[0] + x[4], x[0] - x[4]
    s26, d26 = x[2] + x[6], x[2] - x[6]
    s15, d15 = x[1] + x[5], x[1] - x[5]
    s37, d37 = x[3] + x[7], x[3] - x[7]
    t1, t2 = (d15 - d37) * RC, (d15 + d37) * RC
    e0, o0 = s04 + s26, s15 + s37
    return [e0 + o0, e0 - o0, s04 - s26, s15 - s37, d04 + t1, d26 + t2, d04 - t1, d26 - t2]


def _inv8(z):
    z0, z4, e1, o1, r1, i1, r3, i3 = z
    e0, o0 = z0 + z4, z0 - z4
    s04, s26, s15, s37 = e0 + e1, e0 - e1, o0 + o1, o0 - o1
    d04, d26 = r1 + r3, i1 + i3
    t1, t2 = (r1 - r3) * RC, (i1 - i3) * RC
    d15, d37 = t1 + t2, t2 - t1
    return [s04 + d04, s15 + d15, s26 + d26, s37 + d37, s04 - d04, s15 - d15, s26 - d26, s37 - d37]


def _twiddle16(z, k):
    re, im = z
    k = k % 16
    if k == 0:
        return z
    if k == 4:
        return (im, -re)
    if k == 12:
        return (-im, re)
    if k == 2:
        return ((re + im) * RC, (im - re) * RC)
    if k == 14:
        return ((re - im) * RC, (re + im) * RC)
    if k == 6:
        return ((im - re) * RC, (re + im) * -RC)
    if k == 10:
        return ((re + im) * -RC, (re - im) * RC)
    c, s = float(np.cos(2 * np.pi * k / 16)), float(-np.sin(2 * np.pi * k / 16))
    return (re * c - im * s, re * s + im * c)


def _bfly4(z, sign):
    (ar, ai), (br, bi), (cr, ci), (dr, di) = z
    sr, si, tr, ti = ar + cr, ai + ci, ar - cr, ai - ci
    ur, ui, vr, vi = br + dr, bi + di, br - dr, bi - di
    o0, o2 = (sr + ur, si + ui), (sr - ur, si - ui)
    p, q = (tr + vi, ti - vr), (tr - vi, ti + vr)
    return [o0, p, o2, q] if sign > 0 else [o0, q, o2, p]


class _Pacer:
    def __init__(self, tasks, ntokens):
        self.slots = {}
        for n, task in enumerate(tasks):
            self.slots.setdefault(n * ntokens // len(tasks), []).append(task)
        self.pos = 0

    def feed(self, r):
        for j in range(r.shape[0] // 8):
            for task in self.slots.pop(self.pos, []):
                task(pltpu.bitcast(r[8 * j:8 * j + 8], u32))
            self.pos += 1

    def done(self):
        assert not self.slots


def _pack_rows(m):
    b = np.asarray(m, np.float32).astype(jnp.bfloat16).view(np.uint16).astype(np.uint32)
    return b[..., 0::2, :] | (b[..., 1::2, :] << 16)


@functools.lru_cache(maxsize=None)
def _dft_constants():
    b8 = np.array(_fwd8(list(np.eye(8)))).T
    n = np.arange(D)
    fw = np.zeros((D, D))
    bw = np.zeros((D, D))
    for g in range(4):
        k = np.concatenate([8 * np.arange(64) + r for r in RES[g]])
        ang = 2 * np.pi * ((n[:, None] * k[None, :]) % D) / D
        wgt = np.where(k == 0, 1.0, 2.0) / (D * S)
        fw[:, 256 * g:256 * g + 128] = np.cos(ang)
        fw[:, 256 * g + 128:256 * g + 256] = -np.sin(ang)
        bw[256 * g:256 * g + 128] = (np.cos(ang) * wgt).T
        bw[256 * g + 128:256 * g + 256] = (-np.sin(ang) * wgt).T
    bw[128, :] = (-1.0) ** n / (D * S)
    binv = np.kron(np.linalg.inv(b8), np.eye(128))
    gall = binv @ fw
    giall = bw @ binv.T
    gf = np.zeros((11, 144, 128))
    gi = np.zeros((11, 128, 128))
    sign = []
    half = lambda m, q: np.concatenate([m[64 * q:64 * q + 64], m[128 + 64 * q:192 + 64 * q]])
    for g in range(4):
        sl = slice(256 * g, 256 * g + 256)
        f, b = gall[sl, sl].T, giall[sl, sl]
        if g == 0:
            for q in range(2):
                gf[q, :128] = half(f, q)[:, 128 * q:128 * q + 128]
                gi[q] = half(b, q)[:, 128 * q:128 * q + 128]
            gf[0, 128] = (-1.0) ** np.arange(128)
            continue
        sg = np.sign(f[:128, 0] * f[128:, 128])[:, None]
        sign.append((int(sg[0, 0]), int(sg[64, 0])))
        p, q, r = f[:128, :128], f[:128, 128:], f[128:, :128]
        gf[3 * g - 1:3 * g + 2, :128] = p, q - p, r - sg * p
        p, q, r = b[:128, :128], b[:128, 128:], b[128:, :128]
        gi[3 * g - 1:3 * g + 2] = p, r - sg * p, q - p
    a = np.arange(128)
    mt = np.zeros((4, 16, 128, 128))
    for b in range(16):
        ang = 2 * np.pi * (((16 * a[:, None] + b) * a[None, :]) % S) / S
        c, sn = np.cos(ang), -np.sin(ang)
        mt[:, b] = c, c + sn, sn - c, sn
    return _pack_rows(gf), _pack_rows(gi), _pack_rows(mt), tuple(sign)


def _attn_fill():
    head = np.concatenate([np.arange(64) // 32, np.arange(16) // 8])
    pos = np.concatenate([np.arange(64) % 32, 32 + np.arange(16) % 8])
    ok = (pos[:, None] < M) | (pos[:, None] >= pos[None, :])
    fill = np.where(ok, 0.0, -1e9)
    fill = np.where(head[:, None] == head[None, :], fill, -np.inf)
    return fill.astype(np.float32)


def _strassen(prod, b11, b12, b21, b22, add, sub, emit):
    m2 = prod(1, b11())
    m1 = prod(0, add(b11(), b22()))
    m3 = prod(2, sub(b12(), b22()))
    c22 = prod(5, add(b11(), b12())) + ((m1 - m2) + m3)
    m4 = prod(3, sub(b21(), b11()))
    emit(1, m2 + m4, c22)
    m5 = prod(4, b22())
    emit(0, prod(6, add(b21(), b22())) + ((m1 + m4) - m5), m3 + m5)


class _Blocks(list):
    def __add__(self, other):
        return _Blocks(a + b for a, b in zip(self, other))

    def __sub__(self, other):
        return _Blocks(a - b for a, b in zip(self, other))


def _strassen_left(a11, a12, a21, a22):
    return [a11 + a22, a21 + a22, a11, a22, a11 + a12, a21 - a11, a12 - a22]


def _strassen_left_one(i, blk):
    terms = ((0, 3, 1), (2, 3, 1), (0,), (3,), (0, 1, 1), (2, 0, -1), (1, 3, -1))[i]
    a = blk(*divmod(terms[0], 2))
    if len(terms) == 1:
        return a
    b = blk(*divmod(terms[1], 2))
    return a + b if terms[2] > 0 else a - b


def _kernel(x_hbm, mem_hbm, wq_hbm, wk_hbm, wv_hbm, wo_hbm, bx_hbm, wr_hbm, wi_hbm,
            gf_hbm, gi_hbm, mt_hbm, fill_hbm, out_hbm,
            wraw, wall, wo, xbuf, mem0, x8, xs, xs2, pre, osum, outbuf, fill_ref,
            xb, wt, wl, gf, gi, mt, xd, yb, sems):
    def start(src, dst, sem):
        c = pltpu.make_async_copy(src, dst, sems.at[sem])
        c.start()
        return c

    def wait_all(cs):
        for c in cs:
            c.wait()

    dot = functools.partial(jnp.dot, preferred_element_type=f32)
    dot_nt = lambda a, b: lax.dot_general(a, b, (((1,), (1,)), ((), ())), preferred_element_type=f32)
    cat = lambda *vs: jnp.concatenate(vs, axis=0)
    as_bf16 = lambda w: pltpu.bitcast(w, bf16)
    hi_f32 = lambda w: pltpu.bitcast(w & u32(0xFFFF0000), f32)
    all_ones = lambda tok: ((tok >> 16) | u32(0xFFFF)) | u32(0xFFFF0000)
    after = lambda v, tok: pltpu.bitcast(pltpu.bitcast(v, u32) & all_ones(tok), f32)
    widen = lambda w: as_bf16(w).astype(f32) if w.dtype == u32 else w
    narrow = lambda w: as_bf16(w) if w.dtype == u32 else w.astype(bf16)
    add2 = lambda a, b: widen(a) + widen(b)
    sub2 = lambda a, b: widen(a) - widen(b)
    w_hbm = (wq_hbm, wk_hbm, wv_hbm)

    def start_unit(u):
        return start(w_hbm[u // 2].at[:, :, u % 2], wraw.at[u % NRAW], u % NRAW)

    def start_x(seg0, nseg, sem):
        segs, rows = pl.ds(seg0, nseg), pl.ds(0, SEG - M)
        return start(x_hbm.at[segs, rows, :], xbuf.at[segs], sem)

    def start_filter(row0, nrows, sem):
        rows = pl.ds(row0, nrows)
        return [start(w.at[rows, pl.ds(128 * d, 128)], wt.at[t, d, rows], sem)
                for t, w in enumerate((wr_hbm, wi_hbm)) for d in range(16)]

    def start_piece(n, xsem, parts):
        cols = pl.ds(256 * n, 256)
        cs = [start(x_hbm.at[:, pl.ds(SEG - M, M), cols], x8.at[:, :, cols], xsem)]
        for k, sem in enumerate(parts):
            rows = pl.ds(128 * n + 128 // len(parts) * k, 128 // len(parts))
            cs.append(start(wq_hbm.at[rows, :, 0], wraw.at[0, rows], sem))
        return cs
    c_a = [start_piece(0, 5, (6, 0))] + [start_piece(n, n, (n,)) for n in range(1, 4)]

    xb32 = xb.bitcast(u32)

    def relayout_row(src, dst, r, lo, hi):
        a, b = src.at[r].bitcast(u32)[...]
        dst[pl.ds(r, 8, stride=WP), :] = (a & lo) | (b << 16)
        dst[pl.ds(r + 8 * WP, 8, stride=WP), :] = (a >> 16) | (b & hi)

    def relayout_tasks(u, r0=0, r1=D // 2):
        src, dst = wraw.at[u % NRAW], wall.at[u]

        def make(r):
            def task(tok):
                lo = (tok >> 16) | u32(0xFFFF)
                hi = (tok << 16) | u32(0xFFFF0000)
                relayout_row(src, dst, r, lo, hi)
                relayout_row(src, dst, r + 1, lo, hi)
            return task
        return [make(r) for r in range(r0, r1, 2)]

    def y_blocks(r):
        return pl.ds(4 * (r % 2) + r // 2, 8, stride=8)

    def filter_tasks(blk, wfn):
        def make(phase, k):
            slots = [4 * k + j for j in range(4)] if phase == 1 else [4 * j + k for j in range(4)]

            def task(tok):
                z = [(yb[0, b, blk], yb[1, b, blk]) for b in slots]
                z[0] = tuple(after(v, tok) for v in z[0])
                if phase == 0:
                    o = _bfly4(z, 1)
                    o = [_twiddle16(o[j], k * j) for j in range(4)]
                elif phase == 1:
                    o = _bfly4(z, 1)
                    y = []
                    for j in range(4):
                        wr, wi = wfn(k + 4 * j)
                        xr, xi = o[j]
                        y.append((xr * wr - xi * wi, xr * wi + xi * wr))
                    o = _bfly4(y, -1)
                    o = [_twiddle16(o[j], -k * j) for j in range(4)]
                else:
                    o = _bfly4(z, -1)
                for b, v in zip(slots, o):
                    yb[0, b, blk] = v[0]
                    yb[1, b, blk] = v[1]
            return task
        return [make(phase, k) for phase in range(3) for k in range(4)]

    def butterfly_tasks(par):
        def make(a):
            def task(tok):
                w = [xb32[j, a // 8, a // 2 % 4, pl.ds(8 * (a % 2), 8), :] for j in range(8)]
                if par:
                    hi = (tok << 16) | u32(0xFFFF0000)
                    z = _fwd8([pltpu.bitcast(v & hi, f32) for v in w])
                else:
                    sixteen = ((tok >> 31) | u32(1)) << 4
                    z = _fwd8([pltpu.bitcast(v << sixteen, f32) for v in w])
                for n in range(8):
                    xd[n, pl.ds(8 * XP * par + a, 8, stride=XP), :] = z[n]
            return task
        return [make(a) for a in range(128)]

    sign = _dft_constants()[3]

    def b_dfwd(b, pacer):
        z = lambda n: xd[n, pl.ds(XP * (b // 2 + 8 * (b % 2)), 128), :]
        t0 = dot_nt(as_bf16(gf[0]), z(0).astype(bf16))
        t4 = dot_nt(as_bf16(gf[1, 0:64]), z(1).astype(bf16))
        tr, ti = cat(t0[0:64], t4[0:64]), cat(t0[64:128], t4[64:128])
        ts = [(cat(tr + ti, t0[128:144]).astype(bf16), ti.astype(bf16), cat(tr, t0[128:144]).astype(bf16))]
        for g in range(1, 4):
            x, y = z(2 * g), z(2 * g + 1)
            k1, k2, k3 = [dot_nt(as_bf16(gf[3 * g - 1 + n, 0:64]), v.astype(bf16))
                          for n, v in enumerate((x + y, y, x))]
            pacer.feed(k1)
            tr = k1 + k2
            ti = cat(*[k3[64 * q:64 * q + 64] + k1[64 * q:64 * q + 64] if sign[g - 1][q] > 0
                       else k3[64 * q:64 * q + 64] - k1[64 * q:64 * q + 64] for q in range(2)])
            ts.append(((tr + ti).astype(bf16), ti.astype(bf16), tr.astype(bf16)))
        return ts

    def b_sfwd(b, ts, pacer):
        for g in range(4):
            k1, k2, k3 = [dot(ts[g][n], as_bf16(mt[n, b])) for n in range(3)]
            if g:
                pacer.feed(k2)
            yr, yi = k1[0:128] - k2, k1 + k3
            for q in range(2):
                yb[0, b, y_blocks(RES[g][q])] = yr[64 * q:64 * q + 64].reshape(8, 8, 128)
                yb[1, b, y_blocks(RES[g][q])] = yi[64 * q:64 * q + 64].reshape(8, 8, 128)
            if g == 0:
                yb[0, b, 64] = k1[128:136]
                yb[1, b, 64] = yi[128:136]

    def b_stage1():
        pacer = _Pacer(butterfly_tasks(1), 13 * 48)
        prev = None
        for b in list(range(0, 16, 2)) + list(range(1, 16, 2)):
            ts = b_dfwd(b, pacer)
            if prev is not None:
                b_sfwd(*prev, pacer)
            prev = (b, ts)
        b_sfwd(*prev, pacer)
        pacer.done()

    def b_stage3():
        row0 = lax.broadcasted_iota(jnp.int32, (8, 128), 0) == 0
        low = lax.broadcasted_iota(jnp.int32, (1, 128), 1) < 64
        for b in range(16):
            m = [as_bf16(mt[n, b]) for n in range(4)]
            for g in (1, 2, 3, 0):
                yr, yi = [cat(*[yb[c, b, y_blocks(r)].reshape(64, 128) for r in RES[g]]) for c in range(2)]
                if g == 0:
                    nr = -yr
                    u0 = cat(yr[0:64], jnp.where(row0, yb[0, b, 64], yi[0:8]), yi[8:64])
                    v0 = cat(yi[0:64], jnp.where(row0, yb[1, b, 64], nr[0:8]), nr[8:64])
                    u4, v4 = cat(yr[64:128], yi[64:128]), cat(yi[64:128], nr[64:128])
                    t1 = dot_nt(m[0], u0.astype(bf16)) + dot_nt(m[3], v0.astype(bf16))
                    t2 = dot_nt(m[0], u4.astype(bf16)) + dot_nt(m[3], v4.astype(bf16))
                else:
                    k1, k2, k3 = [dot_nt(m[n], v.astype(bf16)) for n, v in enumerate((yr + yi, yr, yi))]
                    t1, t2 = k1 + k3, k1 - k2
                xd[2 * g, pl.ds(XP * b, 128), :] = t1
                xd[2 * g + 1, pl.ds(XP * b, 128), :] = t2
        for t in range(16):
            rows = lambda j: cat(*[xd[j, pl.ds(8 * t + u, 16, stride=XP), :] for u in range(8)])
            z = [dot(rows(q).astype(bf16), as_bf16(gi[q])) for q in range(2)]
            for g in range(1, 4):
                tr, ti = rows(2 * g), rows(2 * g + 1)
                sg = jnp.where(low, float(sign[g - 1][0]), float(sign[g - 1][1]))
                k1, k2, k3 = [dot(v.astype(bf16), as_bf16(gi[3 * g - 1 + n]))
                              for n, v in enumerate((tr + sg * ti, ti, tr))]
                z += [k1 + k2, k1 + k3]
            y = _inv8(z)
            for j in range(8):
                xb[j, t] = y[j].reshape(4, SEG, 128).astype(bf16)

    HALF = NSEG * M // 2
    pre32 = pre.bitcast(u32)

    def store_pre(pair, row0, cs, packed):
        n = cs[0].shape[0] // M
        segs = pl.ds(row0 // M, n)
        if packed:
            st = jnp.concatenate([c.reshape(n, M, E) for c in cs], axis=1)
            pre32[pair, segs] = pltpu.bitcast(st.reshape(2 * M * n, E).astype(bf16), u32).reshape(n, M, E)
        else:
            for t, c in enumerate(cs):
                pre[pair, segs, pl.ds(M * t, M), :] = c.reshape(n, M, E).astype(bf16)

    def batch(u, p0, p1, tasks=(), t0=0, t1=4):
        mc = HALF // 2 if t1 - t0 == 1 else HALF
        pacer = _Pacer(tasks, (7 * (p1 - p0) - 4 // (t1 - t0)) * HALF // 8)
        w = wall.at[u]
        for p in range(p0, p1):
            for r0 in range(0, HALF, mc):
                def blk(head, par):
                    return lambda: cat(*[w[pl.ds((p + 8 * head) * WP + 64 * (2 * t + par), 64), :]
                                         for t in range(t0, t1)])

                def prod(i, b):
                    lhs = jnp.concatenate([as_bf16(xs32[i, t, pl.ds(r0 // 2, mc // 2), :])
                                           for t in range(t0, t1)], axis=1)
                    r = dot(lhs, narrow(b))
                    pacer.feed(r)
                    return r

                def emit(half, *cs):
                    park = pl.ds((half * HALF + r0) // 8, mc // 8)
                    if t0 > 0:
                        cs = [c + yb[t, p, park].reshape(mc, E) for t, c in enumerate(cs)]
                    if t1 < 4:
                        for t, c in enumerate(cs):
                            yb[t, p, park] = c.reshape(mc // 8, 8, E)
                    else:
                        store_pre(8 * u + p, half * HALF + r0, cs, False)
                if t0 // (t1 - t0) % 2:
                    _strassen(prod, blk(1, 0), blk(0, 0), blk(1, 1), blk(0, 1), add2, sub2,
                              lambda half, c1, c0: emit(half, c0, c1))
                else:
                    _strassen(prod, blk(0, 0), blk(1, 0), blk(0, 1), blk(1, 1), add2, sub2, emit)
        pacer.done()

    QUART = HALF // 2
    xs32, xs2_32 = xs.bitcast(u32), xs2.bitcast(u32)

    def strassen2(right, left, emit, done, pacer, lag):
        def unpack(b):
            if b.dtype == u32 and lag and len(done) >= lag:
                b = b & jnp.tile(all_ones(done[-lag]), (b.shape[0] // 8, 1))
            return widen(b)
        add = lambda a, b: unpack(a) + unpack(b)
        sub = lambda a, b: unpack(a) - unpack(b)

        def outer_prod(i, bs):
            def prod(j, b):
                r = dot(left(7 * i + j), narrow(b))
                pacer.feed(r)
                done.append(pltpu.bitcast(r[0:8], u32))
                return r
            order = (1, 0, 3, 2) if i in (1, 4, 5, 6) else (0, 1, 2, 3)
            cs = {}
            _strassen(prod, *[(lambda b=bs[k]: b) for k in order], add, sub, lambda half, *c: cs.update({half: c}))
            return _Blocks((cs[0] + cs[1])[k] for k in order)

        def outer_emit(half, *cs):
            for col in (1, 0):
                for a in range(2):
                    emit(2 * half + a, 2 * col, cs[col][2 * a], cs[col][2 * a + 1])
        outer = lambda k, c: lambda: [right(2 * k + k2, 2 * c + c2) for k2 in range(2) for c2 in range(2)]
        _strassen(outer_prod, outer(0, 0), outer(0, 1), outer(1, 0), outer(1, 1),
                  lambda x, y: [add(a, b) for a, b in zip(x, y)],
                  lambda x, y: [sub(a, b) for a, b in zip(x, y)], outer_emit)

    def batch2(u, q0, q1, done, tasks=(), lag=LAG):
        pacer = _Pacer(tasks, (49 * (q1 - q0) - 12) * QUART // 8)
        w = wall.at[u]
        for q in range(q0, q1):
            def emit(row, col, *cs):
                store_pre(8 * u + 2 * q + col // 2, row * QUART, cs, True)
            strassen2(lambda k, c: cat(*[w[pl.ds((2 * q + c // 2 + 8 * (c % 2)) * WP + 64 * (k + 4 * t), 64), :]
                                         for t in range(2)]),
                      lambda i: jnp.concatenate([as_bf16(xs2_32[i, t]) for t in range(2)], axis=1),
                      emit, done, pacer, lag)
        pacer.done()

    def left2_tasks():
        def make(i, t, r):
            def task(tok):
                a = _strassen_left_one(i, lambda rh, kh: _Blocks(
                    x8[32 * rh + 16 * rl + r, :, pl.ds(128 * (2 * kh + kl + 4 * t), 128)].astype(f32)
                    for rl in range(2) for kl in range(2)))
                a[0], a[3] = after(a[0], tok), after(a[3], tok)
                for j, v in enumerate(_strassen_left(*a)):
                    xs2[7 * i + j, t, pl.ds(M * r, M), :] = v.astype(bf16)
            return task
        return [make(i, t, r) for i in range(7) for t in range(2) for r in range(16)]

    def left_tasks(n):
        def make(r):
            def task(tok):
                a = [x8[NSEG // 2 * h + r, :, pl.ds(256 * n + 128 * k, 128)].astype(f32)
                     for h in range(2) for k in range(2)]
                a[0], a[3] = after(a[0], tok), after(a[3], tok)
                for i, v in enumerate(_strassen_left(*a)):
                    xs[i, n, pl.ds(M * r, M), :] = v.astype(bf16)
            return task
        return [make(r) for r in range(NSEG // 2)]

    def piece_tasks(n):
        rel, left = relayout_tasks(0, 128 * n, 128 * n + 128), left_tasks(n)
        return [t for r in range(32) for t in (rel[2 * r], left[r], rel[2 * r + 1])]

    run_now = lambda tasks: [task(jnp.zeros((8, 128), u32)) for task in tasks]

    c_a[0][0].wait()
    run_now(left_tasks(0))
    c_a[0][1].wait()
    run_now(relayout_tasks(0, 0, 64))
    c_a[0][2].wait()
    run_now(relayout_tasks(0, 64, 128))
    batch(0, 0, PS[0], (), 0, 1)
    wait_all(c_a[1])
    c_h = [start(wq_hbm.at[pl.ds(256 * n, 256), :, 1], wraw.at[1, pl.ds(256 * n, 256)], n) for n in range(2)]
    batch(0, PS[0], 8, piece_tasks(1), 0, 1)
    batch(0, 0, PS[1], (), 1, 2)
    wait_all(c_a[2])
    batch(0, PS[1], 8, piece_tasks(2), 1, 2)
    batch(0, 0, PS[2], (), 2, 3)
    wait_all(c_a[3])
    c_w2 = start_unit(2)
    batch(0, PS[2], 8, piece_tasks(3), 2, 3)
    batch(0, 0, PS[3], (), 3, 4)
    c_h[0].wait()
    batch(0, PS[3], 8, relayout_tasks(1, 0, 256), 3, 4)
    left2 = left2_tasks()
    batch(1, 0, 5, left2[:128], 0, 2)
    c_h[1].wait()
    start_unit(3)
    batch(1, 5, 8, relayout_tasks(1, 256, 512), 0, 2)
    batch(1, 0, 4, left2[128:], 2, 4)
    c_w2.wait()
    start_unit(4)
    start_unit(5)
    c_b1 = [start(bx_hbm.at[:, :, :, pl.ds(128 * j, 128)], xb.at[j], 5) for j in range(8)]
    c_b1 += [start(gf_hbm, gf.at[pl.ds(0, 11)], 5), start(mt_hbm.at[pl.ds(0, 3)], mt.at[pl.ds(0, 3)], 5)]
    c_loop = [start(wo_hbm.at[:, pl.ds(128 * j, 128)], wo.at[j], 4) for j in range(8)]
    c_loop += [start_x(0, UNROLL, 4), start(mem_hbm, mem0, 4), start(fill_hbm, fill_ref.at[pl.ds(0, 80)], 4)]
    c_loop += start_filter(0, 64, 4)
    batch(1, 4, 8, relayout_tasks(2), 2, 4)
    batch2(2, 0, 2, [])

    def unit_body(u, c):
        slot = (u + 1) % NRAW
        pltpu.make_async_copy(wraw.at[slot], wraw.at[slot], sems.at[slot]).wait()
        done = []
        batch2(u, 2, 4, done, relayout_tasks(u + 1))
        batch2(u + 1, 0, 2, done)
        return c
    lax.fori_loop(2, 5, unit_body, 0)
    wait_all(c_b1)
    batch(5, 6, 8, butterfly_tasks(0))
    batch2(5, 2, 3, [], lag=None)
    b_stage1()
    wait_all(c_loop)
    c_rest = [start_x(UNROLL, NSEG - UNROLL, 6)] + start_filter(64, 448, 6)
    c_b3 = [start(w.at[pl.ds(512, 1), :], wl.at[t], 5) for t, w in enumerate((wr_hbm, wi_hbm))]
    c_b3 += [start(gi_hbm, gi, 5), start(mt_hbm.at[3], mt.at[3], 5)]

    wo32 = wo.bitcast(u32)
    scale = E ** -0.5

    def gated(w, toks):
        if not toks:
            return w
        bits = functools.reduce(
            jnp.bitwise_or, [pltpu.bitcast(jnp.broadcast_to(t, (8, 128)), u32) for t in toks])
        return cat(w[0:8] & all_ones(bits), w[8:])

    def wqkv(i, p, second, toks=(), k0=0, k1=D):
        rows = pl.ds((p % 8 + 8 * second) * WP + k0 // 2, (k1 - k0) // 2)
        return as_bf16(gated(wall[2 * i + p // 8, rows, :], toks))

    def step(n, u, mem, held):
        s = UNROLL * n + u
        rows = cat(mem, xbuf[s].astype(f32))
        lhs = rows.astype(bf16)
        head_start = {}
        if u:
            lo, hi = rows[:, :D // 2].astype(bf16), rows[:, D // 2:].astype(bf16)
            for key in EARLY:
                head_start[key] = dot(lo, wqkv(*key, k1=D // 2))
        fill = fill_ref[pl.ds(0, 80), :]
        heads = [None] * H
        rs = []

        shift = jnp.full((8, 128), 16 - 16 * (n % 2), jnp.int32).astype(u32)
        wblk = pl.ds(pl.multiple_of(64 * (n // 2), 64), 64)
        flt = filter_tasks(
            s, lambda d: [hi_f32(wt.at[t, d, wblk].bitcast(u32)[pl.ds(u, 8, stride=4), :] << shift) for t in range(2)])
        pacer = _Pacer(flt, 48)

        def proj(i, p, toks=()):
            a, b = [
                dot(hi, wqkv(i, p, t, k0=D // 2)) + head_start[i, p, t] if (i, p, t) in head_start
                else dot(lhs, wqkv(i, p, t, toks[t * len(toks) // 2:(t + 1) * len(toks) // 2]))
                for t in range(2)]
            pacer.feed(a)
            pacer.feed(b)
            c = widen(pre32[16 * i + p, s])
            return cat(a, b, c).astype(bf16)

        def probs(q, k):
            sc = dot_nt(q, k) * scale
            sc = jnp.where(fill == 0.0, sc, fill)
            e = jnp.exp(sc - jnp.max(sc, axis=1, keepdims=True))
            l = jnp.sum(e, axis=1, keepdims=True)
            r = pl.reciprocal(l, approx=True)
            r = r * (2.0 - l * r)
            rs.append([r[8 * j:8 * j + 8] for j in range(10)])
            return (e * r).astype(bf16)

        def pv(p, pr, v):
            o = dot(pr, v)
            heads[2 * p] = cat(o[0:8], o[16:32], o[64:72])
            heads[2 * p + 1] = cat(o[32:40], o[48:64], o[72:80])
            held[u, 2 * p], held[u, 2 * p + 1] = o[8:16], o[40:48]

        def left_task(q, i):
            def task(tok):
                a = _strassen_left_one(i, lambda r, k: _Blocks(
                    held[2 * r + r2, 4 * q + 2 * k + k2] for r2 in range(2) for k2 in range(2)))
                a[0], a[3] = after(a[0], tok), after(a[3], tok)
                for j, v in enumerate(_strassen_left(*a)):
                    osum[7 * i + j, q, pl.ds(pl.multiple_of(M * n, M), M), :] = v.astype(bf16)
            return task

        pend = []
        for g in range(4):
            ps = range(4 * g, 4 * g + 4)
            qk = [(proj(0, p), proj(1, p)) for p in ps]
            vs = [proj(2, p, rs[p - 4] if g else ()) for p in ps]
            for a in pend:
                pv(*a)
            pend = [(p, probs(*qk[t]), vs[t]) for t, p in enumerate(ps)]
        pacer.done()

        def wo_part(oc, j, h0, h1, toks=()):
            return dot(oc, as_bf16(gated(wo32[j, pl.ds(64 * h0, 64 * (h1 - h0)), :], toks)))

        acc = []
        pacer = _Pacer([left_task(q, i) for q in range(8) for i in LEFT_AT[u]], 38)
        oc = jnp.concatenate(heads[0:24], axis=1).astype(bf16)
        for j in range(8):
            acc.append(wo_part(oc, j, 0, 24, {3: rs[12] + rs[13], 4: rs[14] + rs[15]}.get(j, ())))
            if j == 4:
                for a in pend:
                    pv(*a)
            if j >= 5:
                pacer.feed(acc[j])
        oc = jnp.concatenate(heads[24:32], axis=1).astype(bf16)
        nxt = []
        for j in range(8):
            r = wo_part(oc, j, 24, 32) + acc[j]
            outbuf[n, u, pl.ds(M, SEG - M), pl.ds(128 * j, 128)] = r[M:].astype(bf16)
            nxt.append(r[0:M])
            pacer.feed(r)
        pacer.done()
        return jnp.concatenate(nxt, axis=1)

    def steps(n, mem):
        pl.when(n == 1)(functools.partial(wait_all, c_rest))
        held = {}
        for u in range(UNROLL):
            mem = step(n, u, mem, held)
        return mem
    lax.fori_loop(0, NSEG // UNROLL, steps, mem0[...].astype(f32))
    tok_rows = pl.ds(M, SEG - M)
    c_out = [start(outbuf.at[:, :, tok_rows, :], out_hbm.at[:, :, tok_rows, pl.ds(0, D)], 0)]

    wait_all(c_b3)
    run_now(filter_tasks(64, lambda d: [wl[t, :, pl.ds(128 * d, 128)].astype(f32) for t in range(2)]))
    b_stage3()
    c_out += [start(xb.at[j], out_hbm.at[:, :, :, pl.ds(D + 128 * j, 128)], 0) for j in range(8)]

    osum32 = osum.bitcast(u32)
    done = []
    for cq in range(2):
        def emit(row, col, *cs):
            for t, c in enumerate(cs):
                outbuf[:, row, pl.ds(0, M), pl.ds(128 * (4 * cq + col + t), 128)] = (
                    c.reshape(NSEG // 4, M, 128).astype(bf16))
            idx = (slice(None), row, pl.ds(0, M), pl.ds(128 * (4 * cq + col), 256))
            c_out.append(start(outbuf.at[idx], out_hbm.at[idx], 0))
        strassen2(lambda k, c: cat(*[wo32[4 * cq + c, pl.ds(64 * (4 * q + k), 64), :] for q in range(8)]),
                  lambda i: jnp.concatenate([as_bf16(osum32[i, q]) for q in range(8)], axis=1),
                  emit, done, _Pacer((), 0), None)
    wait_all(c_out)


@jax.jit
def pallas_concat_heads__memory_aug_recurrent_mem_tr__spectral_gfnet__prompt_kernel(
    A_x: jax.Array,
    A_mem0: jax.Array,
    A_Wq: jax.Array,
    A_Wk: jax.Array,
    A_Wv: jax.Array,
    A_Wo: jax.Array,
    A_seg_len: jax.Array,
    B_x: jax.Array,
    B_w_r: jax.Array,
    B_w_i: jax.Array,
):
    del A_seg_len
    assert A_x.shape == (1, S, D) and A_mem0.shape == (1, M, D) and B_x.shape == (1, S, D)
    assert A_Wq.shape == (D, H, E) and A_Wo.shape == (H, E, D) and B_w_r.shape == (S, D // 2 + 1)
    gf, gi, mt, _ = _dft_constants()
    fill = _attn_fill()
    hbm = pl.BlockSpec(memory_space=pltpu.HBM)
    wshape = (D // 2, 2, 2, 16, E)
    out = pl.pallas_call(
        _kernel,
        out_shape=jax.ShapeDtypeStruct((NSEG // 4, 4, SEG, 2 * D), bf16),
        in_specs=[hbm] * 13,
        out_specs=hbm,
        scratch_shapes=[
            pltpu.VMEM((NRAW, D // 2, 2, 16, E), bf16),
            pltpu.VMEM((6, 16 * WP, E), u32),
            pltpu.VMEM((8, H * E, 128), bf16),
            pltpu.VMEM((NSEG, SEG - M, D), bf16),
            pltpu.VMEM((M, D), bf16),
            pltpu.VMEM((NSEG, M, D), bf16),
            pltpu.VMEM((7, 4, 256, 128), bf16),
            pltpu.VMEM((49, 2, 128, 128), bf16),
            pltpu.VMEM((48, NSEG, 2 * M, E), bf16),
            pltpu.VMEM((49, 8, NSEG * M // 4, E), bf16),
            pltpu.VMEM((NSEG // 4, 4, SEG, D), bf16),
            pltpu.VMEM((96, 80), f32),
            pltpu.VMEM((8, NSEG // 4, 4, SEG, 128), bf16),
            pltpu.VMEM((2, 16, 512, 128), bf16),
            pltpu.VMEM((2, 1, S), bf16),
            pltpu.VMEM((12,) + gf.shape[1:], u32),
            pltpu.VMEM(gi.shape, u32),
            pltpu.VMEM(mt.shape, u32),
            pltpu.VMEM((8, 16 * XP, 128), f32),
            pltpu.VMEM((2, 16, 65, 8, 128), f32),
            pltpu.SemaphoreType.DMA((7,)),
        ],
        compiler_params=pltpu.CompilerParams(vmem_limit_bytes=120 * 1024 * 1024),
    )(A_x.reshape(NSEG, SEG, D), A_mem0.reshape(M, D),
      A_Wq.reshape(wshape), A_Wk.reshape(wshape), A_Wv.reshape(wshape),
      A_Wo.reshape(H * E, D), B_x.reshape(NSEG // 4, 4, SEG, D), B_w_r.T, B_w_i.T, gf, gi, mt, fill)
    return out.reshape(1, S, 2 * D)
```

```python
import functools

import jax
import jax.numpy as jnp
import numpy as np
from jax import lax
from jax.experimental import pallas as pl
from jax.experimental.pallas import tpu as pltpu

S, D, H, E, M, SEG = 2048, 1024, 32, 128, 8, 32
NSEG = S // SEG
WP = 516
XP = 132
NRAW = 4
UNROLL = 4
PS = (6, 4, 4, 4)
BLAG = 4
BM = 0
BT = 29
NB1 = 52
LAG = 8
LEFT_AT = ((), (2,), (4,), (0, 1, 3, 5, 6))
EARLY = ((0, 0, 0), (0, 0, 1), (1, 0, 0), (1, 0, 1), (0, 1, 0))
bf16, f32, u32 = jnp.bfloat16, jnp.float32, jnp.uint32
RES = ((0, 4), (2, 6), (1, 7), (3, 5))
RC = float(np.sqrt(0.5))


def _fwd8(x):
    s04, d04 = x[0] + x[4], x[0] - x[4]
    s26, d26 = x[2] + x[6], x[2] - x[6]
    s15, d15 = x[1] + x[5], x[1] - x[5]
    s37, d37 = x[3] + x[7], x[3] - x[7]
    t1, t2 = (d15 - d37) * RC, (d15 + d37) * RC
    e0, o0 = s04 + s26, s15 + s37
    return [e0 + o0, e0 - o0, s04 - s26, s15 - s37, d04 + t1, d26 + t2, d04 - t1, d26 - t2]


def _inv8(z):
    z0, z4, e1, o1, r1, i1, r3, i3 = z
    e0, o0 = z0 + z4, z0 - z4
    s04, s26, s15, s37 = e0 + e1, e0 - e1, o0 + o1, o0 - o1
    d04, d26 = r1 + r3, i1 + i3
    t1, t2 = (r1 - r3) * RC, (i1 - i3) * RC
    d15, d37 = t1 + t2, t2 - t1
    return [s04 + d04, s15 + d15, s26 + d26, s37 + d37, s04 - d04, s15 - d15, s26 - d26, s37 - d37]


def _twiddle16(z, k):
    re, im = z
    k = k % 16
    if k == 0:
        return z
    if k == 4:
        return (im, -re)
    if k == 12:
        return (-im, re)
    if k == 2:
        return ((re + im) * RC, (im - re) * RC)
    if k == 14:
        return ((re - im) * RC, (re + im) * RC)
    if k == 6:
        return ((im - re) * RC, (re + im) * -RC)
    if k == 10:
        return ((re + im) * -RC, (re - im) * RC)
    c, s = float(np.cos(2 * np.pi * k / 16)), float(-np.sin(2 * np.pi * k / 16))
    return (re * c - im * s, re * s + im * c)


def _bfly4(z, sign):
    (ar, ai), (br, bi), (cr, ci), (dr, di) = z
    sr, si, tr, ti = ar + cr, ai + ci, ar - cr, ai - ci
    ur, ui, vr, vi = br + dr, bi + di, br - dr, bi - di
    o0, o2 = (sr + ur, si + ui), (sr - ur, si - ui)
    p, q = (tr + vi, ti - vr), (tr - vi, ti + vr)
    return [o0, p, o2, q] if sign > 0 else [o0, q, o2, p]


class _Pacer:
    def __init__(self, tasks, ntokens):
        self.slots = {}
        for n, task in enumerate(tasks):
            self.slots.setdefault(n * ntokens // len(tasks), []).append(task)
        self.pos = 0

    def feed(self, r):
        for j in range(r.shape[0] // 8):
            for task in self.slots.pop(self.pos, []):
                task(pltpu.bitcast(r[8 * j:8 * j + 8], u32))
            self.pos += 1

    def done(self):
        assert not self.slots


def _pack_rows(m):
    b = np.asarray(m, np.float32).astype(jnp.bfloat16).view(np.uint16).astype(np.uint32)
    return b[..., 0::2, :] | (b[..., 1::2, :] << 16)


@functools.lru_cache(maxsize=None)
def _dft_constants():
    b8 = np.array(_fwd8(list(np.eye(8)))).T
    n = np.arange(D)
    fw = np.zeros((D, D))
    bw = np.zeros((D, D))
    for g in range(4):
        k = np.concatenate([8 * np.arange(64) + r for r in RES[g]])
        ang = 2 * np.pi * ((n[:, None] * k[None, :]) % D) / D
        wgt = np.where(k == 0, 1.0, 2.0) / (D * S)
        fw[:, 256 * g:256 * g + 128] = np.cos(ang)
        fw[:, 256 * g + 128:256 * g + 256] = -np.sin(ang)
        bw[256 * g:256 * g + 128] = (np.cos(ang) * wgt).T
        bw[256 * g + 128:256 * g + 256] = (-np.sin(ang) * wgt).T
    bw[128, :] = (-1.0) ** n / (D * S)
    binv = np.kron(np.linalg.inv(b8), np.eye(128))
    gall = binv @ fw
    giall = bw @ binv.T
    gf = np.zeros((2, 160, 128))
    gi = np.zeros((11, 128, 128))
    sign = []
    half = lambda m, q: np.concatenate([m[64 * q:64 * q + 64], m[128 + 64 * q:192 + 64 * q]])
    for g in range(4):
        sl = slice(256 * g, 256 * g + 256)
        f, b = gall[sl, sl].T, giall[sl, sl]
        if g == 0:
            for q in range(2):
                gf[q, :128] = half(f, q)[:, 128 * q:128 * q + 128]
                gi[q] = half(b, q)[:, 128 * q:128 * q + 128]
            gf[0, 128] = (-1.0) ** np.arange(128)
            continue
        sg = np.sign(f[:128, 0] * f[128:, 128])[:, None]
        sign.append((int(sg[0, 0]), int(sg[64, 0])))
        p, q, r = b[:128, :128], b[:128, 128:], b[128:, :128]
        gi[3 * g - 1:3 * g + 2] = p, r - sg * p, q - p
    a = np.arange(128)
    mt = np.zeros((4, 16, 128, 128))
    for b in range(16):
        ang = 2 * np.pi * (((16 * a[:, None] + b) * a[None, :]) % S) / S
        c, sn = np.cos(ang), -np.sin(ang)
        mt[:, b] = c, c + sn, sn - c, sn
    tw = np.zeros((8, 8, 128), np.float32)
    for g in range(1, 4):
        ang = 2 * np.pi * a * (RES[g][0] - 4) / D
        tw[2 * g - 2], tw[2 * g - 1] = np.cos(ang), -np.sin(ang)
    return _pack_rows(gf), _pack_rows(gi), _pack_rows(mt), tw, tuple(sign)


def _attn_fill():
    head = np.concatenate([np.arange(64) // 32, np.arange(16) // 8])
    pos = np.concatenate([np.arange(64) % 32, 32 + np.arange(16) % 8])
    ok = (pos[:, None] < M) | (pos[:, None] >= pos[None, :])
    fill = np.where(ok, 0.0, -1e9)
    fill = np.where(head[:, None] == head[None, :], fill, -np.inf)
    return fill.astype(np.float32)


def _strassen(prod, b11, b12, b21, b22, add, sub, emit):
    m2 = prod(1, b11())
    m1 = prod(0, add(b11(), b22()))
    m3 = prod(2, sub(b12(), b22()))
    c22 = prod(5, add(b11(), b12())) + ((m1 - m2) + m3)
    m4 = prod(3, sub(b21(), b11()))
    emit(1, m2 + m4, c22)
    m5 = prod(4, b22())
    emit(0, prod(6, add(b21(), b22())) + ((m1 + m4) - m5), m3 + m5)


class _Blocks(list):
    def __add__(self, other):
        return _Blocks(a + b for a, b in zip(self, other))

    def __sub__(self, other):
        return _Blocks(a - b for a, b in zip(self, other))


def _strassen_left(a11, a12, a21, a22):
    return [a11 + a22, a21 + a22, a11, a22, a11 + a12, a21 - a11, a12 - a22]


def _strassen_left_one(i, blk):
    terms = ((0, 3, 1), (2, 3, 1), (0,), (3,), (0, 1, 1), (2, 0, -1), (1, 3, -1))[i]
    a = blk(*divmod(terms[0], 2))
    if len(terms) == 1:
        return a
    b = blk(*divmod(terms[1], 2))
    return a + b if terms[2] > 0 else a - b


def _kernel(x_hbm, mem_hbm, wq_hbm, wk_hbm, wv_hbm, wo_hbm, bx_hbm, wr_hbm, wi_hbm,
            gf_hbm, gi_hbm, mt_hbm, tw_hbm, fill_hbm, out_hbm,
            wraw, wall, wo, xbuf, mem0, x8, xs, xs2, pre, osum, outbuf, fill_ref,
            xb, wt, wl, gf, gi, mt, tw, xd, yb, sems):
    def start(src, dst, sem):
        c = pltpu.make_async_copy(src, dst, sems.at[sem])
        c.start()
        return c

    def wait_all(cs):
        for c in cs:
            c.wait()

    dot = functools.partial(jnp.dot, preferred_element_type=f32)
    dot_nt = lambda a, b: lax.dot_general(a, b, (((1,), (1,)), ((), ())), preferred_element_type=f32)
    cat = lambda *vs: jnp.concatenate(vs, axis=0)
    as_bf16 = lambda w: pltpu.bitcast(w, bf16)
    hi_f32 = lambda w: pltpu.bitcast(w & u32(0xFFFF0000), f32)
    all_ones = lambda tok: ((tok >> 16) | u32(0xFFFF)) | u32(0xFFFF0000)
    after = lambda v, tok: pltpu.bitcast(pltpu.bitcast(v, u32) & all_ones(tok), f32)
    widen = lambda w: as_bf16(w).astype(f32) if w.dtype == u32 else w
    narrow = lambda w: as_bf16(w) if w.dtype == u32 else w.astype(bf16)
    add2 = lambda a, b: widen(a) + widen(b)
    sub2 = lambda a, b: widen(a) - widen(b)
    w_hbm = (wq_hbm, wk_hbm, wv_hbm)

    def start_unit(u):
        return start(w_hbm[u // 2].at[:, :, u % 2], wraw.at[u % NRAW], u % NRAW)

    def start_x(seg0, nseg, sem):
        segs, rows = pl.ds(seg0, nseg), pl.ds(0, SEG - M)
        return start(x_hbm.at[segs, rows, :], xbuf.at[segs], sem)

    def start_filter(row0, nrows, sem):
        rows = pl.ds(row0, nrows)
        return [start(w.at[rows, pl.ds(128 * d, 128)], wt.at[t, d, rows], sem)
                for t, w in enumerate((wr_hbm, wi_hbm)) for d in range(16)]

    def start_piece(n, xsem, parts):
        cols = pl.ds(256 * n, 256)
        cs = [start(x_hbm.at[:, pl.ds(SEG - M, M), cols], x8.at[:, :, cols], xsem)]
        for k, sem in enumerate(parts):
            rows = pl.ds(128 * n + 128 // len(parts) * k, 128 // len(parts))
            cs.append(start(wq_hbm.at[rows, :, 0], wraw.at[0, rows], sem))
        return cs
    c_a = [start_piece(0, 5, (6, 0))] + [start_piece(n, n, (n,)) for n in range(1, 4)]

    sign = _dft_constants()[4]
    xb32 = xb.bitcast(u32)

    def relayout_row(src, dst, r, lo, hi):
        a, b = src.at[r].bitcast(u32)[...]
        dst[pl.ds(r, 8, stride=WP), :] = (a & lo) | (b << 16)
        dst[pl.ds(r + 8 * WP, 8, stride=WP), :] = (a >> 16) | (b & hi)

    def relayout_tasks(u, r0=0, r1=D // 2):
        src, dst = wraw.at[u % NRAW], wall.at[u]

        def make(r):
            def task(tok):
                lo = (tok >> 16) | u32(0xFFFF)
                hi = (tok << 16) | u32(0xFFFF0000)
                relayout_row(src, dst, r, lo, hi)
                relayout_row(src, dst, r + 1, lo, hi)
            return task
        return [make(r) for r in range(r0, r1, 2)]

    def y_blocks(r):
        return pl.ds(4 * (r % 2) + r // 2, 8, stride=8)

    def filter_tasks(blk, wfn):
        def make(phase, k):
            slots = [4 * k + j for j in range(4)] if phase == 1 else [4 * j + k for j in range(4)]

            def task(tok):
                z = [(yb[0, b, blk], yb[1, b, blk]) for b in slots]
                z[0] = tuple(after(v, tok) for v in z[0])
                if phase == 0:
                    o = _bfly4(z, 1)
                    o = [_twiddle16(o[j], k * j) for j in range(4)]
                elif phase == 1:
                    o = _bfly4(z, 1)
                    y = []
                    for j in range(4):
                        wr, wi = wfn(k + 4 * j)
                        xr, xi = o[j]
                        y.append((xr * wr - xi * wi, xr * wi + xi * wr))
                    o = _bfly4(y, -1)
                    o = [_twiddle16(o[j], -k * j) for j in range(4)]
                else:
                    o = _bfly4(z, -1)
                for b, v in zip(slots, o):
                    yb[0, b, blk] = v[0]
                    yb[1, b, blk] = v[1]
            return task
        return [make(phase, k) for phase in range(3) for k in range(4)]

    def butterfly_tasks(par):
        def make(a):
            def task(tok):
                w = [xb32[j, a // 8, a // 2 % 4, pl.ds(8 * (a % 2), 8), :] for j in range(8)]
                if par:
                    hi = (tok << 16) | u32(0xFFFF0000)
                    z = _fwd8([pltpu.bitcast(v & hi, f32) for v in w])
                else:
                    sixteen = ((tok >> 31) | u32(1)) << 4
                    z = _fwd8([pltpu.bitcast(v << sixteen, f32) for v in w])
                for g in range(1, 4):
                    x, y, c, sn = z[2 * g], z[2 * g + 1], tw[2 * g - 2], tw[2 * g - 1]
                    if sign[g - 1][0] > 0:
                        z[2 * g], z[2 * g + 1] = x * c - y * sn, x * sn + y * c
                    else:
                        z[2 * g], z[2 * g + 1] = x * c + y * sn, x * sn - y * c
                for n in range(8):
                    xd[n, pl.ds(8 * XP * par + a, 8, stride=XP), :] = z[n]
            return task
        return [make(a) for a in range(128)]


    def b_dfwd(b, g, pacer):
        z = lambda n: xd[n, pl.ds(XP * (b // 2 + 8 * (b % 2)), 128), :].astype(bf16)
        tu = dot_nt(as_bf16(gf[1, 0:64] if g else gf[0, 0:72]), z(2 * g))
        tv = dot_nt(as_bf16(gf[1, 0:64]), z(2 * g + 1))
        pacer.feed(tv)
        if g == 0:
            tr, ti = cat(tu[0:64], tv[0:64]), cat(tu[64:128], tv[64:128])
            return cat(tr + ti, tu[128:144]).astype(bf16), ti.astype(bf16), cat(tr, tu[128:144]).astype(bf16)
        tr = cat(tu[0:64] - tv[64:128], tu[0:64] + tv[64:128])
        ti = cat(tu[64:128] + tv[0:64], tu[64:128] - tv[0:64])
        return (tr + ti).astype(bf16), ti.astype(bf16), tr.astype(bf16)

    def b_sfwd(b, g, ts):
        k1, k2, k3 = [dot(ts[n], as_bf16(mt[n, b])) for n in range(3)]
        yr, yi = k1[0:128] - k2, k1 + k3
        for q in range(2):
            yb[0, b, y_blocks(RES[g][q])] = yr[64 * q:64 * q + 64].reshape(8, 8, 128)
            yb[1, b, y_blocks(RES[g][q])] = yi[64 * q:64 * q + 64].reshape(8, 8, 128)
        if g == 0:
            yb[0, b, 64] = k1[128:136]
            yb[1, b, 64] = yi[128:136]

    def b_stage1(tasks):
        pacer = _Pacer(tasks, BT * 16)
        pend = []
        for b in list(range(0, 16, 2)) + list(range(1, 16, 2)):
            for g in range(4):
                pend.append((b, g, b_dfwd(b, g, pacer)))
                if len(pend) > BLAG:
                    b_sfwd(*pend.pop(0))
        for item in pend:
            b_sfwd(*item)
        pacer.done()

    def b_stage3():
        row0 = lax.broadcasted_iota(jnp.int32, (8, 128), 0) == 0
        low = lax.broadcasted_iota(jnp.int32, (1, 128), 1) < 64
        for b in range(16):
            m = [as_bf16(mt[n, b]) for n in range(4)]
            for g in (1, 2, 3, 0):
                yr, yi = [cat(*[yb[c, b, y_blocks(r)].reshape(64, 128) for r in RES[g]]) for c in range(2)]
                if g == 0:
                    nr = -yr
                    u0 = cat(yr[0:64], jnp.where(row0, yb[0, b, 64], yi[0:8]), yi[8:64])
                    v0 = cat(yi[0:64], jnp.where(row0, yb[1, b, 64], nr[0:8]), nr[8:64])
                    u4, v4 = cat(yr[64:128], yi[64:128]), cat(yi[64:128], nr[64:128])
                    t1 = dot_nt(m[0], u0.astype(bf16)) + dot_nt(m[3], v0.astype(bf16))
                    t2 = dot_nt(m[0], u4.astype(bf16)) + dot_nt(m[3], v4.astype(bf16))
                else:
                    k1, k2, k3 = [dot_nt(m[n], v.astype(bf16)) for n, v in enumerate((yr + yi, yr, yi))]
                    t1, t2 = k1 + k3, k1 - k2
                xd[2 * g, pl.ds(XP * b, 128), :] = t1
                xd[2 * g + 1, pl.ds(XP * b, 128), :] = t2
        for t in range(16):
            rows = lambda j: cat(*[xd[j, pl.ds(8 * t + u, 16, stride=XP), :] for u in range(8)])
            z = [dot(rows(q).astype(bf16), as_bf16(gi[q])) for q in range(2)]
            for g in range(1, 4):
                tr, ti = rows(2 * g), rows(2 * g + 1)
                sg = jnp.where(low, float(sign[g - 1][0]), float(sign[g - 1][1]))
                k1, k2, k3 = [dot(v.astype(bf16), as_bf16(gi[3 * g - 1 + n]))
                              for n, v in enumerate((tr + sg * ti, ti, tr))]
                z += [k1 + k2, k1 + k3]
            y = _inv8(z)
            for j in range(8):
                xb[j, t] = y[j].reshape(4, SEG, 128).astype(bf16)

    HALF = NSEG * M // 2
    pre32 = pre.bitcast(u32)

    def store_pre(pair, row0, cs, packed):
        n = cs[0].shape[0] // M
        segs = pl.ds(row0 // M, n)
        if packed:
            st = jnp.concatenate([c.reshape(n, M, E) for c in cs], axis=1)
            pre32[pair, segs] = pltpu.bitcast(st.reshape(2 * M * n, E).astype(bf16), u32).reshape(n, M, E)
        else:
            for t, c in enumerate(cs):
                pre[pair, segs, pl.ds(M * t, M), :] = c.reshape(n, M, E).astype(bf16)

    def batch(u, p0, p1, tasks=(), t0=0, t1=4, margin=4):
        mc = HALF // 2 if t1 - t0 == 1 else HALF
        pacer = _Pacer(tasks, (7 * (p1 - p0) - margin // (t1 - t0)) * HALF // 8)
        w = wall.at[u]
        for p in range(p0, p1):
            for r0 in range(0, HALF, mc):
                def blk(head, par):
                    return lambda: cat(*[w[pl.ds((p + 8 * head) * WP + 64 * (2 * t + par), 64), :]
                                         for t in range(t0, t1)])

                def prod(i, b):
                    lhs = jnp.concatenate([as_bf16(xs32[i, t, pl.ds(r0 // 2, mc // 2), :])
                                           for t in range(t0, t1)], axis=1)
                    r = dot(lhs, narrow(b))
                    pacer.feed(r)
                    return r

                def emit(half, *cs):
                    park = pl.ds((half * HALF + r0) // 8, mc // 8)
                    if t0 > 0:
                        cs = [c + yb[t, p, park].reshape(mc, E) for t, c in enumerate(cs)]
                    if t1 < 4:
                        for t, c in enumerate(cs):
                            yb[t, p, park] = c.reshape(mc // 8, 8, E)
                    else:
                        store_pre(8 * u + p, half * HALF + r0, cs, False)
                if t0 // (t1 - t0) % 2:
                    _strassen(prod, blk(1, 0), blk(0, 0), blk(1, 1), blk(0, 1), add2, sub2,
                              lambda half, c1, c0: emit(half, c0, c1))
                else:
                    _strassen(prod, blk(0, 0), blk(1, 0), blk(0, 1), blk(1, 1), add2, sub2, emit)
        pacer.done()

    QUART = HALF // 2
    xs32, xs2_32 = xs.bitcast(u32), xs2.bitcast(u32)

    def strassen2(right, left, emit, done, pacer, lag):
        def unpack(b):
            if b.dtype == u32 and lag and len(done) >= lag:
                b = b & jnp.tile(all_ones(done[-lag]), (b.shape[0] // 8, 1))
            return widen(b)
        add = lambda a, b: unpack(a) + unpack(b)
        sub = lambda a, b: unpack(a) - unpack(b)

        def outer_prod(i, bs):
            def prod(j, b):
                r = dot(left(7 * i + j), narrow(b))
                pacer.feed(r)
                done.append(pltpu.bitcast(r[0:8], u32))
                return r
            order = (1, 0, 3, 2) if i in (1, 4, 5, 6) else (0, 1, 2, 3)
            cs = {}
            _strassen(prod, *[(lambda b=bs[k]: b) for k in order], add, sub, lambda half, *c: cs.update({half: c}))
            return _Blocks((cs[0] + cs[1])[k] for k in order)

        def outer_emit(half, *cs):
            for col in (1, 0):
                for a in range(2):
                    emit(2 * half + a, 2 * col, cs[col][2 * a], cs[col][2 * a + 1])
        outer = lambda k, c: lambda: [right(2 * k + k2, 2 * c + c2) for k2 in range(2) for c2 in range(2)]
        _strassen(outer_prod, outer(0, 0), outer(0, 1), outer(1, 0), outer(1, 1),
                  lambda x, y: [add(a, b) for a, b in zip(x, y)],
                  lambda x, y: [sub(a, b) for a, b in zip(x, y)], outer_emit)

    def batch2(u, q0, q1, done, tasks=(), lag=LAG):
        pacer = _Pacer(tasks, (49 * (q1 - q0) - 12) * QUART // 8)
        w = wall.at[u]
        for q in range(q0, q1):
            def emit(row, col, *cs):
                store_pre(8 * u + 2 * q + col // 2, row * QUART, cs, True)
            strassen2(lambda k, c: cat(*[w[pl.ds((2 * q + c // 2 + 8 * (c % 2)) * WP + 64 * (k + 4 * t), 64), :]
                                         for t in range(2)]),
                      lambda i: jnp.concatenate([as_bf16(xs2_32[i, t]) for t in range(2)], axis=1),
                      emit, done, pacer, lag)
        pacer.done()

    def left2_tasks():
        def make(i, t, r):
            def task(tok):
                a = _strassen_left_one(i, lambda rh, kh: _Blocks(
                    x8[32 * rh + 16 * rl + r, :, pl.ds(128 * (2 * kh + kl + 4 * t), 128)].astype(f32)
                    for rl in range(2) for kl in range(2)))
                a[0], a[3] = after(a[0], tok), after(a[3], tok)
                for j, v in enumerate(_strassen_left(*a)):
                    xs2[7 * i + j, t, pl.ds(M * r, M), :] = v.astype(bf16)
            return task
        return [make(i, t, r) for i in range(7) for t in range(2) for r in range(16)]

    def left_tasks(n):
        def make(r):
            def task(tok):
                a = [x8[NSEG // 2 * h + r, :, pl.ds(256 * n + 128 * k, 128)].astype(f32)
                     for h in range(2) for k in range(2)]
                a[0], a[3] = after(a[0], tok), after(a[3], tok)
                for i, v in enumerate(_strassen_left(*a)):
                    xs[i, n, pl.ds(M * r, M), :] = v.astype(bf16)
            return task
        return [make(r) for r in range(NSEG // 2)]

    def piece_tasks(n):
        rel, left = relayout_tasks(0, 128 * n, 128 * n + 128), left_tasks(n)
        return [t for r in range(32) for t in (rel[2 * r], left[r], rel[2 * r + 1])]

    run_now = lambda tasks: [task(jnp.zeros((8, 128), u32)) for task in tasks]

    c_a[0][0].wait()
    run_now(left_tasks(0))
    c_a[0][1].wait()
    run_now(relayout_tasks(0, 0, 64))
    c_a[0][2].wait()
    run_now(relayout_tasks(0, 64, 128))
    batch(0, 0, PS[0], (), 0, 1)
    wait_all(c_a[1])
    c_h = [start(wq_hbm.at[pl.ds(256 * n, 256), :, 1], wraw.at[1, pl.ds(256 * n, 256)], n) for n in range(2)]
    batch(0, PS[0], 8, piece_tasks(1), 0, 1)
    batch(0, 0, PS[1], (), 1, 2)
    wait_all(c_a[2])
    batch(0, PS[1], 8, piece_tasks(2), 1, 2)
    batch(0, 0, PS[2], (), 2, 3)
    wait_all(c_a[3])
    c_w2 = start_unit(2)
    batch(0, PS[2], 8, piece_tasks(3), 2, 3)
    batch(0, 0, PS[3], (), 3, 4)
    c_h[0].wait()
    batch(0, PS[3], 8, relayout_tasks(1, 0, 256), 3, 4)
    left2 = left2_tasks()
    batch(1, 0, 4, left2[:112], 0, 2)
    c_h[1].wait()
    start_unit(3)
    batch(1, 4, 7, relayout_tasks(1, 256, 512), 0, 2)
    batch(1, 0, 4, left2[112:], 2, 4)
    c_w2.wait()
    start_unit(4)
    start_unit(5)
    c_b1 = [start(bx_hbm.at[:, :, :, pl.ds(128 * j, 128)], xb.at[j], 5) for j in range(8)]
    c_b1 += [start(gf_hbm, gf, 5), start(tw_hbm, tw, 5), start(mt_hbm.at[pl.ds(0, 3)], mt.at[pl.ds(0, 3)], 5)]
    c_loop = [start(wo_hbm.at[:, pl.ds(128 * j, 128)], wo.at[j], 4) for j in range(8)]
    c_loop += [start_x(0, UNROLL, 4), start(mem_hbm, mem0, 4), start(fill_hbm, fill_ref.at[pl.ds(0, 80)], 4)]
    c_loop += start_filter(0, 64, 4)
    batch(1, 4, 7, relayout_tasks(2), 2, 4)
    batch2(2, 0, 2, [])

    def unit_body(u, c):
        slot = (u + 1) % NRAW
        pltpu.make_async_copy(wraw.at[slot], wraw.at[slot], sems.at[slot]).wait()
        done = []
        batch2(u, 2, 4, done, relayout_tasks(u + 1))
        batch2(u + 1, 0, 2, done)
        return c
    lax.fori_loop(2, 5, unit_body, 0)
    wait_all(c_b1)
    even, odd = butterfly_tasks(0), butterfly_tasks(1)
    both = [t for a in range(128) for t in ((even[a], odd[a]) if a < NB1 else (even[a],))]
    batch(1, 7, 8, both[:len(both) // 3], margin=0)
    batch(5, 6, 8, both[len(both) // 3:], margin=BM)
    batch2(5, 2, 3, [], lag=None)
    b_stage1(odd[NB1:])
    wait_all(c_loop)
    c_rest = [start_x(UNROLL, NSEG - UNROLL, 6)] + start_filter(64, 448, 6)
    c_b3 = [start(w.at[pl.ds(512, 1), :], wl.at[t], 5) for t, w in enumerate((wr_hbm, wi_hbm))]
    c_b3 += [start(gi_hbm, gi, 5), start(mt_hbm.at[3], mt.at[3], 5)]

    wo32 = wo.bitcast(u32)
    scale = E ** -0.5

    def gated(w, toks):
        if not toks:
            return w
        bits = functools.reduce(
            jnp.bitwise_or, [pltpu.bitcast(jnp.broadcast_to(t, (8, 128)), u32) for t in toks])
        return cat(w[0:8] & all_ones(bits), w[8:])

    def wqkv(i, p, second, toks=(), k0=0, k1=D):
        rows = pl.ds((p % 8 + 8 * second) * WP + k0 // 2, (k1 - k0) // 2)
        return as_bf16(gated(wall[2 * i + p // 8, rows, :], toks))

    def step(n, u, mem, held):
        s = UNROLL * n + u
        rows = cat(mem, xbuf[s].astype(f32))
        lhs = rows.astype(bf16)
        head_start = {}
        if u:
            lo, hi = rows[:, :D // 2].astype(bf16), rows[:, D // 2:].astype(bf16)
            for key in EARLY:
                head_start[key] = dot(lo, wqkv(*key, k1=D // 2))
        fill = fill_ref[pl.ds(0, 80), :]
        heads = [None] * H
        rs = []

        shift = jnp.full((8, 128), 16 - 16 * (n % 2), jnp.int32).astype(u32)
        wblk = pl.ds(pl.multiple_of(64 * (n // 2), 64), 64)
        flt = filter_tasks(
            s, lambda d: [hi_f32(wt.at[t, d, wblk].bitcast(u32)[pl.ds(u, 8, stride=4), :] << shift) for t in range(2)])
        pacer = _Pacer(flt, 48)

        def proj(i, p, toks=()):
            a, b = [
                dot(hi, wqkv(i, p, t, k0=D // 2)) + head_start[i, p, t] if (i, p, t) in head_start
                else dot(lhs, wqkv(i, p, t, toks[t * len(toks) // 2:(t + 1) * len(toks) // 2]))
                for t in range(2)]
            pacer.feed(a)
            pacer.feed(b)
            c = widen(pre32[16 * i + p, s])
            return cat(a, b, c).astype(bf16)

        def probs(q, k):
            sc = dot_nt(q, k) * scale
            sc = jnp.where(fill == 0.0, sc, fill)
            e = jnp.exp(sc - jnp.max(sc, axis=1, keepdims=True))
            l = jnp.sum(e, axis=1, keepdims=True)
            r = pl.reciprocal(l, approx=True)
            r = r * (2.0 - l * r)
            rs.append([r[8 * j:8 * j + 8] for j in range(10)])
            return (e * r).astype(bf16)

        def pv(p, pr, v):
            o = dot(pr, v)
            heads[2 * p] = cat(o[0:8], o[16:32], o[64:72])
            heads[2 * p + 1] = cat(o[32:40], o[48:64], o[72:80])
            held[u, 2 * p], held[u, 2 * p + 1] = o[8:16], o[40:48]

        def left_task(q, i):
            def task(tok):
                a = _strassen_left_one(i, lambda r, k: _Blocks(
                    held[2 * r + r2, 4 * q + 2 * k + k2] for r2 in range(2) for k2 in range(2)))
                a[0], a[3] = after(a[0], tok), after(a[3], tok)
                for j, v in enumerate(_strassen_left(*a)):
                    osum[7 * i + j, q, pl.ds(pl.multiple_of(M * n, M), M), :] = v.astype(bf16)
            return task

        pend = []
        for g in range(4):
            ps = range(4 * g, 4 * g + 4)
            qk = [(proj(0, p), proj(1, p)) for p in ps]
            vs = [proj(2, p, rs[p - 4] if g else ()) for p in ps]
            for a in pend:
                pv(*a)
            pend = [(p, probs(*qk[t]), vs[t]) for t, p in enumerate(ps)]
        pacer.done()

        def wo_part(oc, j, h0, h1, toks=()):
            return dot(oc, as_bf16(gated(wo32[j, pl.ds(64 * h0, 64 * (h1 - h0)), :], toks)))

        acc = []
        pacer = _Pacer([left_task(q, i) for q in range(8) for i in LEFT_AT[u]], 38)
        oc = jnp.concatenate(heads[0:24], axis=1).astype(bf16)
        for j in range(8):
            acc.append(wo_part(oc, j, 0, 24, {3: rs[12] + rs[13], 4: rs[14] + rs[15]}.get(j, ())))
            if j == 4:
                for a in pend:
                    pv(*a)
            if j >= 5:
                pacer.feed(acc[j])
        oc = jnp.concatenate(heads[24:32], axis=1).astype(bf16)
        nxt = []
        for j in range(8):
            r = wo_part(oc, j, 24, 32) + acc[j]
            outbuf[n, u, pl.ds(M, SEG - M), pl.ds(128 * j, 128)] = r[M:].astype(bf16)
            nxt.append(r[0:M])
            pacer.feed(r)
        pacer.done()
        return jnp.concatenate(nxt, axis=1)

    def steps(n, mem):
        pl.when(n == 1)(functools.partial(wait_all, c_rest))
        held = {}
        for u in range(UNROLL):
            mem = step(n, u, mem, held)
        return mem
    lax.fori_loop(0, NSEG // UNROLL, steps, mem0[...].astype(f32))
    tok_rows = pl.ds(M, SEG - M)
    c_out = [start(outbuf.at[:, :, tok_rows, :], out_hbm.at[:, :, tok_rows, pl.ds(0, D)], 0)]

    wait_all(c_b3)
    run_now(filter_tasks(64, lambda d: [wl[t, :, pl.ds(128 * d, 128)].astype(f32) for t in range(2)]))
    b_stage3()
    c_out += [start(xb.at[j], out_hbm.at[:, :, :, pl.ds(D + 128 * j, 128)], 0) for j in range(8)]

    osum32 = osum.bitcast(u32)
    done = []
    for cq in range(2):
        def emit(row, col, *cs):
            for t, c in enumerate(cs):
                outbuf[:, row, pl.ds(0, M), pl.ds(128 * (4 * cq + col + t), 128)] = (
                    c.reshape(NSEG // 4, M, 128).astype(bf16))
            idx = (slice(None), row, pl.ds(0, M), pl.ds(128 * (4 * cq + col), 256))
            c_out.append(start(outbuf.at[idx], out_hbm.at[idx], 0))
        strassen2(lambda k, c: cat(*[wo32[4 * cq + c, pl.ds(64 * (4 * q + k), 64), :] for q in range(8)]),
                  lambda i: jnp.concatenate([as_bf16(osum32[i, q]) for q in range(8)], axis=1),
                  emit, done, _Pacer((), 0), None)
    wait_all(c_out)


@jax.jit
def pallas_concat_heads__memory_aug_recurrent_mem_tr__spectral_gfnet__prompt_kernel(
    A_x: jax.Array,
    A_mem0: jax.Array,
    A_Wq: jax.Array,
    A_Wk: jax.Array,
    A_Wv: jax.Array,
    A_Wo: jax.Array,
    A_seg_len: jax.Array,
    B_x: jax.Array,
    B_w_r: jax.Array,
    B_w_i: jax.Array,
):
    del A_seg_len
    assert A_x.shape == (1, S, D) and A_mem0.shape == (1, M, D) and B_x.shape == (1, S, D)
    assert A_Wq.shape == (D, H, E) and A_Wo.shape == (H, E, D) and B_w_r.shape == (S, D // 2 + 1)
    gf, gi, mt, tw, _ = _dft_constants()
    fill = _attn_fill()
    hbm = pl.BlockSpec(memory_space=pltpu.HBM)
    wshape = (D // 2, 2, 2, 16, E)
    out = pl.pallas_call(
        _kernel,
        out_shape=jax.ShapeDtypeStruct((NSEG // 4, 4, SEG, 2 * D), bf16),
        in_specs=[hbm] * 14,
        out_specs=hbm,
        scratch_shapes=[
            pltpu.VMEM((NRAW, D // 2, 2, 16, E), bf16),
            pltpu.VMEM((6, 16 * WP, E), u32),
            pltpu.VMEM((8, H * E, 128), bf16),
            pltpu.VMEM((NSEG, SEG - M, D), bf16),
            pltpu.VMEM((M, D), bf16),
            pltpu.VMEM((NSEG, M, D), bf16),
            pltpu.VMEM((7, 4, 256, 128), bf16),
            pltpu.VMEM((49, 2, 128, 128), bf16),
            pltpu.VMEM((48, NSEG, 2 * M, E), bf16),
            pltpu.VMEM((49, 8, NSEG * M // 4, E), bf16),
            pltpu.VMEM((NSEG // 4, 4, SEG, D), bf16),
            pltpu.VMEM((96, 80), f32),
            pltpu.VMEM((8, NSEG // 4, 4, SEG, 128), bf16),
            pltpu.VMEM((2, 16, 512, 128), bf16),
            pltpu.VMEM((2, 1, S), bf16),
            pltpu.VMEM(gf.shape, u32),
            pltpu.VMEM(gi.shape, u32),
            pltpu.VMEM(mt.shape, u32),
            pltpu.VMEM(tw.shape, f32),
            pltpu.VMEM((8, 16 * XP, 128), f32),
            pltpu.VMEM((2, 16, 65, 8, 128), f32),
            pltpu.SemaphoreType.DMA((7,)),
        ],
        compiler_params=pltpu.CompilerParams(vmem_limit_bytes=120 * 1024 * 1024),
    )(A_x.reshape(NSEG, SEG, D), A_mem0.reshape(M, D),
      A_Wq.reshape(wshape), A_Wk.reshape(wshape), A_Wv.reshape(wshape),
      A_Wo.reshape(H * E, D), B_x.reshape(NSEG // 4, 4, SEG, D), B_w_r.T, B_w_i.T, gf, gi, mt, tw, fill)
    return out.reshape(1, S, 2 * D)
```

```python
import functools

import jax
import jax.numpy as jnp
import numpy as np
from jax import lax
from jax.experimental import pallas as pl
from jax.experimental.pallas import tpu as pltpu

S, D, H, E, M, SEG = 2048, 1024, 32, 128, 8, 32
NSEG = S // SEG
WP = 516
XP = 132
NRAW = 4
UNROLL = 4
PS = (6, 4, 4, 4)
LAG = 8
LEFT_AT = ((), (2,), (4,), (0, 1, 3, 5, 6))
EARLY = ((0, 0, 0), (0, 0, 1), (1, 0, 0), (1, 0, 1), (0, 1, 0))
bf16, f32, u32 = jnp.bfloat16, jnp.float32, jnp.uint32
RES = ((0, 4), (2, 6), (1, 7), (3, 5))
RC = float(np.sqrt(0.5))


def _fwd8(x):
    s04, d04 = x[0] + x[4], x[0] - x[4]
    s26, d26 = x[2] + x[6], x[2] - x[6]
    s15, d15 = x[1] + x[5], x[1] - x[5]
    s37, d37 = x[3] + x[7], x[3] - x[7]
    t1, t2 = (d15 - d37) * RC, (d15 + d37) * RC
    e0, o0 = s04 + s26, s15 + s37
    return [e0 + o0, e0 - o0, s04 - s26, s15 - s37, d04 + t1, d26 + t2, d04 - t1, d26 - t2]


def _inv8(z):
    z0, z4, e1, o1, r1, i1, r3, i3 = z
    e0, o0 = z0 + z4, z0 - z4
    s04, s26, s15, s37 = e0 + e1, e0 - e1, o0 + o1, o0 - o1
    d04, d26 = r1 + r3, i1 + i3
    t1, t2 = (r1 - r3) * RC, (i1 - i3) * RC
    d15, d37 = t1 + t2, t2 - t1
    return [s04 + d04, s15 + d15, s26 + d26, s37 + d37, s04 - d04, s15 - d15, s26 - d26, s37 - d37]


def _twiddle16(z, k):
    re, im = z
    k = k % 16
    if k == 0:
        return z
    if k == 4:
        return (im, -re)
    if k == 12:
        return (-im, re)
    if k == 2:
        return ((re + im) * RC, (im - re) * RC)
    if k == 14:
        return ((re - im) * RC, (re + im) * RC)
    if k == 6:
        return ((im - re) * RC, (re + im) * -RC)
    if k == 10:
        return ((re + im) * -RC, (re - im) * RC)
    c, s = float(np.cos(2 * np.pi * k / 16)), float(-np.sin(2 * np.pi * k / 16))
    return (re * c - im * s, re * s + im * c)


def _bfly4(z, sign):
    (ar, ai), (br, bi), (cr, ci), (dr, di) = z
    sr, si, tr, ti = ar + cr, ai + ci, ar - cr, ai - ci
    ur, ui, vr, vi = br + dr, bi + di, br - dr, bi - di
    o0, o2 = (sr + ur, si + ui), (sr - ur, si - ui)
    p, q = (tr + vi, ti - vr), (tr - vi, ti + vr)
    return [o0, p, o2, q] if sign > 0 else [o0, q, o2, p]


class _Pacer:
    def __init__(self, tasks, ntokens):
        self.slots = {}
        for n, task in enumerate(tasks):
            self.slots.setdefault(n * ntokens // len(tasks), []).append(task)
        self.pos = 0

    def feed(self, r):
        for j in range(r.shape[0] // 8):
            for task in self.slots.pop(self.pos, []):
                task(pltpu.bitcast(r[8 * j:8 * j + 8], u32))
            self.pos += 1

    def done(self):
        assert not self.slots


def _pack_rows(m):
    b = np.asarray(m, np.float32).astype(jnp.bfloat16).view(np.uint16).astype(np.uint32)
    return b[..., 0::2, :] | (b[..., 1::2, :] << 16)


@functools.lru_cache(maxsize=None)
def _dft_constants():
    b8 = np.array(_fwd8(list(np.eye(8)))).T
    n = np.arange(D)
    fw = np.zeros((D, D))
    bw = np.zeros((D, D))
    for g in range(4):
        k = np.concatenate([8 * np.arange(64) + r for r in RES[g]])
        ang = 2 * np.pi * ((n[:, None] * k[None, :]) % D) / D
        wgt = np.where(k == 0, 1.0, 2.0) / (D * S)
        fw[:, 256 * g:256 * g + 128] = np.cos(ang)
        fw[:, 256 * g + 128:256 * g + 256] = -np.sin(ang)
        bw[256 * g:256 * g + 128] = (np.cos(ang) * wgt).T
        bw[256 * g + 128:256 * g + 256] = (-np.sin(ang) * wgt).T
    bw[128, :] = (-1.0) ** n / (D * S)
    binv = np.kron(np.linalg.inv(b8), np.eye(128))
    gall = binv @ fw
    giall = bw @ binv.T
    gf = np.zeros((3, 192, 128))
    gi = np.zeros((11, 128, 128))
    sign = []
    half = lambda m, q: np.concatenate([m[64 * q:64 * q + 64], m[128 + 64 * q:192 + 64 * q]])
    for g in range(4):
        sl = slice(256 * g, 256 * g + 256)
        f, b = gall[sl, sl].T, giall[sl, sl]
        if g == 0:
            for q in range(2):
                gf[q, :128] = half(f, q)[:, 128 * q:128 * q + 128]
                gi[q] = half(b, q)[:, 128 * q:128 * q + 128]
            gf[0, 128] = (-1.0) ** np.arange(128)
            continue
        sg = np.sign(f[:128, 0] * f[128:, 128])[:, None]
        sign.append((int(sg[0, 0]), int(sg[64, 0])))
        p, q, r = b[:128, :128], b[:128, 128:], b[128:, :128]
        gi[3 * g - 1:3 * g + 2] = p, r - sg * p, q - p
    gf[2, :64], gf[2, 64:128] = gf[1, :64], -gf[1, 64:128]
    a = np.arange(128)
    angs = [2 * np.pi * a * (b - 8) / S for b in range(16)] + [2 * np.pi * a * (RES[g][0] - 4) / D for g in range(4)]
    tw = np.zeros((20, 2, 8, 128), np.float32)
    for i, ang in enumerate(angs):
        tw[i, 0], tw[i, 1] = np.cos(ang), -np.sin(ang)
    return _pack_rows(gf), _pack_rows(gi), tw, tuple(sign)


def _attn_fill():
    head = np.concatenate([np.arange(64) // 32, np.arange(16) // 8])
    pos = np.concatenate([np.arange(64) % 32, 32 + np.arange(16) % 8])
    ok = (pos[:, None] < M) | (pos[:, None] >= pos[None, :])
    fill = np.where(ok, 0.0, -1e9)
    fill = np.where(head[:, None] == head[None, :], fill, -np.inf)
    return fill.astype(np.float32)


def _strassen(prod, b11, b12, b21, b22, add, sub, emit):
    m2 = prod(1, b11())
    m1 = prod(0, add(b11(), b22()))
    m3 = prod(2, sub(b12(), b22()))
    c22 = prod(5, add(b11(), b12())) + ((m1 - m2) + m3)
    m4 = prod(3, sub(b21(), b11()))
    emit(1, m2 + m4, c22)
    m5 = prod(4, b22())
    emit(0, prod(6, add(b21(), b22())) + ((m1 + m4) - m5), m3 + m5)


class _Blocks(list):
    def __add__(self, other):
        return _Blocks(a + b for a, b in zip(self, other))

    def __sub__(self, other):
        return _Blocks(a - b for a, b in zip(self, other))


def _strassen_left(a11, a12, a21, a22):
    return [a11 + a22, a21 + a22, a11, a22, a11 + a12, a21 - a11, a12 - a22]


def _strassen_left_one(i, blk):
    terms = ((0, 3, 1), (2, 3, 1), (0,), (3,), (0, 1, 1), (2, 0, -1), (1, 3, -1))[i]
    a = blk(*divmod(terms[0], 2))
    if len(terms) == 1:
        return a
    b = blk(*divmod(terms[1], 2))
    return a + b if terms[2] > 0 else a - b


def _kernel(x_hbm, mem_hbm, wq_hbm, wk_hbm, wv_hbm, wo_hbm, bx_hbm, wr_hbm, wi_hbm,
            gf_hbm, gi_hbm, tw_hbm, fill_hbm, out_hbm,
            wraw, wall, wo, xbuf, mem0, x8, xs, xs2, pre, osum, outbuf, fill_ref,
            xb, wt, wl, gf, gi, tw, xd, yb, sems):
    def start(src, dst, sem):
        c = pltpu.make_async_copy(src, dst, sems.at[sem])
        c.start()
        return c

    def wait_all(cs):
        for c in cs:
            c.wait()

    dot = functools.partial(jnp.dot, preferred_element_type=f32)
    dot_nt = lambda a, b: lax.dot_general(a, b, (((1,), (1,)), ((), ())), preferred_element_type=f32)
    cat = lambda *vs: jnp.concatenate(vs, axis=0)
    as_bf16 = lambda w: pltpu.bitcast(w, bf16)
    hi_f32 = lambda w: pltpu.bitcast(w & u32(0xFFFF0000), f32)
    all_ones = lambda tok: ((tok >> 16) | u32(0xFFFF)) | u32(0xFFFF0000)
    after = lambda v, tok: pltpu.bitcast(pltpu.bitcast(v, u32) & all_ones(tok), f32)
    widen = lambda w: as_bf16(w).astype(f32) if w.dtype == u32 else w
    narrow = lambda w: as_bf16(w) if w.dtype == u32 else w.astype(bf16)
    add2 = lambda a, b: widen(a) + widen(b)
    sub2 = lambda a, b: widen(a) - widen(b)
    w_hbm = (wq_hbm, wk_hbm, wv_hbm)

    def start_unit(u):
        return start(w_hbm[u // 2].at[:, :, u % 2], wraw.at[u % NRAW], u % NRAW)

    def start_x(seg0, nseg, sem):
        segs, rows = pl.ds(seg0, nseg), pl.ds(0, SEG - M)
        return start(x_hbm.at[segs, rows, :], xbuf.at[segs], sem)

    def start_filter(row0, nrows, sem):
        rows = pl.ds(row0, nrows)
        return [start(w.at[rows, pl.ds(128 * d, 128)], wt.at[t, d, rows], sem)
                for t, w in enumerate((wr_hbm, wi_hbm)) for d in range(16)]

    def start_piece(n, xsem, parts):
        cols = pl.ds(256 * n, 256)
        cs = [start(x_hbm.at[:, pl.ds(SEG - M, M), cols], x8.at[:, :, cols], xsem)]
        for k, sem in enumerate(parts):
            rows = pl.ds(128 * n + 128 // len(parts) * k, 128 // len(parts))
            cs.append(start(wq_hbm.at[rows, :, 0], wraw.at[0, rows], sem))
        return cs
    c_a = [start_piece(0, 5, (6, 0))] + [start_piece(n, n, (n,)) for n in range(1, 4)]

    sign = _dft_constants()[3]
    xb32 = xb.bitcast(u32)

    def relayout_row(src, dst, r, lo, hi):
        a, b = src.at[r].bitcast(u32)[...]
        dst[pl.ds(r, 8, stride=WP), :] = (a & lo) | (b << 16)
        dst[pl.ds(r + 8 * WP, 8, stride=WP), :] = (a >> 16) | (b & hi)

    def relayout_tasks(u, r0=0, r1=D // 2):
        src, dst = wraw.at[u % NRAW], wall.at[u]

        def make(r):
            def task(tok):
                lo = (tok >> 16) | u32(0xFFFF)
                hi = (tok << 16) | u32(0xFFFF0000)
                relayout_row(src, dst, r, lo, hi)
                relayout_row(src, dst, r + 1, lo, hi)
            return task
        return [make(r) for r in range(r0, r1, 2)]

    def y_blocks(r):
        return pl.ds(4 * (r % 2) + r // 2, 8, stride=8)

    def filter_tasks(blk, wfn):
        def make(phase, k):
            slots = [4 * k + j for j in range(4)] if phase == 1 else [4 * j + k for j in range(4)]

            def task(tok):
                z = [(yb[0, b, blk], yb[1, b, blk]) for b in slots]
                if phase == 0:
                    z = [(after(zr, tok), zi) for zr, zi in z]
                    z = [(zr * tw[b, 0] - zi * tw[b, 1], zr * tw[b, 1] + zi * tw[b, 0]) if b != 8 else (zr, zi)
                         for b, (zr, zi) in zip(slots, z)]
                else:
                    z[0] = tuple(after(v, tok) for v in z[0])
                if phase == 0:
                    o = _bfly4(z, 1)
                    o = [_twiddle16(o[j], k * j) for j in range(4)]
                elif phase == 1:
                    o = _bfly4(z, 1)
                    y = []
                    for j in range(4):
                        wr, wi = wfn(k + 4 * j)
                        xr, xi = o[j]
                        y.append((xr * wr - xi * wi, xr * wi + xi * wr))
                    o = _bfly4(y, -1)
                    o = [_twiddle16(o[j], -k * j) for j in range(4)]
                else:
                    o = [(zr * tw[b, 0] + zi * tw[b, 1], zi * tw[b, 0] - zr * tw[b, 1]) if b != 8 else (zr, zi)
                         for b, (zr, zi) in zip(slots, _bfly4(z, -1))]
                for b, v in zip(slots, o):
                    yb[0, b, blk] = v[0]
                    yb[1, b, blk] = v[1]
            return task
        return [make(phase, k) for phase in range(3) for k in range(4)]

    mirror = lambda a: a if a < 64 else 191 - a

    def twiddle_d(g, x, y):
        c, sn = [jnp.tile(tw[16 + g, k], (x.shape[0] // 8, 1)) for k in range(2)]
        return (x * c - y * sn, x * sn + y * c) if sign[g - 1][0] > 0 else (x * c + y * sn, x * sn - y * c)

    def butterfly_tasks():
        def make(a, par):
            def task(tok):
                w = [xb32[j, a // 8, a // 2 % 4, pl.ds(8 * (a % 2), 8), :] for j in range(8)]
                if par:
                    hi = (tok << 16) | u32(0xFFFF0000)
                    z = _fwd8([pltpu.bitcast(v & hi, f32) for v in w])
                else:
                    sixteen = ((tok >> 31) | u32(1)) << 4
                    z = _fwd8([pltpu.bitcast(v << sixteen, f32) for v in w])
                for n in range(8):
                    xd[n, pl.ds(8 * XP * par + mirror(a), 8, stride=XP), :] = z[n]
            return task
        return [make(a, par) for a in range(128) for par in range(2)]

    low = lax.broadcasted_iota(jnp.int32, (1, 128), 1) < 64

    def b_dfwd(b, g):
        z = [xd[n, pl.ds(XP * (b // 2 + 8 * (b % 2)), 128), :] for n in (2 * g, 2 * g + 1)]
        if g:
            z = twiddle_d(g, *z)
        z = [cat(v[0:64] + v[64:128], v[0:64] - v[64:128]).astype(bf16) for v in z]
        tu = dot_nt(as_bf16(gf[1, 0:64] if g else gf[0, 0:72]), z[0])
        tv = dot_nt(as_bf16(gf[1, 0:64]), z[1])
        if g == 0:
            tr = cat(tu[0:64], tv[0:64], tu[128:144])
            ti = cat(tu[64:128], tv[64:128], jnp.zeros((16, 128), f32))
        else:
            tr = cat(tu[0:64] - tv[64:128], tu[0:64] + tv[64:128])
            ti = cat(tu[64:128] + tv[0:64], tu[64:128] - tv[0:64])
        return jnp.where(low, tr, ti).astype(bf16), jnp.where(low, ti, tr).astype(bf16)

    def b_sfwd(b, g, ts):
        for c in range(2):
            y = dot(ts[c], as_bf16(gf[2 - c, 0:64]))
            for q in range(2):
                yb[c, b, y_blocks(RES[g][q])] = y[64 * q:64 * q + 64].reshape(8, 8, 128)
            if g == 0:
                yb[c, b, 64] = y[128:136]

    def b_stage1():
        pend = []
        for b in list(range(0, 16, 2)) + list(range(1, 16, 2)):
            for g in range(4):
                pend.append((b, g, b_dfwd(b, g)))
                if len(pend) > 3:
                    b_sfwd(*pend.pop(0))
        for item in pend:
            b_sfwd(*item)

    def b_stage3():
        row0 = lax.broadcasted_iota(jnp.int32, (8, 128), 0) == 0
        for b in range(16):
            for g in (1, 2, 3, 0):
                yr, yi = [cat(*[yb[c, b, y_blocks(r)].reshape(64, 128) for r in RES[g]]) for c in range(2)]
                if g == 0:
                    nr = -yr
                    u0 = cat(yr[0:64], jnp.where(row0, yb[0, b, 64], yi[0:8]), yi[8:64])
                    v0 = cat(yi[0:64], jnp.where(row0, yb[1, b, 64], nr[0:8]), nr[8:64])
                    u4, v4 = cat(yr[64:128], yi[64:128]), cat(yi[64:128], nr[64:128])
                    cu0, cu4 = [dot_nt(as_bf16(gf[2, 0:32]), v.astype(bf16)) for v in (u0, u4)]
                    sv0, sv4 = [dot_nt(as_bf16(gf[2, 32:64]), v.astype(bf16)) for v in (v0, v4)]
                    t1, t2 = cat(cu0 - sv0, cu0 + sv0), cat(cu4 - sv4, cu4 + sv4)
                else:
                    tu, tv = [dot_nt(as_bf16(gf[2, 0:64]), v.astype(bf16)) for v in (yr, yi)]
                    t1 = cat(tu[0:64] - tv[64:128], tu[0:64] + tv[64:128])
                    t2 = cat(tv[0:64] + tu[64:128], tv[0:64] - tu[64:128])
                xd[2 * g, pl.ds(XP * b, 128), :] = t1
                xd[2 * g + 1, pl.ds(XP * b, 128), :] = t2
        for t in range(16):
            rows = lambda j: cat(*[xd[j, pl.ds(mirror(a), 16, stride=XP), :] for a in range(8 * t, 8 * t + 8)])
            z = [dot(rows(q).astype(bf16), as_bf16(gi[q])) for q in range(2)]
            for g in range(1, 4):
                tr, ti = rows(2 * g), rows(2 * g + 1)
                sg = jnp.where(low, float(sign[g - 1][0]), float(sign[g - 1][1]))
                k1, k2, k3 = [dot(v.astype(bf16), as_bf16(gi[3 * g - 1 + n]))
                              for n, v in enumerate((tr + sg * ti, ti, tr))]
                z += [k1 + k2, k1 + k3]
            y = _inv8(z)
            for j in range(8):
                xb[j, t] = y[j].reshape(4, SEG, 128).astype(bf16)

    HALF = NSEG * M // 2
    pre32 = pre.bitcast(u32)

    def store_pre(pair, row0, cs, packed):
        n = cs[0].shape[0] // M
        segs = pl.ds(row0 // M, n)
        if packed:
            st = jnp.concatenate([c.reshape(n, M, E) for c in cs], axis=1)
            pre32[pair, segs] = pltpu.bitcast(st.reshape(2 * M * n, E).astype(bf16), u32).reshape(n, M, E)
        else:
            for t, c in enumerate(cs):
                pre[pair, segs, pl.ds(M * t, M), :] = c.reshape(n, M, E).astype(bf16)

    def batch(u, p0, p1, tasks=(), t0=0, t1=4, margin=4):
        mc = HALF // 2 if t1 - t0 == 1 else HALF
        pacer = _Pacer(tasks, (7 * (p1 - p0) - margin // (t1 - t0)) * HALF // 8)
        w = wall.at[u]
        for p in range(p0, p1):
            for r0 in range(0, HALF, mc):
                def blk(head, par):
                    return lambda: cat(*[w[pl.ds((p + 8 * head) * WP + 64 * (2 * t + par), 64), :]
                                         for t in range(t0, t1)])

                def prod(i, b):
                    lhs = jnp.concatenate([as_bf16(xs32[i, t, pl.ds(r0 // 2, mc // 2), :])
                                           for t in range(t0, t1)], axis=1)
                    r = dot(lhs, narrow(b))
                    pacer.feed(r)
                    return r

                def emit(half, *cs):
                    park = pl.ds((half * HALF + r0) // 8, mc // 8)
                    if t0 > 0:
                        cs = [c + yb[t, p, park].reshape(mc, E) for t, c in enumerate(cs)]
                    if t1 < 4:
                        for t, c in enumerate(cs):
                            yb[t, p, park] = c.reshape(mc // 8, 8, E)
                    else:
                        store_pre(8 * u + p, half * HALF + r0, cs, False)
                if t0 // (t1 - t0) % 2:
                    _strassen(prod, blk(1, 0), blk(0, 0), blk(1, 1), blk(0, 1), add2, sub2,
                              lambda half, c1, c0: emit(half, c0, c1))
                else:
                    _strassen(prod, blk(0, 0), blk(1, 0), blk(0, 1), blk(1, 1), add2, sub2, emit)
        pacer.done()

    QUART = HALF // 2
    xs32, xs2_32 = xs.bitcast(u32), xs2.bitcast(u32)

    def strassen2(right, left, emit, done, pacer, lag):
        def unpack(b):
            if b.dtype == u32 and lag and len(done) >= lag:
                b = b & jnp.tile(all_ones(done[-lag]), (b.shape[0] // 8, 1))
            return widen(b)
        add = lambda a, b: unpack(a) + unpack(b)
        sub = lambda a, b: unpack(a) - unpack(b)

        def outer_prod(i, bs):
            def prod(j, b):
                r = dot(left(7 * i + j), narrow(b))
                pacer.feed(r)
                done.append(pltpu.bitcast(r[0:8], u32))
                return r
            order = (1, 0, 3, 2) if i in (1, 4, 5, 6) else (0, 1, 2, 3)
            cs = {}
            _strassen(prod, *[(lambda b=bs[k]: b) for k in order], add, sub, lambda half, *c: cs.update({half: c}))
            return _Blocks((cs[0] + cs[1])[k] for k in order)

        def outer_emit(half, *cs):
            for col in (1, 0):
                for a in range(2):
                    emit(2 * half + a, 2 * col, cs[col][2 * a], cs[col][2 * a + 1])
        outer = lambda k, c: lambda: [right(2 * k + k2, 2 * c + c2) for k2 in range(2) for c2 in range(2)]
        _strassen(outer_prod, outer(0, 0), outer(0, 1), outer(1, 0), outer(1, 1),
                  lambda x, y: [add(a, b) for a, b in zip(x, y)],
                  lambda x, y: [sub(a, b) for a, b in zip(x, y)], outer_emit)

    def batch2(u, q0, q1, done, tasks=(), lag=LAG):
        pacer = _Pacer(tasks, (49 * (q1 - q0) - 12) * QUART // 8)
        w = wall.at[u]
        for q in range(q0, q1):
            def emit(row, col, *cs):
                store_pre(8 * u + 2 * q + col // 2, row * QUART, cs, True)
            strassen2(lambda k, c: cat(*[w[pl.ds((2 * q + c // 2 + 8 * (c % 2)) * WP + 64 * (k + 4 * t), 64), :]
                                         for t in range(2)]),
                      lambda i: jnp.concatenate([as_bf16(xs2_32[i, t]) for t in range(2)], axis=1),
                      emit, done, pacer, lag)
        pacer.done()

    def left2_tasks():
        def make(i, t, r):
            def task(tok):
                a = _strassen_left_one(i, lambda rh, kh: _Blocks(
                    x8[32 * rh + 16 * rl + r, :, pl.ds(128 * (2 * kh + kl + 4 * t), 128)].astype(f32)
                    for rl in range(2) for kl in range(2)))
                a[0], a[3] = after(a[0], tok), after(a[3], tok)
                for j, v in enumerate(_strassen_left(*a)):
                    xs2[7 * i + j, t, pl.ds(M * r, M), :] = v.astype(bf16)
            return task
        return [make(i, t, r) for i in range(7) for t in range(2) for r in range(16)]

    def left_tasks(n):
        def make(r):
            def task(tok):
                a = [x8[NSEG // 2 * h + r, :, pl.ds(256 * n + 128 * k, 128)].astype(f32)
                     for h in range(2) for k in range(2)]
                a[0], a[3] = after(a[0], tok), after(a[3], tok)
                for i, v in enumerate(_strassen_left(*a)):
                    xs[i, n, pl.ds(M * r, M), :] = v.astype(bf16)
            return task
        return [make(r) for r in range(NSEG // 2)]

    def piece_tasks(n):
        rel, left = relayout_tasks(0, 128 * n, 128 * n + 128), left_tasks(n)
        return [t for r in range(32) for t in (rel[2 * r], left[r], rel[2 * r + 1])]

    run_now = lambda tasks: [task(jnp.zeros((8, 128), u32)) for task in tasks]

    c_a[0][0].wait()
    run_now(left_tasks(0))
    c_a[0][1].wait()
    run_now(relayout_tasks(0, 0, 64))
    c_a[0][2].wait()
    run_now(relayout_tasks(0, 64, 128))
    batch(0, 0, PS[0], (), 0, 1)
    wait_all(c_a[1])
    c_h = [start(wq_hbm.at[pl.ds(256 * n, 256), :, 1], wraw.at[1, pl.ds(256 * n, 256)], n) for n in range(2)]
    batch(0, PS[0], 8, piece_tasks(1), 0, 1)
    batch(0, 0, PS[1], (), 1, 2)
    wait_all(c_a[2])
    batch(0, PS[1], 8, piece_tasks(2), 1, 2)
    batch(0, 0, PS[2], (), 2, 3)
    wait_all(c_a[3])
    c_w2 = start_unit(2)
    batch(0, PS[2], 8, piece_tasks(3), 2, 3)
    batch(0, 0, PS[3], (), 3, 4)
    c_h[0].wait()
    batch(0, PS[3], 8, relayout_tasks(1, 0, 256), 3, 4)
    left2 = left2_tasks()
    batch(1, 0, 5, left2[:128], 0, 2)
    c_h[1].wait()
    start_unit(3)
    batch(1, 5, 8, relayout_tasks(1, 256, 512), 0, 2)
    batch(1, 0, 4, left2[128:], 2, 4)
    c_w2.wait()
    start_unit(4)
    start_unit(5)
    c_b1 = [start(bx_hbm.at[:, :, :, pl.ds(128 * j, 128)], xb.at[j], 5) for j in range(8)]
    c_b1 += [start(gf_hbm, gf, 5), start(tw_hbm, tw, 5)]
    c_loop = [start(wo_hbm.at[:, pl.ds(128 * j, 128)], wo.at[j], 4) for j in range(8)]
    c_loop += [start_x(0, UNROLL, 4), start(mem_hbm, mem0, 4), start(fill_hbm, fill_ref.at[pl.ds(0, 80)], 4)]
    c_loop += start_filter(0, 64, 4)
    batch(1, 4, 8, relayout_tasks(2), 2, 4)
    batch2(2, 0, 2, [])

    def unit_body(u, c):
        slot = (u + 1) % NRAW
        pltpu.make_async_copy(wraw.at[slot], wraw.at[slot], sems.at[slot]).wait()
        done = []
        batch2(u, 2, 4, done, relayout_tasks(u + 1))
        batch2(u + 1, 0, 2, done)
        return c
    lax.fori_loop(2, 5, unit_body, 0)
    wait_all(c_b1)
    batch(5, 6, 8, butterfly_tasks(), margin=0)
    batch2(5, 2, 3, [], lag=None)
    b_stage1()
    wait_all(c_loop)
    c_rest = [start_x(UNROLL, NSEG - UNROLL, 6)] + start_filter(64, 448, 6)
    c_b3 = [start(w.at[pl.ds(512, 1), :], wl.at[t], 5) for t, w in enumerate((wr_hbm, wi_hbm))]
    c_b3 += [start(gi_hbm, gi, 5)]

    wo32 = wo.bitcast(u32)
    scale = E ** -0.5

    def gated(w, toks):
        if not toks:
            return w
        bits = functools.reduce(
            jnp.bitwise_or, [pltpu.bitcast(jnp.broadcast_to(t, (8, 128)), u32) for t in toks])
        return cat(w[0:8] & all_ones(bits), w[8:])

    def wqkv(i, p, second, toks=(), k0=0, k1=D):
        rows = pl.ds((p % 8 + 8 * second) * WP + k0 // 2, (k1 - k0) // 2)
        return as_bf16(gated(wall[2 * i + p // 8, rows, :], toks))

    def step(n, u, mem, held):
        s = UNROLL * n + u
        rows = cat(mem, xbuf[s].astype(f32))
        lhs = rows.astype(bf16)
        head_start = {}
        if u:
            lo, hi = rows[:, :D // 2].astype(bf16), rows[:, D // 2:].astype(bf16)
            for key in EARLY:
                head_start[key] = dot(lo, wqkv(*key, k1=D // 2))
        fill = fill_ref[pl.ds(0, 80), :]
        heads = [None] * H
        rs = []

        shift = jnp.full((8, 128), 16 - 16 * (n % 2), jnp.int32).astype(u32)
        wblk = pl.ds(pl.multiple_of(64 * (n // 2), 64), 64)
        flt = filter_tasks(
            s, lambda d: [hi_f32(wt.at[t, d, wblk].bitcast(u32)[pl.ds(u, 8, stride=4), :] << shift) for t in range(2)])
        pacer = _Pacer(flt, 48)

        def proj(i, p, toks=()):
            a, b = [
                dot(hi, wqkv(i, p, t, k0=D // 2)) + head_start[i, p, t] if (i, p, t) in head_start
                else dot(lhs, wqkv(i, p, t, toks[t * len(toks) // 2:(t + 1) * len(toks) // 2]))
                for t in range(2)]
            pacer.feed(a)
            pacer.feed(b)
            c = widen(pre32[16 * i + p, s])
            return cat(a, b, c).astype(bf16)

        def probs(q, k):
            sc = dot_nt(q, k) * scale
            sc = jnp.where(fill == 0.0, sc, fill)
            e = jnp.exp(sc - jnp.max(sc, axis=1, keepdims=True))
            l = jnp.sum(e, axis=1, keepdims=True)
            r = pl.reciprocal(l, approx=True)
            r = r * (2.0 - l * r)
            rs.append([r[8 * j:8 * j + 8] for j in range(10)])
            return (e * r).astype(bf16)

        def pv(p, pr, v):
            o = dot(pr, v)
            heads[2 * p] = cat(o[0:8], o[16:32], o[64:72])
            heads[2 * p + 1] = cat(o[32:40], o[48:64], o[72:80])
            held[u, 2 * p], held[u, 2 * p + 1] = o[8:16], o[40:48]

        def left_task(q, i):
            def task(tok):
                a = _strassen_left_one(i, lambda r, k: _Blocks(
                    held[2 * r + r2, 4 * q + 2 * k + k2] for r2 in range(2) for k2 in range(2)))
                a[0], a[3] = after(a[0], tok), after(a[3], tok)
                for j, v in enumerate(_strassen_left(*a)):
                    osum[7 * i + j, q, pl.ds(pl.multiple_of(M * n, M), M), :] = v.astype(bf16)
            return task

        pend = []
        for g in range(4):
            ps = range(4 * g, 4 * g + 4)
            qk = [(proj(0, p), proj(1, p)) for p in ps]
            vs = [proj(2, p, rs[p - 4] if g else ()) for p in ps]
            for a in pend:
                pv(*a)
            pend = [(p, probs(*qk[t]), vs[t]) for t, p in enumerate(ps)]
        pacer.done()

        def wo_part(oc, j, h0, h1, toks=()):
            return dot(oc, as_bf16(gated(wo32[j, pl.ds(64 * h0, 64 * (h1 - h0)), :], toks)))

        acc = []
        pacer = _Pacer([left_task(q, i) for q in range(8) for i in LEFT_AT[u]], 38)
        oc = jnp.concatenate(heads[0:24], axis=1).astype(bf16)
        for j in range(8):
            acc.append(wo_part(oc, j, 0, 24, {3: rs[12] + rs[13], 4: rs[14] + rs[15]}.get(j, ())))
            if j == 4:
                for a in pend:
                    pv(*a)
            if j >= 5:
                pacer.feed(acc[j])
        oc = jnp.concatenate(heads[24:32], axis=1).astype(bf16)
        nxt = []
        for j in range(8):
            r = wo_part(oc, j, 24, 32) + acc[j]
            outbuf[n, u, pl.ds(M, SEG - M), pl.ds(128 * j, 128)] = r[M:].astype(bf16)
            nxt.append(r[0:M])
            pacer.feed(r)
        pacer.done()
        return jnp.concatenate(nxt, axis=1)

    def steps(n, mem):
        pl.when(n == 1)(functools.partial(wait_all, c_rest))
        held = {}
        for u in range(UNROLL):
            mem = step(n, u, mem, held)
        return mem
    lax.fori_loop(0, NSEG // UNROLL, steps, mem0[...].astype(f32))
    tok_rows = pl.ds(M, SEG - M)
    c_out = [start(outbuf.at[:, :, tok_rows, :], out_hbm.at[:, :, tok_rows, pl.ds(0, D)], 0)]

    wait_all(c_b3)
    run_now(filter_tasks(64, lambda d: [wl[t, :, pl.ds(128 * d, 128)].astype(f32) for t in range(2)]))
    b_stage3()
    c_out += [start(xb.at[j], out_hbm.at[:, :, :, pl.ds(D + 128 * j, 128)], 0) for j in range(8)]

    osum32 = osum.bitcast(u32)
    done = []
    for cq in range(2):
        def emit(row, col, *cs):
            for t, c in enumerate(cs):
                outbuf[:, row, pl.ds(0, M), pl.ds(128 * (4 * cq + col + t), 128)] = (
                    c.reshape(NSEG // 4, M, 128).astype(bf16))
            idx = (slice(None), row, pl.ds(0, M), pl.ds(128 * (4 * cq + col), 256))
            c_out.append(start(outbuf.at[idx], out_hbm.at[idx], 0))
        strassen2(lambda k, c: cat(*[wo32[4 * cq + c, pl.ds(64 * (4 * q + k), 64), :] for q in range(8)]),
                  lambda i: jnp.concatenate([as_bf16(osum32[i, q]) for q in range(8)], axis=1),
                  emit, done, _Pacer((), 0), None)
    wait_all(c_out)


@jax.jit
def pallas_concat_heads__memory_aug_recurrent_mem_tr__spectral_gfnet__prompt_kernel(
    A_x: jax.Array,
    A_mem0: jax.Array,
    A_Wq: jax.Array,
    A_Wk: jax.Array,
    A_Wv: jax.Array,
    A_Wo: jax.Array,
    A_seg_len: jax.Array,
    B_x: jax.Array,
    B_w_r: jax.Array,
    B_w_i: jax.Array,
):
    del A_seg_len
    assert A_x.shape == (1, S, D) and A_mem0.shape == (1, M, D) and B_x.shape == (1, S, D)
    assert A_Wq.shape == (D, H, E) and A_Wo.shape == (H, E, D) and B_w_r.shape == (S, D // 2 + 1)
    gf, gi, tw, _ = _dft_constants()
    fill = _attn_fill()
    hbm = pl.BlockSpec(memory_space=pltpu.HBM)
    wshape = (D // 2, 2, 2, 16, E)
    out = pl.pallas_call(
        _kernel,
        out_shape=jax.ShapeDtypeStruct((NSEG // 4, 4, SEG, 2 * D), bf16),
        in_specs=[hbm] * 13,
        out_specs=hbm,
        scratch_shapes=[
            pltpu.VMEM((NRAW, D // 2, 2, 16, E), bf16),
            pltpu.VMEM((6, 16 * WP, E), u32),
            pltpu.VMEM((8, H * E, 128), bf16),
            pltpu.VMEM((NSEG, SEG - M, D), bf16),
            pltpu.VMEM((M, D), bf16),
            pltpu.VMEM((NSEG, M, D), bf16),
            pltpu.VMEM((7, 4, 256, 128), bf16),
            pltpu.VMEM((49, 2, 128, 128), bf16),
            pltpu.VMEM((48, NSEG, 2 * M, E), bf16),
            pltpu.VMEM((49, 8, NSEG * M // 4, E), bf16),
            pltpu.VMEM((NSEG // 4, 4, SEG, D), bf16),
            pltpu.VMEM((96, 80), f32),
            pltpu.VMEM((8, NSEG // 4, 4, SEG, 128), bf16),
            pltpu.VMEM((2, 16, 512, 128), bf16),
            pltpu.VMEM((2, 1, S), bf16),
            pltpu.VMEM(gf.shape, u32),
            pltpu.VMEM(gi.shape, u32),
            pltpu.VMEM(tw.shape, f32),
            pltpu.VMEM((8, 16 * XP, 128), f32),
            pltpu.VMEM((2, 16, 65, 8, 128), f32),
            pltpu.SemaphoreType.DMA((7,)),
        ],
        compiler_params=pltpu.CompilerParams(vmem_limit_bytes=120 * 1024 * 1024),
    )(A_x.reshape(NSEG, SEG, D), A_mem0.reshape(M, D),
      A_Wq.reshape(wshape), A_Wk.reshape(wshape), A_Wv.reshape(wshape),
      A_Wo.reshape(H * E, D), B_x.reshape(NSEG // 4, 4, SEG, D), B_w_r.T, B_w_i.T, gf, gi, tw, fill)
    return out.reshape(1, S, 2 * D)
```

```python
import functools

import jax
import jax.numpy as jnp
import numpy as np
from jax import lax
from jax.experimental import pallas as pl
from jax.experimental.pallas import tpu as pltpu

S, D, H, E, M, SEG = 2048, 1024, 32, 128, 8, 32
NSEG = S // SEG
WP = 516
XP = 132
NRAW = 4
UNROLL = 4
PS = (6, 4, 4, 4)
LAG = 8
LEFT_AT = ((), (2,), (4,), (0, 1, 3, 5, 6))
EARLY = ((0, 0, 0), (0, 0, 1), (1, 0, 0), (1, 0, 1), (0, 1, 0))
bf16, f32, u32 = jnp.bfloat16, jnp.float32, jnp.uint32
RES = ((0, 4), (2, 6), (1, 7), (3, 5))
RC = float(np.sqrt(0.5))


def _fwd8(x):
    s04, d04 = x[0] + x[4], x[0] - x[4]
    s26, d26 = x[2] + x[6], x[2] - x[6]
    s15, d15 = x[1] + x[5], x[1] - x[5]
    s37, d37 = x[3] + x[7], x[3] - x[7]
    t1, t2 = (d15 - d37) * RC, (d15 + d37) * RC
    e0, o0 = s04 + s26, s15 + s37
    return [e0 + o0, e0 - o0, s04 - s26, s15 - s37, d04 + t1, d26 + t2, d04 - t1, d26 - t2]


def _inv8(z):
    z0, z4, e1, o1, r1, i1, r3, i3 = z
    e0, o0 = z0 + z4, z0 - z4
    s04, s26, s15, s37 = e0 + e1, e0 - e1, o0 + o1, o0 - o1
    d04, d26 = r1 + r3, i1 + i3
    t1, t2 = (r1 - r3) * RC, (i1 - i3) * RC
    d15, d37 = t1 + t2, t2 - t1
    return [s04 + d04, s15 + d15, s26 + d26, s37 + d37, s04 - d04, s15 - d15, s26 - d26, s37 - d37]


def _twiddle16(z, k):
    re, im = z
    k = k % 16
    if k == 0:
        return z
    if k == 4:
        return (im, -re)
    if k == 12:
        return (-im, re)
    if k == 2:
        return ((re + im) * RC, (im - re) * RC)
    if k == 14:
        return ((re - im) * RC, (re + im) * RC)
    if k == 6:
        return ((im - re) * RC, (re + im) * -RC)
    if k == 10:
        return ((re + im) * -RC, (re - im) * RC)
    c, s = float(np.cos(2 * np.pi * k / 16)), float(-np.sin(2 * np.pi * k / 16))
    return (re * c - im * s, re * s + im * c)


def _bfly4(z, sign):
    (ar, ai), (br, bi), (cr, ci), (dr, di) = z
    sr, si, tr, ti = ar + cr, ai + ci, ar - cr, ai - ci
    ur, ui, vr, vi = br + dr, bi + di, br - dr, bi - di
    o0, o2 = (sr + ur, si + ui), (sr - ur, si - ui)
    p, q = (tr + vi, ti - vr), (tr - vi, ti + vr)
    return [o0, p, o2, q] if sign > 0 else [o0, q, o2, p]


class _Pacer:
    def __init__(self, tasks, ntokens):
        self.slots = {}
        for n, task in enumerate(tasks):
            self.slots.setdefault(n * ntokens // len(tasks), []).append(task)
        self.pos = 0

    def feed(self, r):
        for j in range(r.shape[0] // 8):
            for task in self.slots.pop(self.pos, []):
                task(pltpu.bitcast(r[8 * j:8 * j + 8], u32))
            self.pos += 1

    def done(self):
        assert not self.slots


def _pack_rows(m):
    b = np.asarray(m, np.float32).astype(jnp.bfloat16).view(np.uint16).astype(np.uint32)
    return b[..., 0::2, :] | (b[..., 1::2, :] << 16)


def _dft_constants():
    i, j = np.arange(64)[:, None], np.arange(128)
    whole, half = 2 * np.pi * i * j / 128, 2 * np.pi * (i + 0.5) * j / 128
    gf = np.zeros((3, 192, 128))
    gf[0, :129] = np.concatenate([np.cos(whole), -np.sin(whole), [(-1.0) ** j]])
    gf[1, :128] = np.concatenate([np.cos(half), -np.sin(half)])
    gf[2, :128] = np.concatenate([np.cos(half), np.sin(half)])
    gi = gf[0:2, :128] * (2.0 / (D * S))
    gi[0, 0], gi[0, 64] = gf[0, 0] / (D * S), gf[0, 128] / (D * S)
    angs = [2 * np.pi * j * (b - 8) / S for b in range(16)] + [2 * np.pi * j * (r - 4) / D for r, _ in RES]
    tw = np.zeros((20, 2, 8, 128), np.float32)
    for n, ang in enumerate(angs):
        tw[n, 0], tw[n, 1] = np.cos(ang), -np.sin(ang)
    return _pack_rows(gf), _pack_rows(gi), tw


def _attn_fill():
    head = np.concatenate([np.arange(64) // 32, np.arange(16) // 8])
    pos = np.concatenate([np.arange(64) % 32, 32 + np.arange(16) % 8])
    ok = (pos[:, None] < M) | (pos[:, None] >= pos[None, :])
    fill = np.where(ok, 0.0, -1e9)
    fill = np.where(head[:, None] == head[None, :], fill, -np.inf)
    return fill.astype(np.float32)


def _strassen(prod, b11, b12, b21, b22, add, sub, emit):
    m2 = prod(1, b11())
    m1 = prod(0, add(b11(), b22()))
    m3 = prod(2, sub(b12(), b22()))
    c22 = prod(5, add(b11(), b12())) + ((m1 - m2) + m3)
    m4 = prod(3, sub(b21(), b11()))
    emit(1, m2 + m4, c22)
    m5 = prod(4, b22())
    emit(0, prod(6, add(b21(), b22())) + ((m1 + m4) - m5), m3 + m5)


class _Blocks(list):
    def __add__(self, other):
        return _Blocks(a + b for a, b in zip(self, other))

    def __sub__(self, other):
        return _Blocks(a - b for a, b in zip(self, other))


def _strassen_left(a11, a12, a21, a22):
    return [a11 + a22, a21 + a22, a11, a22, a11 + a12, a21 - a11, a12 - a22]


def _strassen_left_one(i, blk):
    terms = ((0, 3, 1), (2, 3, 1), (0,), (3,), (0, 1, 1), (2, 0, -1), (1, 3, -1))[i]
    a = blk(*divmod(terms[0], 2))
    if len(terms) == 1:
        return a
    b = blk(*divmod(terms[1], 2))
    return a + b if terms[2] > 0 else a - b


def _kernel(x_hbm, mem_hbm, wq_hbm, wk_hbm, wv_hbm, wo_hbm, bx_hbm, wr_hbm, wi_hbm,
            gf_hbm, gi_hbm, tw_hbm, fill_hbm, out_hbm,
            wraw, wall, wo, xbuf, mem0, x8, xs, xs2, pre, osum, outbuf, fill_ref,
            xb, wt, wl, gf, gi, tw, xd, yb, sems):
    def start(src, dst, sem):
        c = pltpu.make_async_copy(src, dst, sems.at[sem])
        c.start()
        return c

    def wait_all(cs):
        for c in cs:
            c.wait()

    dot = functools.partial(jnp.dot, preferred_element_type=f32)
    dot_nt = lambda a, b: lax.dot_general(a, b, (((1,), (1,)), ((), ())), preferred_element_type=f32)
    cat = lambda *vs: jnp.concatenate(vs, axis=0)
    as_bf16 = lambda w: pltpu.bitcast(w, bf16)
    hi_f32 = lambda w: pltpu.bitcast(w & u32(0xFFFF0000), f32)
    all_ones = lambda tok: ((tok >> 16) | u32(0xFFFF)) | u32(0xFFFF0000)
    after = lambda v, tok: pltpu.bitcast(pltpu.bitcast(v, u32) & all_ones(tok), f32)
    widen = lambda w: as_bf16(w).astype(f32) if w.dtype == u32 else w
    narrow = lambda w: as_bf16(w) if w.dtype == u32 else w.astype(bf16)
    add2 = lambda a, b: widen(a) + widen(b)
    sub2 = lambda a, b: widen(a) - widen(b)
    w_hbm = (wq_hbm, wk_hbm, wv_hbm)

    def start_unit(u):
        return start(w_hbm[u // 2].at[:, :, u % 2], wraw.at[u % NRAW], u % NRAW)

    def start_x(seg0, nseg, sem):
        segs, rows = pl.ds(seg0, nseg), pl.ds(0, SEG - M)
        return start(x_hbm.at[segs, rows, :], xbuf.at[segs], sem)

    def start_filter(row0, nrows, sem):
        rows = pl.ds(row0, nrows)
        return [start(w.at[rows, pl.ds(128 * d, 128)], wt.at[t, d, rows], sem)
                for t, w in enumerate((wr_hbm, wi_hbm)) for d in range(16)]

    def start_piece(n, xsem, parts):
        cols = pl.ds(256 * n, 256)
        cs = [start(x_hbm.at[:, pl.ds(SEG - M, M), cols], x8.at[:, :, cols], xsem)]
        for k, sem in enumerate(parts):
            rows = pl.ds(128 * n + 128 // len(parts) * k, 128 // len(parts))
            cs.append(start(wq_hbm.at[rows, :, 0], wraw.at[0, rows], sem))
        return cs
    c_a = [start_piece(0, 5, (6, 0))] + [start_piece(n, n, (n,)) for n in range(1, 4)]

    xb32 = xb.bitcast(u32)

    def relayout_row(src, dst, r, lo, hi):
        a, b = src.at[r].bitcast(u32)[...]
        dst[pl.ds(r, 8, stride=WP), :] = (a & lo) | (b << 16)
        dst[pl.ds(r + 8 * WP, 8, stride=WP), :] = (a >> 16) | (b & hi)

    def relayout_tasks(u, r0=0, r1=D // 2):
        src, dst = wraw.at[u % NRAW], wall.at[u]

        def make(r):
            def task(tok):
                lo = (tok >> 16) | u32(0xFFFF)
                hi = (tok << 16) | u32(0xFFFF0000)
                relayout_row(src, dst, r, lo, hi)
                relayout_row(src, dst, r + 1, lo, hi)
            return task
        return [make(r) for r in range(r0, r1, 2)]

    def y_blocks(r):
        return pl.ds(4 * (r % 2) + r // 2, 8, stride=8)

    def filter_tasks(blk, wfn):
        def make(phase, k):
            slots = [4 * k + j for j in range(4)] if phase == 1 else [4 * j + k for j in range(4)]

            def task(tok):
                z = [(yb[0, b, blk], yb[1, b, blk]) for b in slots]
                if phase == 0:
                    z = [(after(zr, tok), zi) for zr, zi in z]
                    z = [(zr * tw[b, 0] - zi * tw[b, 1], zr * tw[b, 1] + zi * tw[b, 0]) if b != 8 else (zr, zi)
                         for b, (zr, zi) in zip(slots, z)]
                else:
                    z[0] = tuple(after(v, tok) for v in z[0])
                if phase == 0:
                    o = _bfly4(z, 1)
                    o = [_twiddle16(o[j], k * j) for j in range(4)]
                elif phase == 1:
                    o = _bfly4(z, 1)
                    y = []
                    for j in range(4):
                        wr, wi = wfn(k + 4 * j)
                        xr, xi = o[j]
                        y.append((xr * wr - xi * wi, xr * wi + xi * wr))
                    o = _bfly4(y, -1)
                    o = [_twiddle16(o[j], -k * j) for j in range(4)]
                else:
                    o = [(zr * tw[b, 0] + zi * tw[b, 1], zi * tw[b, 0] - zr * tw[b, 1]) if b != 8 else (zr, zi)
                         for b, (zr, zi) in zip(slots, _bfly4(z, -1))]
                for b, v in zip(slots, o):
                    yb[0, b, blk] = v[0]
                    yb[1, b, blk] = v[1]
            return task
        return [make(phase, k) for phase in range(3) for k in range(4)]

    mirror = lambda a: a if a < 64 else 191 - a

    def twiddle_d(g, x, y):
        c, sn = [jnp.tile(tw[16 + g, k], (x.shape[0] // 8, 1)) for k in range(2)]
        return (x * c - y * sn, x * sn + y * c) if g == 3 else (x * c + y * sn, x * sn - y * c)

    def butterfly_tasks():
        def make(a, par):
            def task(tok):
                w = [xb32[j, a // 8, a // 2 % 4, pl.ds(8 * (a % 2), 8), :] for j in range(8)]
                if par:
                    hi = (tok << 16) | u32(0xFFFF0000)
                    z = _fwd8([pltpu.bitcast(v & hi, f32) for v in w])
                else:
                    sixteen = ((tok >> 31) | u32(1)) << 4
                    z = _fwd8([pltpu.bitcast(v << sixteen, f32) for v in w])
                for n in range(8):
                    xd[n, pl.ds(8 * XP * par + mirror(a), 8, stride=XP), :] = z[n]
            return task
        return [make(a, par) for a in range(128) for par in range(2)]

    low = lax.broadcasted_iota(jnp.int32, (1, 128), 1) < 64

    def b_dfwd(b, g):
        z = [xd[n, pl.ds(XP * (b // 2 + 8 * (b % 2)), 128), :] for n in (2 * g, 2 * g + 1)]
        if g:
            z = twiddle_d(g, *z)
        z = [cat(v[0:64] + v[64:128], v[0:64] - v[64:128]).astype(bf16) for v in z]
        tu = dot_nt(as_bf16(gf[1, 0:64] if g else gf[0, 0:72]), z[0])
        tv = dot_nt(as_bf16(gf[1, 0:64]), z[1])
        if g == 0:
            tr = cat(tu[0:64], tv[0:64], tu[128:144])
            ti = cat(tu[64:128], tv[64:128], jnp.zeros((16, 128), f32))
        else:
            tr = cat(tu[0:64] - tv[64:128], tu[0:64] + tv[64:128])
            ti = cat(tu[64:128] + tv[0:64], tu[64:128] - tv[0:64])
        return jnp.where(low, tr, ti).astype(bf16), jnp.where(low, ti, tr).astype(bf16)

    def b_sfwd(b, g, ts):
        for c in range(2):
            y = dot(ts[c], as_bf16(gf[2 - c, 0:64]))
            for q in range(2):
                yb[c, b, y_blocks(RES[g][q])] = y[64 * q:64 * q + 64].reshape(8, 8, 128)
            if g == 0:
                yb[c, b, 64] = y[128:136]

    def b_stage1():
        pend = []
        for b in list(range(0, 16, 2)) + list(range(1, 16, 2)):
            for g in range(4):
                pend.append((b, g, b_dfwd(b, g)))
                if len(pend) > 3:
                    b_sfwd(*pend.pop(0))
        for item in pend:
            b_sfwd(*item)

    def b_sinv(tasks):
        row0 = lax.broadcasted_iota(jnp.int32, (8, 128), 0) == 0
        pacer = _Pacer(tasks, 12 * 8)
        for _, b, g in sorted((b + (6 if g == 0 else 0), b, g) for b in range(16) for g in range(4)):
            (ar, br), (ai, bi) = [[yb[c, b, y_blocks(r)].reshape(64, 128) for r in RES[g]] for c in range(2)]
            if g:
                uv = [(ar + br, ai + bi, -ar - br), (ai - bi, br - ar, bi - ai)]
                uv = [(cat(re, im), cat(im, neg)) for re, im, neg in uv]
            else:
                pacer.done()
                na = -ar
                uv = [(cat(ar, jnp.where(row0, yb[0, b, 64], ai[0:8]), ai[8:]),
                       cat(ai, jnp.where(row0, yb[1, b, 64], na[0:8]), na[8:])),
                      (cat(br, bi), cat(bi, -br))]
            for q, (u, v) in enumerate(uv):
                cu = dot_nt(as_bf16(gf[2, 0:32]), u.astype(bf16))
                sv = dot_nt(as_bf16(gf[2, 32:64]), v.astype(bf16))
                xd[2 * g + q, pl.ds(XP * b, 128), :] = cat(cu - sv, cu + sv)
            pacer.feed(cu)

    def b_dinv(t):
        rows = lambda j: cat(*[xd[j, pl.ds(mirror(a), 16, stride=XP), :] for a in range(8 * t, 8 * t + 8)])
        z = [dot(rows(j).astype(bf16), as_bf16(gi[min(j, 1)])) for j in range(8)]
        for g in range(1, 4):
            u, v = z[2 * g], z[2 * g + 1]
            c, sn = [jnp.tile(tw[16 + g, k], (16, 1)) for k in range(2)]
            z[2 * g] = u * c + v * sn
            z[2 * g + 1] = v * c - u * sn if g == 3 else u * sn - v * c
        y = _inv8(z)
        for j in range(8):
            xb[j, t] = y[j].reshape(4, SEG, 128).astype(bf16)

    HALF = NSEG * M // 2
    pre32 = pre.bitcast(u32)

    def store_pre(pair, row0, cs, packed):
        n = cs[0].shape[0] // M
        segs = pl.ds(row0 // M, n)
        if packed:
            st = jnp.concatenate([c.reshape(n, M, E) for c in cs], axis=1)
            pre32[pair, segs] = pltpu.bitcast(st.reshape(2 * M * n, E).astype(bf16), u32).reshape(n, M, E)
        else:
            for t, c in enumerate(cs):
                pre[pair, segs, pl.ds(M * t, M), :] = c.reshape(n, M, E).astype(bf16)

    def batch(u, p0, p1, tasks=(), t0=0, t1=4, margin=4):
        mc = HALF // 2 if t1 - t0 == 1 else HALF
        pacer = _Pacer(tasks, (7 * (p1 - p0) - margin // (t1 - t0)) * HALF // 8)
        w = wall.at[u]
        for p in range(p0, p1):
            for r0 in range(0, HALF, mc):
                def blk(head, par):
                    return lambda: cat(*[w[pl.ds((p + 8 * head) * WP + 64 * (2 * t + par), 64), :]
                                         for t in range(t0, t1)])

                def prod(i, b):
                    lhs = jnp.concatenate([as_bf16(xs32[i, t, pl.ds(r0 // 2, mc // 2), :])
                                           for t in range(t0, t1)], axis=1)
                    r = dot(lhs, narrow(b))
                    pacer.feed(r)
                    return r

                def emit(half, *cs):
                    park = pl.ds((half * HALF + r0) // 8, mc // 8)
                    if t0 > 0:
                        cs = [c + yb[t, p, park].reshape(mc, E) for t, c in enumerate(cs)]
                    if t1 < 4:
                        for t, c in enumerate(cs):
                            yb[t, p, park] = c.reshape(mc // 8, 8, E)
                    else:
                        store_pre(8 * u + p, half * HALF + r0, cs, False)
                if t0 // (t1 - t0) % 2:
                    _strassen(prod, blk(1, 0), blk(0, 0), blk(1, 1), blk(0, 1), add2, sub2,
                              lambda half, c1, c0: emit(half, c0, c1))
                else:
                    _strassen(prod, blk(0, 0), blk(1, 0), blk(0, 1), blk(1, 1), add2, sub2, emit)
        pacer.done()

    QUART = HALF // 2
    xs32, xs2_32 = xs.bitcast(u32), xs2.bitcast(u32)

    def strassen2(right, left, emit, done, pacer, lag):
        def unpack(b):
            if b.dtype == u32 and lag and len(done) >= lag:
                b = b & jnp.tile(all_ones(done[-lag]), (b.shape[0] // 8, 1))
            return widen(b)
        add = lambda a, b: unpack(a) + unpack(b)
        sub = lambda a, b: unpack(a) - unpack(b)

        def outer_prod(i, bs):
            def prod(j, b):
                r = dot(left(7 * i + j), narrow(b))
                pacer.feed(r)
                done.append(pltpu.bitcast(r[0:8], u32))
                return r
            order = (1, 0, 3, 2) if i in (1, 4, 5, 6) else (0, 1, 2, 3)
            cs = {}
            _strassen(prod, *[(lambda b=bs[k]: b) for k in order], add, sub, lambda half, *c: cs.update({half: c}))
            return _Blocks((cs[0] + cs[1])[k] for k in order)

        def outer_emit(half, *cs):
            for col in (1, 0):
                for a in range(2):
                    emit(2 * half + a, 2 * col, cs[col][2 * a], cs[col][2 * a + 1])
        outer = lambda k, c: lambda: [right(2 * k + k2, 2 * c + c2) for k2 in range(2) for c2 in range(2)]
        _strassen(outer_prod, outer(0, 0), outer(0, 1), outer(1, 0), outer(1, 1),
                  lambda x, y: [add(a, b) for a, b in zip(x, y)],
                  lambda x, y: [sub(a, b) for a, b in zip(x, y)], outer_emit)

    def batch2(u, q0, q1, done, tasks=(), lag=LAG):
        pacer = _Pacer(tasks, (49 * (q1 - q0) - 12) * QUART // 8)
        w = wall.at[u]
        for q in range(q0, q1):
            def emit(row, col, *cs):
                store_pre(8 * u + 2 * q + col // 2, row * QUART, cs, True)
            strassen2(lambda k, c: cat(*[w[pl.ds((2 * q + c // 2 + 8 * (c % 2)) * WP + 64 * (k + 4 * t), 64), :]
                                         for t in range(2)]),
                      lambda i: jnp.concatenate([as_bf16(xs2_32[i, t]) for t in range(2)], axis=1),
                      emit, done, pacer, lag)
        pacer.done()

    def left2_tasks():
        def make(i, t, r):
            def task(tok):
                a = _strassen_left_one(i, lambda rh, kh: _Blocks(
                    x8[32 * rh + 16 * rl + r, :, pl.ds(128 * (2 * kh + kl + 4 * t), 128)].astype(f32)
                    for rl in range(2) for kl in range(2)))
                a[0], a[3] = after(a[0], tok), after(a[3], tok)
                for j, v in enumerate(_strassen_left(*a)):
                    xs2[7 * i + j, t, pl.ds(M * r, M), :] = v.astype(bf16)
            return task
        return [make(i, t, r) for i in range(7) for t in range(2) for r in range(16)]

    def left_tasks(n):
        def make(r):
            def task(tok):
                a = [x8[NSEG // 2 * h + r, :, pl.ds(256 * n + 128 * k, 128)].astype(f32)
                     for h in range(2) for k in range(2)]
                a[0], a[3] = after(a[0], tok), after(a[3], tok)
                for i, v in enumerate(_strassen_left(*a)):
                    xs[i, n, pl.ds(M * r, M), :] = v.astype(bf16)
            return task
        return [make(r) for r in range(NSEG // 2)]

    def piece_tasks(n):
        rel, left = relayout_tasks(0, 128 * n, 128 * n + 128), left_tasks(n)
        return [t for r in range(32) for t in (rel[2 * r], left[r], rel[2 * r + 1])]

    run_now = lambda tasks: [task(jnp.zeros((8, 128), u32)) for task in tasks]

    c_a[0][0].wait()
    run_now(left_tasks(0))
    c_a[0][1].wait()
    run_now(relayout_tasks(0, 0, 64))
    c_a[0][2].wait()
    run_now(relayout_tasks(0, 64, 128))
    batch(0, 0, PS[0], (), 0, 1)
    wait_all(c_a[1])
    c_h = [start(wq_hbm.at[pl.ds(256 * n, 256), :, 1], wraw.at[1, pl.ds(256 * n, 256)], n) for n in range(2)]
    batch(0, PS[0], 8, piece_tasks(1), 0, 1)
    batch(0, 0, PS[1], (), 1, 2)
    wait_all(c_a[2])
    batch(0, PS[1], 8, piece_tasks(2), 1, 2)
    batch(0, 0, PS[2], (), 2, 3)
    wait_all(c_a[3])
    c_w2 = start_unit(2)
    batch(0, PS[2], 8, piece_tasks(3), 2, 3)
    batch(0, 0, PS[3], (), 3, 4)
    c_h[0].wait()
    batch(0, PS[3], 8, relayout_tasks(1, 0, 256), 3, 4)
    left2 = left2_tasks()
    batch(1, 0, 5, left2[:128], 0, 2)
    c_h[1].wait()
    start_unit(3)
    batch(1, 5, 8, relayout_tasks(1, 256, 512), 0, 2)
    batch(1, 0, 4, left2[128:], 2, 4)
    c_w2.wait()
    start_unit(4)
    start_unit(5)
    c_b1 = [start(bx_hbm.at[:, :, :, pl.ds(128 * j, 128)], xb.at[j], 5) for j in range(8)]
    c_b1 += [start(gf_hbm, gf, 5), start(tw_hbm, tw, 5)]
    c_loop = [start(wo_hbm.at[:, pl.ds(128 * j, 128)], wo.at[j], 4) for j in range(8)]
    c_loop += [start_x(0, UNROLL, 4), start(mem_hbm, mem0, 4), start(fill_hbm, fill_ref.at[pl.ds(0, 80)], 4)]
    c_loop += start_filter(0, 64, 4)
    batch(1, 4, 8, relayout_tasks(2), 2, 4)
    batch2(2, 0, 2, [])

    def unit_body(u, c):
        slot = (u + 1) % NRAW
        pltpu.make_async_copy(wraw.at[slot], wraw.at[slot], sems.at[slot]).wait()
        done = []
        batch2(u, 2, 4, done, relayout_tasks(u + 1))
        batch2(u + 1, 0, 2, done)
        return c
    lax.fori_loop(2, 5, unit_body, 0)
    wait_all(c_b1)
    batch(5, 6, 8, butterfly_tasks(), margin=0)
    batch2(5, 2, 3, [], lag=None)
    b_stage1()
    wait_all(c_loop)
    c_rest = [start_x(UNROLL, NSEG - UNROLL, 6)] + start_filter(64, 448, 6)
    c_b3 = [start(w.at[pl.ds(512, 1), :], wl.at[t], 5) for t, w in enumerate((wr_hbm, wi_hbm))]
    c_b3 += [start(gi_hbm, gi, 5)]

    wo32 = wo.bitcast(u32)
    scale = E ** -0.5

    def gated(w, toks):
        if not toks:
            return w
        bits = functools.reduce(
            jnp.bitwise_or, [pltpu.bitcast(jnp.broadcast_to(t, (8, 128)), u32) for t in toks])
        return cat(w[0:8] & all_ones(bits), w[8:])

    def wqkv(i, p, second, toks=(), k0=0, k1=D):
        rows = pl.ds((p % 8 + 8 * second) * WP + k0 // 2, (k1 - k0) // 2)
        return as_bf16(gated(wall[2 * i + p // 8, rows, :], toks))

    def step(n, u, mem, held):
        s = UNROLL * n + u
        rows = cat(mem, xbuf[s].astype(f32))
        lhs = rows.astype(bf16)
        head_start = {}
        if u:
            lo, hi = rows[:, :D // 2].astype(bf16), rows[:, D // 2:].astype(bf16)
            for key in EARLY:
                head_start[key] = dot(lo, wqkv(*key, k1=D // 2))
        fill = fill_ref[pl.ds(0, 80), :]
        heads = [None] * H
        rs = []

        shift = jnp.full((8, 128), 16 - 16 * (n % 2), jnp.int32).astype(u32)
        wblk = pl.ds(pl.multiple_of(64 * (n // 2), 64), 64)
        flt = filter_tasks(
            s, lambda d: [hi_f32(wt.at[t, d, wblk].bitcast(u32)[pl.ds(u, 8, stride=4), :] << shift) for t in range(2)])
        pacer = _Pacer(flt, 84)

        def proj(i, p, toks=()):
            a, b = [
                dot(hi, wqkv(i, p, t, k0=D // 2)) + head_start[i, p, t] if (i, p, t) in head_start
                else dot(lhs, wqkv(i, p, t, toks[t * len(toks) // 2:(t + 1) * len(toks) // 2]))
                for t in range(2)]
            pacer.feed(a)
            pacer.feed(b)
            c = widen(pre32[16 * i + p, s])
            return cat(a, b, c).astype(bf16)

        def probs(q, k):
            sc = dot_nt(q, k) * scale
            sc = jnp.where(fill == 0.0, sc, fill)
            e = jnp.exp(sc - jnp.max(sc, axis=1, keepdims=True))
            l = jnp.sum(e, axis=1, keepdims=True)
            r = pl.reciprocal(l, approx=True)
            r = r * (2.0 - l * r)
            rs.append([r[8 * j:8 * j + 8] for j in range(10)])
            return (e * r).astype(bf16)

        def pv(p, pr, v):
            o = dot(pr, v)
            heads[2 * p] = cat(o[0:8], o[16:32], o[64:72])
            heads[2 * p + 1] = cat(o[32:40], o[48:64], o[72:80])
            held[u, 2 * p], held[u, 2 * p + 1] = o[8:16], o[40:48]

        def left_task(q, i):
            def task(tok):
                a = _strassen_left_one(i, lambda r, k: _Blocks(
                    held[2 * r + r2, 4 * q + 2 * k + k2] for r2 in range(2) for k2 in range(2)))
                a[0], a[3] = after(a[0], tok), after(a[3], tok)
                for j, v in enumerate(_strassen_left(*a)):
                    osum[7 * i + j, q, pl.ds(pl.multiple_of(M * n, M), M), :] = v.astype(bf16)
            return task

        pend = []
        for g in range(4):
            ps = range(4 * g, 4 * g + 4)
            qk = [(proj(0, p), proj(1, p)) for p in ps]
            vs = [proj(2, p, rs[p - 4] if g else ()) for p in ps]
            for a in pend:
                pv(*a)
            pend = [(p, probs(*qk[t]), vs[t]) for t, p in enumerate(ps)]
        pacer.done()

        def wo_part(oc, j, h0, h1, toks=()):
            return dot(oc, as_bf16(gated(wo32[j, pl.ds(64 * h0, 64 * (h1 - h0)), :], toks)))

        acc = []
        pacer = _Pacer([left_task(q, i) for q in range(8) for i in LEFT_AT[u]], 38)
        oc = jnp.concatenate(heads[0:24], axis=1).astype(bf16)
        for j in range(8):
            acc.append(wo_part(oc, j, 0, 24, {3: rs[12] + rs[13], 4: rs[14] + rs[15]}.get(j, ())))
            if j == 4:
                for a in pend:
                    pv(*a)
            if j >= 5:
                pacer.feed(acc[j])
        oc = jnp.concatenate(heads[24:32], axis=1).astype(bf16)
        nxt = []
        for j in range(8):
            r = wo_part(oc, j, 24, 32) + acc[j]
            outbuf[n, u, pl.ds(M, SEG - M), pl.ds(128 * j, 128)] = r[M:].astype(bf16)
            nxt.append(r[0:M])
            pacer.feed(r)
        pacer.done()
        return jnp.concatenate(nxt, axis=1)

    def steps(n, mem):
        pl.when(n == 1)(functools.partial(wait_all, c_rest))
        held = {}
        for u in range(UNROLL):
            mem = step(n, u, mem, held)
        return mem
    lax.fori_loop(0, NSEG // UNROLL, steps, mem0[...].astype(f32))
    tok_rows = pl.ds(M, SEG - M)
    c_out = [start(outbuf.at[:, :, tok_rows, :], out_hbm.at[:, :, tok_rows, pl.ds(0, D)], 0)]

    wait_all(c_b3)
    b_sinv(filter_tasks(64, lambda d: [wl[t, :, pl.ds(128 * d, 128)].astype(f32) for t in range(2)]))
    for t in range(16):
        b_dinv(t)
    c_out += [start(xb.at[j], out_hbm.at[:, :, :, pl.ds(D + 128 * j, 128)], 0) for j in range(8)]

    osum32 = osum.bitcast(u32)
    done = []
    for cq in range(2):
        def emit(row, col, *cs):
            for t, c in enumerate(cs):
                outbuf[:, row, pl.ds(0, M), pl.ds(128 * (4 * cq + col + t), 128)] = (
                    c.reshape(NSEG // 4, M, 128).astype(bf16))
            idx = (slice(None), row, pl.ds(0, M), pl.ds(128 * (4 * cq + col), 256))
            c_out.append(start(outbuf.at[idx], out_hbm.at[idx], 0))
        strassen2(lambda k, c: cat(*[wo32[4 * cq + c, pl.ds(64 * (4 * q + k), 64), :] for q in range(8)]),
                  lambda i: jnp.concatenate([as_bf16(osum32[i, q]) for q in range(8)], axis=1),
                  emit, done, _Pacer((), 0), None)
    wait_all(c_out)


@jax.jit
def pallas_concat_heads__memory_aug_recurrent_mem_tr__spectral_gfnet__prompt_kernel(
    A_x: jax.Array,
    A_mem0: jax.Array,
    A_Wq: jax.Array,
    A_Wk: jax.Array,
    A_Wv: jax.Array,
    A_Wo: jax.Array,
    A_seg_len: jax.Array,
    B_x: jax.Array,
    B_w_r: jax.Array,
    B_w_i: jax.Array,
):
    del A_seg_len
    assert A_x.shape == (1, S, D) and A_mem0.shape == (1, M, D) and B_x.shape == (1, S, D)
    assert A_Wq.shape == (D, H, E) and A_Wo.shape == (H, E, D) and B_w_r.shape == (S, D // 2 + 1)
    gf, gi, tw = _dft_constants()
    fill = _attn_fill()
    hbm = pl.BlockSpec(memory_space=pltpu.HBM)
    wshape = (D // 2, 2, 2, 16, E)
    out = pl.pallas_call(
        _kernel,
        out_shape=jax.ShapeDtypeStruct((NSEG // 4, 4, SEG, 2 * D), bf16),
        in_specs=[hbm] * 13,
        out_specs=hbm,
        scratch_shapes=[
            pltpu.VMEM((NRAW, D // 2, 2, 16, E), bf16),
            pltpu.VMEM((6, 16 * WP, E), u32),
            pltpu.VMEM((8, H * E, 128), bf16),
            pltpu.VMEM((NSEG, SEG - M, D), bf16),
            pltpu.VMEM((M, D), bf16),
            pltpu.VMEM((NSEG, M, D), bf16),
            pltpu.VMEM((7, 4, 256, 128), bf16),
            pltpu.VMEM((49, 2, 128, 128), bf16),
            pltpu.VMEM((48, NSEG, 2 * M, E), bf16),
            pltpu.VMEM((49, 8, NSEG * M // 4, E), bf16),
            pltpu.VMEM((NSEG // 4, 4, SEG, D), bf16),
            pltpu.VMEM((96, 80), f32),
            pltpu.VMEM((8, NSEG // 4, 4, SEG, 128), bf16),
            pltpu.VMEM((2, 16, 512, 128), bf16),
            pltpu.VMEM((2, 1, S), bf16),
            pltpu.VMEM(gf.shape, u32),
            pltpu.VMEM(gi.shape, u32),
            pltpu.VMEM(tw.shape, f32),
            pltpu.VMEM((8, 16 * XP, 128), f32),
            pltpu.VMEM((2, 16, 65, 8, 128), f32),
            pltpu.SemaphoreType.DMA((7,)),
        ],
        compiler_params=pltpu.CompilerParams(vmem_limit_bytes=120 * 1024 * 1024),
    )(A_x.reshape(NSEG, SEG, D), A_mem0.reshape(M, D),
      A_Wq.reshape(wshape), A_Wk.reshape(wshape), A_Wv.reshape(wshape),
      A_Wo.reshape(H * E, D), B_x.reshape(NSEG // 4, 4, SEG, D), B_w_r.T, B_w_i.T, gf, gi, tw, fill)
    return out.reshape(1, S, 2 * D)
```

```python
import functools

import jax
import jax.numpy as jnp
import numpy as np
from jax import lax
from jax.experimental import pallas as pl
from jax.experimental.pallas import tpu as pltpu

S, D, H, E, M, SEG = 2048, 1024, 32, 128, 8, 32
NSEG = S // SEG
WP = 516
XP = 132
NRAW = 4
UNROLL = 4
P0 = 6
NZ = 16
R2 = 256
M0 = 8
L1 = 74
L2 = 150
LEFT_AT = ((), (2,), (4,), (0, 1, 3, 5, 6))
EARLY = ((0, 0, 0), (0, 0, 1), (1, 0, 0), (1, 0, 1), (0, 1, 0))
bf16, f32, u32 = jnp.bfloat16, jnp.float32, jnp.uint32
RES = ((0, 4), (2, 6), (1, 7), (3, 5))
RC = float(np.sqrt(0.5))


def _fwd8(x):
    s04, d04 = x[0] + x[4], x[0] - x[4]
    s26, d26 = x[2] + x[6], x[2] - x[6]
    s15, d15 = x[1] + x[5], x[1] - x[5]
    s37, d37 = x[3] + x[7], x[3] - x[7]
    t1, t2 = (d15 - d37) * RC, (d15 + d37) * RC
    e0, o0 = s04 + s26, s15 + s37
    return [e0 + o0, e0 - o0, s04 - s26, s15 - s37, d04 + t1, d26 + t2, d04 - t1, d26 - t2]


def _inv8(z):
    z0, z4, e1, o1, r1, i1, r3, i3 = z
    e0, o0 = z0 + z4, z0 - z4
    s04, s26, s15, s37 = e0 + e1, e0 - e1, o0 + o1, o0 - o1
    d04, d26 = r1 + r3, i1 + i3
    t1, t2 = (r1 - r3) * RC, (i1 - i3) * RC
    d15, d37 = t1 + t2, t2 - t1
    return [s04 + d04, s15 + d15, s26 + d26, s37 + d37, s04 - d04, s15 - d15, s26 - d26, s37 - d37]


def _twiddle16(z, k):
    re, im = z
    k = k % 16
    if k == 0:
        return z
    if k == 4:
        return (im, -re)
    if k == 12:
        return (-im, re)
    if k == 2:
        return ((re + im) * RC, (im - re) * RC)
    if k == 14:
        return ((re - im) * RC, (re + im) * RC)
    if k == 6:
        return ((im - re) * RC, (re + im) * -RC)
    if k == 10:
        return ((re + im) * -RC, (re - im) * RC)
    c, s = float(np.cos(2 * np.pi * k / 16)), float(-np.sin(2 * np.pi * k / 16))
    return (re * c - im * s, re * s + im * c)


def _bfly4(z, sign):
    (ar, ai), (br, bi), (cr, ci), (dr, di) = z
    sr, si, tr, ti = ar + cr, ai + ci, ar - cr, ai - ci
    ur, ui, vr, vi = br + dr, bi + di, br - dr, bi - di
    o0, o2 = (sr + ur, si + ui), (sr - ur, si - ui)
    p, q = (tr + vi, ti - vr), (tr - vi, ti + vr)
    return [o0, p, o2, q] if sign > 0 else [o0, q, o2, p]


class _Pacer:
    def __init__(self, tasks, ntokens):
        self.slots = {}
        for n, task in enumerate(tasks):
            self.slots.setdefault(n * ntokens // len(tasks), []).append(task)
        self.pos = 0

    def feed(self, r):
        for j in range(r.shape[0] // 8):
            for task in self.slots.pop(self.pos, []):
                task(pltpu.bitcast(r[8 * j:8 * j + 8], u32))
            self.pos += 1

    def done(self):
        assert not self.slots


def _pack_rows(m):
    b = np.asarray(m, np.float32).astype(jnp.bfloat16).view(np.uint16).astype(np.uint32)
    return b[..., 0::2, :] | (b[..., 1::2, :] << 16)


def _dft_constants():
    i, j = np.arange(64)[:, None], np.arange(128)
    whole, half = 2 * np.pi * i * j / 128, 2 * np.pi * (i + 0.5) * j / 128
    gf = np.zeros((3, 192, 128))
    gf[0, :129] = np.concatenate([np.cos(whole), -np.sin(whole), [(-1.0) ** j]])
    gf[1, :128] = np.concatenate([np.cos(half), -np.sin(half)])
    gf[2, :128] = np.concatenate([np.cos(half), np.sin(half)])
    gi = gf[0:2, :128] * (2.0 / (D * S))
    gi[0, 0], gi[0, 64] = gf[0, 0] / (D * S), gf[0, 128] / (D * S)
    angs = [2 * np.pi * j * (b - 8) / S for b in range(16)] + [2 * np.pi * j * (r - 4) / D for r, _ in RES]
    tw = np.zeros((20, 2, 8, 128), np.float32)
    for n, ang in enumerate(angs):
        tw[n, 0], tw[n, 1] = np.cos(ang), -np.sin(ang)
    return _pack_rows(gf), _pack_rows(gi), tw


def _attn_fill():
    head = np.concatenate([np.arange(64) // 32, np.arange(16) // 8])
    pos = np.concatenate([np.arange(64) % 32, 32 + np.arange(16) % 8])
    ok = (pos[:, None] < M) | (pos[:, None] >= pos[None, :])
    fill = np.where(ok, 0.0, -1e9)
    fill = np.where(head[:, None] == head[None, :], fill, -np.inf)
    return fill.astype(np.float32)


def _strassen(prod, b11, b12, b21, b22, add, sub, emit):
    m2 = prod(1, b11())
    m1 = prod(0, add(b11(), b22()))
    m3 = prod(2, sub(b12(), b22()))
    c22 = prod(5, add(b11(), b12())) + ((m1 - m2) + m3)
    m4 = prod(3, sub(b21(), b11()))
    emit(1, m2 + m4, c22)
    m5 = prod(4, b22())
    emit(0, prod(6, add(b21(), b22())) + ((m1 + m4) - m5), m3 + m5)


class _Blocks(list):
    def __add__(self, other):
        return _Blocks(a + b for a, b in zip(self, other))

    def __sub__(self, other):
        return _Blocks(a - b for a, b in zip(self, other))


def _strassen_left(a11, a12, a21, a22):
    return [a11 + a22, a21 + a22, a11, a22, a11 + a12, a21 - a11, a12 - a22]


def _strassen_left_one(i, blk):
    terms = ((0, 3, 1), (2, 3, 1), (0,), (3,), (0, 1, 1), (2, 0, -1), (1, 3, -1))[i]
    a = blk(*divmod(terms[0], 2))
    if len(terms) == 1:
        return a
    b = blk(*divmod(terms[1], 2))
    return a + b if terms[2] > 0 else a - b


def _kernel(x_hbm, mem_hbm, wq_hbm, wk_hbm, wv_hbm, wo_hbm, bx_hbm, wr_hbm, wi_hbm,
            gf_hbm, gi_hbm, tw_hbm, fill_hbm, out_hbm,
            wraw, wall, wo, xbuf, mem0, x8, xs, xs2, pre, osum, outbuf, fill_ref,
            xb, wt, wl, gf, gi, tw, xd, yb, sems):
    def start(src, dst, sem):
        c = pltpu.make_async_copy(src, dst, sems.at[sem])
        c.start()
        return c

    def wait_all(cs):
        for c in cs:
            c.wait()

    dot = functools.partial(jnp.dot, preferred_element_type=f32)
    dot_nt = lambda a, b: lax.dot_general(a, b, (((1,), (1,)), ((), ())), preferred_element_type=f32)
    cat = lambda *vs: jnp.concatenate(vs, axis=0)
    as_bf16 = lambda w: pltpu.bitcast(w, bf16)
    hi_f32 = lambda w: pltpu.bitcast(w & u32(0xFFFF0000), f32)
    all_ones = lambda tok: ((tok >> 16) | u32(0xFFFF)) | u32(0xFFFF0000)
    after = lambda v, tok: pltpu.bitcast(pltpu.bitcast(v, u32) & all_ones(tok), f32)
    widen = lambda w: as_bf16(w).astype(f32) if w.dtype == u32 else w
    narrow = lambda w: as_bf16(w) if w.dtype == u32 else w.astype(bf16)
    add2 = lambda a, b: widen(a) + widen(b)
    sub2 = lambda a, b: widen(a) - widen(b)
    w_hbm = (wq_hbm, wk_hbm, wv_hbm)

    def start_unit(u):
        return start(w_hbm[u // 2].at[:, :, u % 2], wraw.at[u % NRAW], u % NRAW)

    def start_x(seg0, nseg, sem):
        segs, rows = pl.ds(seg0, nseg), pl.ds(0, SEG - M)
        return start(x_hbm.at[segs, rows, :], xbuf.at[segs], sem)

    def start_filter(row0, nrows, sem):
        rows = pl.ds(row0, nrows)
        return [start(w.at[rows, pl.ds(128 * d, 128)], wt.at[t, d, rows], sem)
                for t, w in enumerate((wr_hbm, wi_hbm)) for d in range(16)]

    def start_piece(n, xsem, parts):
        cols = pl.ds(256 * n, 256)
        cs = [start(x_hbm.at[:, pl.ds(SEG - M, M), cols], x8.at[:, :, cols], xsem)]
        for k, sem in enumerate(parts):
            rows = pl.ds(128 * n + 128 // len(parts) * k, 128 // len(parts))
            cs.append(start(wq_hbm.at[rows, :, 0], wraw.at[0, rows], sem))
        return cs
    c_a = [start_piece(0, 5, (6, 0))] + [start_piece(n, n, (n,)) for n in range(1, 4)]

    xb32 = xb.bitcast(u32)

    head_of = lambda slot: slot // 16 * 16 + slot % 8 * 2 + slot % 16 // 8

    def relayout_tasks(u, r0=0, r1=D // 2, pars=(0, 1)):
        src, dst = wraw.at[u % NRAW], wall.at[u]
        step = 4 // len(pars)

        def make(rows):
            def task(tok):
                lo = (tok >> 16) | u32(0xFFFF)
                hi = (tok << 16) | u32(0xFFFF0000)
                for r in rows:
                    a, b = src.at[r].bitcast(u32)[...]
                    for par in pars:
                        dst[pl.ds(r + 8 * WP * par, 8, stride=WP), :] = (
                            (a >> 16) | (b & hi) if par else (a & lo) | (b << 16))
            return task
        return [make(range(r, r + step)) for r in range(r0, r1, step)]

    def y_blocks(r):
        return pl.ds(4 * (r % 2) + r // 2, 8, stride=8)

    def filter_tasks(blk, wfn):
        def make(phase, k):
            slots = [4 * k + j for j in range(4)] if phase == 1 else [4 * j + k for j in range(4)]

            def task(tok):
                z = [(yb[0, b, blk], yb[1, b, blk]) for b in slots]
                if phase == 0:
                    z = [(after(zr, tok), zi) for zr, zi in z]
                    z = [(zr * tw[b, 0] - zi * tw[b, 1], zr * tw[b, 1] + zi * tw[b, 0]) if b != 8 else (zr, zi)
                         for b, (zr, zi) in zip(slots, z)]
                else:
                    z[0] = tuple(after(v, tok) for v in z[0])
                if phase == 0:
                    o = _bfly4(z, 1)
                    o = [_twiddle16(o[j], k * j) for j in range(4)]
                elif phase == 1:
                    o = _bfly4(z, 1)
                    y = []
                    for j in range(4):
                        wr, wi = wfn(k + 4 * j)
                        xr, xi = o[j]
                        y.append((xr * wr - xi * wi, xr * wi + xi * wr))
                    o = _bfly4(y, -1)
                    o = [_twiddle16(o[j], -k * j) for j in range(4)]
                else:
                    o = [(zr * tw[b, 0] + zi * tw[b, 1], zi * tw[b, 0] - zr * tw[b, 1]) if b != 8 else (zr, zi)
                         for b, (zr, zi) in zip(slots, _bfly4(z, -1))]
                for b, v in zip(slots, o):
                    yb[0, b, blk] = v[0]
                    yb[1, b, blk] = v[1]
            return task
        return [make(phase, k) for phase in range(3) for k in range(4)]

    mirror = lambda a: a if a < 64 else 191 - a

    def twiddle_d(g, x, y):
        c, sn = [jnp.tile(tw[16 + g, k], (x.shape[0] // 8, 1)) for k in range(2)]
        return (x * c - y * sn, x * sn + y * c) if g == 3 else (x * c + y * sn, x * sn - y * c)

    def butterfly_tasks():
        def make(a, par):
            def task(tok):
                w = [xb32[j, a // 8, a // 2 % 4, pl.ds(8 * (a % 2), 8), :] for j in range(8)]
                if par:
                    hi = (tok << 16) | u32(0xFFFF0000)
                    z = _fwd8([pltpu.bitcast(v & hi, f32) for v in w])
                else:
                    sixteen = ((tok >> 31) | u32(1)) << 4
                    z = _fwd8([pltpu.bitcast(v << sixteen, f32) for v in w])
                for n in range(8):
                    xd[n, pl.ds(8 * XP * par + mirror(a), 8, stride=XP), :] = z[n]
            return task
        return [make(a, par) for a in range(128) for par in range(2)]

    low = lax.broadcasted_iota(jnp.int32, (1, 128), 1) < 64

    def b_dfwd(b, g):
        z = [xd[n, pl.ds(XP * (b // 2 + 8 * (b % 2)), 128), :] for n in (2 * g, 2 * g + 1)]
        if g:
            z = twiddle_d(g, *z)
        z = [cat(v[0:64] + v[64:128], v[0:64] - v[64:128]).astype(bf16) for v in z]
        tu = dot_nt(as_bf16(gf[1, 0:64] if g else gf[0, 0:72]), z[0])
        tv = dot_nt(as_bf16(gf[1, 0:64]), z[1])
        if g == 0:
            tr = cat(tu[0:64], tv[0:64], tu[128:144])
            ti = cat(tu[64:128], tv[64:128], jnp.zeros((16, 128), f32))
        else:
            tr = cat(tu[0:64] - tv[64:128], tu[0:64] + tv[64:128])
            ti = cat(tu[64:128] + tv[0:64], tu[64:128] - tv[0:64])
        return jnp.where(low, tr, ti).astype(bf16), jnp.where(low, ti, tr).astype(bf16)

    def b_sfwd(b, g, ts):
        for c in range(2):
            y = dot(ts[c], as_bf16(gf[2 - c, 0:64]))
            for q in range(2):
                yb[c, b, y_blocks(RES[g][q])] = y[64 * q:64 * q + 64].reshape(8, 8, 128)
            if g == 0:
                yb[c, b, 64] = y[128:136]

    def b_stage1():
        pend = []
        for b in list(range(0, 16, 2)) + list(range(1, 16, 2)):
            for g in range(4):
                pend.append((b, g, b_dfwd(b, g)))
                if len(pend) > 3:
                    b_sfwd(*pend.pop(0))
        for item in pend:
            b_sfwd(*item)

    def b_sinv(tasks):
        row0 = lax.broadcasted_iota(jnp.int32, (8, 128), 0) == 0
        pacer = _Pacer(tasks, 12 * 8)
        for _, b, g in sorted((b + (6 if g == 0 else 0), b, g) for b in range(16) for g in range(4)):
            (ar, br), (ai, bi) = [[yb[c, b, y_blocks(r)].reshape(64, 128) for r in RES[g]] for c in range(2)]
            if g:
                uv = [(ar + br, ai + bi, -ar - br), (ai - bi, br - ar, bi - ai)]
                uv = [(cat(re, im), cat(im, neg)) for re, im, neg in uv]
            else:
                pacer.done()
                na = -ar
                uv = [(cat(ar, jnp.where(row0, yb[0, b, 64], ai[0:8]), ai[8:]),
                       cat(ai, jnp.where(row0, yb[1, b, 64], na[0:8]), na[8:])),
                      (cat(br, bi), cat(bi, -br))]
            for q, (u, v) in enumerate(uv):
                cu = dot_nt(as_bf16(gf[2, 0:32]), u.astype(bf16))
                sv = dot_nt(as_bf16(gf[2, 32:64]), v.astype(bf16))
                xd[2 * g + q, pl.ds(XP * b, 128), :] = cat(cu - sv, cu + sv)
            pacer.feed(cu)

    def b_dinv(t):
        rows = lambda j: cat(*[xd[j, pl.ds(mirror(a), 16, stride=XP), :] for a in range(8 * t, 8 * t + 8)])
        z = [dot(rows(j).astype(bf16), as_bf16(gi[min(j, 1)])) for j in range(8)]
        for g in range(1, 4):
            u, v = z[2 * g], z[2 * g + 1]
            c, sn = [jnp.tile(tw[16 + g, k], (16, 1)) for k in range(2)]
            z[2 * g] = u * c + v * sn
            z[2 * g + 1] = v * c - u * sn if g == 3 else u * sn - v * c
        y = _inv8(z)
        for j in range(8):
            xb[j, t] = y[j].reshape(4, SEG, 128).astype(bf16)

    HALF = NSEG * M // 2
    pre32 = pre.bitcast(u32)

    def store_pre(pair, row0, cs, packed):
        n = cs[0].shape[0] // M
        segs = pl.ds(row0 // M, n)
        if packed:
            st = jnp.concatenate([c.reshape(n, M, E) for c in cs], axis=1)
            pre32[pair, segs] = pltpu.bitcast(st.reshape(2 * M * n, E).astype(bf16), u32).reshape(n, M, E)
        else:
            for t, c in enumerate(cs):
                pre[pair, segs, pl.ds(M * t, M), :] = c.reshape(n, M, E).astype(bf16)

    def batch(u, p0, p1, tasks=(), t0=0, t1=4, margin=4):
        mc = HALF // 2 if t1 == 1 else HALF
        pacer = _Pacer(tasks, (7 * (p1 - p0) - margin // (t1 - t0)) * HALF // 8)
        w = wall.at[u]
        for p in range(p0, p1):
            for r0 in range(0, HALF, mc):
                def blk(head, par):
                    return lambda: cat(*[w[pl.ds((2 * p + head) * WP + 64 * (2 * t + par), 64), :]
                                         for t in range(t0, t1)])

                def prod(i, b):
                    lhs = jnp.concatenate([as_bf16(xs32[i, t, pl.ds(r0 // 2, mc // 2), :])
                                           for t in range(t0, t1)], axis=1)
                    r = dot(lhs, narrow(b))
                    pacer.feed(r)
                    return r

                def emit(half, *cs):
                    park = pl.ds((half * HALF + r0) // 8, mc // 8)
                    if t0 > 0:
                        cs = [c + yb[t, p, park].reshape(mc, E) for t, c in enumerate(cs)]
                    if t1 < 4:
                        for t, c in enumerate(cs):
                            yb[t, p, park] = c.reshape(mc // 8, 8, E)
                    else:
                        store_pre(8 * u + p, half * HALF + r0, cs, False)
                if t0 // (t1 - t0) % 2:
                    _strassen(prod, blk(1, 0), blk(0, 0), blk(1, 1), blk(0, 1), add2, sub2,
                              lambda half, c1, c0: emit(half, c0, c1))
                else:
                    _strassen(prod, blk(0, 0), blk(1, 0), blk(0, 1), blk(1, 1), add2, sub2, emit)
        pacer.done()

    QUART = HALF // 2
    xs32, xs2_32 = xs.bitcast(u32), xs2.bitcast(u32)

    def strassen2(right, left, emit, pacer):
        def outer_prod(i, bs):
            def prod(j, b):
                r = dot(left(7 * i + j), narrow(b))
                pacer.feed(r)
                return r
            order = (1, 0, 3, 2) if i in (1, 4, 5, 6) else (0, 1, 2, 3)
            cs = {}
            _strassen(prod, *[(lambda b=bs[k]: b) for k in order], add2, sub2, lambda half, *c: cs.update({half: c}))
            return _Blocks((cs[0] + cs[1])[k] for k in order)

        def outer_emit(half, *cs):
            for col in (1, 0):
                for a in range(2):
                    emit(2 * half + a, 2 * col, cs[col][2 * a], cs[col][2 * a + 1])
        outer = lambda k, c: lambda: [right(2 * k + k2, 2 * c + c2) for k2 in range(2) for c2 in range(2)]
        _strassen(outer_prod, outer(0, 0), outer(0, 1), outer(1, 0), outer(1, 1),
                  lambda x, y: [add2(a, b) for a, b in zip(x, y)],
                  lambda x, y: [sub2(a, b) for a, b in zip(x, y)], outer_emit)

    def batch2(u, q0, q1, tasks=()):
        pacer = _Pacer(tasks, (49 * (q1 - q0) - 12) * QUART // 8)
        w = wall.at[u]
        for q in range(q0, q1):
            def emit(row, col, *cs):
                store_pre(8 * u + 2 * q + col // 2, row * QUART, cs, True)
            strassen2(lambda k, c: cat(*[w[pl.ds((4 * q + c) * WP + 64 * (k + 4 * t), 64), :]
                                         for t in range(2)]),
                      lambda i: jnp.concatenate([as_bf16(xs2_32[i, t]) for t in range(2)], axis=1),
                      emit, pacer)
        pacer.done()

    def left2_tasks():
        def make(i, t, r):
            def task(tok):
                a = _strassen_left_one(i, lambda rh, kh: _Blocks(
                    x8[32 * rh + 16 * rl + r, :, pl.ds(128 * (2 * kh + kl + 4 * t), 128)].astype(f32)
                    for rl in range(2) for kl in range(2)))
                a[0], a[3] = after(a[0], tok), after(a[3], tok)
                for j, v in enumerate(_strassen_left(*a)):
                    xs2[7 * i + j, t, pl.ds(M * r, M), :] = v.astype(bf16)
            return task
        return [make(i, t, r) for i in range(7) for t in range(2) for r in range(16)]

    def left_tasks(n):
        def make(r):
            def task(tok):
                a = [x8[NSEG // 2 * h + r, :, pl.ds(256 * n + 128 * k, 128)].astype(f32)
                     for h in range(2) for k in range(2)]
                a[0], a[3] = after(a[0], tok), after(a[3], tok)
                for i, v in enumerate(_strassen_left(*a)):
                    xs[i, n, pl.ds(M * r, M), :] = v.astype(bf16)
            return task
        return [make(r) for r in range(NSEG // 2)]

    def piece_tasks(n):
        return [t for both in zip(relayout_tasks(0, 128 * n, 128 * n + 128, (0,)), left_tasks(n)) for t in both]

    def mix(a, b):
        keyed = [(n / len(a), 0, n) for n in range(len(a))] + [(n / len(b), 1, n) for n in range(len(b))]
        return [(a, b)[w][n] for _, w, n in sorted(keyed)]

    run_now = lambda tasks: [task(jnp.zeros((8, 128), u32)) for task in tasks]

    pre32[0:NZ] = jnp.zeros((NZ, NSEG, M, E), u32)
    c_a[0][0].wait()
    run_now(left_tasks(0))
    c_a[0][1].wait()
    run_now(relayout_tasks(0, 0, 64))
    c_a[0][2].wait()
    run_now(relayout_tasks(0, 64, 128, (0,)))
    batch(0, 0, 4, relayout_tasks(0, 64, 128, (1,)), 0, 1, M0)
    batch(0, 4, P0, (), 0, 1)
    wait_all(c_a[1])
    c_h = [start(wq_hbm.at[pl.ds(256 * n, 256), :, 1], wraw.at[1, pl.ds(256 * n, 256)], n) for n in range(2)]
    batch(0, P0, 8, piece_tasks(1), 0, 1)
    batch(0, 0, 4, relayout_tasks(0, 128, 256, (1,)), 1, 2)
    wait_all(c_a[2])
    batch(0, 4, 8, piece_tasks(2), 1, 2)
    batch(0, 0, 4, relayout_tasks(0, 256, 384, (1,)), 2, 3)
    wait_all(c_a[3])
    c_w2 = start_unit(2)
    batch(0, 4, 8, piece_tasks(3), 2, 3)
    batch(0, 0, 4, relayout_tasks(0, 384, 512, (1,)), 3, 4)
    c_h[0].wait()
    left2 = left2_tasks()
    batch(0, 4, 8, relayout_tasks(1, 0, 256, (0,)), 3, 4)
    batch(1, 0, 4, mix(relayout_tasks(1, 0, 256, (1,)), left2[:L1]), 0, 2)
    c_h[1].wait()
    start_unit(3)
    batch(1, 4, 8, mix(relayout_tasks(1, 256, 512, (0,)), left2[L1:L2]), 0, 2)
    batch(1, 0, 4, mix(relayout_tasks(1, 256, 512, (1,)), left2[L2:]), 2, 4)
    c_w2.wait()
    start_unit(4)
    start_unit(5)
    c_b1 = [start(bx_hbm.at[:, :, :, pl.ds(128 * j, 128)], xb.at[j], 5) for j in range(8)]
    c_b1 += [start(gf_hbm, gf, 5), start(tw_hbm, tw, 5)]
    c_loop = [start(wo_hbm.at[:, pl.ds(128 * j, 128)], wo.at[j], 4) for j in range(8)]
    c_loop += [start_x(0, UNROLL, 4), start(mem_hbm, mem0, 4), start(fill_hbm, fill_ref.at[pl.ds(0, 80)], 4)]
    c_loop += start_filter(0, 64, 4)
    batch(1, 4, 8, mix(relayout_tasks(2, pars=(0,)), relayout_tasks(2, 0, R2, (1,))), 2, 4)
    batch2(2, 0, 2, relayout_tasks(2, R2, 512, (1,)))

    def unit_body(u, c):
        slot = (u + 1) % NRAW
        pltpu.make_async_copy(wraw.at[slot], wraw.at[slot], sems.at[slot]).wait()
        batch2(u, 2, 4, relayout_tasks(u + 1, pars=(0,)))
        batch2(u + 1, 0, 2, relayout_tasks(u + 1, pars=(1,)))
        return c
    lax.fori_loop(2, 5, unit_body, 0)
    wait_all(c_b1)
    batch(5, 6, 8, butterfly_tasks(), margin=0)
    batch2(5, 2, 3)
    b_stage1()
    wait_all(c_loop)
    c_rest = [start_x(UNROLL, NSEG - UNROLL, 6)] + start_filter(64, 448, 6)
    c_b3 = [start(w.at[pl.ds(512, 1), :], wl.at[t], 5) for t, w in enumerate((wr_hbm, wi_hbm))]
    c_b3 += [start(gi_hbm, gi, 5)]

    wo32 = wo.bitcast(u32)
    scale = E ** -0.5

    def gated(w, toks):
        if not toks:
            return w
        bits = functools.reduce(
            jnp.bitwise_or, [pltpu.bitcast(jnp.broadcast_to(t, (8, 128)), u32) for t in toks])
        return cat(w[0:8] & all_ones(bits), w[8:])

    def wqkv(i, p, second, toks=(), k0=0, k1=D):
        rows = pl.ds((p % 8 * 2 + second) * WP + k0 // 2, (k1 - k0) // 2)
        return as_bf16(gated(wall[2 * i + p // 8, rows, :], toks))

    def step(n, u, mem, held):
        s = UNROLL * n + u
        rows = cat(mem, xbuf[s].astype(f32))
        lhs = rows.astype(bf16)
        head_start = {}
        if u:
            lo, hi = rows[:, :D // 2].astype(bf16), rows[:, D // 2:].astype(bf16)
            for key in EARLY:
                head_start[key] = dot(lo, wqkv(*key, k1=D // 2))
        fill = fill_ref[pl.ds(0, 80), :]
        heads = [None] * H
        rs = []

        shift = jnp.full((8, 128), 16 - 16 * (n % 2), jnp.int32).astype(u32)
        wblk = pl.ds(pl.multiple_of(64 * (n // 2), 64), 64)
        flt = filter_tasks(
            s, lambda d: [hi_f32(wt.at[t, d, wblk].bitcast(u32)[pl.ds(u, 8, stride=4), :] << shift) for t in range(2)])
        pacer = _Pacer(flt, 84)

        def proj(i, p, toks=()):
            a, b = [
                dot(hi, wqkv(i, p, t, k0=D // 2)) + head_start[i, p, t] if (i, p, t) in head_start
                else dot(lhs, wqkv(i, p, t, toks[t * len(toks) // 2:(t + 1) * len(toks) // 2]))
                for t in range(2)]
            pacer.feed(a)
            pacer.feed(b)
            c = widen(pre32[16 * i + p, s])
            return cat(a, b, c).astype(bf16)

        def probs(q, k):
            sc = dot_nt(q, k) * scale
            sc = jnp.where(fill == 0.0, sc, fill)
            e = jnp.exp(sc - jnp.max(sc, axis=1, keepdims=True))
            l = jnp.sum(e, axis=1, keepdims=True)
            r = pl.reciprocal(l, approx=True)
            r = r * (2.0 - l * r)
            rs.append([r[8 * j:8 * j + 8] for j in range(10)])
            return (e * r).astype(bf16)

        def pv(p, pr, v):
            o = dot(pr, v)
            heads[2 * p] = cat(o[0:8], o[16:32], o[64:72])
            heads[2 * p + 1] = cat(o[32:40], o[48:64], o[72:80])
            held[u, 2 * p], held[u, 2 * p + 1] = o[8:16], o[40:48]

        def left_task(q, i):
            def task(tok):
                a = _strassen_left_one(i, lambda r, k: _Blocks(
                    held[2 * r + r2, 4 * q + 2 * k + k2] for r2 in range(2) for k2 in range(2)))
                a[0], a[3] = after(a[0], tok), after(a[3], tok)
                for j, v in enumerate(_strassen_left(*a)):
                    osum[7 * i + j, q, pl.ds(pl.multiple_of(M * n, M), M), :] = v.astype(bf16)
            return task

        pend = []
        for g in range(4):
            ps = range(4 * g, 4 * g + 4)
            qk = [(proj(0, p), proj(1, p)) for p in ps]
            vs = [proj(2, p, rs[p - 4] if g else ()) for p in ps]
            for a in pend:
                pv(*a)
            pend = [(p, probs(*qk[t]), vs[t]) for t, p in enumerate(ps)]
        pacer.done()

        def wo_part(oc, j, h0, h1, toks=()):
            w = cat(*[wo32[j, pl.ds(64 * head_of(h), 64), :] for h in range(h0, h1)])
            return dot(oc, as_bf16(gated(w, toks)))

        acc = []
        pacer = _Pacer([left_task(q, i) for q in range(8) for i in LEFT_AT[u]], 38)
        oc = jnp.concatenate(heads[0:24], axis=1).astype(bf16)
        for j in range(8):
            acc.append(wo_part(oc, j, 0, 24, {3: rs[12] + rs[13], 4: rs[14] + rs[15]}.get(j, ())))
            if j == 4:
                for a in pend:
                    pv(*a)
            if j >= 5:
                pacer.feed(acc[j])
        oc = jnp.concatenate(heads[24:32], axis=1).astype(bf16)
        nxt = []
        for j in range(8):
            r = wo_part(oc, j, 24, 32) + acc[j]
            outbuf[n, u, pl.ds(M, SEG - M), pl.ds(128 * j, 128)] = r[M:].astype(bf16)
            nxt.append(r[0:M])
            pacer.feed(r)
        pacer.done()
        return jnp.concatenate(nxt, axis=1)

    def steps(n, mem):
        pl.when(n == 1)(functools.partial(wait_all, c_rest))
        held = {}
        for u in range(UNROLL):
            mem = step(n, u, mem, held)
        return mem
    lax.fori_loop(0, NSEG // UNROLL, steps, mem0[...].astype(f32))
    tok_rows = pl.ds(M, SEG - M)
    c_out = [start(outbuf.at[:, :, tok_rows, :], out_hbm.at[:, :, tok_rows, pl.ds(0, D)], 0)]

    wait_all(c_b3)
    b_sinv(filter_tasks(64, lambda d: [wl[t, :, pl.ds(128 * d, 128)].astype(f32) for t in range(2)]))
    for t in range(16):
        b_dinv(t)
    c_out += [start(xb.at[j], out_hbm.at[:, :, :, pl.ds(D + 128 * j, 128)], 0) for j in range(8)]

    osum32 = osum.bitcast(u32)
    for cq in range(2):
        def emit(row, col, *cs):
            for t, c in enumerate(cs):
                outbuf[:, row, pl.ds(0, M), pl.ds(128 * (4 * cq + col + t), 128)] = (
                    c.reshape(NSEG // 4, M, 128).astype(bf16))
            idx = (slice(None), row, pl.ds(0, M), pl.ds(128 * (4 * cq + col), 256))
            c_out.append(start(outbuf.at[idx], out_hbm.at[idx], 0))
        strassen2(lambda k, c: cat(*[wo32[4 * cq + c, pl.ds(64 * head_of(4 * q + k), 64), :] for q in range(8)]),
                  lambda i: jnp.concatenate([as_bf16(osum32[i, q]) for q in range(8)], axis=1),
                  emit, _Pacer((), 0))
    wait_all(c_out)


@jax.jit
def pallas_concat_heads__memory_aug_recurrent_mem_tr__spectral_gfnet__prompt_kernel(
    A_x: jax.Array,
    A_mem0: jax.Array,
    A_Wq: jax.Array,
    A_Wk: jax.Array,
    A_Wv: jax.Array,
    A_Wo: jax.Array,
    A_seg_len: jax.Array,
    B_x: jax.Array,
    B_w_r: jax.Array,
    B_w_i: jax.Array,
):
    del A_seg_len
    assert A_x.shape == (1, S, D) and A_mem0.shape == (1, M, D) and B_x.shape == (1, S, D)
    assert A_Wq.shape == (D, H, E) and A_Wo.shape == (H, E, D) and B_w_r.shape == (S, D // 2 + 1)
    gf, gi, tw = _dft_constants()
    fill = _attn_fill()
    hbm = pl.BlockSpec(memory_space=pltpu.HBM)
    wshape = (D // 2, 2, 2, 16, E)
    out = pl.pallas_call(
        _kernel,
        out_shape=jax.ShapeDtypeStruct((NSEG // 4, 4, SEG, 2 * D), bf16),
        in_specs=[hbm] * 13,
        out_specs=hbm,
        scratch_shapes=[
            pltpu.VMEM((NRAW, D // 2, 2, 16, E), bf16),
            pltpu.VMEM((6, 16 * WP, E), u32),
            pltpu.VMEM((8, H * E, 128), bf16),
            pltpu.VMEM((NSEG, SEG - M, D), bf16),
            pltpu.VMEM((M, D), bf16),
            pltpu.VMEM((NSEG, M, D), bf16),
            pltpu.VMEM((7, 4, 256, 128), bf16),
            pltpu.VMEM((49, 2, 128, 128), bf16),
            pltpu.VMEM((48, NSEG, 2 * M, E), bf16),
            pltpu.VMEM((49, 8, NSEG * M // 4, E), bf16),
            pltpu.VMEM((NSEG // 4, 4, SEG, D), bf16),
            pltpu.VMEM((96, 80), f32),
            pltpu.VMEM((8, NSEG // 4, 4, SEG, 128), bf16),
            pltpu.VMEM((2, 16, 512, 128), bf16),
            pltpu.VMEM((2, 1, S), bf16),
            pltpu.VMEM(gf.shape, u32),
            pltpu.VMEM(gi.shape, u32),
            pltpu.VMEM(tw.shape, f32),
            pltpu.VMEM((8, 16 * XP, 128), f32),
            pltpu.VMEM((2, 16, 65, 8, 128), f32),
            pltpu.SemaphoreType.DMA((7,)),
        ],
        compiler_params=pltpu.CompilerParams(vmem_limit_bytes=120 * 1024 * 1024),
    )(A_x.reshape(NSEG, SEG, D), A_mem0.reshape(M, D),
      A_Wq.reshape(wshape), A_Wk.reshape(wshape), A_Wv.reshape(wshape),
      A_Wo.reshape(H * E, D), B_x.reshape(NSEG // 4, 4, SEG, D), B_w_r.T, B_w_i.T, gf, gi, tw, fill)
    return out.reshape(1, S, 2 * D)
```

```python
import functools

import jax
import jax.numpy as jnp
import numpy as np
from jax import lax
from jax.experimental import pallas as pl
from jax.experimental.pallas import tpu as pltpu

S, D, H, E, M, SEG = 2048, 1024, 32, 128, 8, 32
NSEG = S // SEG
WP = 516
XP = 132
NRAW = 4
UNROLL = 4
LEFT_AT = ((), (2,), (4,), (0, 1, 3, 5, 6))
EARLY = ((0, 0, 0), (0, 0, 1), (1, 0, 0), (1, 0, 1), (0, 1, 0))
bf16, f32, u32 = jnp.bfloat16, jnp.float32, jnp.uint32
RES = ((0, 4), (2, 6), (1, 7), (3, 5))
RC = float(np.sqrt(0.5))


def _fwd8(x):
    s04, d04 = x[0] + x[4], x[0] - x[4]
    s26, d26 = x[2] + x[6], x[2] - x[6]
    s15, d15 = x[1] + x[5], x[1] - x[5]
    s37, d37 = x[3] + x[7], x[3] - x[7]
    t1, t2 = (d15 - d37) * RC, (d15 + d37) * RC
    e0, o0 = s04 + s26, s15 + s37
    return [e0 + o0, e0 - o0, s04 - s26, s15 - s37, d04 + t1, d26 + t2, d04 - t1, d26 - t2]


def _inv8(z):
    z0, z4, e1, o1, r1, i1, r3, i3 = z
    e0, o0 = z0 + z4, z0 - z4
    s04, s26, s15, s37 = e0 + e1, e0 - e1, o0 + o1, o0 - o1
    d04, d26 = r1 + r3, i1 + i3
    t1, t2 = (r1 - r3) * RC, (i1 - i3) * RC
    d15, d37 = t1 + t2, t2 - t1
    return [s04 + d04, s15 + d15, s26 + d26, s37 + d37, s04 - d04, s15 - d15, s26 - d26, s37 - d37]


def _twiddle16(z, k):
    re, im = z
    k = k % 16
    if k == 0:
        return z
    if k == 4:
        return (im, -re)
    if k == 12:
        return (-im, re)
    if k == 2:
        return ((re + im) * RC, (im - re) * RC)
    if k == 14:
        return ((re - im) * RC, (re + im) * RC)
    if k == 6:
        return ((im - re) * RC, (re + im) * -RC)
    if k == 10:
        return ((re + im) * -RC, (re - im) * RC)
    c, s = float(np.cos(2 * np.pi * k / 16)), float(-np.sin(2 * np.pi * k / 16))
    return (re * c - im * s, re * s + im * c)


def _bfly4(z, sign):
    (ar, ai), (br, bi), (cr, ci), (dr, di) = z
    sr, si, tr, ti = ar + cr, ai + ci, ar - cr, ai - ci
    ur, ui, vr, vi = br + dr, bi + di, br - dr, bi - di
    o0, o2 = (sr + ur, si + ui), (sr - ur, si - ui)
    p, q = (tr + vi, ti - vr), (tr - vi, ti + vr)
    return [o0, p, o2, q] if sign > 0 else [o0, q, o2, p]


class _Pacer:
    def __init__(self, tasks, ntokens):
        self.slots = {}
        for n, task in enumerate(tasks):
            self.slots.setdefault(n * ntokens // len(tasks), []).append(task)
        self.pos = 0

    def feed(self, r):
        for j in range(r.shape[0] // 8):
            for task in self.slots.pop(self.pos, []):
                task(pltpu.bitcast(r[8 * j:8 * j + 8], u32))
            self.pos += 1

    def done(self):
        assert not self.slots


def _pack_rows(m):
    b = np.asarray(m, np.float32).astype(jnp.bfloat16).view(np.uint16).astype(np.uint32)
    return b[..., 0::2, :] | (b[..., 1::2, :] << 16)


def _dft_constants():
    i, j = np.arange(64)[:, None], np.arange(128)
    whole, half = 2 * np.pi * i * j / 128, 2 * np.pi * (i + 0.5) * j / 128
    gf = np.zeros((3, 192, 128))
    gf[0, :129] = np.concatenate([np.cos(whole), -np.sin(whole), [(-1.0) ** j]])
    gf[1, :128] = np.concatenate([np.cos(half), -np.sin(half)])
    gf[2, :128] = np.concatenate([np.cos(half), np.sin(half)])
    gi = gf[0:2, :128] * (2.0 / (D * S))
    gi[0, 0], gi[0, 64] = gf[0, 0] / (D * S), gf[0, 128] / (D * S)
    angs = [2 * np.pi * j * (b - 8) / S for b in range(16)] + [2 * np.pi * j * (r - 4) / D for r, _ in RES]
    tw = np.zeros((20, 2, 8, 128), np.float32)
    for n, ang in enumerate(angs):
        tw[n, 0], tw[n, 1] = np.cos(ang), -np.sin(ang)
    return _pack_rows(gf), _pack_rows(gi), tw


def _attn_fill():
    head = np.concatenate([np.arange(64) // 32, np.arange(16) // 8])
    pos = np.concatenate([np.arange(64) % 32, 32 + np.arange(16) % 8])
    ok = (pos[:, None] < M) | (pos[:, None] >= pos[None, :])
    fill = np.where(ok, 0.0, -1e9)
    fill = np.where(head[:, None] == head[None, :], fill, -np.inf)
    return fill.astype(np.float32)


def _strassen(prod, b11, b12, b21, b22, add, sub, emit):
    m2 = prod(1, b11())
    m1 = prod(0, add(b11(), b22()))
    m3 = prod(2, sub(b12(), b22()))
    c22 = prod(5, add(b11(), b12())) + ((m1 - m2) + m3)
    m4 = prod(3, sub(b21(), b11()))
    emit(1, m2 + m4, c22)
    m5 = prod(4, b22())
    emit(0, prod(6, add(b21(), b22())) + ((m1 + m4) - m5), m3 + m5)


class _Blocks(list):
    def __add__(self, other):
        return _Blocks(a + b for a, b in zip(self, other))

    def __sub__(self, other):
        return _Blocks(a - b for a, b in zip(self, other))


def _strassen_left(a11, a12, a21, a22):
    return [a11 + a22, a21 + a22, a11, a22, a11 + a12, a21 - a11, a12 - a22]


def _strassen_left_one(i, blk):
    terms = ((0, 3, 1), (2, 3, 1), (0,), (3,), (0, 1, 1), (2, 0, -1), (1, 3, -1))[i]
    a = blk(*divmod(terms[0], 2))
    if len(terms) == 1:
        return a
    b = blk(*divmod(terms[1], 2))
    return a + b if terms[2] > 0 else a - b


def _kernel(x_hbm, mem_hbm, wq_hbm, wk_hbm, wv_hbm, wo_hbm, bx_hbm, wr_hbm, wi_hbm,
            gf_hbm, gi_hbm, tw_hbm, fill_hbm, out_hbm,
            wraw, wall, wo, xbuf, mem0, x8, xs, xs2, pre, osum, outbuf, fill_ref,
            xb, wt, wl, gf, gi, tw, xd, yb, sems):
    def start(src, dst, sem):
        c = pltpu.make_async_copy(src, dst, sems.at[sem])
        c.start()
        return c

    def wait_all(cs):
        for c in cs:
            c.wait()

    dot = functools.partial(jnp.dot, preferred_element_type=f32)
    dot_nt = lambda a, b: lax.dot_general(a, b, (((1,), (1,)), ((), ())), preferred_element_type=f32)
    cat = lambda *vs: jnp.concatenate(vs, axis=0)
    as_bf16 = lambda w: pltpu.bitcast(w, bf16)
    hi_f32 = lambda w: pltpu.bitcast(w & u32(0xFFFF0000), f32)
    all_ones = lambda tok: ((tok >> 16) | u32(0xFFFF)) | u32(0xFFFF0000)
    after = lambda v, tok: pltpu.bitcast(pltpu.bitcast(v, u32) & all_ones(tok), f32)
    widen = lambda w: as_bf16(w).astype(f32) if w.dtype == u32 else w
    narrow = lambda w: as_bf16(w) if w.dtype == u32 else w.astype(bf16)
    add2 = lambda a, b: widen(a) + widen(b)
    sub2 = lambda a, b: widen(a) - widen(b)
    w_hbm = (wq_hbm, wk_hbm, wv_hbm)

    def start_unit(u):
        return start(w_hbm[u // 2].at[:, :, u % 2], wraw.at[u % NRAW], u % NRAW)

    def start_x(seg0, nseg, sem):
        segs, rows = pl.ds(seg0, nseg), pl.ds(0, SEG - M)
        return start(x_hbm.at[segs, rows, :], xbuf.at[segs], sem)

    def start_filter(row0, nrows, sem):
        rows = pl.ds(row0, nrows)
        return [start(w.at[rows, pl.ds(128 * d, 128)], wt.at[t, d, rows], sem)
                for t, w in enumerate((wr_hbm, wi_hbm)) for d in range(16)]

    def start_piece(n, xsem, parts):
        cols = pl.ds(256 * n, 256)
        cs = [start(x_hbm.at[:, pl.ds(SEG - M, M), cols], x8.at[:, :, cols], xsem)]
        for k, sem in enumerate(parts):
            rows = pl.ds(128 * n + 128 // len(parts) * k, 128 // len(parts))
            cs.append(start(wq_hbm.at[rows, :, 0], wraw.at[0, rows], sem))
        return cs
    c_a = [start_piece(0, 5, (6, 0))] + [start_piece(n, n, (n,)) for n in range(1, 4)]

    xb32 = xb.bitcast(u32)

    head_of = lambda slot: slot // 16 * 16 + slot % 8 * 2 + slot % 16 // 8

    def relayout_tasks(u, r0=0, r1=D // 2, pars=(0, 1)):
        src, dst = wraw.at[u % NRAW], wall.at[u]
        step = 4 // len(pars)

        def make(rows):
            def task(tok):
                lo = (tok >> 16) | u32(0xFFFF)
                hi = (tok << 16) | u32(0xFFFF0000)
                for r in rows:
                    a, b = src.at[r].bitcast(u32)[...]
                    for par in pars:
                        dst[pl.ds(r + 8 * WP * par, 8, stride=WP), :] = (
                            (a >> 16) | (b & hi) if par else (a & lo) | (b << 16))
            return task
        return [make(range(r, r + step)) for r in range(r0, r1, step)]

    def y_blocks(r):
        return pl.ds(4 * (r % 2) + r // 2, 8, stride=8)

    def filter_tasks(blk, wfn):
        def make(phase, k):
            slots = [4 * k + j for j in range(4)] if phase == 1 else [4 * j + k for j in range(4)]

            def task(tok):
                z = [(yb[0, b, blk], yb[1, b, blk]) for b in slots]
                if phase == 0:
                    z = [(after(zr, tok), zi) for zr, zi in z]
                    z = [(zr * tw[b, 0] - zi * tw[b, 1], zr * tw[b, 1] + zi * tw[b, 0]) if b != 8 else (zr, zi)
                         for b, (zr, zi) in zip(slots, z)]
                else:
                    z[0] = tuple(after(v, tok) for v in z[0])
                if phase == 0:
                    o = _bfly4(z, 1)
                    o = [_twiddle16(o[j], k * j) for j in range(4)]
                elif phase == 1:
                    o = _bfly4(z, 1)
                    y = []
                    for j in range(4):
                        wr, wi = wfn(k + 4 * j)
                        xr, xi = o[j]
                        y.append((xr * wr - xi * wi, xr * wi + xi * wr))
                    o = _bfly4(y, -1)
                    o = [_twiddle16(o[j], -k * j) for j in range(4)]
                else:
                    o = [(zr * tw[b, 0] + zi * tw[b, 1], zi * tw[b, 0] - zr * tw[b, 1]) if b != 8 else (zr, zi)
                         for b, (zr, zi) in zip(slots, _bfly4(z, -1))]
                for b, v in zip(slots, o):
                    yb[0, b, blk] = v[0]
                    yb[1, b, blk] = v[1]
            return task
        return [make(phase, k) for phase in range(3) for k in range(4)]

    mirror = lambda a: a if a < 64 else 191 - a

    def twiddle_d(g, x, y):
        c, sn = [jnp.tile(tw[16 + g, k], (x.shape[0] // 8, 1)) for k in range(2)]
        return (x * c - y * sn, x * sn + y * c) if g == 3 else (x * c + y * sn, x * sn - y * c)

    def butterfly_tasks():
        def make(a, par):
            def task(tok):
                w = [xb32[j, a // 8, a // 2 % 4, pl.ds(8 * (a % 2), 8), :] for j in range(8)]
                if par:
                    hi = (tok << 16) | u32(0xFFFF0000)
                    z = _fwd8([pltpu.bitcast(v & hi, f32) for v in w])
                else:
                    sixteen = ((tok >> 31) | u32(1)) << 4
                    z = _fwd8([pltpu.bitcast(v << sixteen, f32) for v in w])
                for n in range(8):
                    xd[n, pl.ds(8 * XP * par + mirror(a), 8, stride=XP), :] = z[n]
            return task
        return [make(a, par) for a in range(128) for par in range(2)]

    low = lax.broadcasted_iota(jnp.int32, (1, 128), 1) < 64

    def b_dfwd(b, g):
        z = [xd[n, pl.ds(XP * (b // 2 + 8 * (b % 2)), 128), :] for n in (2 * g, 2 * g + 1)]
        if g:
            z = twiddle_d(g, *z)
        z = [cat(v[0:64] + v[64:128], v[0:64] - v[64:128]).astype(bf16) for v in z]
        tu = dot_nt(as_bf16(gf[1, 0:64] if g else gf[0, 0:72]), z[0])
        tv = dot_nt(as_bf16(gf[1, 0:64]), z[1])
        if g == 0:
            tr = cat(tu[0:64], tv[0:64], tu[128:144])
            ti = cat(tu[64:128], tv[64:128], jnp.zeros((16, 128), f32))
        else:
            tr = cat(tu[0:64] - tv[64:128], tu[0:64] + tv[64:128])
            ti = cat(tu[64:128] + tv[0:64], tu[64:128] - tv[0:64])
        return jnp.where(low, tr, ti).astype(bf16), jnp.where(low, ti, tr).astype(bf16)

    def b_sfwd(b, g, ts):
        for c in range(2):
            y = dot(ts[c], as_bf16(gf[2 - c, 0:64]))
            for q in range(2):
                yb[c, b, y_blocks(RES[g][q])] = y[64 * q:64 * q + 64].reshape(8, 8, 128)
            if g == 0:
                yb[c, b, 64] = y[128:136]

    def b_stage1():
        pend = []
        for b in list(range(0, 16, 2)) + list(range(1, 16, 2)):
            for g in range(4):
                pend.append((b, g, b_dfwd(b, g)))
                if len(pend) > 3:
                    b_sfwd(*pend.pop(0))
        for item in pend:
            b_sfwd(*item)

    def b_sinv(tasks):
        row0 = lax.broadcasted_iota(jnp.int32, (8, 128), 0) == 0
        pacer = _Pacer(tasks, 12 * 8)
        for _, b, g in sorted((b + (6 if g == 0 else 0), b, g) for b in range(16) for g in range(4)):
            (ar, br), (ai, bi) = [[yb[c, b, y_blocks(r)].reshape(64, 128) for r in RES[g]] for c in range(2)]
            if g:
                uv = [(ar + br, ai + bi, -ar - br), (ai - bi, br - ar, bi - ai)]
                uv = [(cat(re, im), cat(im, neg)) for re, im, neg in uv]
            else:
                pacer.done()
                na = -ar
                uv = [(cat(ar, jnp.where(row0, yb[0, b, 64], ai[0:8]), ai[8:]),
                       cat(ai, jnp.where(row0, yb[1, b, 64], na[0:8]), na[8:])),
                      (cat(br, bi), cat(bi, -br))]
            for q, (u, v) in enumerate(uv):
                cu = dot_nt(as_bf16(gf[2, 0:32]), u.astype(bf16))
                sv = dot_nt(as_bf16(gf[2, 32:64]), v.astype(bf16))
                xd[2 * g + q, pl.ds(XP * b, 128), :] = cat(cu - sv, cu + sv)
            pacer.feed(cu)

    def b_dinv(t):
        rows = lambda j: cat(*[xd[j, pl.ds(mirror(a), 16, stride=XP), :] for a in range(8 * t, 8 * t + 8)])
        z = [dot(rows(j).astype(bf16), as_bf16(gi[min(j, 1)])) for j in range(8)]
        for g in range(1, 4):
            u, v = z[2 * g], z[2 * g + 1]
            c, sn = [jnp.tile(tw[16 + g, k], (16, 1)) for k in range(2)]
            z[2 * g] = u * c + v * sn
            z[2 * g + 1] = v * c - u * sn if g == 3 else u * sn - v * c
        y = _inv8(z)
        for j in range(8):
            xb[j, t] = y[j].reshape(4, SEG, 128).astype(bf16)

    HALF = NSEG * M // 2
    pre32 = pre.bitcast(u32)

    def store_pre(pair, row0, cs, packed):
        n = cs[0].shape[0] // M
        segs = pl.ds(row0 // M, n)
        if packed:
            st = jnp.concatenate([c.reshape(n, M, E) for c in cs], axis=1)
            pre32[pair, segs] = pltpu.bitcast(st.reshape(2 * M * n, E).astype(bf16), u32).reshape(n, M, E)
        else:
            for t, c in enumerate(cs):
                pre[pair, segs, pl.ds(M * t, M), :] = c.reshape(n, M, E).astype(bf16)

    def batch(u, p0, p1, tasks=(), t0=0, t1=4, margin=4):
        mc = HALF // 2 if t1 == 1 else HALF
        pacer = _Pacer(tasks, (7 * (p1 - p0) - margin // (t1 - t0)) * HALF // 8)
        w = wall.at[u]
        for p in range(p0, p1):
            for r0 in range(0, HALF, mc):
                def blk(head, par):
                    return lambda: cat(*[w[pl.ds((2 * p + head) * WP + 64 * (2 * t + par), 64), :]
                                         for t in range(t0, t1)])

                def prod(i, b):
                    lhs = jnp.concatenate([as_bf16(xs32[i, t, pl.ds(r0 // 2, mc // 2), :])
                                           for t in range(t0, t1)], axis=1)
                    r = dot(lhs, narrow(b))
                    pacer.feed(r)
                    return r

                def emit(half, *cs):
                    park = pl.ds((half * HALF + r0) // 8, mc // 8)
                    if t0 > 0:
                        cs = [c + yb[t, p, park].reshape(mc, E) for t, c in enumerate(cs)]
                    if t1 < 4:
                        for t, c in enumerate(cs):
                            yb[t, p, park] = c.reshape(mc // 8, 8, E)
                    else:
                        store_pre(8 * u + p, half * HALF + r0, cs, False)
                if t0 // (t1 - t0) % 2:
                    _strassen(prod, blk(1, 0), blk(0, 0), blk(1, 1), blk(0, 1), add2, sub2,
                              lambda half, c1, c0: emit(half, c0, c1))
                else:
                    _strassen(prod, blk(0, 0), blk(1, 0), blk(0, 1), blk(1, 1), add2, sub2, emit)
        pacer.done()

    QUART = HALF // 2
    xs32, xs2_32 = xs.bitcast(u32), xs2.bitcast(u32)

    def strassen2(right, left, emit, pacer):
        def outer_prod(i, bs):
            def prod(j, b):
                r = dot(left(7 * i + j), narrow(b))
                pacer.feed(r)
                return r
            order = (1, 0, 3, 2) if i in (1, 4, 5, 6) else (0, 1, 2, 3)
            cs = {}
            _strassen(prod, *[(lambda b=bs[k]: b) for k in order], add2, sub2, lambda half, *c: cs.update({half: c}))
            return _Blocks((cs[0] + cs[1])[k] for k in order)

        def outer_emit(half, *cs):
            for col in (1, 0):
                for a in range(2):
                    emit(2 * half + a, 2 * col, cs[col][2 * a], cs[col][2 * a + 1])
        outer = lambda k, c: lambda: [right(2 * k + k2, 2 * c + c2) for k2 in range(2) for c2 in range(2)]
        _strassen(outer_prod, outer(0, 0), outer(0, 1), outer(1, 0), outer(1, 1),
                  lambda x, y: [add2(a, b) for a, b in zip(x, y)],
                  lambda x, y: [sub2(a, b) for a, b in zip(x, y)], outer_emit)

    def batch2(u, q0, q1, tasks=()):
        pacer = _Pacer(tasks, (49 * (q1 - q0) - 12) * QUART // 8)
        w = wall.at[u]
        for q in range(q0, q1):
            def emit(row, col, *cs):
                store_pre(8 * u + 2 * q + col // 2, row * QUART, cs, True)
            strassen2(lambda k, c: cat(*[w[pl.ds((4 * q + c) * WP + 64 * (k + 4 * t), 64), :]
                                         for t in range(2)]),
                      lambda i: jnp.concatenate([as_bf16(xs2_32[i, t]) for t in range(2)], axis=1),
                      emit, pacer)
        pacer.done()

    def left2_tasks():
        def make(i, t, r):
            def task(tok):
                a = _strassen_left_one(i, lambda rh, kh: _Blocks(
                    x8[32 * rh + 16 * rl + r, :, pl.ds(128 * (2 * kh + kl + 4 * t), 128)].astype(f32)
                    for rl in range(2) for kl in range(2)))
                a[0], a[3] = after(a[0], tok), after(a[3], tok)
                for j, v in enumerate(_strassen_left(*a)):
                    xs2[7 * i + j, t, pl.ds(M * r, M), :] = v.astype(bf16)
            return task
        return [make(i, t, r) for i in range(7) for t in range(2) for r in range(16)]

    def left_tasks(n):
        def make(r):
            def task(tok):
                a = [x8[NSEG // 2 * h + r, :, pl.ds(256 * n + 128 * k, 128)].astype(f32)
                     for h in range(2) for k in range(2)]
                a[0], a[3] = after(a[0], tok), after(a[3], tok)
                for i, v in enumerate(_strassen_left(*a)):
                    xs[i, n, pl.ds(M * r, M), :] = v.astype(bf16)
            return task
        return [make(r) for r in range(NSEG // 2)]

    def piece_tasks(n):
        return [t for both in zip(relayout_tasks(0, 128 * n, 128 * n + 128, (0,)), left_tasks(n)) for t in both]

    def mix(a, b):
        keyed = [(n / len(a), 0, n) for n in range(len(a))] + [(n / len(b), 1, n) for n in range(len(b))]
        return [(a, b)[w][n] for _, w, n in sorted(keyed)]

    run_now = lambda tasks: [task(jnp.zeros((8, 128), u32)) for task in tasks]

    pre32[0:16] = jnp.zeros((16, NSEG, M, E), u32)
    c_a[0][0].wait()
    run_now(left_tasks(0))
    c_a[0][1].wait()
    run_now(relayout_tasks(0, 0, 64))
    c_a[0][2].wait()
    run_now(relayout_tasks(0, 64, 128, (0,)))
    batch(0, 0, 4, relayout_tasks(0, 64, 128, (1,)), 0, 1, margin=8)
    batch(0, 4, 6, (), 0, 1)
    wait_all(c_a[1])
    c_h = [start(wq_hbm.at[pl.ds(256 * n, 256), :, 1], wraw.at[1, pl.ds(256 * n, 256)], n) for n in range(2)]
    batch(0, 6, 8, piece_tasks(1), 0, 1)
    batch(0, 0, 4, relayout_tasks(0, 128, 256, (1,)), 1, 2)
    wait_all(c_a[2])
    batch(0, 4, 8, piece_tasks(2), 1, 2)
    batch(0, 0, 4, relayout_tasks(0, 256, 384, (1,)), 2, 3)
    wait_all(c_a[3])
    c_w2 = start_unit(2)
    batch(0, 4, 8, piece_tasks(3), 2, 3)
    batch(0, 0, 4, relayout_tasks(0, 384, 512, (1,)), 3, 4)
    c_h[0].wait()
    left2 = left2_tasks()
    batch(0, 4, 8, relayout_tasks(1, 0, 256, (0,)), 3, 4)
    batch(1, 0, 4, mix(relayout_tasks(1, 0, 256, (1,)), left2[:74]), 0, 2)
    c_h[1].wait()
    start_unit(3)
    batch(1, 4, 8, mix(relayout_tasks(1, 256, 512, (0,)), left2[74:150]), 0, 2)
    batch(1, 0, 4, mix(relayout_tasks(1, 256, 512, (1,)), left2[150:]), 2, 4)
    c_w2.wait()
    start_unit(4)
    start_unit(5)
    c_b1 = [start(bx_hbm.at[:, :, :, pl.ds(128 * j, 128)], xb.at[j], 5) for j in range(8)]
    c_b1 += [start(gf_hbm, gf, 5), start(tw_hbm, tw, 5)]
    c_loop = [start(wo_hbm.at[:, pl.ds(128 * j, 128)], wo.at[j], 4) for j in range(8)]
    c_loop += [start_x(0, UNROLL, 4), start(mem_hbm, mem0, 4), start(fill_hbm, fill_ref.at[pl.ds(0, 80)], 4)]
    c_loop += start_filter(0, 64, 4)
    batch(1, 4, 8, mix(relayout_tasks(2, pars=(0,)), relayout_tasks(2, 0, 256, (1,))), 2, 4)
    batch2(2, 0, 2, relayout_tasks(2, 256, 512, (1,)))

    def unit_body(u, c):
        slot = (u + 1) % NRAW
        pltpu.make_async_copy(wraw.at[slot], wraw.at[slot], sems.at[slot]).wait()
        batch2(u, 2, 4, relayout_tasks(u + 1, pars=(0,)))
        batch2(u + 1, 0, 2, relayout_tasks(u + 1, pars=(1,)))
        return c
    lax.fori_loop(2, 5, unit_body, 0)
    wait_all(c_b1)
    batch(5, 6, 8, butterfly_tasks(), margin=0)
    batch2(5, 2, 3)
    b_stage1()
    wait_all(c_loop)
    c_rest = [start_x(UNROLL, NSEG - UNROLL, 6)] + start_filter(64, 448, 6)
    c_b3 = [start(w.at[pl.ds(512, 1), :], wl.at[t], 5) for t, w in enumerate((wr_hbm, wi_hbm))]
    c_b3 += [start(gi_hbm, gi, 5)]

    wo32 = wo.bitcast(u32)
    scale = E ** -0.5

    def gated(w, toks):
        if not toks:
            return w
        bits = functools.reduce(
            jnp.bitwise_or, [pltpu.bitcast(jnp.broadcast_to(t, (8, 128)), u32) for t in toks])
        return cat(w[0:8] & all_ones(bits), w[8:])

    def wqkv(i, p, second, toks=(), k0=0, k1=D):
        rows = pl.ds((p % 8 * 2 + second) * WP + k0 // 2, (k1 - k0) // 2)
        return as_bf16(gated(wall[2 * i + p // 8, rows, :], toks))

    def step(n, u, mem, held):
        s = UNROLL * n + u
        rows = cat(mem, xbuf[s].astype(f32))
        lhs = rows.astype(bf16)
        head_start = {}
        if u:
            lo, hi = rows[:, :D // 2].astype(bf16), rows[:, D // 2:].astype(bf16)
            for key in EARLY:
                head_start[key] = dot(lo, wqkv(*key, k1=D // 2))
        fill = fill_ref[pl.ds(0, 80), :]
        heads = [None] * H
        rs = []

        shift = jnp.full((8, 128), 16 - 16 * (n % 2), jnp.int32).astype(u32)
        wblk = pl.ds(pl.multiple_of(64 * (n // 2), 64), 64)
        flt = filter_tasks(
            s, lambda d: [hi_f32(wt.at[t, d, wblk].bitcast(u32)[pl.ds(u, 8, stride=4), :] << shift) for t in range(2)])
        pacer = _Pacer(flt, 84)

        def proj(i, p, toks=()):
            a, b = [
                dot(hi, wqkv(i, p, t, k0=D // 2)) + head_start[i, p, t] if (i, p, t) in head_start
                else dot(lhs, wqkv(i, p, t, toks[t * len(toks) // 2:(t + 1) * len(toks) // 2]))
                for t in range(2)]
            pacer.feed(a)
            pacer.feed(b)
            c = widen(pre32[16 * i + p, s])
            return cat(a, b, c).astype(bf16)

        def probs(q, k):
            sc = dot_nt(q, k) * scale
            sc = jnp.where(fill == 0.0, sc, fill)
            e = jnp.exp(sc - jnp.max(sc, axis=1, keepdims=True))
            l = jnp.sum(e, axis=1, keepdims=True)
            r = pl.reciprocal(l, approx=True)
            r = r * (2.0 - l * r)
            rs.append([r[8 * j:8 * j + 8] for j in range(10)])
            return (e * r).astype(bf16)

        def pv(p, pr, v):
            o = dot(pr, v)
            heads[2 * p] = cat(o[0:8], o[16:32], o[64:72])
            heads[2 * p + 1] = cat(o[32:40], o[48:64], o[72:80])
            held[u, 2 * p], held[u, 2 * p + 1] = o[8:16], o[40:48]

        def left_task(q, i):
            def task(tok):
                a = _strassen_left_one(i, lambda r, k: _Blocks(
                    held[2 * r + r2, 4 * q + 2 * k + k2] for r2 in range(2) for k2 in range(2)))
                a[0], a[3] = after(a[0], tok), after(a[3], tok)
                for j, v in enumerate(_strassen_left(*a)):
                    osum[7 * i + j, q, pl.ds(pl.multiple_of(M * n, M), M), :] = v.astype(bf16)
            return task

        pend = []
        for g in range(4):
            ps = range(4 * g, 4 * g + 4)
            qk = [(proj(0, p), proj(1, p)) for p in ps]
            vs = [proj(2, p, rs[p - 4] if g else ()) for p in ps]
            for a in pend:
                pv(*a)
            pend = [(p, probs(*qk[t]), vs[t]) for t, p in enumerate(ps)]
        pacer.done()

        def wo_part(oc, j, h0, h1, toks=()):
            w = cat(*[wo32[j, pl.ds(64 * head_of(h), 64), :] for h in range(h0, h1)])
            return dot(oc, as_bf16(gated(w, toks)))

        acc = []
        pacer = _Pacer([left_task(q, i) for q in range(8) for i in LEFT_AT[u]], 38)
        oc = jnp.concatenate(heads[0:24], axis=1).astype(bf16)
        for j in range(8):
            acc.append(wo_part(oc, j, 0, 24, {3: rs[12] + rs[13], 4: rs[14] + rs[15]}.get(j, ())))
            if j == 4:
                for a in pend:
                    pv(*a)
            if j >= 5:
                pacer.feed(acc[j])
        oc = jnp.concatenate(heads[24:32], axis=1).astype(bf16)
        nxt = []
        for j in range(8):
            r = wo_part(oc, j, 24, 32) + acc[j]
            outbuf[n, u, pl.ds(M, SEG - M), pl.ds(128 * j, 128)] = r[M:].astype(bf16)
            nxt.append(r[0:M])
            pacer.feed(r)
        pacer.done()
        return jnp.concatenate(nxt, axis=1)

    def steps(n, mem):
        pl.when(n == 1)(functools.partial(wait_all, c_rest))
        held = {}
        for u in range(UNROLL):
            mem = step(n, u, mem, held)
        return mem
    lax.fori_loop(0, NSEG // UNROLL, steps, mem0[...].astype(f32))
    tok_rows = pl.ds(M, SEG - M)
    c_out = [start(outbuf.at[:, :, tok_rows, :], out_hbm.at[:, :, tok_rows, pl.ds(0, D)], 0)]

    wait_all(c_b3)
    b_sinv(filter_tasks(64, lambda d: [wl[t, :, pl.ds(128 * d, 128)].astype(f32) for t in range(2)]))
    for t in range(16):
        b_dinv(t)
    c_out += [start(xb.at[j], out_hbm.at[:, :, :, pl.ds(D + 128 * j, 128)], 0) for j in range(8)]

    osum32 = osum.bitcast(u32)
    for cq in range(2):
        def emit(row, col, *cs):
            for t, c in enumerate(cs):
                outbuf[:, row, pl.ds(0, M), pl.ds(128 * (4 * cq + col + t), 128)] = (
                    c.reshape(NSEG // 4, M, 128).astype(bf16))
            idx = (slice(None), row, pl.ds(0, M), pl.ds(128 * (4 * cq + col), 256))
            c_out.append(start(outbuf.at[idx], out_hbm.at[idx], 0))
        strassen2(lambda k, c: cat(*[wo32[4 * cq + c, pl.ds(64 * head_of(4 * q + k), 64), :] for q in range(8)]),
                  lambda i: jnp.concatenate([as_bf16(osum32[i, q]) for q in range(8)], axis=1),
                  emit, _Pacer((), 0))
    wait_all(c_out)


@jax.jit
def pallas_concat_heads__memory_aug_recurrent_mem_tr__spectral_gfnet__prompt_kernel(
    A_x: jax.Array,
    A_mem0: jax.Array,
    A_Wq: jax.Array,
    A_Wk: jax.Array,
    A_Wv: jax.Array,
    A_Wo: jax.Array,
    A_seg_len: jax.Array,
    B_x: jax.Array,
    B_w_r: jax.Array,
    B_w_i: jax.Array,
):
    del A_seg_len
    assert A_x.shape == (1, S, D) and A_mem0.shape == (1, M, D) and B_x.shape == (1, S, D)
    assert A_Wq.shape == (D, H, E) and A_Wo.shape == (H, E, D) and B_w_r.shape == (S, D // 2 + 1)
    gf, gi, tw = _dft_constants()
    fill = _attn_fill()
    hbm = pl.BlockSpec(memory_space=pltpu.HBM)
    wshape = (D // 2, 2, 2, 16, E)
    out = pl.pallas_call(
        _kernel,
        out_shape=jax.ShapeDtypeStruct((NSEG // 4, 4, SEG, 2 * D), bf16),
        in_specs=[hbm] * 13,
        out_specs=hbm,
        scratch_shapes=[
            pltpu.VMEM((NRAW, D // 2, 2, 16, E), bf16),
            pltpu.VMEM((6, 16 * WP, E), u32),
            pltpu.VMEM((8, H * E, 128), bf16),
            pltpu.VMEM((NSEG, SEG - M, D), bf16),
            pltpu.VMEM((M, D), bf16),
            pltpu.VMEM((NSEG, M, D), bf16),
            pltpu.VMEM((7, 4, 256, 128), bf16),
            pltpu.VMEM((49, 2, 128, 128), bf16),
            pltpu.VMEM((48, NSEG, 2 * M, E), bf16),
            pltpu.VMEM((49, 8, NSEG * M // 4, E), bf16),
            pltpu.VMEM((NSEG // 4, 4, SEG, D), bf16),
            pltpu.VMEM((96, 80), f32),
            pltpu.VMEM((8, NSEG // 4, 4, SEG, 128), bf16),
            pltpu.VMEM((2, 16, 512, 128), bf16),
            pltpu.VMEM((2, 1, S), bf16),
            pltpu.VMEM(gf.shape, u32),
            pltpu.VMEM(gi.shape, u32),
            pltpu.VMEM(tw.shape, f32),
            pltpu.VMEM((8, 16 * XP, 128), f32),
            pltpu.VMEM((2, 16, 65, 8, 128), f32),
            pltpu.SemaphoreType.DMA((7,)),
        ],
        compiler_params=pltpu.CompilerParams(vmem_limit_bytes=120 * 1024 * 1024),
    )(A_x.reshape(NSEG, SEG, D), A_mem0.reshape(M, D),
      A_Wq.reshape(wshape), A_Wk.reshape(wshape), A_Wv.reshape(wshape),
      A_Wo.reshape(H * E, D), B_x.reshape(NSEG // 4, 4, SEG, D), B_w_r.T, B_w_i.T, gf, gi, tw, fill)
    return out.reshape(1, S, 2 * D)
```

```python
import functools

import jax
import jax.numpy as jnp
import numpy as np
from jax import lax
from jax.experimental import pallas as pl
from jax.experimental.pallas import tpu as pltpu

S, D, H, E, M, SEG = 2048, 1024, 32, 128, 8, 32
NSEG = S // SEG
WP = 516
XP = 132
NRAW = 4
UNROLL = 4
LEFT_AT = ((), (2,), (4,), (0, 1, 3, 5, 6))
EARLY = ((0, 0, 0), (0, 0, 1), (1, 0, 0), (1, 0, 1), (0, 1, 0))
bf16, f32, u32 = jnp.bfloat16, jnp.float32, jnp.uint32
RES = ((0, 4), (2, 6), (1, 7), (3, 5))
RC = float(np.sqrt(0.5))


def _fwd8(x):
    s04, d04 = x[0] + x[4], x[0] - x[4]
    s26, d26 = x[2] + x[6], x[2] - x[6]
    s15, d15 = x[1] + x[5], x[1] - x[5]
    s37, d37 = x[3] + x[7], x[3] - x[7]
    t1, t2 = (d15 - d37) * RC, (d15 + d37) * RC
    e0, o0 = s04 + s26, s15 + s37
    return [e0 + o0, e0 - o0, s04 - s26, s15 - s37, d04 + t1, d26 + t2, d04 - t1, d26 - t2]


def _inv8(z):
    z0, z4, e1, o1, r1, i1, r3, i3 = z
    e0, o0 = z0 + z4, z0 - z4
    s04, s26, s15, s37 = e0 + e1, e0 - e1, o0 + o1, o0 - o1
    d04, d26 = r1 + r3, i1 + i3
    t1, t2 = (r1 - r3) * RC, (i1 - i3) * RC
    d15, d37 = t1 + t2, t2 - t1
    return [s04 + d04, s15 + d15, s26 + d26, s37 + d37, s04 - d04, s15 - d15, s26 - d26, s37 - d37]


def _twiddle16(z, k):
    re, im = z
    k = k % 16
    if k == 0:
        return z
    if k == 4:
        return (im, -re)
    if k == 12:
        return (-im, re)
    if k == 2:
        return ((re + im) * RC, (im - re) * RC)
    if k == 14:
        return ((re - im) * RC, (re + im) * RC)
    if k == 6:
        return ((im - re) * RC, (re + im) * -RC)
    if k == 10:
        return ((re + im) * -RC, (re - im) * RC)
    c, s = float(np.cos(2 * np.pi * k / 16)), float(-np.sin(2 * np.pi * k / 16))
    return (re * c - im * s, re * s + im * c)


def _bfly4(z, sign):
    (ar, ai), (br, bi), (cr, ci), (dr, di) = z
    sr, si, tr, ti = ar + cr, ai + ci, ar - cr, ai - ci
    ur, ui, vr, vi = br + dr, bi + di, br - dr, bi - di
    o0, o2 = (sr + ur, si + ui), (sr - ur, si - ui)
    p, q = (tr + vi, ti - vr), (tr - vi, ti + vr)
    return [o0, p, o2, q] if sign > 0 else [o0, q, o2, p]


class _Pacer:
    def __init__(self, tasks, ntokens):
        self.slots = {}
        for n, task in enumerate(tasks):
            self.slots.setdefault(n * ntokens // len(tasks), []).append(task)
        self.pos = 0

    def feed(self, r):
        for j in range(r.shape[0] // 8):
            for task in self.slots.pop(self.pos, []):
                task(pltpu.bitcast(r[8 * j:8 * j + 8], u32))
            self.pos += 1

    def done(self):
        assert not self.slots


def _pack_rows(m):
    b = np.asarray(m, np.float32).astype(jnp.bfloat16).view(np.uint16).astype(np.uint32)
    return b[..., 0::2, :] | (b[..., 1::2, :] << 16)


def _dft_constants():
    i, j = np.arange(64)[:, None], np.arange(128)
    whole, half = 2 * np.pi * i * j / 128, 2 * np.pi * (i + 0.5) * j / 128
    gf = np.zeros((3, 192, 128))
    gf[0, :129] = np.concatenate([np.cos(whole), -np.sin(whole), [(-1.0) ** j]])
    gf[1, :128] = np.concatenate([np.cos(half), -np.sin(half)])
    gf[2, :128] = np.concatenate([np.cos(half), np.sin(half)])
    gi = gf[0:2, :128] * (2.0 / (D * S))
    gi[0, 0], gi[0, 64] = gf[0, 0] / (D * S), gf[0, 128] / (D * S)
    angs = [2 * np.pi * j * (b - 8) / S for b in range(16)] + [2 * np.pi * j * (r - 4) / D for r, _ in RES]
    tw = np.zeros((20, 2, 8, 128), np.float32)
    for n, ang in enumerate(angs):
        tw[n, 0], tw[n, 1] = np.cos(ang), -np.sin(ang)
    return _pack_rows(gf), _pack_rows(gi), tw


def _attn_fill():
    head = np.concatenate([np.arange(64) // 32, np.arange(16) // 8])
    pos = np.concatenate([np.arange(64) % 32, 32 + np.arange(16) % 8])
    ok = (pos[:, None] < M) | (pos[:, None] >= pos[None, :])
    fill = np.where(ok, 0.0, -1e9)
    fill = np.where(head[:, None] == head[None, :], fill, -np.inf)
    return fill.astype(np.float32)


def _strassen(prod, b11, b12, b21, b22, add, sub, emit):
    m2 = prod(1, b11())
    m1 = prod(0, add(b11(), b22()))
    m3 = prod(2, sub(b12(), b22()))
    c22 = prod(5, add(b11(), b12())) + ((m1 - m2) + m3)
    m4 = prod(3, sub(b21(), b11()))
    emit(1, m2 + m4, c22)
    m5 = prod(4, b22())
    emit(0, prod(6, add(b21(), b22())) + ((m1 + m4) - m5), m3 + m5)


class _Blocks(list):
    def __add__(self, other):
        return _Blocks(a + b for a, b in zip(self, other))

    def __sub__(self, other):
        return _Blocks(a - b for a, b in zip(self, other))


def _strassen_left(a11, a12, a21, a22):
    return [a11 + a22, a21 + a22, a11, a22, a11 + a12, a21 - a11, a12 - a22]


def _strassen_left_one(i, blk):
    terms = ((0, 3, 1), (2, 3, 1), (0,), (3,), (0, 1, 1), (2, 0, -1), (1, 3, -1))[i]
    a = blk(*divmod(terms[0], 2))
    if len(terms) == 1:
        return a
    b = blk(*divmod(terms[1], 2))
    return a + b if terms[2] > 0 else a - b


def _kernel(x_hbm, mem_hbm, wq_hbm, wk_hbm, wv_hbm, wo_hbm, bx_hbm, wr_hbm, wi_hbm,
            gf_hbm, gi_hbm, tw_hbm, fill_hbm, out_hbm,
            wraw, wall, wo, xbuf, mem0, x8, xs, xs2, pre, osum, outbuf, fill_ref,
            xb, wt, wl, gf, gi, tw, xd, yb, sems):
    def start(src, dst, sem):
        c = pltpu.make_async_copy(src, dst, sems.at[sem])
        c.start()
        return c

    def wait_all(cs):
        for c in cs:
            c.wait()

    dot = functools.partial(jnp.dot, preferred_element_type=f32)
    dot_nt = lambda a, b: lax.dot_general(a, b, (((1,), (1,)), ((), ())), preferred_element_type=f32)
    cat = lambda *vs: jnp.concatenate(vs, axis=0)
    as_bf16 = lambda w: pltpu.bitcast(w, bf16)
    hi_f32 = lambda w: pltpu.bitcast(w & u32(0xFFFF0000), f32)
    all_ones = lambda tok: ((tok >> 16) | u32(0xFFFF)) | u32(0xFFFF0000)
    after = lambda v, tok: pltpu.bitcast(pltpu.bitcast(v, u32) & all_ones(tok), f32)
    widen = lambda w: as_bf16(w).astype(f32) if w.dtype == u32 else w
    narrow = lambda w: as_bf16(w) if w.dtype == u32 else w.astype(bf16)
    add2 = lambda a, b: widen(a) + widen(b)
    sub2 = lambda a, b: widen(a) - widen(b)
    w_hbm = (wq_hbm, wk_hbm, wv_hbm)

    def start_unit(u):
        return start(w_hbm[u // 2].at[:, :, u % 2], wraw.at[u % NRAW], u % NRAW)

    def start_x(seg0, nseg, sem):
        segs, rows = pl.ds(seg0, nseg), pl.ds(0, SEG - M)
        return start(x_hbm.at[segs, rows, :], xbuf.at[segs], sem)

    def start_filter(row0, nrows, sem):
        rows = pl.ds(row0, nrows)
        return [start(w.at[rows, pl.ds(128 * d, 128)], wt.at[t, d, rows], sem)
                for t, w in enumerate((wr_hbm, wi_hbm)) for d in range(16)]

    def start_piece(n, xsem, parts):
        cols = pl.ds(256 * n, 256)
        cs = [start(x_hbm.at[:, pl.ds(SEG - M, M), cols], x8.at[:, :, cols], xsem)]
        for k, sem in enumerate(parts):
            rows = pl.ds(128 * n + 128 // len(parts) * k, 128 // len(parts))
            cs.append(start(wq_hbm.at[rows, :, 0], wraw.at[0, rows], sem))
        return cs
    c_a = [start_piece(0, 5, (6, 0))] + [start_piece(n, n, (n,)) for n in range(1, 4)]

    xb32 = xb.bitcast(u32)

    head_of = lambda slot: slot // 16 * 16 + slot % 8 * 2 + slot % 16 // 8

    def relayout_tasks(u, r0=0, r1=D // 2, pars=(0, 1)):
        src, dst = wraw.at[u % NRAW], wall.at[u]
        step = 4 // len(pars)

        def make(rows):
            def task(tok):
                lo = (tok >> 16) | u32(0xFFFF)
                hi = (tok << 16) | u32(0xFFFF0000)
                for r in rows:
                    a, b = src.at[r].bitcast(u32)[...]
                    for par in pars:
                        dst[pl.ds(r + 8 * WP * par, 8, stride=WP), :] = (
                            (a >> 16) | (b & hi) if par else (a & lo) | (b << 16))
            return task
        return [make(range(r, r + step)) for r in range(r0, r1, step)]

    def y_blocks(r):
        return pl.ds(4 * (r % 2) + r // 2, 8, stride=8)

    def filter_tasks(blk, wfn):
        def make(phase, k):
            slots = [4 * k + j for j in range(4)] if phase == 1 else [4 * j + k for j in range(4)]

            def task(tok):
                z = [(yb[0, b, blk], yb[1, b, blk]) for b in slots]
                if phase == 0:
                    z = [(after(zr, tok), zi) for zr, zi in z]
                    z = [(zr * tw[b, 0] - zi * tw[b, 1], zr * tw[b, 1] + zi * tw[b, 0]) if b != 8 else (zr, zi)
                         for b, (zr, zi) in zip(slots, z)]
                else:
                    z[0] = tuple(after(v, tok) for v in z[0])
                if phase == 0:
                    o = _bfly4(z, 1)
                    o = [_twiddle16(o[j], k * j) for j in range(4)]
                elif phase == 1:
                    o = _bfly4(z, 1)
                    y = []
                    for j in range(4):
                        wr, wi = wfn(k + 4 * j)
                        xr, xi = o[j]
                        y.append((xr * wr - xi * wi, xr * wi + xi * wr))
                    o = _bfly4(y, -1)
                    o = [_twiddle16(o[j], -k * j) for j in range(4)]
                else:
                    o = [(zr * tw[b, 0] + zi * tw[b, 1], zi * tw[b, 0] - zr * tw[b, 1]) if b != 8 else (zr, zi)
                         for b, (zr, zi) in zip(slots, _bfly4(z, -1))]
                for b, v in zip(slots, o):
                    yb[0, b, blk] = v[0]
                    yb[1, b, blk] = v[1]
            return task
        return [make(phase, k) for phase in range(3) for k in range(4)]

    mirror = lambda a: a if a < 64 else 191 - a

    def twiddle_d(g, x, y):
        c, sn = [jnp.tile(tw[16 + g, k], (x.shape[0] // 8, 1)) for k in range(2)]
        return (x * c - y * sn, x * sn + y * c) if g == 3 else (x * c + y * sn, x * sn - y * c)

    def butterfly_tasks():
        def make(a, par):
            def task(tok):
                w = [xb32[j, a // 8, a // 2 % 4, pl.ds(8 * (a % 2), 8), :] for j in range(8)]
                if par:
                    hi = (tok << 16) | u32(0xFFFF0000)
                    z = _fwd8([pltpu.bitcast(v & hi, f32) for v in w])
                else:
                    sixteen = ((tok >> 31) | u32(1)) << 4
                    z = _fwd8([pltpu.bitcast(v << sixteen, f32) for v in w])
                for n in range(8):
                    xd[n, pl.ds(8 * XP * par + mirror(a), 8, stride=XP), :] = z[n]
            return task
        return [make(a, par) for a in range(128) for par in range(2)]

    low = lax.broadcasted_iota(jnp.int32, (1, 128), 1) < 64

    def b_dfwd(b, g):
        z = [xd[n, pl.ds(XP * (b // 2 + 8 * (b % 2)), 128), :] for n in (2 * g, 2 * g + 1)]
        if g:
            z = twiddle_d(g, *z)
        z = [cat(v[0:64] + v[64:128], v[0:64] - v[64:128]).astype(bf16) for v in z]
        tu = dot_nt(as_bf16(gf[1, 0:64] if g else gf[0, 0:72]), z[0])
        tv = dot_nt(as_bf16(gf[1, 0:64]), z[1])
        if g == 0:
            tr = cat(tu[0:64], tv[0:64], tu[128:144])
            ti = cat(tu[64:128], tv[64:128], jnp.zeros((16, 128), f32))
        else:
            tr = cat(tu[0:64] - tv[64:128], tu[0:64] + tv[64:128])
            ti = cat(tu[64:128] + tv[0:64], tu[64:128] - tv[0:64])
        return jnp.where(low, tr, ti).astype(bf16), jnp.where(low, ti, tr).astype(bf16)

    def b_sfwd(b, g, ts):
        for c in range(2):
            y = dot(ts[c], as_bf16(gf[2 - c, 0:64]))
            for q in range(2):
                yb[c, b, y_blocks(RES[g][q])] = y[64 * q:64 * q + 64].reshape(8, 8, 128)
            if g == 0:
                yb[c, b, 64] = y[128:136]

    def b_stage1():
        pend = []
        for b in list(range(0, 16, 2)) + list(range(1, 16, 2)):
            for g in range(4):
                pend.append((b, g, b_dfwd(b, g)))
                if len(pend) > 3:
                    b_sfwd(*pend.pop(0))
        for item in pend:
            b_sfwd(*item)

    def b_sinv(tasks):
        row0 = lax.broadcasted_iota(jnp.int32, (8, 128), 0) == 0
        pacer = _Pacer(tasks, 12 * 8)
        for _, b, g in sorted((b + (6 if g == 0 else 0), b, g) for b in range(16) for g in range(4)):
            (ar, br), (ai, bi) = [[yb[c, b, y_blocks(r)].reshape(64, 128) for r in RES[g]] for c in range(2)]
            if g:
                uv = [(ar + br, ai + bi, -ar - br), (ai - bi, br - ar, bi - ai)]
                uv = [(cat(re, im), cat(im, neg)) for re, im, neg in uv]
            else:
                pacer.done()
                na = -ar
                uv = [(cat(ar, jnp.where(row0, yb[0, b, 64], ai[0:8]), ai[8:]),
                       cat(ai, jnp.where(row0, yb[1, b, 64], na[0:8]), na[8:])),
                      (cat(br, bi), cat(bi, -br))]
            for q, (u, v) in enumerate(uv):
                cu = dot_nt(as_bf16(gf[2, 0:32]), u.astype(bf16))
                sv = dot_nt(as_bf16(gf[2, 32:64]), v.astype(bf16))
                xd[2 * g + q, pl.ds(XP * b, 128), :] = cat(cu - sv, cu + sv)
            pacer.feed(cu)

    def b_dinv(t):
        rows = lambda j: cat(*[xd[j, pl.ds(mirror(a), 16, stride=XP), :] for a in range(8 * t, 8 * t + 8)])
        z = [None] * 8
        for j in (4, 5, 6, 7, 2, 3, 0, 1):
            z[j] = dot(rows(j).astype(bf16), as_bf16(gi[min(j, 1)]))
        for g in range(1, 4):
            u, v = z[2 * g], z[2 * g + 1]
            c, sn = [jnp.tile(tw[16 + g, k], (16, 1)) for k in range(2)]
            z[2 * g] = u * c + v * sn
            z[2 * g + 1] = v * c - u * sn if g == 3 else u * sn - v * c
        y = _inv8(z)
        for j in range(8):
            xb[j, t] = y[j].reshape(4, SEG, 128).astype(bf16)

    HALF = NSEG * M // 2
    pre32 = pre.bitcast(u32)

    def store_pre(pair, row0, cs):
        n = cs[0].shape[0] // M
        pre[pair, pl.ds(row0 // M, n)] = jnp.concatenate([c.reshape(n, M, E) for c in cs], axis=1).astype(bf16)

    def batch(u, p0, p1, tasks=(), t0=0, t1=4, margin=4):
        mc = HALF // 2 if t1 == 1 else HALF
        pacer = _Pacer(tasks, (7 * (p1 - p0) - margin // (t1 - t0)) * HALF // 8)
        w = wall.at[u]
        for p in range(p0, p1):
            for r0 in range(0, HALF, mc):
                def blk(head, par):
                    return lambda: cat(*[w[pl.ds((2 * p + head) * WP + 64 * (2 * t + par), 64), :]
                                         for t in range(t0, t1)])

                def prod(i, b):
                    lhs = jnp.concatenate([as_bf16(xs32[i, t, pl.ds(r0 // 2, mc // 2), :])
                                           for t in range(t0, t1)], axis=1)
                    r = dot(lhs, narrow(b))
                    pacer.feed(r)
                    return r

                def emit(half, *cs):
                    park = pl.ds((half * HALF + r0) // 8, mc // 8)
                    if t0 > 0:
                        cs = [c + yb[t, p, park].reshape(mc, E) for t, c in enumerate(cs)]
                    if t1 < 4:
                        for t, c in enumerate(cs):
                            yb[t, p, park] = c.reshape(mc // 8, 8, E)
                    else:
                        store_pre(8 * u + p, half * HALF + r0, cs)
                if t0 // (t1 - t0) % 2:
                    _strassen(prod, blk(1, 0), blk(0, 0), blk(1, 1), blk(0, 1), add2, sub2,
                              lambda half, c1, c0: emit(half, c0, c1))
                else:
                    _strassen(prod, blk(0, 0), blk(1, 0), blk(0, 1), blk(1, 1), add2, sub2, emit)
        pacer.done()

    QUART = HALF // 2
    xs32, xs2_32 = xs.bitcast(u32), xs2.bitcast(u32)

    def strassen2(right, left, emit, pacer):
        def outer_prod(i, bs):
            def prod(j, b):
                r = dot(left(7 * i + j), narrow(b))
                pacer.feed(r)
                return r
            order = (1, 0, 3, 2) if i in (1, 4, 5, 6) else (0, 1, 2, 3)
            cs = {}
            _strassen(prod, *[(lambda b=bs[k]: b) for k in order], add2, sub2, lambda half, *c: cs.update({half: c}))
            return _Blocks((cs[0] + cs[1])[k] for k in order)

        def outer_emit(half, *cs):
            for col in (1, 0):
                for a in range(2):
                    emit(2 * half + a, 2 * col, cs[col][2 * a], cs[col][2 * a + 1])
        outer = lambda k, c: lambda: [right(2 * k + k2, 2 * c + c2) for k2 in range(2) for c2 in range(2)]
        _strassen(outer_prod, outer(0, 0), outer(0, 1), outer(1, 0), outer(1, 1),
                  lambda x, y: [add2(a, b) for a, b in zip(x, y)],
                  lambda x, y: [sub2(a, b) for a, b in zip(x, y)], outer_emit)

    def batch2(u, q0, q1, tasks=(), margin=12):
        pacer = _Pacer(tasks, (49 * (q1 - q0) - margin) * QUART // 8)
        w = wall.at[u]
        for q in range(q0, q1):
            def emit(row, col, *cs):
                store_pre(8 * u + 2 * q + col // 2, row * QUART, cs)
            strassen2(lambda k, c: cat(*[w[pl.ds((4 * q + c) * WP + 64 * (k + 4 * t), 64), :]
                                         for t in range(2)]),
                      lambda i: jnp.concatenate([as_bf16(xs2_32[i, t]) for t in range(2)], axis=1),
                      emit, pacer)
        pacer.done()

    def left2_tasks():
        def make(i, t, r):
            def task(tok):
                a = _strassen_left_one(i, lambda rh, kh: _Blocks(
                    x8[32 * rh + 16 * rl + r, :, pl.ds(128 * (2 * kh + kl + 4 * t), 128)].astype(f32)
                    for rl in range(2) for kl in range(2)))
                a[0], a[3] = after(a[0], tok), after(a[3], tok)
                for j, v in enumerate(_strassen_left(*a)):
                    xs2[7 * i + j, t, pl.ds(M * r, M), :] = v.astype(bf16)
            return task
        return [make(i, t, r) for i in range(7) for t in range(2) for r in range(16)]

    def left_tasks(n):
        def make(r):
            def task(tok):
                a = [x8[NSEG // 2 * h + r, :, pl.ds(256 * n + 128 * k, 128)].astype(f32)
                     for h in range(2) for k in range(2)]
                a[0], a[3] = after(a[0], tok), after(a[3], tok)
                for i, v in enumerate(_strassen_left(*a)):
                    xs[i, n, pl.ds(M * r, M), :] = v.astype(bf16)
            return task
        return [make(r) for r in range(NSEG // 2)]

    def piece_tasks(n):
        return [t for both in zip(relayout_tasks(0, 128 * n, 128 * n + 128, (0,)), left_tasks(n)) for t in both]

    def mix(a, b):
        keyed = [(n / len(a), 0, n) for n in range(len(a))] + [(n / len(b), 1, n) for n in range(len(b))]
        return [(a, b)[w][n] for _, w, n in sorted(keyed)]

    run_now = lambda tasks: [task(jnp.zeros((8, 128), u32)) for task in tasks]

    pre32[0:16] = jnp.zeros((16, NSEG, M, E), u32)
    c_a[0][0].wait()
    run_now(left_tasks(0))
    c_a[0][1].wait()
    run_now(relayout_tasks(0, 0, 64))
    c_a[0][2].wait()
    run_now(relayout_tasks(0, 64, 128, (0,)))
    batch(0, 0, 4, relayout_tasks(0, 64, 128, (1,)), 0, 1, margin=8)
    batch(0, 4, 6, (), 0, 1)
    wait_all(c_a[1])
    c_h = [start(wq_hbm.at[pl.ds(256 * n, 256), :, 1], wraw.at[1, pl.ds(256 * n, 256)], n) for n in range(2)]
    batch(0, 6, 8, piece_tasks(1), 0, 1)
    batch(0, 0, 4, relayout_tasks(0, 128, 256, (1,)), 1, 2)
    wait_all(c_a[2])
    batch(0, 4, 8, piece_tasks(2), 1, 2)
    batch(0, 0, 4, relayout_tasks(0, 256, 384, (1,)), 2, 3)
    wait_all(c_a[3])
    c_w2 = start_unit(2)
    batch(0, 4, 8, piece_tasks(3), 2, 3)
    batch(0, 0, 4, relayout_tasks(0, 384, 512, (1,)), 3, 4)
    c_h[0].wait()
    left2 = left2_tasks()
    batch(0, 4, 8, relayout_tasks(1, 0, 256, (0,)), 3, 4)
    batch(1, 0, 4, mix(relayout_tasks(1, 0, 256, (1,)), left2[:74]), 0, 2)
    c_h[1].wait()
    start_unit(3)
    batch(1, 4, 8, mix(relayout_tasks(1, 256, 512, (0,)), left2[74:150]), 0, 2)
    batch(1, 0, 4, mix(relayout_tasks(1, 256, 512, (1,)), left2[150:]), 2, 4)
    c_w2.wait()
    start_unit(4)
    start_unit(5)
    c_b1 = [start(bx_hbm.at[:, :, :, pl.ds(128 * j, 128)], xb.at[j], 5) for j in range(8)]
    c_b1 += [start(gf_hbm, gf, 5), start(tw_hbm, tw, 5)]
    c_loop = [start(wo_hbm.at[:, pl.ds(128 * j, 128)], wo.at[j], 4) for j in range(8)]
    c_loop += [start_x(0, UNROLL, 4), start(mem_hbm, mem0, 4), start(fill_hbm, fill_ref.at[pl.ds(0, 80)], 4)]
    c_loop += start_filter(0, 64, 4)
    batch(1, 4, 8, mix(relayout_tasks(2, pars=(0,)), relayout_tasks(2, 0, 256, (1,))), 2, 4)
    batch2(2, 0, 2, relayout_tasks(2, 256, 512, (1,)))

    def unit_body(u, c):
        slot = (u + 1) % NRAW
        pltpu.make_async_copy(wraw.at[slot], wraw.at[slot], sems.at[slot]).wait()
        batch2(u, 2, 4, relayout_tasks(u + 1, pars=(0,)), 16)
        batch2(u + 1, 0, 2, relayout_tasks(u + 1, pars=(1,)), 4)
        return c
    lax.fori_loop(2, 5, unit_body, 0)
    wait_all(c_b1)
    batch(5, 6, 8, butterfly_tasks(), margin=0)
    batch2(5, 2, 3)
    b_stage1()
    wait_all(c_loop)
    c_rest = [start_x(UNROLL, NSEG - UNROLL, 6)] + start_filter(64, 448, 6)
    c_b3 = [start(w.at[pl.ds(512, 1), :], wl.at[t], 5) for t, w in enumerate((wr_hbm, wi_hbm))]
    c_b3 += [start(gi_hbm, gi, 5)]

    wo32 = wo.bitcast(u32)
    scale = E ** -0.5

    def gated(w, toks):
        if not toks:
            return w
        bits = functools.reduce(
            jnp.bitwise_or, [pltpu.bitcast(jnp.broadcast_to(t, (8, 128)), u32) for t in toks])
        return cat(w[0:8] & all_ones(bits), w[8:])

    def wqkv(i, p, second, toks=(), k0=0, k1=D):
        rows = pl.ds((p % 8 * 2 + second) * WP + k0 // 2, (k1 - k0) // 2)
        return as_bf16(gated(wall[2 * i + p // 8, rows, :], toks))

    def step(n, u, mem, held):
        s = UNROLL * n + u
        rows = cat(mem, xbuf[s].astype(f32))
        lhs = rows.astype(bf16)
        head_start = {}
        if u:
            lo, hi = rows[:, :D // 2].astype(bf16), rows[:, D // 2:].astype(bf16)
            for key in EARLY:
                head_start[key] = dot(lo, wqkv(*key, k1=D // 2))
        fill = fill_ref[pl.ds(0, 80), :]
        heads = [None] * H
        rs = []

        shift = jnp.full((8, 128), 16 - 16 * (n % 2), jnp.int32).astype(u32)
        wblk = pl.ds(pl.multiple_of(64 * (n // 2), 64), 64)
        flt = filter_tasks(
            s, lambda d: [hi_f32(wt.at[t, d, wblk].bitcast(u32)[pl.ds(u, 8, stride=4), :] << shift) for t in range(2)])
        pacer = _Pacer(flt, 84)

        def proj(i, p, toks=()):
            a, b = [
                dot(hi, wqkv(i, p, t, k0=D // 2)) + head_start[i, p, t] if (i, p, t) in head_start
                else dot(lhs, wqkv(i, p, t, toks[t * len(toks) // 2:(t + 1) * len(toks) // 2]))
                for t in range(2)]
            pacer.feed(a)
            pacer.feed(b)
            c = widen(pre32[16 * i + p, s])
            return cat(a, b, c).astype(bf16)

        def probs(q, k):
            sc = dot_nt(q, k) * scale
            sc = jnp.where(fill == 0.0, sc, fill)
            e = jnp.exp(sc - jnp.max(sc, axis=1, keepdims=True))
            l = jnp.sum(e, axis=1, keepdims=True)
            r = pl.reciprocal(l, approx=True)
            r = r * (2.0 - l * r)
            rs.append([r[8 * j:8 * j + 8] for j in range(10)])
            return (e * r).astype(bf16)

        def pv(p, pr, v):
            o = dot(pr, v)
            heads[2 * p] = cat(o[0:8], o[16:32], o[64:72])
            heads[2 * p + 1] = cat(o[32:40], o[48:64], o[72:80])
            held[u, 2 * p], held[u, 2 * p + 1] = o[8:16], o[40:48]

        def left_task(q, i):
            def task(tok):
                a = _strassen_left_one(i, lambda r, k: _Blocks(
                    held[2 * r + r2, 4 * q + 2 * k + k2] for r2 in range(2) for k2 in range(2)))
                a[0], a[3] = after(a[0], tok), after(a[3], tok)
                for j, v in enumerate(_strassen_left(*a)):
                    osum[7 * i + j, q, pl.ds(pl.multiple_of(M * n, M), M), :] = v.astype(bf16)
            return task

        pend = []
        for g in range(4):
            ps = range(4 * g, 4 * g + 4)
            qk = [(proj(0, p), proj(1, p)) for p in ps]
            vs = [proj(2, p, rs[p - 4] if g else ()) for p in ps]
            for a in pend:
                pv(*a)
            pend = [(p, probs(*qk[t]), vs[t]) for t, p in enumerate(ps)]
        pacer.done()

        def wo_part(oc, j, h0, h1, toks=()):
            w = cat(*[wo32[j, pl.ds(64 * head_of(h), 64), :] for h in range(h0, h1)])
            return dot(oc, as_bf16(gated(w, toks)))

        acc = []
        pacer = _Pacer([left_task(q, i) for q in range(8) for i in LEFT_AT[u]], 38)
        oc = jnp.concatenate(heads[0:24], axis=1).astype(bf16)
        for j in range(8):
            acc.append(wo_part(oc, j, 0, 24, {3: rs[12] + rs[13], 4: rs[14] + rs[15]}.get(j, ())))
            if j == 4:
                for a in pend:
                    pv(*a)
            if j >= 5:
                pacer.feed(acc[j])
        oc = jnp.concatenate(heads[24:32], axis=1).astype(bf16)
        nxt = []
        for j in range(8):
            r = wo_part(oc, j, 24, 32) + acc[j]
            outbuf[n, u, pl.ds(M, SEG - M), pl.ds(128 * j, 128)] = r[M:].astype(bf16)
            nxt.append(r[0:M])
            pacer.feed(r)
        pacer.done()
        return jnp.concatenate(nxt, axis=1)

    def steps(n, mem):
        pl.when(n == 1)(functools.partial(wait_all, c_rest))
        held = {}
        for u in range(UNROLL):
            mem = step(n, u, mem, held)
        return mem
    lax.fori_loop(0, NSEG // UNROLL, steps, mem0[...].astype(f32))
    tok_rows = pl.ds(M, SEG - M)
    c_out = [start(outbuf.at[:, :, tok_rows, :], out_hbm.at[:, :, tok_rows, pl.ds(0, D)], 0)]

    wait_all(c_b3)
    b_sinv(filter_tasks(64, lambda d: [wl[t, :, pl.ds(128 * d, 128)].astype(f32) for t in range(2)]))
    for t in range(16):
        b_dinv(t)
    c_out += [start(xb.at[j], out_hbm.at[:, :, :, pl.ds(D + 128 * j, 128)], 0) for j in range(8)]

    osum32 = osum.bitcast(u32)
    for cq in range(2):
        def emit(row, col, *cs):
            idx = (slice(None), row, pl.ds(0, M), pl.ds(128 * (4 * cq + col), 256))
            outbuf[idx] = jnp.concatenate(cs, axis=1).reshape(NSEG // 4, M, 256).astype(bf16)
            c_out.append(start(outbuf.at[idx], out_hbm.at[idx], 0))
        strassen2(lambda k, c: cat(*[wo32[4 * cq + c, pl.ds(64 * head_of(4 * q + k), 64), :] for q in range(8)]),
                  lambda i: jnp.concatenate([as_bf16(osum32[i, q]) for q in range(8)], axis=1),
                  emit, _Pacer((), 0))
    wait_all(c_out)


@jax.jit
def pallas_concat_heads__memory_aug_recurrent_mem_tr__spectral_gfnet__prompt_kernel(
    A_x: jax.Array,
    A_mem0: jax.Array,
    A_Wq: jax.Array,
    A_Wk: jax.Array,
    A_Wv: jax.Array,
    A_Wo: jax.Array,
    A_seg_len: jax.Array,
    B_x: jax.Array,
    B_w_r: jax.Array,
    B_w_i: jax.Array,
):
    del A_seg_len
    assert A_x.shape == (1, S, D) and A_mem0.shape == (1, M, D) and B_x.shape == (1, S, D)
    assert A_Wq.shape == (D, H, E) and A_Wo.shape == (H, E, D) and B_w_r.shape == (S, D // 2 + 1)
    gf, gi, tw = _dft_constants()
    fill = _attn_fill()
    hbm = pl.BlockSpec(memory_space=pltpu.HBM)
    wshape = (D // 2, 2, 2, 16, E)
    out = pl.pallas_call(
        _kernel,
        out_shape=jax.ShapeDtypeStruct((NSEG // 4, 4, SEG, 2 * D), bf16),
        in_specs=[hbm] * 13,
        out_specs=hbm,
        scratch_shapes=[
            pltpu.VMEM((NRAW, D // 2, 2, 16, E), bf16),
            pltpu.VMEM((6, 16 * WP, E), u32),
            pltpu.VMEM((8, H * E, 128), bf16),
            pltpu.VMEM((NSEG, SEG - M, D), bf16),
            pltpu.VMEM((M, D), bf16),
            pltpu.VMEM((NSEG, M, D), bf16),
            pltpu.VMEM((7, 4, 256, 128), bf16),
            pltpu.VMEM((49, 2, 128, 128), bf16),
            pltpu.VMEM((48, NSEG, 2 * M, E), bf16),
            pltpu.VMEM((49, 8, NSEG * M // 4, E), bf16),
            pltpu.VMEM((NSEG // 4, 4, SEG, D), bf16),
            pltpu.VMEM((96, 80), f32),
            pltpu.VMEM((8, NSEG // 4, 4, SEG, 128), bf16),
            pltpu.VMEM((2, 16, 512, 128), bf16),
            pltpu.VMEM((2, 1, S), bf16),
            pltpu.VMEM(gf.shape, u32),
            pltpu.VMEM(gi.shape, u32),
            pltpu.VMEM(tw.shape, f32),
            pltpu.VMEM((8, 16 * XP, 128), f32),
            pltpu.VMEM((2, 16, 65, 8, 128), f32),
            pltpu.SemaphoreType.DMA((7,)),
        ],
        compiler_params=pltpu.CompilerParams(vmem_limit_bytes=120 * 1024 * 1024),
    )(A_x.reshape(NSEG, SEG, D), A_mem0.reshape(M, D),
      A_Wq.reshape(wshape), A_Wk.reshape(wshape), A_Wv.reshape(wshape),
      A_Wo.reshape(H * E, D), B_x.reshape(NSEG // 4, 4, SEG, D), B_w_r.T, B_w_i.T, gf, gi, tw, fill)
    return out.reshape(1, S, 2 * D)
```

```python
import functools

import jax
import jax.numpy as jnp
import numpy as np
from jax import lax
from jax.experimental import pallas as pl
from jax.experimental.pallas import tpu as pltpu

S, D, H, E, M, SEG = 2048, 1024, 32, 128, 8, 32
NSEG = S // SEG
WP = 516
XP = 132
NRAW = 4
UNROLL = 4
LEFT_AT = ((), (2,), (4,), (0, 1, 3, 5, 6))
EARLY = ((0, 0, 0), (0, 0, 1), (1, 0, 0), (1, 0, 1), (0, 1, 0))
bf16, f32, u32 = jnp.bfloat16, jnp.float32, jnp.uint32
RES = ((0, 4), (2, 6), (1, 7), (3, 5))
RC = float(np.sqrt(0.5))


def _fwd8(x):
    s04, d04 = x[0] + x[4], x[0] - x[4]
    s26, d26 = x[2] + x[6], x[2] - x[6]
    s15, d15 = x[1] + x[5], x[1] - x[5]
    s37, d37 = x[3] + x[7], x[3] - x[7]
    t1, t2 = (d15 - d37) * RC, (d15 + d37) * RC
    e0, o0 = s04 + s26, s15 + s37
    return [e0 + o0, e0 - o0, s04 - s26, s15 - s37, d04 + t1, d26 + t2, d04 - t1, d26 - t2]


def _inv8(z):
    z0, z4, e1, o1, r1, i1, r3, i3 = z
    e0, o0 = z0 + z4, z0 - z4
    s04, s26, s15, s37 = e0 + e1, e0 - e1, o0 + o1, o0 - o1
    d04, d26 = r1 + r3, i1 + i3
    t1, t2 = (r1 - r3) * RC, (i1 - i3) * RC
    d15, d37 = t1 + t2, t2 - t1
    return [s04 + d04, s15 + d15, s26 + d26, s37 + d37, s04 - d04, s15 - d15, s26 - d26, s37 - d37]


def _twiddle16(z, k):
    re, im = z
    k = k % 16
    if k == 0:
        return z
    if k == 4:
        return (im, -re)
    if k == 12:
        return (-im, re)
    if k == 2:
        return ((re + im) * RC, (im - re) * RC)
    if k == 14:
        return ((re - im) * RC, (re + im) * RC)
    if k == 6:
        return ((im - re) * RC, (re + im) * -RC)
    if k == 10:
        return ((re + im) * -RC, (re - im) * RC)
    c, s = float(np.cos(2 * np.pi * k / 16)), float(-np.sin(2 * np.pi * k / 16))
    return (re * c - im * s, re * s + im * c)


def _bfly4(z, sign):
    (ar, ai), (br, bi), (cr, ci), (dr, di) = z
    sr, si, tr, ti = ar + cr, ai + ci, ar - cr, ai - ci
    ur, ui, vr, vi = br + dr, bi + di, br - dr, bi - di
    o0, o2 = (sr + ur, si + ui), (sr - ur, si - ui)
    p, q = (tr + vi, ti - vr), (tr - vi, ti + vr)
    return [o0, p, o2, q] if sign > 0 else [o0, q, o2, p]


class _Pacer:
    def __init__(self, tasks, ntokens):
        self.slots = {}
        for n, task in enumerate(tasks):
            self.slots.setdefault(n * ntokens // len(tasks), []).append(task)
        self.pos = 0

    def feed(self, r):
        for j in range(r.shape[0] // 8):
            for task in self.slots.pop(self.pos, []):
                task(pltpu.bitcast(r[8 * j:8 * j + 8], u32))
            self.pos += 1

    def done(self):
        assert not self.slots


def _pack_rows(m):
    b = np.asarray(m, np.float32).astype(jnp.bfloat16).view(np.uint16).astype(np.uint32)
    return b[..., 0::2, :] | (b[..., 1::2, :] << 16)


def _dft_constants():
    i, j = np.arange(64)[:, None], np.arange(128)
    whole, half = 2 * np.pi * i * j / 128, 2 * np.pi * (i + 0.5) * j / 128
    gf = np.zeros((3, 192, 128))
    gf[0, :129] = np.concatenate([np.cos(whole), -np.sin(whole), [(-1.0) ** j]])
    gf[1, :128] = np.concatenate([np.cos(half), -np.sin(half)])
    gf[2, :128] = np.concatenate([np.cos(half), np.sin(half)])
    gi = gf[0:2, :128] * (2.0 / (D * S))
    gi[0, 0], gi[0, 64] = gf[0, 0] / (D * S), gf[0, 128] / (D * S)
    angs = [2 * np.pi * j * (b - 8) / S for b in range(16)] + [2 * np.pi * j * (r - 4) / D for r, _ in RES]
    tw = np.zeros((20, 2, 8, 128), np.float32)
    for n, ang in enumerate(angs):
        tw[n, 0], tw[n, 1] = np.cos(ang), -np.sin(ang)
    return _pack_rows(gf), _pack_rows(gi), tw


def _attn_fill():
    head = np.concatenate([np.arange(64) // 32, np.arange(16) // 8])
    pos = np.concatenate([np.arange(64) % 32, 32 + np.arange(16) % 8])
    ok = (pos[:, None] < M) | (pos[:, None] >= pos[None, :])
    fill = np.where(ok, 0.0, -1e9)
    fill = np.where(head[:, None] == head[None, :], fill, -np.inf)
    return fill.astype(np.float32)


def _strassen(prod, b11, b12, b21, b22, add, sub, emit):
    m2 = prod(1, b11())
    m1 = prod(0, add(b11(), b22()))
    m3 = prod(2, sub(b12(), b22()))
    c22 = prod(5, add(b11(), b12())) + ((m1 - m2) + m3)
    m4 = prod(3, sub(b21(), b11()))
    emit(1, m2 + m4, c22)
    m5 = prod(4, b22())
    emit(0, prod(6, add(b21(), b22())) + ((m1 + m4) - m5), m3 + m5)


class _Blocks(list):
    def __add__(self, other):
        return _Blocks(a + b for a, b in zip(self, other))

    def __sub__(self, other):
        return _Blocks(a - b for a, b in zip(self, other))


def _strassen_left(a11, a12, a21, a22):
    return [a11 + a22, a21 + a22, a11, a22, a11 + a12, a21 - a11, a12 - a22]


def _strassen_left_one(i, blk):
    terms = ((0, 3, 1), (2, 3, 1), (0,), (3,), (0, 1, 1), (2, 0, -1), (1, 3, -1))[i]
    a = blk(*divmod(terms[0], 2))
    if len(terms) == 1:
        return a
    b = blk(*divmod(terms[1], 2))
    return a + b if terms[2] > 0 else a - b


def _kernel(x_hbm, mem_hbm, wq_hbm, wk_hbm, wv_hbm, wo_hbm, bx_hbm, wr_hbm, wi_hbm,
            gf_hbm, gi_hbm, tw_hbm, fill_hbm, out_hbm,
            wraw, wall, wo, xbuf, mem0, x8, xs, xs2, pre, osum, outbuf, fill_ref,
            xb, wt, wl, gf, gi, tw, xd, yb, sems):
    def start(src, dst, sem):
        c = pltpu.make_async_copy(src, dst, sems.at[sem])
        c.start()
        return c

    def wait_all(cs):
        for c in cs:
            c.wait()

    dot = functools.partial(jnp.dot, preferred_element_type=f32)
    dot_nt = lambda a, b: lax.dot_general(a, b, (((1,), (1,)), ((), ())), preferred_element_type=f32)
    cat = lambda *vs: jnp.concatenate(vs, axis=0)
    as_bf16 = lambda w: pltpu.bitcast(w, bf16)
    hi_f32 = lambda w: pltpu.bitcast(w & u32(0xFFFF0000), f32)
    all_ones = lambda tok: ((tok >> 16) | u32(0xFFFF)) | u32(0xFFFF0000)

    def after(tok, *vs):
        ones = all_ones(tok)
        return [pltpu.bitcast(pltpu.bitcast(v, u32) & ones, f32) for v in vs]

    widen = lambda w: as_bf16(w).astype(f32) if w.dtype == u32 else w
    narrow = lambda w: as_bf16(w) if w.dtype == u32 else w.astype(bf16)
    add2 = lambda a, b: widen(a) + widen(b)
    sub2 = lambda a, b: widen(a) - widen(b)
    w_hbm = (wq_hbm, wk_hbm, wv_hbm)

    def start_unit(u):
        return start(w_hbm[u // 2].at[:, :, u % 2], wraw.at[u % NRAW], u % NRAW)

    def start_x(seg0, nseg, sem):
        segs, rows = pl.ds(seg0, nseg), pl.ds(0, SEG - M)
        return start(x_hbm.at[segs, rows, :], xbuf.at[segs], sem)

    def start_filter(row0, nrows, sem):
        rows = pl.ds(row0, nrows)
        return [start(w.at[rows, pl.ds(128 * d, 128)], wt.at[t, d, rows], sem)
                for t, w in enumerate((wr_hbm, wi_hbm)) for d in range(16)]

    def start_piece(n, xsem, parts):
        cols = pl.ds(256 * n, 256)
        cs = [start(x_hbm.at[:, pl.ds(SEG - M, M), cols], x8.at[:, :, cols], xsem)]
        for k, sem in enumerate(parts):
            rows = pl.ds(128 * n + 128 // len(parts) * k, 128 // len(parts))
            cs.append(start(wq_hbm.at[rows, :, 0], wraw.at[0, rows], sem))
        return cs
    c_a = [start_piece(0, 5, (6, 0))] + [start_piece(n, n, (n,)) for n in range(1, 4)]

    xb32 = xb.bitcast(u32)

    head_of = lambda slot: slot // 16 * 16 + slot % 8 * 2 + slot % 16 // 8

    def relayout_tasks(u, r0=0, r1=D // 2, pars=(0, 1)):
        src, dst = wraw.at[u % NRAW], wall.at[u]
        step = 4 // len(pars)

        def make(rows):
            def task(tok):
                mask = [(tok << 16) | u32(0xFFFF0000) if par else (tok >> 16) | u32(0xFFFF) for par in pars]
                for r in rows:
                    words = src.at[r].bitcast(u32)
                    a, b = words[0], words[1]
                    for par, m in zip(pars, mask):
                        dst[pl.ds(r + 8 * WP * par, 8, stride=WP), :] = (
                            (a >> 16) | (b & m) if par else (a & m) | (b << 16))
            return task
        return [make(range(r, r + step)) for r in range(r0, r1, step)]

    def y_blocks(r):
        return pl.ds(4 * (r % 2) + r // 2, 8, stride=8)

    def filter_tasks(blk, wfn):
        def make(phase, k):
            slots = [4 * k + j for j in range(4)] if phase == 1 else [4 * j + k for j in range(4)]

            def task(tok):
                z = [(yb[0, b, blk], yb[1, b, blk]) for b in slots]
                if phase == 0:
                    z = list(zip(after(tok, *[zr for zr, _ in z]), [zi for _, zi in z]))
                    z = [(zr * tw[b, 0] - zi * tw[b, 1], zr * tw[b, 1] + zi * tw[b, 0]) if b != 8 else (zr, zi)
                         for b, (zr, zi) in zip(slots, z)]
                else:
                    z[0] = after(tok, *z[0])
                if phase == 0:
                    o = _bfly4(z, 1)
                    o = [_twiddle16(o[j], k * j) for j in range(4)]
                elif phase == 1:
                    o = _bfly4(z, 1)
                    y = []
                    for j in range(4):
                        wr, wi = wfn(k + 4 * j)
                        xr, xi = o[j]
                        y.append((xr * wr - xi * wi, xr * wi + xi * wr))
                    o = _bfly4(y, -1)
                    o = [_twiddle16(o[j], -k * j) for j in range(4)]
                else:
                    o = [(zr * tw[b, 0] + zi * tw[b, 1], zi * tw[b, 0] - zr * tw[b, 1]) if b != 8 else (zr, zi)
                         for b, (zr, zi) in zip(slots, _bfly4(z, -1))]
                for b, v in zip(slots, o):
                    yb[0, b, blk] = v[0]
                    yb[1, b, blk] = v[1]
            return task
        return [make(phase, k) for phase in range(3) for k in range(4)]

    mirror = lambda a: a if a < 64 else 191 - a

    def twiddle_d(g, x, y):
        c, sn = [jnp.tile(tw[16 + g, k], (x.shape[0] // 8, 1)) for k in range(2)]
        return (x * c - y * sn, x * sn + y * c) if g == 3 else (x * c + y * sn, x * sn - y * c)

    def butterfly_tasks():
        def make(a, par):
            def task(tok):
                w = [xb32[j, a // 8, a // 2 % 4, pl.ds(8 * (a % 2), 8), :] for j in range(8)]
                if par:
                    hi = (tok << 16) | u32(0xFFFF0000)
                    z = _fwd8([pltpu.bitcast(v & hi, f32) for v in w])
                else:
                    sixteen = ((tok >> 31) | u32(1)) << 4
                    z = _fwd8([pltpu.bitcast(v << sixteen, f32) for v in w])
                for n in range(8):
                    xd[n, pl.ds(8 * XP * par + mirror(a), 8, stride=XP), :] = z[n]
            return task
        return [make(a, par) for a in range(128) for par in range(2)]

    low = lax.broadcasted_iota(jnp.int32, (1, 128), 1) < 64

    def b_dfwd(b, g):
        z = [xd[n, pl.ds(XP * (b // 2 + 8 * (b % 2)), 128), :] for n in (2 * g, 2 * g + 1)]
        if g:
            z = twiddle_d(g, *z)
        z = [cat(v[0:64] + v[64:128], v[0:64] - v[64:128]).astype(bf16) for v in z]
        tu = dot_nt(as_bf16(gf[1, 0:64] if g else gf[0, 0:72]), z[0])
        tv = dot_nt(as_bf16(gf[1, 0:64]), z[1])
        if g == 0:
            tr = cat(tu[0:64], tv[0:64], tu[128:144])
            ti = cat(tu[64:128], tv[64:128], jnp.zeros((16, 128), f32))
        else:
            tr = cat(tu[0:64] - tv[64:128], tu[0:64] + tv[64:128])
            ti = cat(tu[64:128] + tv[0:64], tu[64:128] - tv[0:64])
        return jnp.where(low, tr, ti).astype(bf16), jnp.where(low, ti, tr).astype(bf16)

    def b_sfwd(b, g, ts):
        for c in range(2):
            y = dot(ts[c], as_bf16(gf[2 - c, 0:64]))
            for q in range(2):
                yb[c, b, y_blocks(RES[g][q])] = y[64 * q:64 * q + 64].reshape(8, 8, 128)
            if g == 0:
                yb[c, b, 64] = y[128:136]

    def b_stage1():
        pend = []
        for b in list(range(0, 16, 2)) + list(range(1, 16, 2)):
            for g in range(4):
                pend.append((b, g, b_dfwd(b, g)))
                if len(pend) > 3:
                    b_sfwd(*pend.pop(0))
        for item in pend:
            b_sfwd(*item)

    def b_sinv(tasks):
        row0 = lax.broadcasted_iota(jnp.int32, (8, 128), 0) == 0
        pacer = _Pacer(tasks, 12 * 8)
        for _, b, g in sorted((b + (6 if g == 0 else 0), b, g) for b in range(16) for g in range(4)):
            (ar, br), (ai, bi) = [[yb[c, b, y_blocks(r)].reshape(64, 128) for r in RES[g]] for c in range(2)]
            if g:
                uv = [(ar + br, ai + bi, -ar - br), (ai - bi, br - ar, bi - ai)]
                uv = [(cat(re, im), cat(im, neg)) for re, im, neg in uv]
            else:
                pacer.done()
                na = -ar
                uv = [(cat(ar, jnp.where(row0, yb[0, b, 64], ai[0:8]), ai[8:]),
                       cat(ai, jnp.where(row0, yb[1, b, 64], na[0:8]), na[8:])),
                      (cat(br, bi), cat(bi, -br))]
            for q, (u, v) in enumerate(uv):
                cu = dot_nt(as_bf16(gf[2, 0:32]), u.astype(bf16))
                sv = dot_nt(as_bf16(gf[2, 32:64]), v.astype(bf16))
                xd[2 * g + q, pl.ds(XP * b, 128), :] = cat(cu - sv, cu + sv)
            pacer.feed(cu)

    def b_dinv(t):
        rows = lambda j: cat(*[xd[j, pl.ds(mirror(a), 16, stride=XP), :] for a in range(8 * t, 8 * t + 8)])
        z = [None] * 8
        for j in (4, 5, 6, 7, 2, 3, 0, 1):
            z[j] = dot(rows(j).astype(bf16), as_bf16(gi[min(j, 1)]))
        for g in range(1, 4):
            u, v = z[2 * g], z[2 * g + 1]
            c, sn = [jnp.tile(tw[16 + g, k], (16, 1)) for k in range(2)]
            z[2 * g] = u * c + v * sn
            z[2 * g + 1] = v * c - u * sn if g == 3 else u * sn - v * c
        y = _inv8(z)
        for j in range(8):
            xb[j, t] = y[j].reshape(4, SEG, 128).astype(bf16)

    HALF = NSEG * M // 2
    pre32 = pre.bitcast(u32)

    def store_pre(pair, row0, cs):
        n = cs[0].shape[0] // M
        pre[pair, pl.ds(row0 // M, n)] = jnp.concatenate([c.reshape(n, M, E) for c in cs], axis=1).astype(bf16)

    def batch(u, p0, p1, tasks=(), t0=0, t1=4, margin=4):
        mc = HALF // 2 if t1 == 1 else HALF
        pacer = _Pacer(tasks, (7 * (p1 - p0) - margin // (t1 - t0)) * HALF // 8)
        w = wall.at[u]
        for p in range(p0, p1):
            for r0 in range(0, HALF, mc):
                def blk(head, par):
                    return lambda: cat(*[w[pl.ds((2 * p + head) * WP + 64 * (2 * t + par), 64), :]
                                         for t in range(t0, t1)])

                def prod(i, b):
                    lhs = jnp.concatenate([as_bf16(xs32[i, t, pl.ds(r0 // 2, mc // 2), :])
                                           for t in range(t0, t1)], axis=1)
                    r = dot(lhs, narrow(b))
                    pacer.feed(r)
                    return r

                def emit(half, *cs):
                    park = pl.ds((half * HALF + r0) // 8, mc // 8)
                    if t0 > 0:
                        cs = [c + yb[t, p, park].reshape(mc, E) for t, c in enumerate(cs)]
                    if t1 < 4:
                        for t, c in enumerate(cs):
                            yb[t, p, park] = c.reshape(mc // 8, 8, E)
                    else:
                        store_pre(8 * u + p, half * HALF + r0, cs)
                if t0 // (t1 - t0) % 2:
                    _strassen(prod, blk(1, 0), blk(0, 0), blk(1, 1), blk(0, 1), add2, sub2,
                              lambda half, c1, c0: emit(half, c0, c1))
                else:
                    _strassen(prod, blk(0, 0), blk(1, 0), blk(0, 1), blk(1, 1), add2, sub2, emit)
        pacer.done()

    QUART = HALF // 2
    xs32, xs2_32 = xs.bitcast(u32), xs2.bitcast(u32)

    def strassen2(right, left, emit, pacer):
        def outer_prod(i, bs):
            def prod(j, b):
                r = dot(left(7 * i + j), narrow(b))
                pacer.feed(r)
                return r
            order = (1, 0, 3, 2) if i in (1, 4, 5, 6) else (0, 1, 2, 3)
            cs = {}
            _strassen(prod, *[(lambda b=bs[k]: b) for k in order], add2, sub2, lambda half, *c: cs.update({half: c}))
            return _Blocks((cs[0] + cs[1])[k] for k in order)

        def outer_emit(half, *cs):
            for col in (1, 0):
                for a in range(2):
                    emit(2 * half + a, 2 * col, cs[col][2 * a], cs[col][2 * a + 1])
        outer = lambda k, c: lambda: [right(2 * k + k2, 2 * c + c2) for k2 in range(2) for c2 in range(2)]
        _strassen(outer_prod, outer(0, 0), outer(0, 1), outer(1, 0), outer(1, 1),
                  lambda x, y: [add2(a, b) for a, b in zip(x, y)],
                  lambda x, y: [sub2(a, b) for a, b in zip(x, y)], outer_emit)

    def batch2(u, q0, q1, tasks=(), margin=12):
        pacer = _Pacer(tasks, (49 * (q1 - q0) - margin) * QUART // 8)
        w = wall.at[u]
        for q in range(q0, q1):
            def emit(row, col, *cs):
                store_pre(8 * u + 2 * q + col // 2, row * QUART, cs)
            strassen2(lambda k, c: cat(*[w[pl.ds((4 * q + c) * WP + 64 * (k + 4 * t), 64), :]
                                         for t in range(2)]),
                      lambda i: jnp.concatenate([as_bf16(xs2_32[i, t]) for t in range(2)], axis=1),
                      emit, pacer)
        pacer.done()

    def left2_tasks():
        def make(i, t, r):
            def task(tok):
                a = _strassen_left_one(i, lambda rh, kh: _Blocks(
                    x8[32 * rh + 16 * rl + r, :, pl.ds(128 * (2 * kh + kl + 4 * t), 128)].astype(f32)
                    for rl in range(2) for kl in range(2)))
                a[0], a[3] = after(tok, a[0], a[3])
                for j, v in enumerate(_strassen_left(*a)):
                    xs2[7 * i + j, t, pl.ds(M * r, M), :] = v.astype(bf16)
            return task
        return [make(i, t, r) for i in range(7) for t in range(2) for r in range(16)]

    def left_tasks(n):
        def make(r):
            def task(tok):
                a = [x8[NSEG // 2 * h + r, :, pl.ds(256 * n + 128 * k, 128)].astype(f32)
                     for h in range(2) for k in range(2)]
                a[0], a[3] = after(tok, a[0], a[3])
                for i, v in enumerate(_strassen_left(*a)):
                    xs[i, n, pl.ds(M * r, M), :] = v.astype(bf16)
            return task
        return [make(r) for r in range(NSEG // 2)]

    def piece_tasks(n):
        return [t for both in zip(relayout_tasks(0, 128 * n, 128 * n + 128, (0,)), left_tasks(n)) for t in both]

    def mix(a, b):
        keyed = [(n / len(a), 0, n) for n in range(len(a))] + [(n / len(b), 1, n) for n in range(len(b))]
        return [(a, b)[w][n] for _, w, n in sorted(keyed)]

    run_now = lambda tasks: [task(jnp.zeros((8, 128), u32)) for task in tasks]

    pre32[0:16] = jnp.zeros((16, NSEG, M, E), u32)
    c_a[0][0].wait()
    run_now(left_tasks(0))
    c_a[0][1].wait()
    run_now(relayout_tasks(0, 0, 64))
    c_a[0][2].wait()
    run_now(relayout_tasks(0, 64, 128, (0,)))
    batch(0, 0, 4, relayout_tasks(0, 64, 128, (1,)), 0, 1, margin=8)
    batch(0, 4, 6, (), 0, 1)
    wait_all(c_a[1])
    c_h = [start(wq_hbm.at[pl.ds(256 * n, 256), :, 1], wraw.at[1, pl.ds(256 * n, 256)], n) for n in range(2)]
    batch(0, 6, 8, piece_tasks(1), 0, 1)
    batch(0, 0, 4, relayout_tasks(0, 128, 256, (1,)), 1, 2)
    wait_all(c_a[2])
    batch(0, 4, 8, piece_tasks(2), 1, 2)
    batch(0, 0, 4, relayout_tasks(0, 256, 384, (1,)), 2, 3)
    wait_all(c_a[3])
    c_w2 = start_unit(2)
    batch(0, 4, 8, piece_tasks(3), 2, 3)
    batch(0, 0, 4, relayout_tasks(0, 384, 512, (1,)), 3, 4)
    c_h[0].wait()
    left2 = left2_tasks()
    batch(0, 4, 8, relayout_tasks(1, 0, 256, (0,)), 3, 4)
    batch(1, 0, 4, mix(relayout_tasks(1, 0, 256, (1,)), left2[:74]), 0, 2)
    c_h[1].wait()
    start_unit(3)
    batch(1, 4, 8, mix(relayout_tasks(1, 256, 512, (0,)), left2[74:150]), 0, 2)
    batch(1, 0, 4, mix(relayout_tasks(1, 256, 512, (1,)), left2[150:]), 2, 4)
    c_w2.wait()
    start_unit(4)
    start_unit(5)
    c_b1 = [start(bx_hbm.at[:, :, :, pl.ds(128 * j, 128)], xb.at[j], 5) for j in range(8)]
    c_b1 += [start(gf_hbm, gf, 5), start(tw_hbm, tw, 5)]
    c_loop = [start(wo_hbm.at[:, pl.ds(128 * j, 128)], wo.at[j], 4) for j in range(8)]
    c_loop += [start_x(0, UNROLL, 4), start(mem_hbm, mem0, 4), start(fill_hbm, fill_ref.at[pl.ds(0, 80)], 4)]
    c_loop += start_filter(0, 64, 4)
    batch(1, 4, 8, mix(relayout_tasks(2, pars=(0,)), relayout_tasks(2, 0, 320, (1,))), 2, 4)
    batch2(2, 0, 2, relayout_tasks(2, 320, 512, (1,)), 0)

    def unit_body(u, c):
        slot = (u + 1) % NRAW
        pltpu.make_async_copy(wraw.at[slot], wraw.at[slot], sems.at[slot]).wait()
        batch2(u, 2, 4, relayout_tasks(u + 1, pars=(0,)), 16)
        batch2(u + 1, 0, 2, relayout_tasks(u + 1, pars=(1,)), 4)
        return c
    lax.fori_loop(2, 5, unit_body, 0)
    wait_all(c_b1)
    batch(5, 6, 8, butterfly_tasks(), margin=0)
    batch2(5, 2, 3)
    b_stage1()
    wait_all(c_loop)
    c_rest = [start_x(UNROLL, NSEG - UNROLL, 6)] + start_filter(64, 448, 6)
    c_b3 = [start(w.at[pl.ds(512, 1), :], wl.at[t], 5) for t, w in enumerate((wr_hbm, wi_hbm))]
    c_b3 += [start(gi_hbm, gi, 5)]

    wo32 = wo.bitcast(u32)
    scale = E ** -0.5

    def gated(w, toks):
        if not toks:
            return w
        bits = functools.reduce(
            jnp.bitwise_or, [pltpu.bitcast(jnp.broadcast_to(t, (8, 128)), u32) for t in toks])
        return cat(w[0:8] & all_ones(bits), w[8:])

    def wqkv(i, p, second, toks=(), k0=0, k1=D):
        rows = pl.ds((p % 8 * 2 + second) * WP + k0 // 2, (k1 - k0) // 2)
        return as_bf16(gated(wall[2 * i + p // 8, rows, :], toks))

    def step(n, u, mem, held):
        s = UNROLL * n + u
        rows = cat(mem, xbuf[s].astype(f32))
        lhs = rows.astype(bf16)
        head_start = {}
        if u:
            lo, hi = rows[:, :D // 2].astype(bf16), rows[:, D // 2:].astype(bf16)
            for key in EARLY:
                head_start[key] = dot(lo, wqkv(*key, k1=D // 2))
        fill = fill_ref[pl.ds(0, 80), :]
        heads = [None] * H
        rs = []

        shift = jnp.full((8, 128), 16 - 16 * (n % 2), jnp.int32).astype(u32)
        wblk = pl.ds(pl.multiple_of(64 * (n // 2), 64), 64)
        flt = filter_tasks(
            s, lambda d: [hi_f32(wt.at[t, d, wblk].bitcast(u32)[pl.ds(u, 8, stride=4), :] << shift) for t in range(2)])
        pacer = _Pacer(flt, 84)

        def proj(i, p, toks=()):
            a, b = [
                dot(hi, wqkv(i, p, t, k0=D // 2)) + head_start[i, p, t] if (i, p, t) in head_start
                else dot(lhs, wqkv(i, p, t, toks[t * len(toks) // 2:(t + 1) * len(toks) // 2]))
                for t in range(2)]
            pacer.feed(a)
            pacer.feed(b)
            c = widen(pre32[16 * i + p, s])
            return cat(a, b, c).astype(bf16)

        def probs(q, k):
            sc = dot_nt(q, k) * scale
            sc = jnp.where(fill == 0.0, sc, fill)
            e = jnp.exp(sc - jnp.max(sc, axis=1, keepdims=True))
            l = jnp.sum(e, axis=1, keepdims=True)
            r = pl.reciprocal(l, approx=True)
            r = r * (2.0 - l * r)
            rs.append([r[8 * j:8 * j + 8] for j in range(10)])
            return (e * r).astype(bf16)

        def pv(p, pr, v):
            o = dot(pr, v)
            heads[2 * p] = cat(o[0:8], o[16:32], o[64:72])
            heads[2 * p + 1] = cat(o[32:40], o[48:64], o[72:80])
            held[u, 2 * p], held[u, 2 * p + 1] = o[8:16], o[40:48]

        osum_rows = pl.ds(pl.multiple_of(M * n, M), M)

        def left_task(q, i):
            def task(tok):
                a = _strassen_left_one(i, lambda r, k: _Blocks(
                    held[2 * r + r2, 4 * q + 2 * k + k2] for r2 in range(2) for k2 in range(2)))
                a[0], a[3] = after(tok, a[0], a[3])
                for j, v in enumerate(_strassen_left(*a)):
                    osum[7 * i + j, q, osum_rows, :] = v.astype(bf16)
            return task

        pend = []
        for g in range(4):
            ps = range(4 * g, 4 * g + 4)
            qk = [(proj(0, p), proj(1, p)) for p in ps]
            vs = [proj(2, p, rs[p - 4] if g else ()) for p in ps]
            for a in pend:
                pv(*a)
            pend = [(p, probs(*qk[t]), vs[t]) for t, p in enumerate(ps)]
        pacer.done()

        def wo_part(oc, j, h0, h1, toks=()):
            w = cat(*[wo32[j, pl.ds(64 * head_of(h), 64), :] for h in range(h0, h1)])
            return dot(oc, as_bf16(gated(w, toks)))

        acc = []
        pacer = _Pacer([left_task(q, i) for q in range(8) for i in LEFT_AT[u]], 38)
        oc = jnp.concatenate(heads[0:24], axis=1).astype(bf16)
        for j in range(8):
            acc.append(wo_part(oc, j, 0, 24, {3: rs[12] + rs[13], 4: rs[14] + rs[15]}.get(j, ())))
            if j == 4:
                for a in pend:
                    pv(*a)
            if j >= 5:
                pacer.feed(acc[j])
        oc = jnp.concatenate(heads[24:32], axis=1).astype(bf16)
        nxt = []
        for j in range(8):
            r = wo_part(oc, j, 24, 32) + acc[j]
            outbuf[n, u, pl.ds(M, SEG - M), pl.ds(128 * j, 128)] = r[M:].astype(bf16)
            nxt.append(r[0:M])
            pacer.feed(r)
        pacer.done()
        return jnp.concatenate(nxt, axis=1)

    def steps(n, mem):
        pl.when(n == 1)(functools.partial(wait_all, c_rest))
        held = {}
        for u in range(UNROLL):
            mem = step(n, u, mem, held)
        return mem
    lax.fori_loop(0, NSEG // UNROLL, steps, mem0[...].astype(f32))
    tok_rows = pl.ds(M, SEG - M)
    c_out = [start(outbuf.at[:, :, tok_rows, :], out_hbm.at[:, :, tok_rows, pl.ds(0, D)], 0)]

    wait_all(c_b3)
    b_sinv(filter_tasks(64, lambda d: [wl[t, :, pl.ds(128 * d, 128)].astype(f32) for t in range(2)]))
    for t in range(16):
        b_dinv(t)
    c_out += [start(xb.at[j], out_hbm.at[:, :, :, pl.ds(D + 128 * j, 128)], 0) for j in range(8)]

    osum32 = osum.bitcast(u32)
    for cq in range(2):
        def emit(row, col, *cs):
            idx = (slice(None), row, pl.ds(0, M), pl.ds(128 * (4 * cq + col), 256))
            outbuf[idx] = jnp.concatenate(cs, axis=1).reshape(NSEG // 4, M, 256).astype(bf16)
            c_out.append(start(outbuf.at[idx], out_hbm.at[idx], 0))
        strassen2(lambda k, c: cat(*[wo32[4 * cq + c, pl.ds(64 * head_of(4 * q + k), 64), :] for q in range(8)]),
                  lambda i: jnp.concatenate([as_bf16(osum32[i, q]) for q in range(8)], axis=1),
                  emit, _Pacer((), 0))
    wait_all(c_out)


@jax.jit
def pallas_concat_heads__memory_aug_recurrent_mem_tr__spectral_gfnet__prompt_kernel(
    A_x: jax.Array,
    A_mem0: jax.Array,
    A_Wq: jax.Array,
    A_Wk: jax.Array,
    A_Wv: jax.Array,
    A_Wo: jax.Array,
    A_seg_len: jax.Array,
    B_x: jax.Array,
    B_w_r: jax.Array,
    B_w_i: jax.Array,
):
    del A_seg_len
    assert A_x.shape == (1, S, D) and A_mem0.shape == (1, M, D) and B_x.shape == (1, S, D)
    assert A_Wq.shape == (D, H, E) and A_Wo.shape == (H, E, D) and B_w_r.shape == (S, D // 2 + 1)
    gf, gi, tw = _dft_constants()
    fill = _attn_fill()
    hbm = pl.BlockSpec(memory_space=pltpu.HBM)
    wshape = (D // 2, 2, 2, 16, E)
    out = pl.pallas_call(
        _kernel,
        out_shape=jax.ShapeDtypeStruct((NSEG // 4, 4, SEG, 2 * D), bf16),
        in_specs=[hbm] * 13,
        out_specs=hbm,
        scratch_shapes=[
            pltpu.VMEM((NRAW, D // 2, 2, 16, E), bf16),
            pltpu.VMEM((6, 16 * WP, E), u32),
            pltpu.VMEM((8, H * E, 128), bf16),
            pltpu.VMEM((NSEG, SEG - M, D), bf16),
            pltpu.VMEM((M, D), bf16),
            pltpu.VMEM((NSEG, M, D), bf16),
            pltpu.VMEM((7, 4, 256, 128), bf16),
            pltpu.VMEM((49, 2, 128, 128), bf16),
            pltpu.VMEM((48, NSEG, 2 * M, E), bf16),
            pltpu.VMEM((49, 8, NSEG * M // 4, E), bf16),
            pltpu.VMEM((NSEG // 4, 4, SEG, D), bf16),
            pltpu.VMEM((96, 80), f32),
            pltpu.VMEM((8, NSEG // 4, 4, SEG, 128), bf16),
            pltpu.VMEM((2, 16, 512, 128), bf16),
            pltpu.VMEM((2, 1, S), bf16),
            pltpu.VMEM(gf.shape, u32),
            pltpu.VMEM(gi.shape, u32),
            pltpu.VMEM(tw.shape, f32),
            pltpu.VMEM((8, 16 * XP, 128), f32),
            pltpu.VMEM((2, 16, 65, 8, 128), f32),
            pltpu.SemaphoreType.DMA((7,)),
        ],
        compiler_params=pltpu.CompilerParams(vmem_limit_bytes=120 * 1024 * 1024),
    )(A_x.reshape(NSEG, SEG, D), A_mem0.reshape(M, D),
      A_Wq.reshape(wshape), A_Wk.reshape(wshape), A_Wv.reshape(wshape),
      A_Wo.reshape(H * E, D), B_x.reshape(NSEG // 4, 4, SEG, D), B_w_r.T, B_w_i.T, gf, gi, tw, fill)
    return out.reshape(1, S, 2 * D)
```

```python
import functools

import jax
import jax.numpy as jnp
import numpy as np
from jax import lax
from jax.experimental import pallas as pl
from jax.experimental.pallas import tpu as pltpu

S, D, H, E, M, SEG = 2048, 1024, 32, 128, 8, 32
NSEG = S // SEG
WP = 516
XP = 132
NRAW = 4
UNROLL = 4
LEFT_AT = ((), (2,), (4,), (0, 1, 3, 5, 6))
EARLY = ((0, 0, 0), (0, 0, 1), (1, 0, 0), (1, 0, 1), (0, 1, 0))
bf16, f32, u32 = jnp.bfloat16, jnp.float32, jnp.uint32
RES = ((0, 4), (2, 6), (1, 7), (3, 5))
RC = float(np.sqrt(0.5))


def _fwd8(x):
    s04, d04 = x[0] + x[4], x[0] - x[4]
    s26, d26 = x[2] + x[6], x[2] - x[6]
    s15, d15 = x[1] + x[5], x[1] - x[5]
    s37, d37 = x[3] + x[7], x[3] - x[7]
    t1, t2 = (d15 - d37) * RC, (d15 + d37) * RC
    e0, o0 = s04 + s26, s15 + s37
    return [e0 + o0, e0 - o0, s04 - s26, s15 - s37, d04 + t1, d26 + t2, d04 - t1, d26 - t2]


def _inv8(z):
    z0, z4, e1, o1, r1, i1, r3, i3 = z
    e0, o0 = z0 + z4, z0 - z4
    s04, s26, s15, s37 = e0 + e1, e0 - e1, o0 + o1, o0 - o1
    d04, d26 = r1 + r3, i1 + i3
    t1, t2 = (r1 - r3) * RC, (i1 - i3) * RC
    d15, d37 = t1 + t2, t2 - t1
    return [s04 + d04, s15 + d15, s26 + d26, s37 + d37, s04 - d04, s15 - d15, s26 - d26, s37 - d37]


def _twiddle16(z, k):
    re, im = z
    k = k % 16
    if k == 0:
        return z
    if k == 4:
        return (im, -re)
    if k == 12:
        return (-im, re)
    if k == 2:
        return ((re + im) * RC, (im - re) * RC)
    if k == 14:
        return ((re - im) * RC, (re + im) * RC)
    if k == 6:
        return ((im - re) * RC, (re + im) * -RC)
    if k == 10:
        return ((re + im) * -RC, (re - im) * RC)
    c, s = float(np.cos(2 * np.pi * k / 16)), float(-np.sin(2 * np.pi * k / 16))
    return (re * c - im * s, re * s + im * c)


def _bfly4(z, sign):
    (ar, ai), (br, bi), (cr, ci), (dr, di) = z
    sr, si, tr, ti = ar + cr, ai + ci, ar - cr, ai - ci
    ur, ui, vr, vi = br + dr, bi + di, br - dr, bi - di
    o0, o2 = (sr + ur, si + ui), (sr - ur, si - ui)
    p, q = (tr + vi, ti - vr), (tr - vi, ti + vr)
    return [o0, p, o2, q] if sign > 0 else [o0, q, o2, p]


class _Pacer:
    def __init__(self, tasks, ntokens):
        self.slots = {}
        for n, task in enumerate(tasks):
            self.slots.setdefault(n * ntokens // len(tasks), []).append(task)
        self.pos = 0

    def feed(self, r):
        for j in range(r.shape[0] // 8):
            for task in self.slots.pop(self.pos, []):
                task(pltpu.bitcast(r[8 * j:8 * j + 8], u32))
            self.pos += 1

    def done(self):
        assert not self.slots


def _pack_rows(m):
    b = np.asarray(m, np.float32).astype(jnp.bfloat16).view(np.uint16).astype(np.uint32)
    return b[..., 0::2, :] | (b[..., 1::2, :] << 16)


def _dft_constants():
    i, j = np.arange(64)[:, None], np.arange(128)
    whole, half = 2 * np.pi * i * j / 128, 2 * np.pi * (i + 0.5) * j / 128
    gf = np.zeros((3, 192, 128))
    gf[0, :129] = np.concatenate([np.cos(whole), -np.sin(whole), [(-1.0) ** j]])
    gf[1, :128] = np.concatenate([np.cos(half), -np.sin(half)])
    gf[2, :128] = np.concatenate([np.cos(half), np.sin(half)])
    gi = gf[0:2, :128] * (2.0 / (D * S))
    gi[0, 0], gi[0, 64] = gf[0, 0] / (D * S), gf[0, 128] / (D * S)
    angs = [2 * np.pi * j * (b - 8) / S for b in range(16)] + [2 * np.pi * j * (r - 4) / D for r, _ in RES]
    tw = np.zeros((20, 2, 8, 128), np.float32)
    for n, ang in enumerate(angs):
        tw[n, 0], tw[n, 1] = np.cos(ang), -np.sin(ang)
    return _pack_rows(gf), _pack_rows(gi), tw


def _attn_fill():
    head = np.concatenate([np.arange(64) // 32, np.arange(16) // 8])
    pos = np.concatenate([np.arange(64) % 32, 32 + np.arange(16) % 8])
    ok = (pos[:, None] < M) | (pos[:, None] >= pos[None, :])
    fill = np.where(ok, 0.0, -1e9)
    fill = np.where(head[:, None] == head[None, :], fill, -np.inf)
    return fill.astype(np.float32)


def _strassen(prod, b11, b12, b21, b22, add, sub, emit):
    m2 = prod(1, b11())
    m1 = prod(0, add(b11(), b22()))
    m3 = prod(2, sub(b12(), b22()))
    c22 = prod(5, add(b11(), b12())) + ((m1 - m2) + m3)
    m4 = prod(3, sub(b21(), b11()))
    emit(1, m2 + m4, c22)
    m5 = prod(4, b22())
    emit(0, prod(6, add(b21(), b22())) + ((m1 + m4) - m5), m3 + m5)


class _Blocks(list):
    def __add__(self, other):
        return _Blocks(a + b for a, b in zip(self, other))

    def __sub__(self, other):
        return _Blocks(a - b for a, b in zip(self, other))


def _strassen_left(a11, a12, a21, a22):
    return [a11 + a22, a21 + a22, a11, a22, a11 + a12, a21 - a11, a12 - a22]


def _strassen_left_one(i, blk):
    terms = ((0, 3, 1), (2, 3, 1), (0,), (3,), (0, 1, 1), (2, 0, -1), (1, 3, -1))[i]
    a = blk(*divmod(terms[0], 2))
    if len(terms) == 1:
        return a
    b = blk(*divmod(terms[1], 2))
    return a + b if terms[2] > 0 else a - b


def _kernel(x_hbm, mem_hbm, wq_hbm, wk_hbm, wv_hbm, wo_hbm, bx_hbm, wr_hbm, wi_hbm,
            gf_hbm, gi_hbm, tw_hbm, fill_hbm, out_hbm,
            wraw, wall, wo, xbuf, mem0, x8, xs, xs2, pre, osum, outbuf, fill_ref,
            xb, wt, wl, gf, gi, tw, xd, yb, sems):
    def start(src, dst, sem):
        c = pltpu.make_async_copy(src, dst, sems.at[sem])
        c.start()
        return c

    def wait_all(cs):
        for c in cs:
            c.wait()

    dot = functools.partial(jnp.dot, preferred_element_type=f32)
    dot_nt = lambda a, b: lax.dot_general(a, b, (((1,), (1,)), ((), ())), preferred_element_type=f32)
    cat = lambda *vs: jnp.concatenate(vs, axis=0)
    as_bf16 = lambda w: pltpu.bitcast(w, bf16)
    hi_f32 = lambda w: pltpu.bitcast(w & u32(0xFFFF0000), f32)
    all_ones = lambda tok: ((tok >> 16) | u32(0xFFFF)) | u32(0xFFFF0000)

    def after(tok, *vs):
        ones = all_ones(tok)
        return [pltpu.bitcast(pltpu.bitcast(v, u32) & ones, f32) for v in vs]

    widen = lambda w: as_bf16(w).astype(f32) if w.dtype == u32 else w
    narrow = lambda w: as_bf16(w) if w.dtype == u32 else w.astype(bf16)
    add2 = lambda a, b: widen(a) + widen(b)
    sub2 = lambda a, b: widen(a) - widen(b)
    w_hbm = (wq_hbm, wk_hbm, wv_hbm)

    def start_unit(u):
        return start(w_hbm[u // 2].at[:, :, u % 2], wraw.at[u % NRAW], u % NRAW)

    def start_x(seg0, nseg, sem):
        segs, rows = pl.ds(seg0, nseg), pl.ds(0, SEG - M)
        return start(x_hbm.at[segs, rows, :], xbuf.at[segs], sem)

    def start_filter(row0, nrows, sem):
        rows = pl.ds(row0, nrows)
        return [start(w.at[rows, pl.ds(128 * d, 128)], wt.at[t, d, rows], sem)
                for t, w in enumerate((wr_hbm, wi_hbm)) for d in range(16)]

    def start_piece(n, xsem, parts):
        cols = pl.ds(256 * n, 256)
        cs = [start(x_hbm.at[:, pl.ds(SEG - M, M), cols], x8.at[:, :, cols], xsem)]
        for k, sem in enumerate(parts):
            rows = pl.ds(128 * n + 128 // len(parts) * k, 128 // len(parts))
            cs.append(start(wq_hbm.at[rows, :, 0], wraw.at[0, rows], sem))
        return cs
    c_a = [start_piece(0, 5, (6, 0))] + [start_piece(n, n, (n,)) for n in range(1, 4)]

    xb32 = xb.bitcast(u32)

    head_of = lambda slot: slot // 16 * 16 + slot % 8 * 2 + slot % 16 // 8

    def relayout_tasks(u, r0=0, r1=D // 2, pars=(0, 1)):
        src, dst = wraw.at[u % NRAW], wall.at[u]
        step = 4 // len(pars)

        def make(rows):
            def task(tok):
                mask = [(tok << 16) | u32(0xFFFF0000) if par else (tok >> 16) | u32(0xFFFF) for par in pars]
                for r in rows:
                    words = src.at[r].bitcast(u32)
                    a, b = words[0], words[1]
                    for par, m in zip(pars, mask):
                        dst[pl.ds(r + 8 * WP * par, 8, stride=WP), :] = (
                            (a >> 16) | (b & m) if par else (a & m) | (b << 16))
            return task
        return [make(range(r, r + step)) for r in range(r0, r1, step)]

    def y_blocks(r):
        return pl.ds(4 * (r % 2) + r // 2, 8, stride=8)

    def filter_tasks(blk, wfn):
        def make(phase, k):
            slots = [4 * k + j for j in range(4)] if phase == 1 else [4 * j + k for j in range(4)]

            def task(tok):
                z = [(yb[0, b, blk], yb[1, b, blk]) for b in slots]
                if phase == 0:
                    z = list(zip(after(tok, *[zr for zr, _ in z]), [zi for _, zi in z]))
                    z = [(zr * tw[b, 0] - zi * tw[b, 1], zr * tw[b, 1] + zi * tw[b, 0]) if b != 8 else (zr, zi)
                         for b, (zr, zi) in zip(slots, z)]
                else:
                    z[0] = after(tok, *z[0])
                if phase == 0:
                    o = _bfly4(z, 1)
                    o = [_twiddle16(o[j], k * j) for j in range(4)]
                elif phase == 1:
                    o = _bfly4(z, 1)
                    y = []
                    for j in range(4):
                        wr, wi = wfn(k + 4 * j)
                        xr, xi = o[j]
                        y.append((xr * wr - xi * wi, xr * wi + xi * wr))
                    o = _bfly4(y, -1)
                    o = [_twiddle16(o[j], -k * j) for j in range(4)]
                else:
                    o = [(zr * tw[b, 0] + zi * tw[b, 1], zi * tw[b, 0] - zr * tw[b, 1]) if b != 8 else (zr, zi)
                         for b, (zr, zi) in zip(slots, _bfly4(z, -1))]
                for b, v in zip(slots, o):
                    yb[0, b, blk] = v[0]
                    yb[1, b, blk] = v[1]
            return task
        return [make(phase, k) for phase in range(3) for k in range(4)]

    mirror = lambda a: a if a < 64 else 191 - a

    def twiddle_d(g, x, y):
        c, sn = [jnp.tile(tw[16 + g, k], (x.shape[0] // 8, 1)) for k in range(2)]
        return (x * c - y * sn, x * sn + y * c) if g == 3 else (x * c + y * sn, x * sn - y * c)

    def butterfly_tasks():
        def make(a, par):
            def task(tok):
                w = [xb32[j, a // 8, a // 2 % 4, pl.ds(8 * (a % 2), 8), :] for j in range(8)]
                if par:
                    hi = (tok << 16) | u32(0xFFFF0000)
                    z = _fwd8([pltpu.bitcast(v & hi, f32) for v in w])
                else:
                    sixteen = ((tok >> 31) | u32(1)) << 4
                    z = _fwd8([pltpu.bitcast(v << sixteen, f32) for v in w])
                for n in range(8):
                    xd[n, pl.ds(8 * XP * par + mirror(a), 8, stride=XP), :] = z[n]
            return task
        return [make(a, par) for a in range(128) for par in range(2)]

    low = lax.broadcasted_iota(jnp.int32, (1, 128), 1) < 64

    def b_dfwd(b, g):
        z = [xd[n, pl.ds(XP * (b // 2 + 8 * (b % 2)), 128), :] for n in (2 * g, 2 * g + 1)]
        if g:
            z = twiddle_d(g, *z)
        z = [cat(v[0:64] + v[64:128], v[0:64] - v[64:128]).astype(bf16) for v in z]
        tu = dot_nt(as_bf16(gf[1, 0:64] if g else gf[0, 0:72]), z[0])
        tv = dot_nt(as_bf16(gf[1, 0:64]), z[1])
        if g == 0:
            tr = cat(tu[0:64], tv[0:64], tu[128:144])
            ti = cat(tu[64:128], tv[64:128], jnp.zeros((16, 128), f32))
        else:
            tr = cat(tu[0:64] - tv[64:128], tu[0:64] + tv[64:128])
            ti = cat(tu[64:128] + tv[0:64], tu[64:128] - tv[0:64])
        return jnp.where(low, tr, ti).astype(bf16), jnp.where(low, ti, tr).astype(bf16)

    def b_sfwd(b, g, ts):
        for c in range(2):
            y = dot(ts[c], as_bf16(gf[2 - c, 0:64]))
            for q in range(2):
                yb[c, b, y_blocks(RES[g][q])] = y[64 * q:64 * q + 64].reshape(8, 8, 128)
            if g == 0:
                yb[c, b, 64] = y[128:136]

    def b_stage1():
        pend = []
        for b in list(range(0, 16, 2)) + list(range(1, 16, 2)):
            for g in range(4):
                pend.append((b, g, b_dfwd(b, g)))
                if len(pend) > 3:
                    b_sfwd(*pend.pop(0))
        for item in pend:
            b_sfwd(*item)

    def b_sinv(tasks):
        row0 = lax.broadcasted_iota(jnp.int32, (8, 128), 0) == 0
        pacer = _Pacer(tasks, 12 * 8)
        for _, b, g in sorted((b + (6 if g == 0 else 0), b, g) for b in range(16) for g in range(4)):
            (ar, br), (ai, bi) = [[yb[c, b, y_blocks(r)].reshape(64, 128) for r in RES[g]] for c in range(2)]
            if g:
                uv = [(ar + br, ai + bi, -ar - br), (ai - bi, br - ar, bi - ai)]
                uv = [(cat(re, im), cat(im, neg)) for re, im, neg in uv]
            else:
                pacer.done()
                na = -ar
                uv = [(cat(ar, jnp.where(row0, yb[0, b, 64], ai[0:8]), ai[8:]),
                       cat(ai, jnp.where(row0, yb[1, b, 64], na[0:8]), na[8:])),
                      (cat(br, bi), cat(bi, -br))]
            for q, (u, v) in enumerate(uv):
                cu = dot_nt(as_bf16(gf[2, 0:32]), u.astype(bf16))
                sv = dot_nt(as_bf16(gf[2, 32:64]), v.astype(bf16))
                xd[2 * g + q, pl.ds(XP * b, 128), :] = cat(cu - sv, cu + sv)
            pacer.feed(cu)

    def b_dinv(t):
        rows = lambda j: cat(*[xd[j, pl.ds(mirror(a), 16, stride=XP), :] for a in range(8 * t, 8 * t + 8)])
        z = [None] * 8
        for j in (4, 5, 6, 7, 2, 3, 0, 1):
            z[j] = dot(rows(j).astype(bf16), as_bf16(gi[min(j, 1)]))
        for g in range(1, 4):
            u, v = z[2 * g], z[2 * g + 1]
            c, sn = [jnp.tile(tw[16 + g, k], (16, 1)) for k in range(2)]
            z[2 * g] = u * c + v * sn
            z[2 * g + 1] = v * c - u * sn if g == 3 else u * sn - v * c
        y = _inv8(z)
        for j in range(8):
            xb[j, t] = y[j].reshape(4, SEG, 128).astype(bf16)

    HALF = NSEG * M // 2
    pre32 = pre.bitcast(u32)

    def store_pre(pair, row0, cs):
        n = cs[0].shape[0] // M
        pre[pair, pl.ds(row0 // M, n)] = jnp.concatenate([c.reshape(n, M, E) for c in cs], axis=1).astype(bf16)

    def batch(u, p0, p1, tasks=(), t0=0, t1=4, margin=4):
        pacer = _Pacer(tasks, (7 * (p1 - p0) - margin // (t1 - t0)) * HALF // 8)
        w = wall.at[u]
        for p in range(p0, p1):
            def blk(head, par):
                return lambda: cat(*[w[pl.ds((2 * p + head) * WP + 64 * (2 * t + par), 64), :]
                                     for t in range(t0, t1)])

            def prod(i, b):
                r = dot(jnp.concatenate([as_bf16(xs32[i, t]) for t in range(t0, t1)], axis=1), narrow(b))
                pacer.feed(r)
                return r

            def emit(half, *cs):
                park = pl.ds(half * HALF // 8, HALF // 8)
                if t0 > 0:
                    cs = [c + yb[t, p, park].reshape(HALF, E) for t, c in enumerate(cs)]
                if t1 < 4:
                    for t, c in enumerate(cs):
                        yb[t, p, park] = c.reshape(HALF // 8, 8, E)
                else:
                    store_pre(8 * u + p, half * HALF, cs)
            if t0 // (t1 - t0) % 2:
                _strassen(prod, blk(1, 0), blk(0, 0), blk(1, 1), blk(0, 1), add2, sub2,
                          lambda half, c1, c0: emit(half, c0, c1))
            else:
                _strassen(prod, blk(0, 0), blk(1, 0), blk(0, 1), blk(1, 1), add2, sub2, emit)
        pacer.done()

    QUART = HALF // 2
    xs32, xs2_32 = xs.bitcast(u32), xs2.bitcast(u32)

    def strassen2(right, left, emit, pacer):
        def outer_prod(i, bs):
            def prod(j, b):
                r = dot(left(7 * i + j), narrow(b))
                pacer.feed(r)
                return r
            order = (1, 0, 3, 2) if i in (1, 4, 5, 6) else (0, 1, 2, 3)
            cs = {}
            _strassen(prod, *[(lambda b=bs[k]: b) for k in order], add2, sub2, lambda half, *c: cs.update({half: c}))
            return _Blocks((cs[0] + cs[1])[k] for k in order)

        def outer_emit(half, *cs):
            for col in (1, 0):
                for a in range(2):
                    emit(2 * half + a, 2 * col, cs[col][2 * a], cs[col][2 * a + 1])
        outer = lambda k, c: lambda: [right(2 * k + k2, 2 * c + c2) for k2 in range(2) for c2 in range(2)]
        _strassen(outer_prod, outer(0, 0), outer(0, 1), outer(1, 0), outer(1, 1),
                  lambda x, y: [add2(a, b) for a, b in zip(x, y)],
                  lambda x, y: [sub2(a, b) for a, b in zip(x, y)], outer_emit)

    def batch2(u, q0, q1, tasks=(), margin=12):
        pacer = _Pacer(tasks, (49 * (q1 - q0) - margin) * QUART // 8)
        w = wall.at[u]
        for q in range(q0, q1):
            def emit(row, col, *cs):
                store_pre(8 * u + 2 * q + col // 2, row * QUART, cs)
            strassen2(lambda k, c: cat(*[w[pl.ds((4 * q + c) * WP + 64 * (k + 4 * t), 64), :]
                                         for t in range(2)]),
                      lambda i: jnp.concatenate([as_bf16(xs2_32[i, t]) for t in range(2)], axis=1),
                      emit, pacer)
        pacer.done()

    def left2_tasks():
        def make(i, t, r):
            def task(tok):
                a = _strassen_left_one(i, lambda rh, kh: _Blocks(
                    x8[32 * rh + 16 * rl + r, :, pl.ds(128 * (2 * kh + kl + 4 * t), 128)].astype(f32)
                    for rl in range(2) for kl in range(2)))
                a[0], a[3] = after(tok, a[0], a[3])
                for j, v in enumerate(_strassen_left(*a)):
                    xs2[7 * i + j, t, pl.ds(M * r, M), :] = v.astype(bf16)
            return task
        return [make(i, t, r) for i in range(7) for t in range(2) for r in range(16)]

    def left_tasks(n):
        def make(r):
            def task(tok):
                a = [x8[NSEG // 2 * h + r, :, pl.ds(256 * n + 128 * k, 128)].astype(f32)
                     for h in range(2) for k in range(2)]
                a[0], a[3] = after(tok, a[0], a[3])
                for i, v in enumerate(_strassen_left(*a)):
                    xs[i, n, pl.ds(M * r, M), :] = v.astype(bf16)
            return task
        return [make(r) for r in range(NSEG // 2)]

    def piece_tasks(n):
        return [t for both in zip(relayout_tasks(0, 128 * n, 128 * n + 128, (0,)), left_tasks(n)) for t in both]

    def mix(a, b):
        keyed = [(n / len(a), 0, n) for n in range(len(a))] + [(n / len(b), 1, n) for n in range(len(b))]
        return [(a, b)[w][n] for _, w, n in sorted(keyed)]

    run_now = lambda tasks: [task(jnp.zeros((8, 128), u32)) for task in tasks]

    pre32[0:16] = jnp.zeros((16, NSEG, M, E), u32)
    c_a[0][0].wait()
    run_now(left_tasks(0))
    c_a[0][1].wait()
    run_now(relayout_tasks(0, 0, 64))
    c_a[0][2].wait()
    run_now(relayout_tasks(0, 64, 128, (0,)))
    batch(0, 0, 4, relayout_tasks(0, 64, 128, (1,)), 0, 1, margin=8)
    batch(0, 4, 8, (), 0, 1)
    wait_all(c_a[1])
    c_h = [start(wq_hbm.at[pl.ds(256 * n, 256), :, 1], wraw.at[1, pl.ds(256 * n, 256)], n) for n in range(2)]
    run_now(piece_tasks(1))
    batch(0, 0, 4, relayout_tasks(0, 128, 256, (1,)), 1, 2)
    wait_all(c_a[2])
    batch(0, 4, 8, piece_tasks(2), 1, 2)
    batch(0, 0, 4, relayout_tasks(0, 256, 384, (1,)), 2, 3)
    wait_all(c_a[3])
    c_w2 = start_unit(2)
    batch(0, 4, 8, piece_tasks(3), 2, 3)
    batch(0, 0, 4, relayout_tasks(0, 384, 512, (1,)), 3, 4)
    c_h[0].wait()
    left2 = left2_tasks()
    batch(0, 4, 8, relayout_tasks(1, 0, 256, (0,)), 3, 4)
    batch(1, 0, 4, mix(relayout_tasks(1, 0, 256, (1,)), left2[:74]), 0, 2)
    c_h[1].wait()
    start_unit(3)
    batch(1, 4, 8, mix(relayout_tasks(1, 256, 512, (0,)), left2[74:150]), 0, 2)
    batch(1, 0, 4, mix(relayout_tasks(1, 256, 512, (1,)), left2[150:]), 2, 4)
    c_w2.wait()
    start_unit(4)
    start_unit(5)
    c_b1 = [start(bx_hbm.at[:, :, :, pl.ds(128 * j, 128)], xb.at[j], 5) for j in range(8)]
    c_b1 += [start(gf_hbm, gf, 5), start(tw_hbm, tw, 5)]
    c_loop = [start(wo_hbm.at[:, pl.ds(128 * j, 128)], wo.at[j], 4) for j in range(8)]
    c_loop += [start_x(0, UNROLL, 4), start(mem_hbm, mem0, 4), start(fill_hbm, fill_ref.at[pl.ds(0, 80)], 4)]
    c_loop += start_filter(0, 64, 4)
    batch(1, 4, 8, mix(relayout_tasks(2, pars=(0,)), relayout_tasks(2, 0, 320, (1,))), 2, 4)
    batch2(2, 0, 2, relayout_tasks(2, 320, 512, (1,)), 0)

    def unit_body(u, c):
        slot = (u + 1) % NRAW
        pltpu.make_async_copy(wraw.at[slot], wraw.at[slot], sems.at[slot]).wait()
        batch2(u, 2, 4, relayout_tasks(u + 1, pars=(0,)), 16)
        batch2(u + 1, 0, 2, relayout_tasks(u + 1, pars=(1,)), 4)
        return c
    lax.fori_loop(2, 5, unit_body, 0)
    wait_all(c_b1)
    batch(5, 6, 8, butterfly_tasks(), margin=0)
    batch2(5, 2, 3)
    b_stage1()
    wait_all(c_loop)
    c_rest = [start_x(UNROLL, NSEG - UNROLL, 6)] + start_filter(64, 448, 6)
    c_b3 = [start(w.at[pl.ds(512, 1), :], wl.at[t], 5) for t, w in enumerate((wr_hbm, wi_hbm))]
    c_b3 += [start(gi_hbm, gi, 5)]

    wo32 = wo.bitcast(u32)
    scale = E ** -0.5

    def gated(w, toks):
        if not toks:
            return w
        bits = functools.reduce(
            jnp.bitwise_or, [pltpu.bitcast(jnp.broadcast_to(t, (8, 128)), u32) for t in toks])
        return cat(w[0:8] & all_ones(bits), w[8:])

    def wqkv(i, p, second, toks=(), k0=0, k1=D):
        rows = pl.ds((p % 8 * 2 + second) * WP + k0 // 2, (k1 - k0) // 2)
        return as_bf16(gated(wall[2 * i + p // 8, rows, :], toks))

    def step(n, u, mem, held):
        s = UNROLL * n + u
        rows = cat(mem, xbuf[s].astype(f32))
        lhs = rows.astype(bf16)
        head_start = {}
        if u:
            lo, hi = rows[:, :D // 2].astype(bf16), rows[:, D // 2:].astype(bf16)
            for key in EARLY:
                head_start[key] = dot(lo, wqkv(*key, k1=D // 2))
        fill = fill_ref[pl.ds(0, 80), :]
        heads = [None] * H
        rs = []

        shift = jnp.full((8, 128), 16 - 16 * (n % 2), jnp.int32).astype(u32)
        wblk = pl.ds(pl.multiple_of(64 * (n // 2), 64), 64)
        flt = filter_tasks(
            s, lambda d: [hi_f32(wt.at[t, d, wblk].bitcast(u32)[pl.ds(u, 8, stride=4), :] << shift) for t in range(2)])
        pacer = _Pacer(flt, 84)

        def proj(i, p, toks=()):
            a, b = [
                dot(hi, wqkv(i, p, t, k0=D // 2)) + head_start[i, p, t] if (i, p, t) in head_start
                else dot(lhs, wqkv(i, p, t, toks[t * len(toks) // 2:(t + 1) * len(toks) // 2]))
                for t in range(2)]
            pacer.feed(a)
            pacer.feed(b)
            c = widen(pre32[16 * i + p, s])
            return cat(a, b, c).astype(bf16)

        def probs(q, k):
            sc = dot_nt(q, k) * scale
            sc = jnp.where(fill == 0.0, sc, fill)
            e = jnp.exp(sc - jnp.max(sc, axis=1, keepdims=True))
            l = jnp.sum(e, axis=1, keepdims=True)
            r = pl.reciprocal(l, approx=True)
            r = r * (2.0 - l * r)
            rs.append([r[8 * j:8 * j + 8] for j in range(10)])
            return (e * r).astype(bf16)

        def pv(p, pr, v):
            o = dot(pr, v)
            heads[2 * p] = cat(o[0:8], o[16:32], o[64:72])
            heads[2 * p + 1] = cat(o[32:40], o[48:64], o[72:80])
            held[u, 2 * p], held[u, 2 * p + 1] = o[8:16], o[40:48]

        osum_rows = pl.ds(pl.multiple_of(M * n, M), M)

        def left_task(q, i):
            def task(tok):
                a = _strassen_left_one(i, lambda r, k: _Blocks(
                    held[2 * r + r2, 4 * q + 2 * k + k2] for r2 in range(2) for k2 in range(2)))
                a[0], a[3] = after(tok, a[0], a[3])
                for j, v in enumerate(_strassen_left(*a)):
                    osum[7 * i + j, q, osum_rows, :] = v.astype(bf16)
            return task

        pend = []
        for g in range(4):
            ps = range(4 * g, 4 * g + 4)
            qk = [(proj(0, p), proj(1, p)) for p in ps]
            vs = [proj(2, p, rs[p - 4] if g else ()) for p in ps]
            for a in pend:
                pv(*a)
            pend = [(p, probs(*qk[t]), vs[t]) for t, p in enumerate(ps)]
        pacer.done()

        def wo_part(oc, j, h0, h1, toks=()):
            w = cat(*[wo32[j, pl.ds(64 * head_of(h), 64), :] for h in range(h0, h1)])
            return dot(oc, as_bf16(gated(w, toks)))

        acc = []
        pacer = _Pacer([left_task(q, i) for q in range(8) for i in LEFT_AT[u]], 38)
        oc = jnp.concatenate(heads[0:24], axis=1).astype(bf16)
        for j in range(8):
            acc.append(wo_part(oc, j, 0, 24, {3: rs[12] + rs[13], 4: rs[14] + rs[15]}.get(j, ())))
            if j == 4:
                for a in pend:
                    pv(*a)
            if j >= 5:
                pacer.feed(acc[j])
        oc = jnp.concatenate(heads[24:32], axis=1).astype(bf16)
        nxt = []
        for j in range(8):
            r = wo_part(oc, j, 24, 32) + acc[j]
            outbuf[n, u, pl.ds(M, SEG - M), pl.ds(128 * j, 128)] = r[M:].astype(bf16)
            nxt.append(r[0:M])
            pacer.feed(r)
        pacer.done()
        return jnp.concatenate(nxt, axis=1)

    def steps(n, mem):
        pl.when(n == 1)(functools.partial(wait_all, c_rest))
        held = {}
        for u in range(UNROLL):
            mem = step(n, u, mem, held)
        return mem
    lax.fori_loop(0, NSEG // UNROLL, steps, mem0[...].astype(f32))
    tok_rows = pl.ds(M, SEG - M)
    c_out = [start(outbuf.at[:, :, tok_rows, :], out_hbm.at[:, :, tok_rows, pl.ds(0, D)], 0)]

    wait_all(c_b3)
    b_sinv(filter_tasks(64, lambda d: [wl[t, :, pl.ds(128 * d, 128)].astype(f32) for t in range(2)]))
    for t in range(16):
        b_dinv(t)
    c_out += [start(xb.at[j], out_hbm.at[:, :, :, pl.ds(D + 128 * j, 128)], 0) for j in range(8)]

    osum32 = osum.bitcast(u32)
    for cq in range(2):
        def emit(row, col, *cs):
            idx = (slice(None), row, pl.ds(0, M), pl.ds(128 * (4 * cq + col), 256))
            outbuf[idx] = jnp.concatenate(cs, axis=1).reshape(NSEG // 4, M, 256).astype(bf16)
            c_out.append(start(outbuf.at[idx], out_hbm.at[idx], 0))
        strassen2(lambda k, c: cat(*[wo32[4 * cq + c, pl.ds(64 * head_of(4 * q + k), 64), :] for q in range(8)]),
                  lambda i: jnp.concatenate([as_bf16(osum32[i, q]) for q in range(8)], axis=1),
                  emit, _Pacer((), 0))
    wait_all(c_out)


@jax.jit
def pallas_concat_heads__memory_aug_recurrent_mem_tr__spectral_gfnet__prompt_kernel(
    A_x: jax.Array,
    A_mem0: jax.Array,
    A_Wq: jax.Array,
    A_Wk: jax.Array,
    A_Wv: jax.Array,
    A_Wo: jax.Array,
    A_seg_len: jax.Array,
    B_x: jax.Array,
    B_w_r: jax.Array,
    B_w_i: jax.Array,
):
    del A_seg_len
    assert A_x.shape == (1, S, D) and A_mem0.shape == (1, M, D) and B_x.shape == (1, S, D)
    assert A_Wq.shape == (D, H, E) and A_Wo.shape == (H, E, D) and B_w_r.shape == (S, D // 2 + 1)
    gf, gi, tw = _dft_constants()
    fill = _attn_fill()
    hbm = pl.BlockSpec(memory_space=pltpu.HBM)
    wshape = (D // 2, 2, 2, 16, E)
    out = pl.pallas_call(
        _kernel,
        out_shape=jax.ShapeDtypeStruct((NSEG // 4, 4, SEG, 2 * D), bf16),
        in_specs=[hbm] * 13,
        out_specs=hbm,
        scratch_shapes=[
            pltpu.VMEM((NRAW, D // 2, 2, 16, E), bf16),
            pltpu.VMEM((6, 16 * WP, E), u32),
            pltpu.VMEM((8, H * E, 128), bf16),
            pltpu.VMEM((NSEG, SEG - M, D), bf16),
            pltpu.VMEM((M, D), bf16),
            pltpu.VMEM((NSEG, M, D), bf16),
            pltpu.VMEM((7, 4, 256, 128), bf16),
            pltpu.VMEM((49, 2, 128, 128), bf16),
            pltpu.VMEM((48, NSEG, 2 * M, E), bf16),
            pltpu.VMEM((49, 8, NSEG * M // 4, E), bf16),
            pltpu.VMEM((NSEG // 4, 4, SEG, D), bf16),
            pltpu.VMEM((96, 80), f32),
            pltpu.VMEM((8, NSEG // 4, 4, SEG, 128), bf16),
            pltpu.VMEM((2, 16, 512, 128), bf16),
            pltpu.VMEM((2, 1, S), bf16),
            pltpu.VMEM(gf.shape, u32),
            pltpu.VMEM(gi.shape, u32),
            pltpu.VMEM(tw.shape, f32),
            pltpu.VMEM((8, 16 * XP, 128), f32),
            pltpu.VMEM((2, 16, 65, 8, 128), f32),
            pltpu.SemaphoreType.DMA((7,)),
        ],
        compiler_params=pltpu.CompilerParams(vmem_limit_bytes=120 * 1024 * 1024),
    )(A_x.reshape(NSEG, SEG, D), A_mem0.reshape(M, D),
      A_Wq.reshape(wshape), A_Wk.reshape(wshape), A_Wv.reshape(wshape),
      A_Wo.reshape(H * E, D), B_x.reshape(NSEG // 4, 4, SEG, D), B_w_r.T, B_w_i.T, gf, gi, tw, fill)
    return out.reshape(1, S, 2 * D)
```
